```python
import jax
import jax.numpy as jnp

def _softmax(x, axis=-1):
    return jax.nn.softmax(x, axis=axis)

def _gelu(x):
    return jax.nn.gelu(x, approximate=True)

def _silu(x):
    return jax.nn.silu(x)

def _sigmoid(x):
    return jax.nn.sigmoid(x)

def _layernorm(x, axis=-1, eps=1e-05):
    m = jnp.mean(x, axis=axis, keepdims=True)
    v = jnp.var(x, axis=axis, keepdims=True)
    return (x - m) / jnp.sqrt(v + eps)

def _scatter_add(tgt, idx, src, axis=0):
    return tgt.at[idx].add(src)

def _segment_sum(src, seg, n):
    return jax.ops.segment_sum(src, seg, n)

class _Rng:

    def __init__(self, key):
        self._k = key

    def _next(self):
        self._k, sub = jax.random.split(self._k)
        return sub

    def normal(self, shape):
        return jax.random.normal(self._next(), shape, dtype=jnp.bfloat16)

    def randint(self, lo, hi, shape):
        return jax.random.randint(self._next(), shape, lo, hi, dtype=jnp.int32)

    def uniform(self, shape, lo=0.0, hi=1.0):
        return jax.random.uniform(self._next(), shape, jnp.bfloat16, lo, hi)

    def permutation(self, n):
        return jax.random.permutation(self._next(), n)
kernel_name = 'sequential_preLN__memory_aug_infini_attn__moe_arch_mod__prompt'

def setup_inputs():
    _rng = _Rng(jax.random.key(int.from_bytes(__import__("os").urandom(4), "little")))
    _w = lambda a: (lambda t: t.astype(jnp.bfloat16) if jnp.issubdtype(t.dtype, jnp.floating) else t)(jnp.asarray(a))

    def _A_setup():
        B, S, D, H = (1, 2048, 576, 32)
        N = 4
        L = max(1, S // N)
        sc = D ** (-0.5)
        return {'x': _w((lambda *s: _rng.normal(s) * 0.05)(B, N * L, D)), 'wq': _w((lambda *s: _rng.normal(s) * 0.05)(D, D) * sc), 'wk': _w((lambda *s: _rng.normal(s) * 0.05)(D, D) * sc), 'wv': _w((lambda *s: _rng.normal(s) * 0.05)(D, D) * sc), 'wo': _w((lambda *s: _rng.normal(s) * 0.05)(D, D) * sc), 'beta': _w((lambda *s: _rng.normal(s) * 0.05)(H))}
    _A_in = _A_setup()

    def _B_setup():
        B, S, D, F, C = (1, 2048, 576, 4608, 1)
        return {'x': _w((lambda *s: _rng.normal(s) * 0.05)(B, S, D)), 'w_r': _w((lambda *s: _rng.normal(s) * 0.05)(D)), 'w_gate': _w((lambda *s: _rng.normal(s) * 0.05)(D, F)), 'w_up': _w((lambda *s: _rng.normal(s) * 0.05)(D, F)), 'w_down': _w((lambda *s: _rng.normal(s) * 0.05)(F, D))}
    _B_in = _B_setup()
    return {'A_x': _A_in['x'], 'A_wq': _A_in['wq'], 'A_wk': _A_in['wk'], 'A_wv': _A_in['wv'], 'A_wo': _A_in['wo'], 'A_beta': _A_in['beta'], 'B_x': _B_in['x'], 'B_w_r': _B_in['w_r'], 'B_w_gate': _B_in['w_gate'], 'B_w_up': _B_in['w_up'], 'B_w_down': _B_in['w_down']}

def reference(A_x, A_wq, A_wk, A_wv, A_wo, A_beta, B_x, B_w_r, B_w_gate, B_w_up, B_w_down):

    def _A_ref(x, wq, wk, wv, wo, beta):
        B, S, D = x.shape
        H = 32
        Dh = D // H
        N = 4
        L = S // N
        q = (lambda x, *d: x.transpose(*d))((x @ wq).reshape(B, S, H, Dh), 0, 2, 1, 3).reshape(B, H, N, L, Dh)
        k = (lambda x, *d: x.transpose(*d))((x @ wk).reshape(B, S, H, Dh), 0, 2, 1, 3).reshape(B, H, N, L, Dh)
        v = (lambda x, *d: x.transpose(*d))((x @ wv).reshape(B, S, H, Dh), 0, 2, 1, 3).reshape(B, H, N, L, Dh)
        phi = lambda t: jnp.where(t > 0, t + 1.0, jnp.exp(t))
        scale = Dh ** (-0.5)
        ar = jnp.arange(L)
        mask = (lambda x, dt: x.astype(dt))(ar[:, None] < ar[None, :], x.dtype) * -1000000000.0
        g = _sigmoid(beta).reshape(1, H, 1, 1)
        M = jnp.einsum('bhd,bhe->bhde', q[:, :, 0, 0, :] * 0.0, q[:, :, 0, 0, :] * 0.0)
        z = q[:, :, 0, 0, :] * 0.0
        outs = []
        for s in range(N):
            qs, ks, vs = (q[:, :, s].copy(), k[:, :, s].copy(), v[:, :, s].copy())
            logits = jnp.einsum('bhqd,bhkd->bhqk', qs, ks) * scale + mask
            p = _softmax(logits, axis=-1)
            a_dot = jnp.einsum('bhqk,bhkd->bhqd', p, vs)
            pq = phi(qs)
            num = jnp.einsum('bhld,bhde->bhle', pq, M)
            den = jnp.einsum('bhld,bhd->bhl', pq, z)[..., None] + 1e-06
            a_mem = num / den
            o = g * a_mem + (1.0 - g) * a_dot
            outs.append(o)
            pk = phi(ks)
            M = M + jnp.einsum('bhld,bhle->bhde', pk, vs)
            z = z + jnp.einsum('bhld->bhd', pk)
        o = (lambda x, *d: x.transpose(*d))(jnp.stack(outs, 2).reshape(B, H, S, Dh), 0, 2, 1, 3).reshape(B, S, D)
        return o @ wo

    def _B_ref(x, w_r, w_gate, w_up, w_down):
        B, S, D = x.shape
        C = 1
        r = x @ w_r
        idx = jnp.argsort(-r, axis=-1)[:, :C]
        idx_e = jnp.repeat(idx.reshape(B, C, 1), D, axis=2)
        x_sel = jnp.take_along_axis(x, idx_e, axis=1)
        g = _silu(x_sel @ w_gate)
        u = x_sel @ w_up
        y = g * u @ w_down
        r_sel = _sigmoid(jnp.take_along_axis(r, idx, axis=1))
        y = y * r_sel.reshape(B, C, 1)
        b_off = (jnp.arange(B) * S).reshape(B, 1)
        flat_idx = (idx + b_off).reshape(B * C)
        zero = (x * 0.0).reshape(B * S, D)
        upd = _scatter_add(zero, flat_idx, y.reshape(B * C, D), axis=0)
        return x + upd.reshape(B, S, D)
    x = A_x
    h = x + _A_ref(_layernorm(x, axis=-1), A_wq, A_wk, A_wv, A_wo, A_beta)
    h2 = h + _B_ref(_layernorm(h, axis=-1), B_w_r, B_w_gate, B_w_up, B_w_down)
    return h2
```

```python
import functools

import jax
import jax.numpy as jnp
from jax import lax
import jax.experimental.pallas as pl
import jax.experimental.pallas.tpu as pltpu

S = 2048
D = 576
H = 32
DH = 18
NSEG = 4
L = 512
F = 4608
T = 128
NT = L // T
EPS = 1e-5
LOG2E = 1.4426950408889634
QSCALE = (DH ** -0.5) * LOG2E
WIN = 112
GROUPS = (tuple(range(0, 7)), tuple(range(7, 13)), tuple(range(13, 19)),
          tuple(range(19, 25)), tuple(range(25, 32)))
NG = len(GROUPS)
MROWS = T + 16
SAFE_LOGIT = 60.0
SAFE_V = 2.0 ** 40

bf16 = jnp.bfloat16
f32 = jnp.float32


def _layernorm_t(x):
    m = jnp.mean(x, axis=0, keepdims=True)
    xc = x - m
    v = jnp.mean(xc * xc, axis=0, keepdims=True)
    return xc * lax.rsqrt(v + EPS)


def _phi(t):
    return jnp.where(t > 0, t + 1.0, jnp.exp(t))


def _dot(a, b):
    return jnp.dot(a, b, preferred_element_type=f32)


def _dot_nt(a, b):
    return lax.dot_general(a, b, (((1,), (1,)), ((), ())), preferred_element_type=f32)


def _dot_tn(a, b):
    return lax.dot_general(a, b, (((0,), (0,)), ((), ())), preferred_element_type=f32)


def _masked_q(qt_ref, g, j):
    ws = WIN * g
    row64 = lax.broadcasted_iota(jnp.int32, (64, T), 0)
    qw32 = pltpu.bitcast(qt_ref[ws:ws + T, j * T:(j + 1) * T], jnp.uint32)
    qms = []
    for h in GROUPS[g]:
        lo2 = (h * DH - ws) // 2
        qmask = (row64 >= lo2) & (row64 < lo2 + DH // 2)
        qms.append(pltpu.bitcast(jnp.where(qmask, qw32, jnp.uint32(0)), bf16))
    return jnp.concatenate(qms, axis=1)


def _scores_fast(g, kp_ref, qt_ref, p_ref):
    kk = lax.broadcasted_iota(jnp.int32, (T, T), 0)
    qq = lax.broadcasted_iota(jnp.int32, (T, T), 1)
    causal = kk <= qq
    for j in range(NT):
        qm = _masked_q(qt_ref, g, j)
        nk = T * (j + 1)
        p = jnp.exp2(_dot(kp_ref[g, 0:nk, :], qm))
        for u in range(len(GROUPS[g])):
            pu = p[:, u * T:(u + 1) * T]
            if j > 0:
                p_ref[u, j, 0:j * T, :] = pu[0:j * T].astype(bf16)
            p_ref[u, j, j * T:(j + 1) * T, :] = jnp.where(
                causal, pu[j * T:(j + 1) * T], 0.0).astype(bf16)


def _scores_safe(g, kp_ref, qt_ref, p_ref):
    for j in range(NT):
        nk = T * (j + 1)
        kk = lax.broadcasted_iota(jnp.int32, (nk, T), 0)
        qq = lax.broadcasted_iota(jnp.int32, (nk, T), 1) + j * T
        causal = kk <= qq
        qm = _masked_q(qt_ref, g, j)
        for u in range(len(GROUPS[g])):
            s = _dot(kp_ref[g, 0:nk, :], qm[:, u * T:(u + 1) * T])
            s = jnp.where(causal, s, -jnp.inf)
            m = jnp.max(s, axis=0, keepdims=True)
            p_ref[u, j, 0:nk, :] = jnp.exp2(s - m).astype(bf16)


def _pv(g, vh_ref, p_ref, g1_ref, ot_ref):
    row32 = lax.broadcasted_iota(jnp.int32, (32, T), 0)
    for u, h in enumerate(GROUPS[g]):
        vs = ((h * DH) // 16) * 16
        off = h * DH - vs
        omask = (row32 >= off) & (row32 < off + DH)
        g1 = g1_ref[h]
        for j in range(NT):
            nk = T * (j + 1)
            acc = _dot(vh_ref[h, :, 0:nk], p_ref[u, j, 0:nk, :])
            l8 = acc[24:32] if off <= 6 else acc[0:8]
            rl = g1 / l8
            o = acc * jnp.concatenate([rl] * 4, axis=0) + ot_ref[vs:vs + 32, j * T:(j + 1) * T]
            pltpu.store(ot_ref.at[vs:vs + 32, j * T:(j + 1) * T], o, mask=omask)


def _kernel(x_hbm, wq_hbm, wk_hbm, wv_hbm, wo_hbm, beta_ref, wr_ref, wg_hbm, wu_hbm, wd_hbm,
            out_hbm,
            x_v, w_in, wt, wot, wg_v, wu_v, wd_v,
            xn, qt, pqt, kt, pkt, vt, kp, vh, p0, p1, ot,
            macc, mb, bmask, gtab, g1tab, wrtab, xn2_all, out_v, best_v, best_i,
            sem_x, sem_w, sem_o):
    def x_copy(s):
        return pltpu.make_async_copy(x_hbm.at[0, :, pl.ds(s * L, L)],
                                     x_v.at[:, pl.ds(s * L, L)], sem_x.at[s])

    def out_copy(s):
        return pltpu.make_async_copy(out_v.at[:, pl.ds(s * L, L)],
                                     out_hbm.at[0, :, pl.ds(s * L, L)], sem_o.at[s])

    w_copies = [
        pltpu.make_async_copy(wq_hbm, w_in.at[0], sem_w.at[0]),
        pltpu.make_async_copy(wk_hbm, w_in.at[1], sem_w.at[1]),
        pltpu.make_async_copy(wv_hbm, w_in.at[2], sem_w.at[2]),
        pltpu.make_async_copy(wo_hbm, w_in.at[3], sem_w.at[3]),
        pltpu.make_async_copy(wg_hbm, wg_v, sem_w.at[4]),
        pltpu.make_async_copy(wu_hbm, wu_v, sem_w.at[5]),
        pltpu.make_async_copy(wd_hbm, wd_v, sem_w.at[6]),
    ]
    x_copy(0).start()
    for c in w_copies[:4]:
        c.start()

    gate = jax.nn.sigmoid(beta_ref[...].astype(f32))
    rr = lax.broadcasted_iota(jnp.int32, (D, H), 0)
    hh = lax.broadcasted_iota(jnp.int32, (D, H), 1)
    onehot = (rr >= hh * DH) & (rr < (hh + 1) * DH)
    gcol = jnp.sum(jnp.where(onehot, gate, 0.0), axis=1, keepdims=True)
    gtab[...] = jnp.broadcast_to(gcol, (D, T))
    hh8 = lax.broadcasted_iota(jnp.int32, (8, H), 1)
    for h in range(H):
        gh = jnp.sum(jnp.where(hh8 == h, gate, 0.0), axis=1, keepdims=True)
        g1tab[h] = jnp.broadcast_to(1.0 - gh, (8, T))
    wr_row = wr_ref[...].astype(f32).reshape(1, D)
    wr_pad = jnp.concatenate([wr_row, jnp.zeros((1, 5 * T - D), f32)], axis=1)
    wrtab[...] = jnp.broadcast_to(wr_pad, (T, 5 * T)).T[0:D]
    mr = lax.broadcasted_iota(jnp.int32, (MROWS, T), 0)
    mc = lax.broadcasted_iota(jnp.int32, (MROWS, T), 1)
    for g in range(NG):
        ws = WIN * g
        m = jnp.zeros((MROWS, T), jnp.bool_)
        for i, h in enumerate(GROUPS[g]):
            lo = h * DH - ws
            cols = (mc >= lo) & (mc < lo + DH)
            rows = ((mr >= lo) & (mr < lo + DH) & (mr < T)) | (mr == T + i)
            m = m | (cols & rows)
        bmask[g] = jnp.where(m, 1.0, 0.0)
    macc[...] = jnp.zeros_like(macc)
    mb[...] = jnp.zeros_like(mb)
    best_v[...] = jnp.full(best_v.shape, -jnp.inf, f32)
    best_i[...] = jnp.zeros(best_i.shape, jnp.int32)

    cmax = []
    for i in range(3):
        w_copies[i].wait()
        w = w_in[i]
        wt[i * D:(i + 1) * D, :] = w.T
        wf = w.astype(f32)
        cmax.append(jnp.max(jnp.sum(wf * wf, axis=0, keepdims=True)))
    for s in range(1, NSEG):
        x_copy(s).start()
    for c in w_copies[4:]:
        c.start()
    w_copies[3].wait()
    wot[...] = w_in[3].T
    slack = 1.05
    logit_bound2 = (cmax[0] * cmax[1]) * (slack * D * DH * QSCALE) ** 2
    v_bound2 = cmax[2] * (slack * D)
    safe = (logit_bound2 <= SAFE_LOGIT ** 2) & (v_bound2 <= SAFE_V ** 2)

    ones_rows = jnp.ones((16, L), bf16)
    row32u = lax.broadcasted_iota(jnp.int32, (16, L), 0)

    def segment(s, fast):
        x_copy(s).wait()
        col0 = pl.multiple_of(s * L, L)
        xs = x_v[:, pl.ds(col0, L)].astype(f32)
        xn[...] = _layernorm_t(xs).astype(bf16)
        qkv = _dot(wt[...], xn[...])
        q = qkv[0:D]
        qt[...] = (q * QSCALE).astype(bf16)
        pqt[...] = _phi(q).astype(bf16)
        k = qkv[D:2 * D]
        kt[...] = k.astype(bf16)
        pkt[...] = _phi(k).astype(bf16)
        vt[...] = qkv[2 * D:3 * D].astype(bf16)
        for g in range(NG):
            kp[g] = kt[WIN * g:WIN * g + T, :].T
        one32 = jnp.uint32(0x3F803F80)
        for h in range(H):
            vs = ((h * DH) // 16) * 16
            off2 = (h * DH - vs) // 2
            v32 = pltpu.bitcast(vt[vs:vs + 32, :], jnp.uint32)
            keep = (row32u >= off2) & (row32u < off2 + DH // 2)
            vh[h] = pltpu.bitcast(jnp.where(keep, v32, one32), bf16)

        row128 = lax.broadcasted_iota(jnp.int32, (T, T), 0)
        row8 = lax.broadcasted_iota(jnp.int32, (8, T), 0)
        for g in range(NG):
            ws = WIN * g
            heads = GROUPS[g]
            lo_g, hi_g = heads[0] * DH - ws, (heads[-1] + 1) * DH - ws
            wmask = (row128 >= lo_g) & (row128 < hi_g)
            for j in range(NT):
                nd = _dot(mb[g], pqt[ws:ws + T, j * T:(j + 1) * T])
                rden = 1.0 / (nd[T:T + 8] + 1e-6)
                rb = [jnp.broadcast_to(rden[i:i + 1], (8, T)) for i in range(len(heads))]
                blocks = []
                for b in range(T // 8):
                    r_lo, r_hi = 8 * b, 8 * b + 7
                    i_lo = min(max((r_lo + ws) // DH - heads[0], 0), len(heads) - 1)
                    i_hi = min(max((r_hi + ws) // DH - heads[0], 0), len(heads) - 1)
                    if i_lo == i_hi:
                        blocks.append(rb[i_lo])
                    else:
                        cut = (heads[0] + i_hi) * DH - ws - r_lo
                        blocks.append(jnp.where(row8 < cut, rb[i_lo], rb[i_hi]))
                am = nd[0:T] * jnp.concatenate(blocks, axis=0) * gtab[ws:ws + T, :]
                pltpu.store(ot.at[ws:ws + T, j * T:(j + 1) * T], am, mask=wmask)

        ps = (p0, p1)
        scores = _scores_fast if fast else _scores_safe
        scores(0, kp, qt, ps[0])
        for g in range(NG):
            if g + 1 < NG:
                scores(g + 1, kp, qt, ps[(g + 1) % 2])
            _pv(g, vh, ps[g % 2], g1tab, ot)

        for g in range(NG):
            ws = WIN * g
            lhs = jnp.concatenate([vt[ws:ws + T, :], ones_rows], axis=0)
            upd = macc[g] + _dot_nt(lhs, pkt[ws:ws + T, :])
            macc[g] = upd
            mb[g] = jnp.where(bmask[g] != 0.0, upd, 0.0).astype(bf16)

        hres = xs + _dot(wot[...], ot[...].astype(bf16))
        x2 = _layernorm_t(hres)
        x2b = x2.astype(bf16)
        xn2_all[:, pl.ds(col0, L)] = x2b
        out_v[:, pl.ds(col0, L)] = (hres + x2).astype(bf16)
        out_copy(s).start()
        wr4 = jnp.concatenate([wrtab[...]] * NT, axis=1)
        r = jnp.sum(x2b.astype(f32) * wr4, axis=0, keepdims=True)
        r = r.astype(bf16).astype(f32)
        rmax = jnp.max(r, axis=1, keepdims=True)
        ids = lax.broadcasted_iota(jnp.int32, (1, L), 1) + col0
        rid = jnp.min(jnp.where(r == rmax, ids, S), axis=1, keepdims=True)
        better = rmax > best_v[0:1, 0:1]
        best_i[...] = jnp.broadcast_to(jnp.where(better, rid, best_i[0:1, 0:1]), best_i.shape)
        best_v[...] = jnp.broadcast_to(jnp.where(better, rmax, best_v[0:1, 0:1]), best_v.shape)

    @pl.when(safe)
    def _():
        lax.fori_loop(0, NSEG, lambda s, c: (segment(s, True), c)[1], 0)

    @pl.when(jnp.logical_not(safe))
    def _():
        lax.fori_loop(0, NSEG, lambda s, c: (segment(s, False), c)[1], 0)

    idx = jnp.clip(jnp.max(best_i[...]), 0, S - 1)
    base = pl.multiple_of((idx // T) * T, T)
    lane = idx - base
    blk = xn2_all[:, pl.ds(base, T)]
    pick = jnp.where(lax.broadcasted_iota(jnp.int32, (16, T), 1) == lane, 1.0, 0.0).astype(bf16)
    xg = _dot_nt(pick, blk).astype(bf16)
    for c in w_copies[4:]:
        c.wait()
    gt = _dot(xg, wg_v[...])
    up = _dot(xg, wu_v[...])
    act = (gt * jax.nn.sigmoid(gt) * up)[0:1].astype(bf16).astype(f32)
    yacc = jnp.zeros((D, T), f32)
    for c in range(F // T):
        yacc = yacc + wd_v[:, c * T:(c + 1) * T].astype(f32) * act[:, c * T:(c + 1) * T]
    y = jnp.sum(yacc, axis=1, keepdims=True) * jax.nn.sigmoid(best_v[0:1, 0:1])
    for s in range(NSEG):
        out_copy(s).wait()
    sel = lax.broadcasted_iota(jnp.int32, (D, T), 1) == lane
    cur = out_v[:, pl.ds(base, T)].astype(f32)
    out_v[:, pl.ds(base, T)] = (cur + jnp.where(sel, y, 0.0)).astype(bf16)
    patch = pltpu.make_async_copy(out_v.at[:, pl.ds(base, T)],
                                  out_hbm.at[0, :, pl.ds(base, T)], sem_o.at[NSEG])
    patch.start()
    patch.wait()


@jax.jit
def pallas_sequential_preLN__memory_aug_infini_attn__moe_arch_mod__prompt_kernel(
    A_x: jax.Array,
    A_wq: jax.Array,
    A_wk: jax.Array,
    A_wv: jax.Array,
    A_wo: jax.Array,
    A_beta: jax.Array,
    B_x: jax.Array,
    B_w_r: jax.Array,
    B_w_gate: jax.Array,
    B_w_up: jax.Array,
    B_w_down: jax.Array,
):
    del B_x
    hbm_spec = pl.BlockSpec(memory_space=pltpu.HBM)
    vmem_spec = pl.BlockSpec(memory_space=pltpu.VMEM)
    scratch = [
        pltpu.VMEM((D, S), bf16),
        pltpu.VMEM((4, D, D), bf16),
        pltpu.VMEM((3 * D, D), bf16),
        pltpu.VMEM((D, D), bf16),
        pltpu.VMEM((D, F), bf16),
        pltpu.VMEM((D, F), bf16),
        pltpu.VMEM((D, F), bf16),
        pltpu.VMEM((D, L), bf16),
        pltpu.VMEM((D, L), bf16),
        pltpu.VMEM((D, L), bf16),
        pltpu.VMEM((D, L), bf16),
        pltpu.VMEM((D, L), bf16),
        pltpu.VMEM((D, L), bf16),
        pltpu.VMEM((NG, L, T), bf16),
        pltpu.VMEM((H, 32, L), bf16),
        pltpu.VMEM((7, NT, L, T), bf16),
        pltpu.VMEM((7, NT, L, T), bf16),
        pltpu.VMEM((D, L), f32),
        pltpu.VMEM((NG, MROWS, T), f32),
        pltpu.VMEM((NG, MROWS, T), bf16),
        pltpu.VMEM((NG, MROWS, T), f32),
        pltpu.VMEM((D, T), f32),
        pltpu.VMEM((H, 8, T), f32),
        pltpu.VMEM((D, T), f32),
        pltpu.VMEM((D, S), bf16),
        pltpu.VMEM((D, S), bf16),
        pltpu.VMEM((8, T), f32),
        pltpu.VMEM((8, T), jnp.int32),
        pltpu.SemaphoreType.DMA((NSEG,)),
        pltpu.SemaphoreType.DMA((7,)),
        pltpu.SemaphoreType.DMA((NSEG + 1,)),
    ]
    out_t = pl.pallas_call(
        _kernel,
        out_shape=jax.ShapeDtypeStruct((1, D, S), bf16),
        in_specs=[hbm_spec, hbm_spec, hbm_spec, hbm_spec, hbm_spec, vmem_spec, vmem_spec,
                  hbm_spec, hbm_spec, hbm_spec],
        out_specs=hbm_spec,
        scratch_shapes=scratch,
        compiler_params=pltpu.CompilerParams(vmem_limit_bytes=100 * 1024 * 1024),
    )(jnp.transpose(A_x, (0, 2, 1)), A_wq, A_wk, A_wv, A_wo, A_beta.reshape(1, H),
      B_w_r, B_w_gate, B_w_up, B_w_down.T)
    return jnp.transpose(out_t, (0, 2, 1))
```

```python
import contextlib

import jax
import jax.numpy as jnp
from jax import lax
import jax.experimental.pallas as pl
import jax.experimental.pallas.tpu as pltpu

S = 2048
D = 576
H = 32
DH = 18
NSEG = 4
L = 512
F = 4608
T = 128
NT = L // T
EPS = 1e-5
LOG2E = 1.4426950408889634
QSCALE = (DH ** -0.5) * LOG2E
WIN = 112
GROUPS = (tuple(range(0, 7)), tuple(range(7, 13)), tuple(range(13, 19)),
          tuple(range(19, 25)), tuple(range(25, 32)))
NG = len(GROUPS)
MROWS = T + 16
SAFE_LOGIT = 60.0
SAFE_V = 2.0 ** 40

bf16 = jnp.bfloat16
f32 = jnp.float32
_SIDE_A = {}
_ORDER_B = ["MU", "OP", "LN1", "PR", "MR", "FINC"]
_PROFILE = False


def _scope(name):
    return jax.named_scope(name) if _PROFILE else contextlib.nullcontext()


def _colsum(x):
    n = x.shape[0] // 4
    parts = [jnp.sum(x[i * n:(i + 1) * n].reshape(n // 8, 8, x.shape[1]), axis=0) for i in range(4)]
    return jnp.sum((parts[0] + parts[1]) + (parts[2] + parts[3]), axis=0, keepdims=True)


def _ln_stats(x):
    m = _colsum(x) * (1.0 / D)
    v = jnp.maximum(_colsum(x * x) * (1.0 / D) - m * m, 0.0)
    a = lax.rsqrt(v + EPS)
    return a, -m * a


def _phi(t):
    return jnp.where(t > 0, t + 1.0, jnp.exp(t))


def _dot(a, b):
    return jnp.dot(a, b, preferred_element_type=f32)


def _dot_nt(a, b):
    return lax.dot_general(a, b, (((1,), (1,)), ((), ())), preferred_element_type=f32)


def _dot_tn(a, b):
    return lax.dot_general(a, b, (((0,), (0,)), ((), ())), preferred_element_type=f32)


def _swapped(g, u):
    return u % 2 == 1


def _masked_q(qt_ref, g, j):
    ws = WIN * g
    row64 = lax.broadcasted_iota(jnp.int32, (64, T), 0)
    qw32 = pltpu.bitcast(qt_ref[ws:ws + T, j * T:(j + 1) * T], jnp.uint32)
    qw32_sw = pltpu.roll(qw32, T // 2, axis=1)
    qms = []
    for u, h in enumerate(GROUPS[g]):
        lo2 = (h * DH - ws) // 2
        qmask = (row64 >= lo2) & (row64 < lo2 + DH // 2)
        src = qw32_sw if _swapped(g, u) else qw32
        qms.append(jnp.where(qmask, src, jnp.uint32(0)))
    return qms


def _causal_masks(nk, j):
    kk = lax.broadcasted_iota(jnp.int32, (nk, T), 0)
    qq = lax.broadcasted_iota(jnp.int32, (nk, T), 1)
    return kk <= qq + j * T, kk <= ((qq + T // 2) & (T - 1)) + j * T


def _scores_fast(g, kp_ref, qt_ref, p_ref):
    nh = len(GROUPS[g])
    causal = _causal_masks(T, 0)
    lane64 = lax.broadcasted_iota(jnp.int32, (64, T), 1)
    for j in range(NT):
        qms = _masked_q(qt_ref, g, j)
        qm = jnp.concatenate([pltpu.bitcast(q, bf16) for q in qms], axis=1)
        pairs = []
        for u in range(0, nh, 2):
            w = qms[u] if u + 1 == nh else jnp.where(lane64 < T // 2, qms[u + 1], qms[u])
            pairs.append(pltpu.bitcast(w, bf16))
        n1 = T * j + T // 2
        p1 = jnp.exp2(_dot(kp_ref[g, 0:n1, :], qm))
        p2 = jnp.exp2(_dot(kp_ref[g, n1:n1 + T // 2, :], jnp.concatenate(pairs, axis=1)))
        for u in range(nh):
            pu = p1[:, u * T:(u + 1) * T]
            if j > 0:
                p_ref[u, j, 0:j * T, :] = pu[0:j * T].astype(bf16)
            diag = jnp.concatenate(
                [pu[j * T:n1], p2[:, (u // 2) * T:(u // 2 + 1) * T]], axis=0)
            p_ref[u, j, j * T:(j + 1) * T, :] = jnp.where(
                causal[1 if _swapped(g, u) else 0], diag, 0.0).astype(bf16)


def _attention_safe(h, kp_ref, qt_ref, vh_ref, g1_ref, am_ref, ot_ref):
    g = jnp.minimum(jnp.maximum(h - 1, 0) // 6, NG - 1)
    ws = pl.multiple_of(g * WIN, 16)
    lo = h * DH - ws
    row128 = lax.broadcasted_iota(jnp.int32, (T, T), 0)
    qmask = (row128 >= lo) & (row128 < lo + DH)
    vs = pl.multiple_of(((h * DH) // 16) * 16, 16)
    off = h * DH - vs
    row32 = lax.broadcasted_iota(jnp.int32, (32, T), 0)
    omask = (row32 >= off) & (row32 < off + DH)
    kk = lax.broadcasted_iota(jnp.int32, (L, T), 0)
    qq = lax.broadcasted_iota(jnp.int32, (L, T), 1)

    def tile(j, c):
        c0 = pl.multiple_of(j * T, T)
        qm = jnp.where(qmask, qt_ref[pl.ds(ws, T), pl.ds(c0, T)].astype(f32), 0.0).astype(bf16)
        s = _dot(kp_ref[g], qm)
        s = jnp.where(kk <= qq + c0, s, -jnp.inf)
        m = jnp.max(s, axis=0, keepdims=True)
        p = jnp.exp2(s - m).astype(bf16)
        acc = _dot(vh_ref[h], p)
        l8 = jnp.where(off <= 6, acc[24:32], acc[0:8])
        rl = g1_ref[h] / l8
        o = acc * jnp.concatenate([rl] * 4, axis=0) + am_ref[pl.ds(vs, 32), pl.ds(c0, T)]
        pltpu.store(ot_ref.at[pl.ds(vs, 32), pl.ds(c0, T)], o, mask=omask)
        return c

    lax.fori_loop(0, NT, tile, 0)


def _pv(g, vh_ref, p_ref, g1_ref, am_ref, ot_ref):
    row32 = lax.broadcasted_iota(jnp.int32, (32, T), 0)
    for u, h in enumerate(GROUPS[g]):
        vs = ((h * DH) // 16) * 16
        off = h * DH - vs
        omask = (row32 >= off) & (row32 < off + DH)
        g1 = g1_ref[h]
        for j in range(NT):
            nk = T * (j + 1)
            acc = _dot(vh_ref[h, :, 0:nk], p_ref[u, j, 0:nk, :])
            l8 = acc[24:32] if off <= 6 else acc[0:8]
            rl = g1 / l8
            o = acc * jnp.concatenate([rl] * 4, axis=0)
            if _swapped(g, u):
                o = pltpu.roll(o, T // 2, axis=1)
            o = o + am_ref[vs:vs + 32, j * T:(j + 1) * T]
            pltpu.store(ot_ref.at[vs:vs + 32, j * T:(j + 1) * T], o, mask=omask)


def _kernel(x_hbm, wq_hbm, wk_hbm, wv_hbm, wo_hbm, beta_hbm, wr_hbm, wg_hbm, wu_hbm, wd_hbm,
            out_hbm,
            x_v, w_in, wt, at, wg_v, wu_v, wd_v,
            xn, qt, pqt, kt, pkt, vt, kp, vh, p0, p1, am_v, ot,
            macc, mb, bmask, gtab, g1tab, wrtab, xn2_all, out_v, best_v, best_i, wrsum, beta_ref, wr_ref,
            sem_x, sem_w, sem_o):
    def x_copy(s):
        return pltpu.make_async_copy(x_hbm.at[0, :, pl.ds(s * L, L)],
                                     x_v.at[:, pl.ds(s * L, L)], sem_x.at[s])

    def out_copy(s):
        return pltpu.make_async_copy(out_v.at[:, pl.ds(s * L, L)],
                                     out_hbm.at[0, :, pl.ds(s * L, L)], sem_o.at[s])

    w_copies = [
        pltpu.make_async_copy(wq_hbm, w_in.at[0], sem_w.at[0]),
        pltpu.make_async_copy(wk_hbm, w_in.at[1], sem_w.at[1]),
        pltpu.make_async_copy(wv_hbm, w_in.at[2], sem_w.at[2]),
        pltpu.make_async_copy(wo_hbm, w_in.at[3], sem_w.at[3]),
        pltpu.make_async_copy(wg_hbm, wg_v, sem_w.at[4]),
        pltpu.make_async_copy(wu_hbm, wu_v, sem_w.at[5]),
        pltpu.make_async_copy(wd_hbm, wd_v, sem_w.at[6]),
    ]
    small_b = pltpu.make_async_copy(beta_hbm, beta_ref, sem_w.at[7])
    small_r = pltpu.make_async_copy(wr_hbm, wr_ref, sem_w.at[8])
    w_copies[0].start()
    x_copy(0).start()
    small_b.start()
    small_r.start()

    class _Small:
        @staticmethod
        def wait():
            small_b.wait()
            small_r.wait()
    small = _Small

    def build_tables():
        gate = jax.nn.sigmoid(beta_ref[...].astype(f32).reshape(1, H))
        rr = lax.broadcasted_iota(jnp.int32, (D, H), 0)
        hh = lax.broadcasted_iota(jnp.int32, (D, H), 1)
        onehot = (rr >= hh * DH) & (rr < (hh + 1) * DH)
        gcol = jnp.sum(jnp.where(onehot, gate, 0.0), axis=1, keepdims=True)
        gtab[...] = jnp.broadcast_to(gcol, (D, T))
        hh8 = lax.broadcasted_iota(jnp.int32, (8, H), 1)
        for h in range(H):
            gh = jnp.sum(jnp.where(hh8 == h, gate, 0.0), axis=1, keepdims=True)
            g1tab[h] = jnp.broadcast_to(1.0 - gh, (8, T))
        wr_row = wr_ref[...].astype(f32).reshape(1, D)
        wr_pad = jnp.concatenate([wr_row, jnp.zeros((1, 5 * T - D), f32)], axis=1)
        wrtab[...] = jnp.broadcast_to(wr_pad, (T, 5 * T)).T[0:D]
        wrsum[...] = jnp.broadcast_to(jnp.sum(wr_row, axis=1, keepdims=True), wrsum.shape)

    mr = lax.broadcasted_iota(jnp.int32, (MROWS, T), 0)
    mc = lax.broadcasted_iota(jnp.int32, (MROWS, T), 1)
    for g in range(NG):
        ws = WIN * g
        m = jnp.zeros((MROWS, T), jnp.bool_)
        for i, h in enumerate(GROUPS[g]):
            lo = h * DH - ws
            cols = (mc >= lo) & (mc < lo + DH)
            rows = ((mr >= lo) & (mr < lo + DH) & (mr < T)) | (mr == T + i)
            m = m | (cols & rows)
        bmask[g] = jnp.where(m, 1.0, 0.0)
    macc[...] = jnp.zeros_like(macc)
    mb[...] = jnp.zeros_like(mb)
    best_v[...] = jnp.full(best_v.shape, -jnp.inf, f32)
    best_i[...] = jnp.zeros(best_i.shape, jnp.int32)

    ones_rows = jnp.ones((16, L), bf16)
    row32u = lax.broadcasted_iota(jnp.int32, (16, L), 0)

    def ln1(s):
        col0 = pl.multiple_of(s * L, L)
        xs = x_v[:, pl.ds(col0, L)].astype(f32)
        a, b = _ln_stats(xs)
        xn[...] = (xs * a + b).astype(bf16)

    def finalize(s, t0, nt, attn, valid):
        w = nt * T
        col0 = pl.multiple_of(s * L + t0 * T, T)
        hres = x_v[:, pl.ds(col0, w)].astype(f32) + attn
        a, b = _ln_stats(hres)
        x2 = hres * a + b
        xn2_all[:, pl.ds(col0, w)] = x2.astype(bf16)
        out_v[:, pl.ds(col0, w)] = (hres + x2).astype(bf16)
        wr = jnp.concatenate([wrtab[...]] * nt, axis=1)
        r = _colsum(hres * wr) * a + b * wrsum[0:1, 0:1]
        r = r.astype(bf16).astype(f32)
        if valid is not None:
            r = jnp.where(valid, r, -jnp.inf)
        bv, bi = best_v[0:1, :], best_i[0:1, :]
        for t in range(nt):
            rt = r[:, t * T:(t + 1) * T]
            better = rt > bv
            bi = jnp.where(better, col0 + t * T, bi)
            bv = jnp.where(better, rt, bv)
        best_i[...] = jnp.broadcast_to(bi, best_i.shape)
        best_v[...] = jnp.broadcast_to(bv, best_v.shape)

    def store_q(q):
        qt[...] = (q * QSCALE).astype(bf16)
        pqt[...] = _phi(q).astype(bf16)

    def store_k(k):
        kt[...] = k.astype(bf16)
        pkt[...] = _phi(k).astype(bf16)
        for g in range(NG):
            kp[g] = kt[WIN * g:WIN * g + T, :].T

    def store_v(v):
        vt[...] = v.astype(bf16)
        one32 = jnp.uint32(0x3F803F80)
        for h in range(H):
            vs = ((h * DH) // 16) * 16
            off2 = (h * DH - vs) // 2
            v32 = pltpu.bitcast(vt[vs:vs + 32, :], jnp.uint32)
            keep = (row32u >= off2) & (row32u < off2 + DH // 2)
            vh[h] = pltpu.bitcast(jnp.where(keep, v32, one32), bf16)

    def project():
        qkv = _dot(wt[...], xn[...])
        store_q(qkv[0:D])
        store_k(qkv[D:2 * D])
        store_v(qkv[2 * D:3 * D])

    def mem_read():
        row128 = lax.broadcasted_iota(jnp.int32, (T, T), 0)
        row8 = lax.broadcasted_iota(jnp.int32, (8, T), 0)
        for g in range(NG):
            ws = WIN * g
            heads = GROUPS[g]
            lo_g, hi_g = heads[0] * DH - ws, (heads[-1] + 1) * DH - ws
            wmask = (row128 >= lo_g) & (row128 < hi_g)
            for j in range(NT):
                nd = _dot(mb[g], pqt[ws:ws + T, j * T:(j + 1) * T])
                rden = 1.0 / (nd[T:T + 8] + 1e-6)
                rb = [jnp.broadcast_to(rden[i:i + 1], (8, T)) for i in range(len(heads))]
                blocks = []
                for b in range(T // 8):
                    r_lo, r_hi = 8 * b, 8 * b + 7
                    i_lo = min(max((r_lo + ws) // DH - heads[0], 0), len(heads) - 1)
                    i_hi = min(max((r_hi + ws) // DH - heads[0], 0), len(heads) - 1)
                    if i_lo == i_hi:
                        blocks.append(rb[i_lo])
                    else:
                        cut = (heads[0] + i_hi) * DH - ws - r_lo
                        blocks.append(jnp.where(row8 < cut, rb[i_lo], rb[i_hi]))
                amv = nd[0:T] * jnp.concatenate(blocks, axis=0) * gtab[ws:ws + T, :]
                pltpu.store(am_v.at[ws:ws + T, j * T:(j + 1) * T], amv, mask=wmask)

    def attention(fast, side):
        def run_side(pos):
            for job in side.get(pos, ()):
                job()
        ps = (p0, p1)
        if fast:
            run_side(0)
            _scores_fast(0, kp, qt, ps[0])
            for g in range(NG):
                run_side(g + 1)
                if g + 1 < NG:
                    _scores_fast(g + 1, kp, qt, ps[(g + 1) % 2])
                _pv(g, vh, ps[g % 2], g1tab, am_v, ot)
            run_side(NG + 1)
        else:
            for pos in range(NG + 2):
                run_side(pos)
            lax.fori_loop(0, H, lambda h, c: (_attention_safe(h, kp, qt, vh, g1tab, am_v, ot), c)[1], 0)

    def mem_update():
        for g in range(NG):
            ws = WIN * g
            lhs = jnp.concatenate([vt[ws:ws + T, :], ones_rows], axis=0)
            upd = macc[g] + _dot_nt(lhs, pkt[ws:ws + T, :])
            macc[g] = upd
            mb[g] = jnp.where(bmask[g] != 0.0, upd, 0.0).astype(bf16)

    def out_project():
        at[...] = _dot_tn(w_in[3], ot[...].astype(bf16))

    def load_weight(i):
        w = w_in[i]
        wt[i * D:(i + 1) * D, :] = w.T
        wf = w.astype(f32)
        return jnp.max(jnp.sum(wf * wf, axis=0, keepdims=True))

    am_v[...] = jnp.zeros_like(am_v)
    at[...] = jnp.zeros_like(at)
    with _scope("p_wq_wait"):
        w_copies[0].wait()
    w_copies[1].start()
    w_copies[2].start()
    x_copy(1).start()
    w_copies[3].start()
    with _scope("p_wq_T"):
        cq = load_weight(0)
    with _scope("p_x0_wait"):
        x_copy(0).wait()
    for s in range(2, NSEG):
        x_copy(s).start()
    for c in w_copies[4:]:
        c.start()
    HALF = 288
    with _scope("p_ln1_qlo"):
        ln1(0)
        q_lo = _dot(wt[0:HALF, :], xn[...])
        qt[0:HALF, :] = (q_lo * QSCALE).astype(bf16)
        pqt[0:HALF, :] = _phi(q_lo).astype(bf16)
    with _scope("p_wk_wait"):
        w_copies[1].wait()
    with _scope("p_wkT_qhi"):
        ck = load_weight(1)
        q_hi = _dot(wt[HALF:D, :], xn[...])
        qt[HALF:D, :] = (q_hi * QSCALE).astype(bf16)
        pqt[HALF:D, :] = _phi(q_hi).astype(bf16)
    with _scope("p_wv_wait"):
        w_copies[2].wait()
    with _scope("p_wvT_KV"):
        cv = load_weight(2)
        store_k(_dot(wt[D:2 * D, :], xn[...]))
        store_v(_dot(wt[2 * D:3 * D, :], xn[...]))
    slack = 1.05
    logit_bound2 = (cq * ck) * (slack * D * DH * QSCALE) ** 2
    v_bound2 = cv * (slack * D)
    safe = (logit_bound2 <= SAFE_LOGIT ** 2) & (v_bound2 <= SAFE_V ** 2)
    with _scope("p_tables"):
        small.wait()
        build_tables()
        w_copies[3].wait()

    def body(s, carry):
        more = s + 1 < NSEG
        nxt = jnp.minimum(s + 1, NSEG - 1)
        prev = jnp.maximum(s - 1, 0)

        @pl.when(more)
        def _():
            x_copy(nxt).wait()

        steps = {
            "LN1": lambda: ln1(nxt),
            "FINP": lambda: finalize(prev, 0, NT, at[...], s > 0),
            "FINC": lambda: finalize(s, 0, NT, at[...], None),
            "MU": mem_update, "PR": project, "MR": mem_read, "OP": out_project,
        }
        side = {k: [steps[n] for n in v] for k, v in _SIDE_A.items()}

        @pl.when(safe)
        def _():
            with _scope("attn"):
                attention(True, side)

        @pl.when(jnp.logical_not(safe))
        def _():
            attention(False, side)

        @pl.when(more)
        def _():
            with _scope("blockB"):
                for n in _ORDER_B:
                    steps[n]()

        if "FINP" in _ORDER_B:
            @pl.when(jnp.logical_and(s > 0, more))
            def _():
                out_copy(prev).start()
        else:
            @pl.when(more)
            def _():
                out_copy(s).start()
        return carry

    lax.fori_loop(0, NSEG, body, 0)
    with _scope("fin"):
        otb = ot[...].astype(bf16)
        a3 = [_dot_tn(w_in[3], otb[:, t * T:(t + 1) * T]) for t in range(NT)]
        if "FINP" in _ORDER_B:
            finalize(NSEG - 2, 0, NT, at[...], None)
            out_copy(NSEG - 2).start()
        for t in range(NT):
            finalize(NSEG - 1, t, 1, a3[t], None)
        out_copy(NSEG - 1).start()

    bv = best_v[...]
    rmax = jnp.max(bv, axis=1, keepdims=True)
    cand = best_i[...] + lax.broadcasted_iota(jnp.int32, best_i.shape, 1)
    idx = jnp.clip(jnp.min(jnp.where(bv == rmax, cand, S)), 0, S - 1)
    base = pl.multiple_of((idx // T) * T, T)
    lane = idx - base
    blk = xn2_all[:, pl.ds(base, T)]
    pick = jnp.where(lax.broadcasted_iota(jnp.int32, (16, T), 1) == lane, 1.0, 0.0).astype(bf16)
    xg = _dot_nt(pick, blk).astype(bf16)
    for c in w_copies[4:]:
        c.wait()
    yacc = jnp.zeros((D, T), f32)
    FC = 4 * T
    for c in range(F // FC):
        gt = _dot(xg, wg_v[:, c * FC:(c + 1) * FC])
        up = _dot(xg, wu_v[:, c * FC:(c + 1) * FC])
        act = (gt * jax.nn.sigmoid(gt) * up)[0:1].astype(bf16).astype(f32)
        for t in range(FC // T):
            f0 = c * FC + t * T
            yacc = yacc + wd_v[:, f0:f0 + T].astype(f32) * act[:, t * T:(t + 1) * T]
    y = jnp.sum(yacc, axis=1, keepdims=True) * jax.nn.sigmoid(rmax[0:1])
    for s in range(NSEG):
        out_copy(s).wait()
    sel = lax.broadcasted_iota(jnp.int32, (D, T), 1) == lane
    cur = out_v[:, pl.ds(base, T)].astype(f32)
    out_v[:, pl.ds(base, T)] = (cur + jnp.where(sel, y, 0.0)).astype(bf16)
    patch = pltpu.make_async_copy(out_v.at[:, pl.ds(base, T)],
                                  out_hbm.at[0, :, pl.ds(base, T)], sem_o.at[NSEG])
    patch.start()
    patch.wait()


@jax.jit
def pallas_sequential_preLN__memory_aug_infini_attn__moe_arch_mod__prompt_kernel(
    A_x: jax.Array,
    A_wq: jax.Array,
    A_wk: jax.Array,
    A_wv: jax.Array,
    A_wo: jax.Array,
    A_beta: jax.Array,
    B_x: jax.Array,
    B_w_r: jax.Array,
    B_w_gate: jax.Array,
    B_w_up: jax.Array,
    B_w_down: jax.Array,
):
    del B_x
    hbm_spec = pl.BlockSpec(memory_space=pltpu.HBM)
    scratch = [
        pltpu.VMEM((D, S), bf16),
        pltpu.VMEM((4, D, D), bf16),
        pltpu.VMEM((3 * D, D), bf16),
        pltpu.VMEM((D, L), f32),
        pltpu.VMEM((D, F), bf16),
        pltpu.VMEM((D, F), bf16),
        pltpu.VMEM((D, F), bf16),
        pltpu.VMEM((D, L), bf16),
        pltpu.VMEM((D, L), bf16),
        pltpu.VMEM((D, L), bf16),
        pltpu.VMEM((D, L), bf16),
        pltpu.VMEM((D, L), bf16),
        pltpu.VMEM((D, L), bf16),
        pltpu.VMEM((NG, L, T), bf16),
        pltpu.VMEM((H, 32, L), bf16),
        pltpu.VMEM((7, NT, L, T), bf16),
        pltpu.VMEM((7, NT, L, T), bf16),
        pltpu.VMEM((D, L), f32),
        pltpu.VMEM((D, L), f32),
        pltpu.VMEM((NG, MROWS, T), f32),
        pltpu.VMEM((NG, MROWS, T), bf16),
        pltpu.VMEM((NG, MROWS, T), f32),
        pltpu.VMEM((D, T), f32),
        pltpu.VMEM((H, 8, T), f32),
        pltpu.VMEM((D, T), f32),
        pltpu.VMEM((D, S), bf16),
        pltpu.VMEM((D, S), bf16),
        pltpu.VMEM((8, T), f32),
        pltpu.VMEM((8, T), jnp.int32),
        pltpu.VMEM((8, T), f32),
        pltpu.VMEM((H,), bf16),
        pltpu.VMEM((D,), bf16),
        pltpu.SemaphoreType.DMA((NSEG,)),
        pltpu.SemaphoreType.DMA((9,)),
        pltpu.SemaphoreType.DMA((NSEG + 1,)),
    ]
    out_t = pl.pallas_call(
        _kernel,
        out_shape=jax.ShapeDtypeStruct((1, D, S), bf16),
        in_specs=[hbm_spec] * 10,
        out_specs=hbm_spec,
        scratch_shapes=scratch,
        compiler_params=pltpu.CompilerParams(vmem_limit_bytes=100 * 1024 * 1024),
    )(jnp.transpose(A_x, (0, 2, 1)), A_wq, A_wk, A_wv, A_wo, A_beta,
      B_w_r, B_w_gate, B_w_up, B_w_down.T)
    return jnp.transpose(out_t, (0, 2, 1))
```

```python
import contextlib

import jax
import jax.numpy as jnp
from jax import lax
import jax.experimental.pallas as pl
import jax.experimental.pallas.tpu as pltpu

S = 2048
D = 576
H = 32
DH = 18
NSEG = 4
L = 512
F = 4608
T = 128
NT = L // T
EPS = 1e-5
LOG2E = 1.4426950408889634
QSCALE = (DH ** -0.5) * LOG2E
WIN = 112
GROUPS = (tuple(range(0, 7)), tuple(range(7, 13)), tuple(range(13, 19)),
          tuple(range(19, 25)), tuple(range(25, 32)))
NG = len(GROUPS)
KP = 640
MROWS = T + 16
SAFE_LOGIT = 60.0
SAFE_V = 2.0 ** 40

bf16 = jnp.bfloat16
f32 = jnp.float32
_ORDER_B = ["MU", "OP", "LN1", "PR", "MR", "FIN"]
_PROFILE = False


def _scope(name):
    return jax.named_scope(name) if _PROFILE else contextlib.nullcontext()


def _colsum(x):
    n = x.shape[0] // 4
    parts = [jnp.sum(x[i * n:(i + 1) * n].reshape(n // 8, 8, x.shape[1]), axis=0) for i in range(4)]
    return jnp.sum((parts[0] + parts[1]) + (parts[2] + parts[3]), axis=0, keepdims=True)


def _ln_stats(x):
    m = _colsum(x) * (1.0 / D)
    v = jnp.maximum(_colsum(x * x) * (1.0 / D) - m * m, 0.0)
    a = lax.rsqrt(v + EPS)
    return a, -m * a


def _phi(t):
    return jnp.where(t > 0, t + 1.0, jnp.exp(t))


def _dot(a, b):
    return jnp.dot(a, b, preferred_element_type=f32)


def _dot_nt(a, b):
    return lax.dot_general(a, b, (((1,), (1,)), ((), ())), preferred_element_type=f32)


def _dot_tn(a, b):
    return lax.dot_general(a, b, (((0,), (0,)), ((), ())), preferred_element_type=f32)


def _swapped(g, u):
    return u % 2 == 1


def _masked_q(qt_ref, g, j):
    ws = WIN * g
    row64 = lax.broadcasted_iota(jnp.int32, (64, T), 0)
    qw32 = pltpu.bitcast(qt_ref[ws:ws + T, j * T:(j + 1) * T], jnp.uint32)
    qw32_sw = pltpu.roll(qw32, T // 2, axis=1)
    qms = []
    for u, h in enumerate(GROUPS[g]):
        lo2 = (h * DH - ws) // 2
        qmask = (row64 >= lo2) & (row64 < lo2 + DH // 2)
        src = qw32_sw if _swapped(g, u) else qw32
        qms.append(jnp.where(qmask, src, jnp.uint32(0)))
    return qms


def _causal_masks(nk, j):
    kk = lax.broadcasted_iota(jnp.int32, (nk, T), 0)
    qq = lax.broadcasted_iota(jnp.int32, (nk, T), 1)
    return kk <= qq + j * T, kk <= ((qq + T // 2) & (T - 1)) + j * T


def _scores_fast(g, kp_ref, qt_ref, p_ref):
    nh = len(GROUPS[g])
    causal = _causal_masks(T, 0)
    lane64 = lax.broadcasted_iota(jnp.int32, (64, T), 1)
    for j in range(NT):
        qms = _masked_q(qt_ref, g, j)
        qm = jnp.concatenate([pltpu.bitcast(q, bf16) for q in qms], axis=1)
        pairs = []
        for u in range(0, nh, 2):
            w = qms[u] if u + 1 == nh else jnp.where(lane64 < T // 2, qms[u + 1], qms[u])
            pairs.append(pltpu.bitcast(w, bf16))
        n1 = T * j + T // 2
        p1 = jnp.exp2(_dot(kp_ref[g, 0:n1, :], qm))
        p2 = jnp.exp2(_dot(kp_ref[g, n1:n1 + T // 2, :], jnp.concatenate(pairs, axis=1)))
        for u in range(nh):
            pu = p1[:, u * T:(u + 1) * T]
            if j > 0:
                p_ref[u, j, 0:j * T, :] = pu[0:j * T].astype(bf16)
            diag = jnp.concatenate(
                [pu[j * T:n1], p2[:, (u // 2) * T:(u // 2 + 1) * T]], axis=0)
            p_ref[u, j, j * T:(j + 1) * T, :] = jnp.where(
                causal[1 if _swapped(g, u) else 0], diag, 0.0).astype(bf16)


def _attention_safe(h, kp_ref, qt_ref, vh_ref, g1_ref, am_ref, ot_ref):
    g = jnp.minimum(jnp.maximum(h - 1, 0) // 6, NG - 1)
    ws = pl.multiple_of(g * WIN, 16)
    lo = h * DH - ws
    row128 = lax.broadcasted_iota(jnp.int32, (T, T), 0)
    qmask = (row128 >= lo) & (row128 < lo + DH)
    vs = pl.multiple_of(((h * DH) // 16) * 16, 16)
    off = h * DH - vs
    row32 = lax.broadcasted_iota(jnp.int32, (32, T), 0)
    omask = (row32 >= off) & (row32 < off + DH)
    kk = lax.broadcasted_iota(jnp.int32, (L, T), 0)
    qq = lax.broadcasted_iota(jnp.int32, (L, T), 1)

    def tile(j, c):
        c0 = pl.multiple_of(j * T, T)
        qm = jnp.where(qmask, qt_ref[pl.ds(ws, T), pl.ds(c0, T)].astype(f32), 0.0).astype(bf16)
        s = _dot(kp_ref[g], qm)
        s = jnp.where(kk <= qq + c0, s, -jnp.inf)
        m = jnp.max(s, axis=0, keepdims=True)
        p = jnp.exp2(s - m).astype(bf16)
        acc = _dot(vh_ref[h], p)
        l8 = jnp.where(off <= 6, acc[24:32], acc[0:8])
        rl = g1_ref[h] / l8
        o = acc * jnp.concatenate([rl] * 4, axis=0) + am_ref[pl.ds(vs, 32), pl.ds(c0, T)]
        pltpu.store(ot_ref.at[pl.ds(vs, 32), pl.ds(c0, T)], o, mask=omask)
        return c

    lax.fori_loop(0, NT, tile, 0)


def _pv(g, vh_ref, p_ref, g1_ref, am_ref, ot_ref):
    row32 = lax.broadcasted_iota(jnp.int32, (32, T), 0)
    for u, h in enumerate(GROUPS[g]):
        vs = ((h * DH) // 16) * 16
        off = h * DH - vs
        omask = (row32 >= off) & (row32 < off + DH)
        g1 = g1_ref[h]
        for j in range(NT):
            nk = T * (j + 1)
            acc = _dot(vh_ref[h, :, 0:nk], p_ref[u, j, 0:nk, :])
            l8 = acc[24:32] if off <= 6 else acc[0:8]
            rl = g1 / l8
            o = acc * jnp.concatenate([rl] * 4, axis=0)
            if _swapped(g, u):
                o = pltpu.roll(o, T // 2, axis=1)
            o = o + am_ref[vs:vs + 32, j * T:(j + 1) * T]
            pltpu.store(ot_ref.at[vs:vs + 32, j * T:(j + 1) * T], o, mask=omask)


def _kernel(x_hbm, wq_hbm, wk_hbm, wv_hbm, wo_hbm, beta_hbm, wr_hbm, wg_hbm, wu_hbm, wd_hbm,
            out_hbm,
            x_v, w_in, wt, hbuf, wg_v, wu_v, wd_v,
            aug, arow, qt, pqt, kt, pkt, vt, kp, vh, p0, p1, am_v, ot,
            macc, mb, bmask, gtab, g1tab, wrtab, ab_all, out_v, best_v, best_i, wrsum, beta_ref, wr_ref,
            sem_x, sem_w, sem_o):
    def x_copy(s):
        return pltpu.make_async_copy(x_hbm.at[0, :, pl.ds(s * L, L)],
                                     x_v.at[:, pl.ds(s * L, L)], sem_x.at[s])

    def out_copy(s):
        return pltpu.make_async_copy(out_v.at[:, pl.ds(s * L, L)],
                                     out_hbm.at[0, :, pl.ds(s * L, L)], sem_o.at[s])

    w_copies = [
        pltpu.make_async_copy(wq_hbm, w_in.at[0], sem_w.at[0]),
        pltpu.make_async_copy(wk_hbm, w_in.at[1], sem_w.at[1]),
        pltpu.make_async_copy(wv_hbm, w_in.at[2], sem_w.at[2]),
        pltpu.make_async_copy(wo_hbm, w_in.at[3], sem_w.at[3]),
        pltpu.make_async_copy(wg_hbm, wg_v, sem_w.at[4]),
        pltpu.make_async_copy(wu_hbm, wu_v, sem_w.at[5]),
        pltpu.make_async_copy(wd_hbm, wd_v, sem_w.at[6]),
    ]
    small_b = pltpu.make_async_copy(beta_hbm, beta_ref, sem_w.at[7])
    small_r = pltpu.make_async_copy(wr_hbm, wr_ref, sem_w.at[8])
    small_b.start()
    small_r.start()
    x_copy(0).start()
    w_copies[0].start()
    w_copies[1].start()

    def build_tables():
        gate = jax.nn.sigmoid(beta_ref[...].astype(f32).reshape(1, H))
        rr = lax.broadcasted_iota(jnp.int32, (D, H), 0)
        hh = lax.broadcasted_iota(jnp.int32, (D, H), 1)
        onehot = (rr >= hh * DH) & (rr < (hh + 1) * DH)
        gcol = jnp.sum(jnp.where(onehot, gate, 0.0), axis=1, keepdims=True)
        gtab[...] = jnp.broadcast_to(gcol, (D, T))
        hh8 = lax.broadcasted_iota(jnp.int32, (8, H), 1)
        for h in range(H):
            gh = jnp.sum(jnp.where(hh8 == h, gate, 0.0), axis=1, keepdims=True)
            g1tab[h] = jnp.broadcast_to(1.0 - gh, (8, T))
        wr_row = wr_ref[...].astype(f32).reshape(1, D)
        wr_pad = jnp.concatenate([wr_row, jnp.zeros((1, 5 * T - D), f32)], axis=1)
        wrtab[...] = jnp.broadcast_to(wr_pad, (T, 5 * T)).T[0:D]
        wrsum[...] = jnp.broadcast_to(jnp.sum(wr_row, axis=1, keepdims=True), wrsum.shape)

    mr = lax.broadcasted_iota(jnp.int32, (MROWS, T), 0)
    mc = lax.broadcasted_iota(jnp.int32, (MROWS, T), 1)
    for g in range(NG):
        ws = WIN * g
        m = jnp.zeros((MROWS, T), jnp.bool_)
        for i, h in enumerate(GROUPS[g]):
            lo = h * DH - ws
            cols = (mc >= lo) & (mc < lo + DH)
            rows = ((mr >= lo) & (mr < lo + DH) & (mr < T)) | (mr == T + i)
            m = m | (cols & rows)
        bmask[g] = jnp.where(m, 1.0, 0.0)
    macc[...] = jnp.zeros_like(macc)
    mb[...] = jnp.zeros_like(mb)
    best_v[...] = jnp.full(best_v.shape, -jnp.inf, f32)
    best_i[...] = jnp.zeros(best_i.shape, jnp.int32)

    ones_rows = jnp.ones((16, L), bf16)
    row32u = lax.broadcasted_iota(jnp.int32, (16, L), 0)

    def ln1(s):
        col0 = pl.multiple_of(s * L, L)
        xs = x_v[:, pl.ds(col0, L)].astype(f32)
        m = _colsum(xs) * (1.0 / D)
        v = jnp.maximum(_colsum(xs * xs) * (1.0 / D) - m * m, 0.0)
        arow[:, pl.ds(col0, L)] = jnp.broadcast_to(lax.rsqrt(v + EPS), (8, L))
        m_hi = (-m).astype(bf16).astype(f32)
        m_lo = -m - m_hi
        r16 = lax.broadcasted_iota(jnp.int32, (16, L), 0)
        rows = jnp.where(r16 >= 4, 0.0, jnp.where((r16 & 1) == 0, m_hi, m_lo))
        aug[:, pl.ds(col0, L)] = rows.astype(bf16)

    def finalize(s, t0, nt, attn):
        w = nt * T
        col0 = pl.multiple_of(s * L + t0 * T, T)
        hres = x_v[:, pl.ds(col0, w)].astype(f32) + attn
        hbuf[:, pl.ds(col0, w)] = hres
        a, b = _ln_stats(hres)
        wr = jnp.concatenate([wrtab[...]] * nt, axis=1)
        r = _colsum(hres * wr) * a + b * wrsum[0:1, 0:1]
        ab_all[0:8, pl.ds(col0, w)] = jnp.broadcast_to(a, (8, w))
        ab_all[8:16, pl.ds(col0, w)] = jnp.broadcast_to(b, (8, w))
        out_v[:, pl.ds(col0, w)] = (hbuf[:, pl.ds(col0, w)] * (1.0 + a) + b).astype(bf16)
        r = r.astype(bf16).astype(f32)
        bv, bi = best_v[0:1, :], best_i[0:1, :]
        for t in range(nt):
            rt = r[:, t * T:(t + 1) * T]
            better = rt > bv
            bi = jnp.where(better, col0 + t * T, bi)
            bv = jnp.where(better, rt, bv)
        best_i[...] = jnp.broadcast_to(bi, best_i.shape)
        best_v[...] = jnp.broadcast_to(bv, best_v.shape)

    def proj_rhs(s):
        col0 = pl.multiple_of(s * L, L)
        return jnp.concatenate([x_v[:, pl.ds(col0, L)], aug[:, pl.ds(col0, L)],
                                jnp.zeros((KP - D - 16, L), bf16)], axis=0)

    def ln_scale(s):
        return arow[0:1, pl.ds(pl.multiple_of(s * L, L), L)]

    def store_q(raw, a, r0, r1):
        qt[r0:r1, :] = (raw * (a * QSCALE)).astype(bf16)
        pqt[r0:r1, :] = _phi(raw * a).astype(bf16)

    def store_k(raw, a):
        k = raw * a
        kt[...] = k.astype(bf16)
        pkt[...] = _phi(k).astype(bf16)
        for g in range(NG):
            kp[g] = kt[WIN * g:WIN * g + T, :].T

    def store_v(raw, a):
        vt[...] = (raw * a).astype(bf16)
        one32 = jnp.uint32(0x3F803F80)
        for h in range(H):
            vs = ((h * DH) // 16) * 16
            off2 = (h * DH - vs) // 2
            v32 = pltpu.bitcast(vt[vs:vs + 32, :], jnp.uint32)
            keep = (row32u >= off2) & (row32u < off2 + DH // 2)
            vh[h] = pltpu.bitcast(jnp.where(keep, v32, one32), bf16)

    def project(s):
        qkv = _dot(wt[...], proj_rhs(s))
        a = ln_scale(s)
        store_q(qkv[0:D], a, 0, D)
        store_k(qkv[D:2 * D], a)
        store_v(qkv[2 * D:3 * D], a)

    def mem_read():
        row128 = lax.broadcasted_iota(jnp.int32, (T, T), 0)
        row8 = lax.broadcasted_iota(jnp.int32, (8, T), 0)
        for g in range(NG):
            ws = WIN * g
            heads = GROUPS[g]
            lo_g, hi_g = heads[0] * DH - ws, (heads[-1] + 1) * DH - ws
            wmask = (row128 >= lo_g) & (row128 < hi_g)
            for j in range(NT):
                nd = _dot(mb[g], pqt[ws:ws + T, j * T:(j + 1) * T])
                rden = 1.0 / (nd[T:T + 8] + 1e-6)
                rb = [jnp.broadcast_to(rden[i:i + 1], (8, T)) for i in range(len(heads))]
                blocks = []
                for b in range(T // 8):
                    r_lo, r_hi = 8 * b, 8 * b + 7
                    i_lo = min(max((r_lo + ws) // DH - heads[0], 0), len(heads) - 1)
                    i_hi = min(max((r_hi + ws) // DH - heads[0], 0), len(heads) - 1)
                    if i_lo == i_hi:
                        blocks.append(rb[i_lo])
                    else:
                        cut = (heads[0] + i_hi) * DH - ws - r_lo
                        blocks.append(jnp.where(row8 < cut, rb[i_lo], rb[i_hi]))
                amv = nd[0:T] * jnp.concatenate(blocks, axis=0) * gtab[ws:ws + T, :]
                pltpu.store(am_v.at[ws:ws + T, j * T:(j + 1) * T], amv, mask=wmask)

    def attention(fast):
        ps = (p0, p1)
        if fast:
            _scores_fast(0, kp, qt, ps[0])
            for g in range(NG):
                if g + 1 < NG:
                    _scores_fast(g + 1, kp, qt, ps[(g + 1) % 2])
                _pv(g, vh, ps[g % 2], g1tab, am_v, ot)
        else:
            lax.fori_loop(0, H, lambda h, c: (_attention_safe(h, kp, qt, vh, g1tab, am_v, ot), c)[1], 0)

    def mem_update():
        for g in range(NG):
            ws = WIN * g
            lhs = jnp.concatenate([vt[ws:ws + T, :], ones_rows], axis=0)
            upd = macc[g] + _dot_nt(lhs, pkt[ws:ws + T, :])
            macc[g] = upd
            mb[g] = jnp.where(bmask[g] != 0.0, upd, 0.0).astype(bf16)

    def out_project():
        return _dot_tn(w_in[3], ot[...].astype(bf16))

    def load_weight(i):
        w = w_in[i]
        wf = w.astype(f32)
        c = jnp.sum(wf, axis=0, keepdims=True)
        c_hi = c.astype(bf16).astype(f32)
        r16 = lax.broadcasted_iota(jnp.int32, (16, D), 0)
        extra = jnp.where(r16 >= 4, 0.0, jnp.where(r16 < 2, c_hi, c - c_hi)).astype(bf16)
        w_aug = jnp.concatenate([w, extra, jnp.zeros((KP - D - 16, D), bf16)], axis=0)
        w_t = w_aug.T
        wt[i * D:(i + 1) * D, :] = w_t
        return w_t, jnp.max(jnp.sum(wf * wf, axis=0, keepdims=True))

    am_v[...] = jnp.zeros_like(am_v)
    with _scope("p_tables"):
        small_b.wait()
        small_r.wait()
        build_tables()
    with _scope("p_x0_wait"):
        x_copy(0).wait()
    w_copies[2].start()
    x_copy(1).start()
    w_copies[3].start()
    with _scope("p_ln1"):
        ln1(0)
    with _scope("p_wq_wait"):
        w_copies[0].wait()
    for s in range(2, NSEG):
        x_copy(s).start()
    for c in w_copies[4:]:
        c.start()
    HALF = 288
    with _scope("p_wqT_qlo"):
        wq_t, cq = load_weight(0)
        store_q(_dot(wq_t[0:HALF], proj_rhs(0)), ln_scale(0), 0, HALF)
    with _scope("p_wk_wait"):
        w_copies[1].wait()
    with _scope("p_wkT_qhi"):
        _, ck = load_weight(1)
        store_q(_dot(wt[HALF:D, :], proj_rhs(0)), ln_scale(0), HALF, D)
    with _scope("p_wv_wait"):
        w_copies[2].wait()
    with _scope("p_wvT_KV"):
        _, cv = load_weight(2)
        store_k(_dot(wt[D:2 * D, :], proj_rhs(0)), ln_scale(0))
        store_v(_dot(wt[2 * D:3 * D, :], proj_rhs(0)), ln_scale(0))
    slack = 1.05
    logit_bound2 = (cq * ck) * (slack * D * DH * QSCALE) ** 2
    v_bound2 = cv * (slack * D)
    safe = (logit_bound2 <= SAFE_LOGIT ** 2) & (v_bound2 <= SAFE_V ** 2)
    w_copies[3].wait()

    def body(s, carry):
        more = s + 1 < NSEG
        nxt = jnp.minimum(s + 1, NSEG - 1)

        @pl.when(more)
        def _():
            x_copy(nxt).wait()

        @pl.when(safe)
        def _():
            with _scope("attn"):
                attention(True)

        @pl.when(jnp.logical_not(safe))
        def _():
            attention(False)

        @pl.when(more)
        def _():
            with _scope("blockB"):
                hold = {}
                steps = {
                    "MU": mem_update,
                    "OP": lambda: hold.update(a=out_project()),
                    "LN1": lambda: ln1(nxt),
                    "PR": lambda: project(nxt),
                    "MR": mem_read,
                    "FIN": lambda: finalize(s, 0, NT, hold["a"]),
                }
                for n in _ORDER_B:
                    steps[n]()
            out_copy(s).start()
        return carry

    lax.fori_loop(0, NSEG, body, 0)
    with _scope("fin"):
        otb = ot[...].astype(bf16)
        for t in range(NT):
            finalize(NSEG - 1, t, 1, _dot_tn(w_in[3], otb[:, t * T:(t + 1) * T]))
        out_copy(NSEG - 1).start()

    bv = best_v[...]
    rmax = jnp.max(bv, axis=1, keepdims=True)
    cand = best_i[...] + lax.broadcasted_iota(jnp.int32, best_i.shape, 1)
    idx = jnp.clip(jnp.min(jnp.where(bv == rmax, cand, S)), 0, S - 1)
    base = pl.multiple_of((idx // T) * T, T)
    lane = idx - base
    blk = (hbuf[:, pl.ds(base, T)] * ab_all[0:1, pl.ds(base, T)]
           + ab_all[8:9, pl.ds(base, T)]).astype(bf16)
    pick = jnp.where(lax.broadcasted_iota(jnp.int32, (16, T), 1) == lane, 1.0, 0.0).astype(bf16)
    xg = _dot_nt(pick, blk).astype(bf16)
    for c in w_copies[4:]:
        c.wait()
    yacc = jnp.zeros((D, T), f32)
    FC = 4 * T
    for c in range(F // FC):
        gt = _dot(xg, wg_v[:, c * FC:(c + 1) * FC])
        up = _dot(xg, wu_v[:, c * FC:(c + 1) * FC])
        act = (gt * jax.nn.sigmoid(gt) * up)[0:1].astype(bf16).astype(f32)
        for t in range(FC // T):
            f0 = c * FC + t * T
            yacc = yacc + wd_v[:, f0:f0 + T].astype(f32) * act[:, t * T:(t + 1) * T]
    y = jnp.sum(yacc, axis=1, keepdims=True) * jax.nn.sigmoid(rmax[0:1])
    for s in range(NSEG):
        out_copy(s).wait()
    sel = lax.broadcasted_iota(jnp.int32, (D, T), 1) == lane
    cur = out_v[:, pl.ds(base, T)].astype(f32)
    out_v[:, pl.ds(base, T)] = (cur + jnp.where(sel, y, 0.0)).astype(bf16)
    patch = pltpu.make_async_copy(out_v.at[:, pl.ds(base, T)],
                                  out_hbm.at[0, :, pl.ds(base, T)], sem_o.at[NSEG])
    patch.start()
    patch.wait()


@jax.jit
def pallas_sequential_preLN__memory_aug_infini_attn__moe_arch_mod__prompt_kernel(
    A_x: jax.Array,
    A_wq: jax.Array,
    A_wk: jax.Array,
    A_wv: jax.Array,
    A_wo: jax.Array,
    A_beta: jax.Array,
    B_x: jax.Array,
    B_w_r: jax.Array,
    B_w_gate: jax.Array,
    B_w_up: jax.Array,
    B_w_down: jax.Array,
):
    del B_x
    hbm_spec = pl.BlockSpec(memory_space=pltpu.HBM)
    scratch = [
        pltpu.VMEM((D, S), bf16),
        pltpu.VMEM((4, D, D), bf16),
        pltpu.VMEM((3 * D, KP), bf16),
        pltpu.VMEM((D, S), f32),
        pltpu.VMEM((D, F), bf16),
        pltpu.VMEM((D, F), bf16),
        pltpu.VMEM((D, F), bf16),
        pltpu.VMEM((16, S), bf16),
        pltpu.VMEM((8, S), f32),
        pltpu.VMEM((D, L), bf16),
        pltpu.VMEM((D, L), bf16),
        pltpu.VMEM((D, L), bf16),
        pltpu.VMEM((D, L), bf16),
        pltpu.VMEM((D, L), bf16),
        pltpu.VMEM((NG, L, T), bf16),
        pltpu.VMEM((H, 32, L), bf16),
        pltpu.VMEM((7, NT, L, T), bf16),
        pltpu.VMEM((7, NT, L, T), bf16),
        pltpu.VMEM((D, L), f32),
        pltpu.VMEM((D, L), f32),
        pltpu.VMEM((NG, MROWS, T), f32),
        pltpu.VMEM((NG, MROWS, T), bf16),
        pltpu.VMEM((NG, MROWS, T), f32),
        pltpu.VMEM((D, T), f32),
        pltpu.VMEM((H, 8, T), f32),
        pltpu.VMEM((D, T), f32),
        pltpu.VMEM((16, S), f32),
        pltpu.VMEM((D, S), bf16),
        pltpu.VMEM((8, T), f32),
        pltpu.VMEM((8, T), jnp.int32),
        pltpu.VMEM((8, T), f32),
        pltpu.VMEM((H,), bf16),
        pltpu.VMEM((D,), bf16),
        pltpu.SemaphoreType.DMA((NSEG,)),
        pltpu.SemaphoreType.DMA((9,)),
        pltpu.SemaphoreType.DMA((NSEG + 1,)),
    ]
    out_t = pl.pallas_call(
        _kernel,
        out_shape=jax.ShapeDtypeStruct((1, D, S), bf16),
        in_specs=[hbm_spec] * 10,
        out_specs=hbm_spec,
        scratch_shapes=scratch,
        compiler_params=pltpu.CompilerParams(vmem_limit_bytes=100 * 1024 * 1024),
    )(jnp.transpose(A_x, (0, 2, 1)), A_wq, A_wk, A_wv, A_wo, A_beta,
      B_w_r, B_w_gate, B_w_up, B_w_down.T)
    return jnp.transpose(out_t, (0, 2, 1))
```

```python
import contextlib

import jax
import jax.numpy as jnp
from jax import lax
import jax.experimental.pallas as pl
import jax.experimental.pallas.tpu as pltpu

S = 2048
D = 576
H = 32
DH = 18
NSEG = 4
L = 512
F = 4608
T = 128
NT = L // T
EPS = 1e-5
LOG2E = 1.4426950408889634
QSCALE = (DH ** -0.5) * LOG2E
WIN = 112
GROUPS = (tuple(range(0, 7)), tuple(range(7, 13)), tuple(range(13, 19)),
          tuple(range(19, 25)), tuple(range(25, 32)))
NG = len(GROUPS)
KP = 640
MROWS = T + 16
SAFE_LOGIT = 60.0
SAFE_V = 2.0 ** 40

bf16 = jnp.bfloat16
f32 = jnp.float32
_ORDER_B = ["MU", "OP", "LN1", "PR", "MR", "FIN"]
_PROFILE = False


def _scope(name):
    return jax.named_scope(name) if _PROFILE else contextlib.nullcontext()


def _colsum(x):
    n = x.shape[0] // 4
    parts = [jnp.sum(x[i * n:(i + 1) * n].reshape(n // 8, 8, x.shape[1]), axis=0) for i in range(4)]
    return jnp.sum((parts[0] + parts[1]) + (parts[2] + parts[3]), axis=0, keepdims=True)


def _ln_stats(x):
    m = _colsum(x) * (1.0 / D)
    v = jnp.maximum(_colsum(x * x) * (1.0 / D) - m * m, 0.0)
    a = lax.rsqrt(v + EPS)
    return a, -m * a


def _phi(t):
    return jnp.where(t > 0, t + 1.0, jnp.exp(t))


def _dot(a, b):
    return jnp.dot(a, b, preferred_element_type=f32)


def _dot_nt(a, b):
    return lax.dot_general(a, b, (((1,), (1,)), ((), ())), preferred_element_type=f32)


def _dot_tn(a, b):
    return lax.dot_general(a, b, (((0,), (0,)), ((), ())), preferred_element_type=f32)


def _swapped(g, u):
    return u % 2 == 1


def _masked_q(qt_ref, g, j):
    ws = WIN * g
    row64 = lax.broadcasted_iota(jnp.int32, (64, T), 0)
    qw32 = pltpu.bitcast(qt_ref[ws:ws + T, j * T:(j + 1) * T], jnp.uint32)
    qw32_sw = pltpu.roll(qw32, T // 2, axis=1)
    qms = []
    for u, h in enumerate(GROUPS[g]):
        lo2 = (h * DH - ws) // 2
        qmask = (row64 >= lo2) & (row64 < lo2 + DH // 2)
        src = qw32_sw if _swapped(g, u) else qw32
        qms.append(jnp.where(qmask, src, jnp.uint32(0)))
    return qms


def _causal_masks(nk, j):
    kk = lax.broadcasted_iota(jnp.int32, (nk, T), 0)
    qq = lax.broadcasted_iota(jnp.int32, (nk, T), 1)
    return kk <= qq + j * T, kk <= ((qq + T // 2) & (T - 1)) + j * T


def _scores_fast(g, kp_ref, qt_ref, p_ref):
    nh = len(GROUPS[g])
    causal = _causal_masks(T, 0)
    lane64 = lax.broadcasted_iota(jnp.int32, (64, T), 1)
    for j in range(NT):
        qms = _masked_q(qt_ref, g, j)
        qm = jnp.concatenate([pltpu.bitcast(q, bf16) for q in qms], axis=1)
        pairs = []
        for u in range(0, nh, 2):
            w = qms[u] if u + 1 == nh else jnp.where(lane64 < T // 2, qms[u + 1], qms[u])
            pairs.append(pltpu.bitcast(w, bf16))
        n1 = T * j + T // 2
        p1 = jnp.exp2(_dot(kp_ref[g, 0:n1, :], qm))
        p2 = jnp.exp2(_dot(kp_ref[g, n1:n1 + T // 2, :], jnp.concatenate(pairs, axis=1)))
        for u in range(nh):
            pu = p1[:, u * T:(u + 1) * T]
            if j > 0:
                p_ref[u, j, 0:j * T, :] = pu[0:j * T].astype(bf16)
            diag = jnp.concatenate(
                [pu[j * T:n1], p2[:, (u // 2) * T:(u // 2 + 1) * T]], axis=0)
            p_ref[u, j, j * T:(j + 1) * T, :] = jnp.where(
                causal[1 if _swapped(g, u) else 0], diag, 0.0).astype(bf16)


def _attention_safe(h, kp_ref, qt_ref, vh_ref, g1_ref, am_ref, ot_ref):
    g = jnp.minimum(jnp.maximum(h - 1, 0) // 6, NG - 1)
    ws = pl.multiple_of(g * WIN, 16)
    lo = h * DH - ws
    row128 = lax.broadcasted_iota(jnp.int32, (T, T), 0)
    qmask = (row128 >= lo) & (row128 < lo + DH)
    vs = pl.multiple_of(((h * DH) // 16) * 16, 16)
    off = h * DH - vs
    row32 = lax.broadcasted_iota(jnp.int32, (32, T), 0)
    omask = (row32 >= off) & (row32 < off + DH)
    kk = lax.broadcasted_iota(jnp.int32, (L, T), 0)
    qq = lax.broadcasted_iota(jnp.int32, (L, T), 1)

    def tile(j, c):
        c0 = pl.multiple_of(j * T, T)
        qm = jnp.where(qmask, qt_ref[pl.ds(ws, T), pl.ds(c0, T)].astype(f32), 0.0).astype(bf16)
        s = _dot(kp_ref[g], qm)
        s = jnp.where(kk <= qq + c0, s, -jnp.inf)
        m = jnp.max(s, axis=0, keepdims=True)
        p = jnp.exp2(s - m).astype(bf16)
        acc = _dot(vh_ref[h], p)
        l8 = jnp.where(off <= 6, acc[24:32], acc[0:8])
        rl = g1_ref[h] / l8
        o = acc * jnp.concatenate([rl] * 4, axis=0) + am_ref[pl.ds(vs, 32), pl.ds(c0, T)]
        pltpu.store(ot_ref.at[pl.ds(vs, 32), pl.ds(c0, T)], o, mask=omask)
        return c

    lax.fori_loop(0, NT, tile, 0)


def _pv(g, vh_ref, p_ref, g1_ref, am_ref, ot_ref):
    row32 = lax.broadcasted_iota(jnp.int32, (32, T), 0)
    for u, h in enumerate(GROUPS[g]):
        vs = ((h * DH) // 16) * 16
        off = h * DH - vs
        omask = (row32 >= off) & (row32 < off + DH)
        g1 = g1_ref[h]
        for j in range(NT):
            nk = T * (j + 1)
            acc = _dot(vh_ref[h, :, 0:nk], p_ref[u, j, 0:nk, :])
            l8 = acc[24:32] if off <= 6 else acc[0:8]
            rl = g1 / l8
            o = acc * jnp.concatenate([rl] * 4, axis=0)
            if _swapped(g, u):
                o = pltpu.roll(o, T // 2, axis=1)
            o = o + am_ref[vs:vs + 32, j * T:(j + 1) * T]
            pltpu.store(ot_ref.at[vs:vs + 32, j * T:(j + 1) * T], o, mask=omask)


def _kernel(x_hbm, wq_hbm, wk_hbm, wv_hbm, wo_hbm, beta_hbm, wr_hbm, wg_hbm, wu_hbm, wd_hbm,
            out_hbm,
            x_v, w_in, wt, hbuf, wg_v, wu_v, wd_v,
            aug, arow, qt, pqt, kt, pkt, vt, kp, vh, p0, p1, am_v, ot,
            macc, mb, bmask, gtab, g1tab, wrtab, ab_all, out_v, best_v, best_i, wrsum, beta_ref, wr_ref,
            sem_x, sem_w, sem_o):
    def x_copy(s):
        return pltpu.make_async_copy(x_hbm.at[0, :, pl.ds(s * L, L)],
                                     x_v.at[:, pl.ds(s * L, L)], sem_x.at[s])

    def out_copy(s):
        return pltpu.make_async_copy(out_v.at[:, pl.ds(s * L, L)],
                                     out_hbm.at[0, :, pl.ds(s * L, L)], sem_o.at[s])

    w_copies = [
        pltpu.make_async_copy(wq_hbm, w_in.at[0], sem_w.at[0]),
        pltpu.make_async_copy(wk_hbm, w_in.at[1], sem_w.at[1]),
        pltpu.make_async_copy(wv_hbm, w_in.at[2], sem_w.at[2]),
        pltpu.make_async_copy(wo_hbm, w_in.at[3], sem_w.at[3]),
        pltpu.make_async_copy(wg_hbm, wg_v, sem_w.at[4]),
        pltpu.make_async_copy(wu_hbm, wu_v, sem_w.at[5]),
        pltpu.make_async_copy(wd_hbm, wd_v, sem_w.at[6]),
    ]
    small_b = pltpu.make_async_copy(beta_hbm, beta_ref, sem_w.at[7])
    small_r = pltpu.make_async_copy(wr_hbm, wr_ref, sem_w.at[8])
    small_b.start()
    small_r.start()
    x_copy(0).start()
    w_copies[0].start()
    w_copies[1].start()

    def build_tables():
        gate = jax.nn.sigmoid(beta_ref[...].astype(f32).reshape(1, H))
        rr = lax.broadcasted_iota(jnp.int32, (D, H), 0)
        hh = lax.broadcasted_iota(jnp.int32, (D, H), 1)
        onehot = (rr >= hh * DH) & (rr < (hh + 1) * DH)
        gcol = jnp.sum(jnp.where(onehot, gate, 0.0), axis=1, keepdims=True)
        gtab[...] = jnp.broadcast_to(gcol, (D, T))
        hh8 = lax.broadcasted_iota(jnp.int32, (8, H), 1)
        for h in range(H):
            gh = jnp.sum(jnp.where(hh8 == h, gate, 0.0), axis=1, keepdims=True)
            g1tab[h] = jnp.broadcast_to(1.0 - gh, (8, T))
        wr_row = wr_ref[...].astype(f32).reshape(1, D)
        wr_pad = jnp.concatenate([wr_row, jnp.zeros((1, 5 * T - D), f32)], axis=1)
        wrtab[...] = jnp.broadcast_to(wr_pad, (T, 5 * T)).T[0:D]
        wrsum[...] = jnp.broadcast_to(jnp.sum(wr_row, axis=1, keepdims=True), wrsum.shape)

    mr = lax.broadcasted_iota(jnp.int32, (MROWS, T), 0)
    mc = lax.broadcasted_iota(jnp.int32, (MROWS, T), 1)
    for g in range(NG):
        ws = WIN * g
        m = jnp.zeros((MROWS, T), jnp.bool_)
        for i, h in enumerate(GROUPS[g]):
            lo = h * DH - ws
            cols = (mc >= lo) & (mc < lo + DH)
            rows = ((mr >= lo) & (mr < lo + DH) & (mr < T)) | (mr == T + i)
            m = m | (cols & rows)
        bmask[g] = jnp.where(m, 1.0, 0.0)
    macc[...] = jnp.zeros_like(macc)
    mb[...] = jnp.zeros_like(mb)
    best_v[...] = jnp.full(best_v.shape, -jnp.inf, f32)
    best_i[...] = jnp.zeros(best_i.shape, jnp.int32)

    ones_rows = jnp.ones((16, L), bf16)
    row32u = lax.broadcasted_iota(jnp.int32, (16, L), 0)

    def ln1(s):
        col0 = pl.multiple_of(s * L, L)
        xs = x_v[:, pl.ds(col0, L)].astype(f32)
        m = _colsum(xs) * (1.0 / D)
        v = jnp.maximum(_colsum(xs * xs) * (1.0 / D) - m * m, 0.0)
        arow[:, pl.ds(col0, L)] = jnp.broadcast_to(lax.rsqrt(v + EPS), (8, L))
        m_hi = (-m).astype(bf16).astype(f32)
        m_lo = -m - m_hi
        r16 = lax.broadcasted_iota(jnp.int32, (16, L), 0)
        rows = jnp.where(r16 >= 4, 0.0, jnp.where((r16 & 1) == 0, m_hi, m_lo))
        aug[:, pl.ds(col0, L)] = rows.astype(bf16)

    def finalize(s, t0, nt, attn):
        w = nt * T
        col0 = pl.multiple_of(s * L + t0 * T, T)
        hres = x_v[:, pl.ds(col0, w)].astype(f32) + attn
        hbuf[:, pl.ds(col0, w)] = hres
        a, b = _ln_stats(hres)
        wr = jnp.concatenate([wrtab[...]] * nt, axis=1)
        r = _colsum(hres * wr) * a + b * wrsum[0:1, 0:1]
        ab_all[0:8, pl.ds(col0, w)] = jnp.broadcast_to(a, (8, w))
        ab_all[8:16, pl.ds(col0, w)] = jnp.broadcast_to(b, (8, w))
        out_v[:, pl.ds(col0, w)] = (hbuf[:, pl.ds(col0, w)] * (1.0 + a) + b).astype(bf16)
        r = r.astype(bf16).astype(f32)
        bv, bi = best_v[0:1, :], best_i[0:1, :]
        for t in range(nt):
            rt = r[:, t * T:(t + 1) * T]
            better = rt > bv
            bi = jnp.where(better, col0 + t * T, bi)
            bv = jnp.where(better, rt, bv)
        best_i[...] = jnp.broadcast_to(bi, best_i.shape)
        best_v[...] = jnp.broadcast_to(bv, best_v.shape)

    def proj_rhs(s):
        col0 = pl.multiple_of(s * L, L)
        return jnp.concatenate([x_v[:, pl.ds(col0, L)], aug[:, pl.ds(col0, L)],
                                jnp.zeros((KP - D - 16, L), bf16)], axis=0)

    def ln_scale(s):
        return arow[0:1, pl.ds(pl.multiple_of(s * L, L), L)]

    def store_q(raw, a, r0, r1):
        qt[r0:r1, :] = (raw * (a * QSCALE)).astype(bf16)
        pqt[r0:r1, :] = _phi(raw * a).astype(bf16)

    def store_k_rows(raw, a, r0, r1):
        k = raw * a
        kt[r0:r1, :] = k.astype(bf16)
        pkt[r0:r1, :] = _phi(k).astype(bf16)

    def transpose_k():
        for g in range(NG):
            kp[g] = kt[WIN * g:WIN * g + T, :].T

    def store_k(raw, a):
        store_k_rows(raw, a, 0, D)
        transpose_k()

    def store_v(raw, a):
        vt[...] = (raw * a).astype(bf16)
        one32 = jnp.uint32(0x3F803F80)
        for h in range(H):
            vs = ((h * DH) // 16) * 16
            off2 = (h * DH - vs) // 2
            v32 = pltpu.bitcast(vt[vs:vs + 32, :], jnp.uint32)
            keep = (row32u >= off2) & (row32u < off2 + DH // 2)
            vh[h] = pltpu.bitcast(jnp.where(keep, v32, one32), bf16)

    def project(s):
        qkv = _dot(wt[...], proj_rhs(s))
        a = ln_scale(s)
        store_q(qkv[0:D], a, 0, D)
        store_k(qkv[D:2 * D], a)
        store_v(qkv[2 * D:3 * D], a)

    def mem_read():
        row128 = lax.broadcasted_iota(jnp.int32, (T, T), 0)
        row8 = lax.broadcasted_iota(jnp.int32, (8, T), 0)
        for g in range(NG):
            ws = WIN * g
            heads = GROUPS[g]
            lo_g, hi_g = heads[0] * DH - ws, (heads[-1] + 1) * DH - ws
            wmask = (row128 >= lo_g) & (row128 < hi_g)
            for j in range(NT):
                nd = _dot(mb[g], pqt[ws:ws + T, j * T:(j + 1) * T])
                rden = 1.0 / (nd[T:T + 8] + 1e-6)
                rb = [jnp.broadcast_to(rden[i:i + 1], (8, T)) for i in range(len(heads))]
                blocks = []
                for b in range(T // 8):
                    r_lo, r_hi = 8 * b, 8 * b + 7
                    i_lo = min(max((r_lo + ws) // DH - heads[0], 0), len(heads) - 1)
                    i_hi = min(max((r_hi + ws) // DH - heads[0], 0), len(heads) - 1)
                    if i_lo == i_hi:
                        blocks.append(rb[i_lo])
                    else:
                        cut = (heads[0] + i_hi) * DH - ws - r_lo
                        blocks.append(jnp.where(row8 < cut, rb[i_lo], rb[i_hi]))
                amv = nd[0:T] * jnp.concatenate(blocks, axis=0) * gtab[ws:ws + T, :]
                pltpu.store(am_v.at[ws:ws + T, j * T:(j + 1) * T], amv, mask=wmask)

    def attention(fast):
        ps = (p0, p1)
        if fast:
            _scores_fast(0, kp, qt, ps[0])
            for g in range(NG):
                if g + 1 < NG:
                    _scores_fast(g + 1, kp, qt, ps[(g + 1) % 2])
                _pv(g, vh, ps[g % 2], g1tab, am_v, ot)
        else:
            lax.fori_loop(0, H, lambda h, c: (_attention_safe(h, kp, qt, vh, g1tab, am_v, ot), c)[1], 0)

    def mem_update():
        for g in range(NG):
            ws = WIN * g
            lhs = jnp.concatenate([vt[ws:ws + T, :], ones_rows], axis=0)
            upd = macc[g] + _dot_nt(lhs, pkt[ws:ws + T, :])
            macc[g] = upd
            mb[g] = jnp.where(bmask[g] != 0.0, upd, 0.0).astype(bf16)

    def out_project():
        return _dot_tn(w_in[3], ot[...].astype(bf16))

    def load_weight(i):
        w = w_in[i]
        wf = w.astype(f32)
        c = jnp.sum(wf, axis=0, keepdims=True)
        c_hi = c.astype(bf16).astype(f32)
        r16 = lax.broadcasted_iota(jnp.int32, (16, D), 0)
        extra = jnp.where(r16 >= 4, 0.0, jnp.where(r16 < 2, c_hi, c - c_hi)).astype(bf16)
        w_aug = jnp.concatenate([w, extra, jnp.zeros((KP - D - 16, D), bf16)], axis=0)
        w_t = w_aug.T
        wt[i * D:(i + 1) * D, :] = w_t
        return w_t, jnp.max(jnp.sum(wf * wf, axis=0, keepdims=True))

    am_v[...] = jnp.zeros_like(am_v)
    with _scope("p_tables"):
        small_b.wait()
        small_r.wait()
        build_tables()
    with _scope("p_wq_wait"):
        w_copies[0].wait()
    w_copies[2].start()
    x_copy(1).start()
    w_copies[3].start()
    with _scope("p_wqT"):
        _, cq = load_weight(0)
    with _scope("p_x0_wait"):
        x_copy(0).wait()
    for s in range(2, NSEG):
        x_copy(s).start()
    for c in w_copies[4:]:
        c.start()
    HALF = 288
    with _scope("p_qlo"):
        ln1(0)
        store_q(_dot(wt[0:HALF, :], proj_rhs(0)), ln_scale(0), 0, HALF)
    with _scope("p_wk_wait"):
        w_copies[1].wait()
    with _scope("p_qhi_wkT_klo"):
        wk_t, ck = load_weight(1)
        store_q(_dot(wt[HALF:D, :], proj_rhs(0)), ln_scale(0), HALF, D)
        store_k_rows(_dot(wk_t[0:HALF], proj_rhs(0)), ln_scale(0), 0, HALF)
    with _scope("p_wv_wait"):
        w_copies[2].wait()
    with _scope("p_khi_wvT_v"):
        wv_t, cv = load_weight(2)
        store_k_rows(_dot(wt[D + HALF:2 * D, :], proj_rhs(0)), ln_scale(0), HALF, D)
        transpose_k()
        store_v(_dot(wv_t, proj_rhs(0)), ln_scale(0))
    slack = 1.05
    logit_bound2 = (cq * ck) * (slack * D * DH * QSCALE) ** 2
    v_bound2 = cv * (slack * D)
    safe = (logit_bound2 <= SAFE_LOGIT ** 2) & (v_bound2 <= SAFE_V ** 2)
    w_copies[3].wait()

    def body(s, carry):
        more = s + 1 < NSEG
        nxt = jnp.minimum(s + 1, NSEG - 1)

        @pl.when(more)
        def _():
            x_copy(nxt).wait()

        @pl.when(safe)
        def _():
            with _scope("attn"):
                attention(True)

        @pl.when(jnp.logical_not(safe))
        def _():
            attention(False)

        @pl.when(more)
        def _():
            with _scope("blockB"):
                hold = {}
                steps = {
                    "MU": mem_update,
                    "OP": lambda: hold.update(a=out_project()),
                    "LN1": lambda: ln1(nxt),
                    "PR": lambda: project(nxt),
                    "MR": mem_read,
                    "FIN": lambda: finalize(s, 0, NT, hold["a"]),
                }
                for n in _ORDER_B:
                    steps[n]()
            out_copy(s).start()
        return carry

    lax.fori_loop(0, NSEG, body, 0)
    with _scope("fin"):
        finalize(NSEG - 1, 0, NT, out_project())
        out_copy(NSEG - 1).start()

    bv = best_v[...]
    rmax = jnp.max(bv, axis=1, keepdims=True)
    cand = best_i[...] + lax.broadcasted_iota(jnp.int32, best_i.shape, 1)
    idx = jnp.clip(jnp.min(jnp.where(bv == rmax, cand, S)), 0, S - 1)
    base = pl.multiple_of((idx // T) * T, T)
    lane = idx - base
    blk = (hbuf[:, pl.ds(base, T)] * ab_all[0:1, pl.ds(base, T)]
           + ab_all[8:9, pl.ds(base, T)]).astype(bf16)
    pick = jnp.where(lax.broadcasted_iota(jnp.int32, (16, T), 1) == lane, 1.0, 0.0).astype(bf16)
    xg = _dot_nt(pick, blk).astype(bf16)
    for c in w_copies[4:]:
        c.wait()
    yacc = jnp.zeros((D, T), f32)
    FC = 4 * T
    for c in range(F // FC):
        gt = _dot(xg, wg_v[:, c * FC:(c + 1) * FC])
        up = _dot(xg, wu_v[:, c * FC:(c + 1) * FC])
        act = (gt * jax.nn.sigmoid(gt) * up)[0:1].astype(bf16).astype(f32)
        for t in range(FC // T):
            f0 = c * FC + t * T
            wd = jnp.concatenate([wd_v[r:r + 8, f0:f0 + T].astype(f32) for r in range(0, D, 8)], axis=0)
            yacc = yacc + wd * act[:, t * T:(t + 1) * T]
    y = jnp.sum(yacc, axis=1, keepdims=True) * jax.nn.sigmoid(rmax[0:1])
    for s in range(NSEG):
        out_copy(s).wait()
    sel = lax.broadcasted_iota(jnp.int32, (D, T), 1) == lane
    cur = out_v[:, pl.ds(base, T)].astype(f32)
    out_v[:, pl.ds(base, T)] = (cur + jnp.where(sel, y, 0.0)).astype(bf16)
    patch = pltpu.make_async_copy(out_v.at[:, pl.ds(base, T)],
                                  out_hbm.at[0, :, pl.ds(base, T)], sem_o.at[NSEG])
    patch.start()
    patch.wait()


@jax.jit
def pallas_sequential_preLN__memory_aug_infini_attn__moe_arch_mod__prompt_kernel(
    A_x: jax.Array,
    A_wq: jax.Array,
    A_wk: jax.Array,
    A_wv: jax.Array,
    A_wo: jax.Array,
    A_beta: jax.Array,
    B_x: jax.Array,
    B_w_r: jax.Array,
    B_w_gate: jax.Array,
    B_w_up: jax.Array,
    B_w_down: jax.Array,
):
    del B_x
    hbm_spec = pl.BlockSpec(memory_space=pltpu.HBM)
    scratch = [
        pltpu.VMEM((D, S), bf16),
        pltpu.VMEM((4, D, D), bf16),
        pltpu.VMEM((3 * D, KP), bf16),
        pltpu.VMEM((D, S), f32),
        pltpu.VMEM((D, F), bf16),
        pltpu.VMEM((D, F), bf16),
        pltpu.VMEM((D, F), bf16),
        pltpu.VMEM((16, S), bf16),
        pltpu.VMEM((8, S), f32),
        pltpu.VMEM((D, L), bf16),
        pltpu.VMEM((D, L), bf16),
        pltpu.VMEM((D, L), bf16),
        pltpu.VMEM((D, L), bf16),
        pltpu.VMEM((D, L), bf16),
        pltpu.VMEM((NG, L, T), bf16),
        pltpu.VMEM((H, 32, L), bf16),
        pltpu.VMEM((7, NT, L, T), bf16),
        pltpu.VMEM((7, NT, L, T), bf16),
        pltpu.VMEM((D, L), f32),
        pltpu.VMEM((D, L), f32),
        pltpu.VMEM((NG, MROWS, T), f32),
        pltpu.VMEM((NG, MROWS, T), bf16),
        pltpu.VMEM((NG, MROWS, T), f32),
        pltpu.VMEM((D, T), f32),
        pltpu.VMEM((H, 8, T), f32),
        pltpu.VMEM((D, T), f32),
        pltpu.VMEM((16, S), f32),
        pltpu.VMEM((D, S), bf16),
        pltpu.VMEM((8, T), f32),
        pltpu.VMEM((8, T), jnp.int32),
        pltpu.VMEM((8, T), f32),
        pltpu.VMEM((H,), bf16),
        pltpu.VMEM((D,), bf16),
        pltpu.SemaphoreType.DMA((NSEG,)),
        pltpu.SemaphoreType.DMA((9,)),
        pltpu.SemaphoreType.DMA((NSEG + 1,)),
    ]
    out_t = pl.pallas_call(
        _kernel,
        out_shape=jax.ShapeDtypeStruct((1, D, S), bf16),
        in_specs=[hbm_spec] * 10,
        out_specs=hbm_spec,
        scratch_shapes=scratch,
        compiler_params=pltpu.CompilerParams(vmem_limit_bytes=100 * 1024 * 1024),
    )(jnp.transpose(A_x, (0, 2, 1)), A_wq, A_wk, A_wv, A_wo, A_beta,
      B_w_r, B_w_gate, B_w_up, B_w_down.T)
    return jnp.transpose(out_t, (0, 2, 1))
```

```python
import contextlib

import jax
import jax.numpy as jnp
from jax import lax
import jax.experimental.pallas as pl
import jax.experimental.pallas.tpu as pltpu

S = 2048
D = 576
H = 32
DH = 18
NSEG = 4
L = 512
F = 4608
T = 128
NT = L // T
EPS = 1e-5
LOG2E = 1.4426950408889634
QSCALE = (DH ** -0.5) * LOG2E
WIN = 112
GROUPS = (tuple(range(0, 7)), tuple(range(7, 13)), tuple(range(13, 19)),
          tuple(range(19, 25)), tuple(range(25, 32)))
NG = len(GROUPS)
KP = 640
MROWS = T + 16
SAFE_LOGIT = 60.0
SAFE_V = 2.0 ** 40

bf16 = jnp.bfloat16
f32 = jnp.float32
_ORDER_B = ["MU", "OP", "LN1", "PR", "MR", "FIN"]
_PROFILE = False


def _scope(name):
    return jax.named_scope(name) if _PROFILE else contextlib.nullcontext()


def _colsum(x):
    n = x.shape[0] // 4
    parts = [jnp.sum(x[i * n:(i + 1) * n].reshape(n // 8, 8, x.shape[1]), axis=0) for i in range(4)]
    return jnp.sum((parts[0] + parts[1]) + (parts[2] + parts[3]), axis=0, keepdims=True)


def _ln_stats(x):
    m = _colsum(x) * (1.0 / D)
    v = jnp.maximum(_colsum(x * x) * (1.0 / D) - m * m, 0.0)
    a = lax.rsqrt(v + EPS)
    return a, -m * a


def _phi(t):
    return jnp.where(t > 0, t + 1.0, jnp.exp(t))


def _dot(a, b):
    return jnp.dot(a, b, preferred_element_type=f32)


def _dot_nt(a, b):
    return lax.dot_general(a, b, (((1,), (1,)), ((), ())), preferred_element_type=f32)


def _dot_tn(a, b):
    return lax.dot_general(a, b, (((0,), (0,)), ((), ())), preferred_element_type=f32)


def _swapped(g, u):
    return u % 2 == 1


def _masked_q(qt_ref, g, j):
    ws = WIN * g
    row64 = lax.broadcasted_iota(jnp.int32, (64, T), 0)
    qw32 = pltpu.bitcast(qt_ref[ws:ws + T, j * T:(j + 1) * T], jnp.uint32)
    qw32_sw = pltpu.roll(qw32, T // 2, axis=1)
    qms = []
    for u, h in enumerate(GROUPS[g]):
        lo2 = (h * DH - ws) // 2
        qmask = (row64 >= lo2) & (row64 < lo2 + DH // 2)
        src = qw32_sw if _swapped(g, u) else qw32
        qms.append(jnp.where(qmask, src, jnp.uint32(0)))
    return qms


def _causal_masks(nk, j):
    kk = lax.broadcasted_iota(jnp.int32, (nk, T), 0)
    qq = lax.broadcasted_iota(jnp.int32, (nk, T), 1)
    return kk <= qq + j * T, kk <= ((qq + T // 2) & (T - 1)) + j * T


def _scores_fast(g, kp_ref, qt_ref, p_ref):
    nh = len(GROUPS[g])
    causal = _causal_masks(T, 0)
    lane64 = lax.broadcasted_iota(jnp.int32, (64, T), 1)
    for j in range(NT):
        qms = _masked_q(qt_ref, g, j)
        qm = jnp.concatenate([pltpu.bitcast(q, bf16) for q in qms], axis=1)
        pairs = []
        for u in range(0, nh, 2):
            w = qms[u] if u + 1 == nh else jnp.where(lane64 < T // 2, qms[u + 1], qms[u])
            pairs.append(pltpu.bitcast(w, bf16))
        n1 = T * j + T // 2
        p1 = jnp.exp2(_dot(kp_ref[g, 0:n1, :], qm))
        p2 = jnp.exp2(_dot(kp_ref[g, n1:n1 + T // 2, :], jnp.concatenate(pairs, axis=1)))
        for u in range(nh):
            pu = p1[:, u * T:(u + 1) * T]
            if j > 0:
                p_ref[u, j, 0:j * T, :] = pu[0:j * T].astype(bf16)
            diag = jnp.concatenate(
                [pu[j * T:n1], p2[:, (u // 2) * T:(u // 2 + 1) * T]], axis=0)
            p_ref[u, j, j * T:(j + 1) * T, :] = jnp.where(
                causal[1 if _swapped(g, u) else 0], diag, 0.0).astype(bf16)


def _attention_safe(h, kp_ref, qt_ref, vt_ref, g1_ref, am_ref, ot_ref):
    g = jnp.minimum(jnp.maximum(h - 1, 0) // 6, NG - 1)
    ws = pl.multiple_of(g * WIN, 16)
    lo = h * DH - ws
    row128 = lax.broadcasted_iota(jnp.int32, (T, T), 0)
    qmask = (row128 >= lo) & (row128 < lo + DH)
    vs = pl.multiple_of(((h * DH) // 16) * 16, 16)
    off = h * DH - vs
    row32 = lax.broadcasted_iota(jnp.int32, (32, T), 0)
    omask = (row32 >= off) & (row32 < off + DH)
    kk = lax.broadcasted_iota(jnp.int32, (L, T), 0)
    qq = lax.broadcasted_iota(jnp.int32, (L, T), 1)

    def tile(j, c):
        c0 = pl.multiple_of(j * T, T)
        qm = jnp.where(qmask, qt_ref[pl.ds(ws, T), pl.ds(c0, T)].astype(f32), 0.0).astype(bf16)
        s = _dot(kp_ref[g], qm)
        s = jnp.where(kk <= qq + c0, s, -jnp.inf)
        m = jnp.max(s, axis=0, keepdims=True)
        p = jnp.exp2(s - m).astype(bf16)
        acc = _dot(_v_rows(vt_ref, vs, off // 2, L), p)
        l8 = jnp.where(off <= 6, acc[24:32], acc[0:8])
        rl = g1_ref[h] / l8
        o = acc * jnp.concatenate([rl] * 4, axis=0) + am_ref[pl.ds(vs, 32), pl.ds(c0, T)]
        pltpu.store(ot_ref.at[pl.ds(vs, 32), pl.ds(c0, T)], o, mask=omask)
        return c

    lax.fori_loop(0, NT, tile, 0)


def _v_rows(vt_ref, vs, off2, nk):
    row16 = lax.broadcasted_iota(jnp.int32, (16, nk), 0)
    keep = (row16 >= off2) & (row16 < off2 + DH // 2)
    v32 = pltpu.bitcast(vt_ref[pl.ds(vs, 32), 0:nk], jnp.uint32)
    return pltpu.bitcast(jnp.where(keep, v32, jnp.uint32(0x3F803F80)), bf16)


def _pv(g, vt_ref, p_ref, g1_ref, am_ref, ot_ref):
    row32 = lax.broadcasted_iota(jnp.int32, (32, T), 0)
    for u, h in enumerate(GROUPS[g]):
        vs = ((h * DH) // 16) * 16
        off = h * DH - vs
        omask = (row32 >= off) & (row32 < off + DH)
        g1 = g1_ref[h]
        vrows = _v_rows(vt_ref, vs, off // 2, L)
        for j in range(NT):
            nk = T * (j + 1)
            acc = _dot(vrows[:, 0:nk], p_ref[u, j, 0:nk, :])
            l8 = acc[24:32] if off <= 6 else acc[0:8]
            rl = g1 / l8
            o = acc * jnp.concatenate([rl] * 4, axis=0)
            if _swapped(g, u):
                o = pltpu.roll(o, T // 2, axis=1)
            o = o + am_ref[vs:vs + 32, j * T:(j + 1) * T]
            pltpu.store(ot_ref.at[vs:vs + 32, j * T:(j + 1) * T], o, mask=omask)


def _kernel(x_hbm, wq_hbm, wk_hbm, wv_hbm, wo_hbm, beta_hbm, wr_hbm, wg_hbm, wu_hbm, wd_hbm,
            out_hbm,
            x_v, w_in, wt, hbuf, wg_v, wu_v, wd_v,
            aug, arow, qt, pqt, kt, pkt, vt, kp, p0, p1, am_v, ot,
            macc, mb, bmask, gtab, g1tab, wrtab, ab_all, out_v, best_v, best_i, wrsum, beta_ref, wr_ref,
            sem_x, sem_w, sem_o):
    def x_copy(s):
        return pltpu.make_async_copy(x_hbm.at[0, :, pl.ds(s * L, L)],
                                     x_v.at[:, pl.ds(s * L, L)], sem_x.at[s])

    def out_copy(s):
        return pltpu.make_async_copy(out_v.at[:, pl.ds(s * L, L)],
                                     out_hbm.at[0, :, pl.ds(s * L, L)], sem_o.at[s])

    w_copies = [
        pltpu.make_async_copy(wq_hbm, w_in.at[0], sem_w.at[0]),
        pltpu.make_async_copy(wk_hbm, w_in.at[1], sem_w.at[1]),
        pltpu.make_async_copy(wv_hbm, w_in.at[2], sem_w.at[2]),
        pltpu.make_async_copy(wo_hbm, w_in.at[3], sem_w.at[3]),
        pltpu.make_async_copy(wg_hbm, wg_v, sem_w.at[4]),
        pltpu.make_async_copy(wu_hbm, wu_v, sem_w.at[5]),
        pltpu.make_async_copy(wd_hbm, wd_v, sem_w.at[6]),
    ]
    small_b = pltpu.make_async_copy(beta_hbm, beta_ref, sem_w.at[7])
    small_r = pltpu.make_async_copy(wr_hbm, wr_ref, sem_w.at[8])
    small_b.start()
    small_r.start()
    x_copy(0).start()
    w_copies[0].start()
    w_copies[1].start()

    def build_tables():
        gate = jax.nn.sigmoid(beta_ref[...].astype(f32).reshape(1, H))
        rr = lax.broadcasted_iota(jnp.int32, (D, H), 0)
        hh = lax.broadcasted_iota(jnp.int32, (D, H), 1)
        onehot = (rr >= hh * DH) & (rr < (hh + 1) * DH)
        gcol = jnp.sum(jnp.where(onehot, gate, 0.0), axis=1, keepdims=True)
        gtab[...] = jnp.broadcast_to(gcol, (D, T))
        hh8 = lax.broadcasted_iota(jnp.int32, (8, H), 1)
        for h in range(H):
            gh = jnp.sum(jnp.where(hh8 == h, gate, 0.0), axis=1, keepdims=True)
            g1tab[h] = jnp.broadcast_to(1.0 - gh, (8, T))
        wr_row = wr_ref[...].astype(f32).reshape(1, D)
        wr_pad = jnp.concatenate([wr_row, jnp.zeros((1, 5 * T - D), f32)], axis=1)
        wrtab[...] = jnp.broadcast_to(wr_pad, (T, 5 * T)).T[0:D]
        wrsum[...] = jnp.broadcast_to(jnp.sum(wr_row, axis=1, keepdims=True), wrsum.shape)

    mr = lax.broadcasted_iota(jnp.int32, (MROWS, T), 0)
    mc = lax.broadcasted_iota(jnp.int32, (MROWS, T), 1)
    for g in range(NG):
        ws = WIN * g
        m = jnp.zeros((MROWS, T), jnp.bool_)
        for i, h in enumerate(GROUPS[g]):
            lo = h * DH - ws
            cols = (mc >= lo) & (mc < lo + DH)
            rows = ((mr >= lo) & (mr < lo + DH) & (mr < T)) | (mr == T + i)
            m = m | (cols & rows)
        bmask[g] = jnp.where(m, 1.0, 0.0)
    macc[...] = jnp.zeros_like(macc)
    mb[...] = jnp.zeros_like(mb)
    best_v[...] = jnp.full(best_v.shape, -jnp.inf, f32)
    best_i[...] = jnp.zeros(best_i.shape, jnp.int32)

    ones_rows = jnp.ones((16, L), bf16)

    def ln1(s):
        col0 = pl.multiple_of(s * L, L)
        xs = x_v[:, pl.ds(col0, L)].astype(f32)
        m = _colsum(xs) * (1.0 / D)
        v = jnp.maximum(_colsum(xs * xs) * (1.0 / D) - m * m, 0.0)
        arow[:, pl.ds(col0, L)] = jnp.broadcast_to(lax.rsqrt(v + EPS), (8, L))
        m_hi = (-m).astype(bf16).astype(f32)
        m_lo = -m - m_hi
        r16 = lax.broadcasted_iota(jnp.int32, (16, L), 0)
        rows = jnp.where(r16 >= 4, 0.0, jnp.where((r16 & 1) == 0, m_hi, m_lo))
        aug[:, pl.ds(col0, L)] = rows.astype(bf16)

    def finalize(s, t0, nt, attn):
        w = nt * T
        col0 = pl.multiple_of(s * L + t0 * T, T)
        hres = x_v[:, pl.ds(col0, w)].astype(f32) + attn
        hbuf[:, pl.ds(col0, w)] = hres
        a, b = _ln_stats(hres)
        wr = jnp.concatenate([wrtab[...]] * nt, axis=1)
        r = _colsum(hres * wr) * a + b * wrsum[0:1, 0:1]
        ab_all[0:8, pl.ds(col0, w)] = jnp.broadcast_to(a, (8, w))
        ab_all[8:16, pl.ds(col0, w)] = jnp.broadcast_to(b, (8, w))
        out_v[:, pl.ds(col0, w)] = (hbuf[:, pl.ds(col0, w)] * (1.0 + a) + b).astype(bf16)
        r = r.astype(bf16).astype(f32)
        bv, bi = best_v[0:1, :], best_i[0:1, :]
        for t in range(nt):
            rt = r[:, t * T:(t + 1) * T]
            better = rt > bv
            bi = jnp.where(better, col0 + t * T, bi)
            bv = jnp.where(better, rt, bv)
        best_i[...] = jnp.broadcast_to(bi, best_i.shape)
        best_v[...] = jnp.broadcast_to(bv, best_v.shape)

    def proj_rhs(s):
        col0 = pl.multiple_of(s * L, L)
        return jnp.concatenate([x_v[:, pl.ds(col0, L)], aug[:, pl.ds(col0, L)],
                                jnp.zeros((KP - D - 16, L), bf16)], axis=0)

    def ln_scale(s):
        return arow[0:1, pl.ds(pl.multiple_of(s * L, L), L)]

    def store_q(raw, a, r0, r1):
        qt[r0:r1, :] = (raw * (a * QSCALE)).astype(bf16)
        pqt[r0:r1, :] = _phi(raw * a).astype(bf16)

    def store_k_rows(raw, a, r0, r1):
        k = raw * a
        kt[r0:r1, :] = k.astype(bf16)
        pkt[r0:r1, :] = _phi(k).astype(bf16)

    def transpose_k():
        for g in range(NG):
            kp[g] = kt[WIN * g:WIN * g + T, :].T

    def store_k(raw, a):
        k = raw * a
        kb = k.astype(bf16)
        pkt[...] = _phi(k).astype(bf16)
        for g in range(NG):
            kp[g] = kb[WIN * g:WIN * g + T, :].T

    def store_v(raw, a):
        vt[...] = (raw * a).astype(bf16)

    def project(s):
        qkv = _dot(wt[...], proj_rhs(s))
        a = ln_scale(s)
        store_q(qkv[0:D], a, 0, D)
        store_k(qkv[D:2 * D], a)
        store_v(qkv[2 * D:3 * D], a)

    def mem_read():
        row128 = lax.broadcasted_iota(jnp.int32, (T, T), 0)
        row8 = lax.broadcasted_iota(jnp.int32, (8, T), 0)
        for g in range(NG):
            ws = WIN * g
            heads = GROUPS[g]
            lo_g, hi_g = heads[0] * DH - ws, (heads[-1] + 1) * DH - ws
            wmask = (row128 >= lo_g) & (row128 < hi_g)
            for j in range(NT):
                nd = _dot(mb[g], pqt[ws:ws + T, j * T:(j + 1) * T])
                rden = 1.0 / (nd[T:T + 8] + 1e-6)
                rb = [jnp.broadcast_to(rden[i:i + 1], (8, T)) for i in range(len(heads))]
                blocks = []
                for b in range(T // 8):
                    r_lo, r_hi = 8 * b, 8 * b + 7
                    i_lo = min(max((r_lo + ws) // DH - heads[0], 0), len(heads) - 1)
                    i_hi = min(max((r_hi + ws) // DH - heads[0], 0), len(heads) - 1)
                    if i_lo == i_hi:
                        blocks.append(rb[i_lo])
                    else:
                        cut = (heads[0] + i_hi) * DH - ws - r_lo
                        blocks.append(jnp.where(row8 < cut, rb[i_lo], rb[i_hi]))
                amv = nd[0:T] * jnp.concatenate(blocks, axis=0) * gtab[ws:ws + T, :]
                pltpu.store(am_v.at[ws:ws + T, j * T:(j + 1) * T], amv, mask=wmask)

    def attention(fast):
        ps = (p0, p1)
        if fast:
            _scores_fast(0, kp, qt, ps[0])
            for g in range(NG):
                if g + 1 < NG:
                    _scores_fast(g + 1, kp, qt, ps[(g + 1) % 2])
                _pv(g, vt, ps[g % 2], g1tab, am_v, ot)
        else:
            lax.fori_loop(0, H, lambda h, c: (_attention_safe(h, kp, qt, vt, g1tab, am_v, ot), c)[1], 0)

    def mem_update():
        for g in range(NG):
            ws = WIN * g
            lhs = jnp.concatenate([vt[ws:ws + T, :], ones_rows], axis=0)
            upd = macc[g] + _dot_nt(lhs, pkt[ws:ws + T, :])
            macc[g] = upd
            mb[g] = jnp.where(bmask[g] != 0.0, upd, 0.0).astype(bf16)

    def out_project():
        return _dot_tn(w_in[3], ot[...].astype(bf16))

    def load_weight(i):
        w = w_in[i]
        wf = w.astype(f32)
        c = jnp.sum(wf, axis=0, keepdims=True)
        c_hi = c.astype(bf16).astype(f32)
        r16 = lax.broadcasted_iota(jnp.int32, (16, D), 0)
        extra = jnp.where(r16 >= 4, 0.0, jnp.where(r16 < 2, c_hi, c - c_hi)).astype(bf16)
        w_aug = jnp.concatenate([w, extra, jnp.zeros((KP - D - 16, D), bf16)], axis=0)
        w_t = w_aug.T
        wt[i * D:(i + 1) * D, :] = w_t
        return w_t, jnp.max(jnp.sum(wf * wf, axis=0, keepdims=True))

    am_v[...] = jnp.zeros_like(am_v)
    with _scope("p_tables"):
        small_b.wait()
        small_r.wait()
        build_tables()
    with _scope("p_wq_wait"):
        w_copies[0].wait()
    w_copies[2].start()
    x_copy(1).start()
    w_copies[3].start()
    with _scope("p_wqT"):
        _, cq = load_weight(0)
    with _scope("p_x0_wait"):
        x_copy(0).wait()
    for s in range(2, NSEG):
        x_copy(s).start()
    for c in w_copies[4:]:
        c.start()
    HALF = 288
    with _scope("p_qlo"):
        ln1(0)
        store_q(_dot(wt[0:HALF, :], proj_rhs(0)), ln_scale(0), 0, HALF)
    with _scope("p_wk_wait"):
        w_copies[1].wait()
    with _scope("p_qhi_wkT_klo"):
        wk_t, ck = load_weight(1)
        store_q(_dot(wt[HALF:D, :], proj_rhs(0)), ln_scale(0), HALF, D)
        store_k_rows(_dot(wk_t[0:HALF], proj_rhs(0)), ln_scale(0), 0, HALF)
    with _scope("p_wv_wait"):
        w_copies[2].wait()
    with _scope("p_khi_wvT_v"):
        wv_t, cv = load_weight(2)
        store_k_rows(_dot(wt[D + HALF:2 * D, :], proj_rhs(0)), ln_scale(0), HALF, D)
        transpose_k()
        store_v(_dot(wv_t, proj_rhs(0)), ln_scale(0))
    slack = 1.05
    logit_bound2 = (cq * ck) * (slack * D * DH * QSCALE) ** 2
    v_bound2 = cv * (slack * D)
    safe = (logit_bound2 <= SAFE_LOGIT ** 2) & (v_bound2 <= SAFE_V ** 2)
    w_copies[3].wait()

    def body(s, carry):
        more = s + 1 < NSEG
        nxt = jnp.minimum(s + 1, NSEG - 1)

        @pl.when(more)
        def _():
            x_copy(nxt).wait()

        @pl.when(safe)
        def _():
            with _scope("attn"):
                attention(True)

        @pl.when(jnp.logical_not(safe))
        def _():
            attention(False)

        @pl.when(more)
        def _():
            with _scope("blockB"):
                hold = {}
                steps = {
                    "MU": mem_update,
                    "OP": lambda: hold.update(a=out_project()),
                    "LN1": lambda: ln1(nxt),
                    "PR": lambda: project(nxt),
                    "MR": mem_read,
                    "FIN": lambda: finalize(s, 0, NT, hold["a"]),
                }
                for n in _ORDER_B:
                    steps[n]()
            out_copy(s).start()
        return carry

    lax.fori_loop(0, NSEG, body, 0)
    with _scope("fin"):
        finalize(NSEG - 1, 0, NT, out_project())
        out_copy(NSEG - 1).start()

    bv = best_v[...]
    rmax = jnp.max(bv, axis=1, keepdims=True)
    cand = best_i[...] + lax.broadcasted_iota(jnp.int32, best_i.shape, 1)
    idx = jnp.clip(jnp.min(jnp.where(bv == rmax, cand, S)), 0, S - 1)
    base = pl.multiple_of((idx // T) * T, T)
    lane = idx - base
    blk = (hbuf[:, pl.ds(base, T)] * ab_all[0:1, pl.ds(base, T)]
           + ab_all[8:9, pl.ds(base, T)]).astype(bf16)
    pick = jnp.where(lax.broadcasted_iota(jnp.int32, (16, T), 1) == lane, 1.0, 0.0).astype(bf16)
    xg = _dot_nt(pick, blk).astype(bf16)
    for c in w_copies[4:]:
        c.wait()
    yacc = jnp.zeros((D, T), f32)
    FC = 4 * T
    for c in range(F // FC):
        gt = _dot(xg, wg_v[:, c * FC:(c + 1) * FC])
        up = _dot(xg, wu_v[:, c * FC:(c + 1) * FC])
        act = (gt * jax.nn.sigmoid(gt) * up)[0:1].astype(bf16).astype(f32)
        for t in range(FC // T):
            f0 = c * FC + t * T
            wd = jnp.concatenate([wd_v[r:r + 8, f0:f0 + T].astype(f32) for r in range(0, D, 8)], axis=0)
            yacc = yacc + wd * act[:, t * T:(t + 1) * T]
    y = jnp.sum(yacc, axis=1, keepdims=True) * jax.nn.sigmoid(rmax[0:1])
    for s in range(NSEG):
        out_copy(s).wait()
    sel = lax.broadcasted_iota(jnp.int32, (D, T), 1) == lane
    cur = out_v[:, pl.ds(base, T)].astype(f32)
    out_v[:, pl.ds(base, T)] = (cur + jnp.where(sel, y, 0.0)).astype(bf16)
    patch = pltpu.make_async_copy(out_v.at[:, pl.ds(base, T)],
                                  out_hbm.at[0, :, pl.ds(base, T)], sem_o.at[NSEG])
    patch.start()
    patch.wait()


@jax.jit
def pallas_sequential_preLN__memory_aug_infini_attn__moe_arch_mod__prompt_kernel(
    A_x: jax.Array,
    A_wq: jax.Array,
    A_wk: jax.Array,
    A_wv: jax.Array,
    A_wo: jax.Array,
    A_beta: jax.Array,
    B_x: jax.Array,
    B_w_r: jax.Array,
    B_w_gate: jax.Array,
    B_w_up: jax.Array,
    B_w_down: jax.Array,
):
    del B_x
    hbm_spec = pl.BlockSpec(memory_space=pltpu.HBM)
    scratch = [
        pltpu.VMEM((D, S), bf16),
        pltpu.VMEM((4, D, D), bf16),
        pltpu.VMEM((3 * D, KP), bf16),
        pltpu.VMEM((D, S), f32),
        pltpu.VMEM((D, F), bf16),
        pltpu.VMEM((D, F), bf16),
        pltpu.VMEM((D, F), bf16),
        pltpu.VMEM((16, S), bf16),
        pltpu.VMEM((8, S), f32),
        pltpu.VMEM((D, L), bf16),
        pltpu.VMEM((D, L), bf16),
        pltpu.VMEM((D, L), bf16),
        pltpu.VMEM((D, L), bf16),
        pltpu.VMEM((D, L), bf16),
        pltpu.VMEM((NG, L, T), bf16),
        pltpu.VMEM((7, NT, L, T), bf16),
        pltpu.VMEM((7, NT, L, T), bf16),
        pltpu.VMEM((D, L), f32),
        pltpu.VMEM((D, L), f32),
        pltpu.VMEM((NG, MROWS, T), f32),
        pltpu.VMEM((NG, MROWS, T), bf16),
        pltpu.VMEM((NG, MROWS, T), f32),
        pltpu.VMEM((D, T), f32),
        pltpu.VMEM((H, 8, T), f32),
        pltpu.VMEM((D, T), f32),
        pltpu.VMEM((16, S), f32),
        pltpu.VMEM((D, S), bf16),
        pltpu.VMEM((8, T), f32),
        pltpu.VMEM((8, T), jnp.int32),
        pltpu.VMEM((8, T), f32),
        pltpu.VMEM((H,), bf16),
        pltpu.VMEM((D,), bf16),
        pltpu.SemaphoreType.DMA((NSEG,)),
        pltpu.SemaphoreType.DMA((9,)),
        pltpu.SemaphoreType.DMA((NSEG + 1,)),
    ]
    out_t = pl.pallas_call(
        _kernel,
        out_shape=jax.ShapeDtypeStruct((1, D, S), bf16),
        in_specs=[hbm_spec] * 10,
        out_specs=hbm_spec,
        scratch_shapes=scratch,
        compiler_params=pltpu.CompilerParams(vmem_limit_bytes=100 * 1024 * 1024),
    )(jnp.transpose(A_x, (0, 2, 1)), A_wq, A_wk, A_wv, A_wo, A_beta,
      B_w_r, B_w_gate, B_w_up, B_w_down.T)
    return jnp.transpose(out_t, (0, 2, 1))
```

```python
import contextlib

import jax
import jax.numpy as jnp
from jax import lax
import jax.experimental.pallas as pl
import jax.experimental.pallas.tpu as pltpu

S = 2048
D = 576
H = 32
DH = 18
NSEG = 4
L = 512
F = 4608
T = 128
NT = L // T
EPS = 1e-5
LOG2E = 1.4426950408889634
QSCALE = (DH ** -0.5) * LOG2E
WIN = 112
GROUPS = (tuple(range(0, 7)), tuple(range(7, 13)), tuple(range(13, 19)),
          tuple(range(19, 25)), tuple(range(25, 32)))
NG = len(GROUPS)
KP = 640
MROWS = T + 16
SAFE_LOGIT = 60.0
SAFE_V = 2.0 ** 40

bf16 = jnp.bfloat16
f32 = jnp.float32
_ORDER_B = ["MU", "OP", "LN1", "PR", "MR", "FIN"]
_PROFILE = False


def _scope(name):
    return jax.named_scope(name) if _PROFILE else contextlib.nullcontext()


def _colsum(x):
    n = x.shape[0] // 4
    parts = [jnp.sum(x[i * n:(i + 1) * n].reshape(n // 8, 8, x.shape[1]), axis=0) for i in range(4)]
    return jnp.sum((parts[0] + parts[1]) + (parts[2] + parts[3]), axis=0, keepdims=True)


def _ln_stats(x):
    m = _colsum(x) * (1.0 / D)
    v = jnp.maximum(_colsum(x * x) * (1.0 / D) - m * m, 0.0)
    a = lax.rsqrt(v + EPS)
    return a, -m * a


def _phi(t):
    return jnp.where(t > 0, t + 1.0, jnp.exp(t))


def _dot(a, b):
    return jnp.dot(a, b, preferred_element_type=f32)


def _dot_nt(a, b):
    return lax.dot_general(a, b, (((1,), (1,)), ((), ())), preferred_element_type=f32)


def _dot_tn(a, b):
    return lax.dot_general(a, b, (((0,), (0,)), ((), ())), preferred_element_type=f32)


def _swapped(g, u):
    return u % 2 == 1


def _masked_q(qt_ref, g, j):
    ws = WIN * g
    row64 = lax.broadcasted_iota(jnp.int32, (64, T), 0)
    qw32 = pltpu.bitcast(qt_ref[ws:ws + T, j * T:(j + 1) * T], jnp.uint32)
    qw32_sw = pltpu.roll(qw32, T // 2, axis=1)
    qms = []
    for u, h in enumerate(GROUPS[g]):
        lo2 = (h * DH - ws) // 2
        qmask = (row64 >= lo2) & (row64 < lo2 + DH // 2)
        src = qw32_sw if _swapped(g, u) else qw32
        qms.append(jnp.where(qmask, src, jnp.uint32(0)))
    return qms


def _causal_masks(nk, j):
    kk = lax.broadcasted_iota(jnp.int32, (nk, T), 0)
    qq = lax.broadcasted_iota(jnp.int32, (nk, T), 1)
    return kk <= qq + j * T, kk <= ((qq + T // 2) & (T - 1)) + j * T


def _scores_fast(g, kp_ref, qt_ref, p_ref):
    nh = len(GROUPS[g])
    causal = _causal_masks(T, 0)
    lane64 = lax.broadcasted_iota(jnp.int32, (64, T), 1)
    for j in range(NT):
        qms = _masked_q(qt_ref, g, j)
        qm = jnp.concatenate([pltpu.bitcast(q, bf16) for q in qms], axis=1)
        pairs = []
        for u in range(0, nh, 2):
            w = qms[u] if u + 1 == nh else jnp.where(lane64 < T // 2, qms[u + 1], qms[u])
            pairs.append(pltpu.bitcast(w, bf16))
        n1 = T * j + T // 2
        p1 = jnp.exp2(_dot(kp_ref[g, 0:n1, :], qm))
        p2 = jnp.exp2(_dot(kp_ref[g, n1:n1 + T // 2, :], jnp.concatenate(pairs, axis=1)))
        for u in range(nh):
            pu = p1[:, u * T:(u + 1) * T]
            if j > 0:
                p_ref[u, j, 0:j * T, :] = pu[0:j * T].astype(bf16)
            diag = jnp.concatenate(
                [pu[j * T:n1], p2[:, (u // 2) * T:(u // 2 + 1) * T]], axis=0)
            p_ref[u, j, j * T:(j + 1) * T, :] = jnp.where(
                causal[1 if _swapped(g, u) else 0], diag, 0.0).astype(bf16)


def _attention_safe(h, kp_ref, qt_ref, vt_ref, g1_ref, am_ref, ot_ref):
    g = jnp.minimum(jnp.maximum(h - 1, 0) // 6, NG - 1)
    ws = pl.multiple_of(g * WIN, 16)
    lo = h * DH - ws
    row128 = lax.broadcasted_iota(jnp.int32, (T, T), 0)
    qmask = (row128 >= lo) & (row128 < lo + DH)
    vs = pl.multiple_of(((h * DH) // 16) * 16, 16)
    off = h * DH - vs
    row32 = lax.broadcasted_iota(jnp.int32, (32, T), 0)
    omask = (row32 >= off) & (row32 < off + DH)
    kk = lax.broadcasted_iota(jnp.int32, (L, T), 0)
    qq = lax.broadcasted_iota(jnp.int32, (L, T), 1)

    def tile(j, c):
        c0 = pl.multiple_of(j * T, T)
        qm = jnp.where(qmask, qt_ref[pl.ds(ws, T), pl.ds(c0, T)].astype(f32), 0.0).astype(bf16)
        s = _dot(kp_ref[g], qm)
        s = jnp.where(kk <= qq + c0, s, -jnp.inf)
        m = jnp.max(s, axis=0, keepdims=True)
        p = jnp.exp2(s - m).astype(bf16)
        acc = _dot(_v_rows(vt_ref, vs, off // 2, L), p)
        l8 = jnp.where(off <= 6, acc[24:32], acc[0:8])
        rl = g1_ref[h] / l8
        o = acc * jnp.concatenate([rl] * 4, axis=0) + am_ref[pl.ds(vs, 32), pl.ds(c0, T)]
        pltpu.store(ot_ref.at[pl.ds(vs, 32), pl.ds(c0, T)], o, mask=omask)
        return c

    lax.fori_loop(0, NT, tile, 0)


def _v_rows(vt_ref, vs, off2, nk):
    row16 = lax.broadcasted_iota(jnp.int32, (16, nk), 0)
    keep = (row16 >= off2) & (row16 < off2 + DH // 2)
    v32 = pltpu.bitcast(vt_ref[pl.ds(vs, 32), 0:nk], jnp.uint32)
    return pltpu.bitcast(jnp.where(keep, v32, jnp.uint32(0x3F803F80)), bf16)


def _pv(g, vt_ref, p_ref, g1_ref, am_ref, ot_ref):
    row32 = lax.broadcasted_iota(jnp.int32, (32, T), 0)
    for u, h in enumerate(GROUPS[g]):
        vs = ((h * DH) // 16) * 16
        off = h * DH - vs
        omask = (row32 >= off) & (row32 < off + DH)
        g1 = g1_ref[h]
        vrows = _v_rows(vt_ref, vs, off // 2, L)
        for j in range(NT):
            nk = T * (j + 1)
            acc = _dot(vrows[:, 0:nk], p_ref[u, j, 0:nk, :])
            l8 = acc[24:32] if off <= 6 else acc[0:8]
            rl = g1 / l8
            o = acc * jnp.concatenate([rl] * 4, axis=0)
            if _swapped(g, u):
                o = pltpu.roll(o, T // 2, axis=1)
            o = o + am_ref[vs:vs + 32, j * T:(j + 1) * T]
            pltpu.store(ot_ref.at[vs:vs + 32, j * T:(j + 1) * T], o, mask=omask)


def _kernel(x_hbm, wq_hbm, wk_hbm, wv_hbm, wo_hbm, beta_hbm, wr_hbm, wg_hbm, wu_hbm, wd_hbm,
            out_hbm,
            x_v, w_in, wt, hbuf, wg_v, wu_v, wd_v,
            aug, arow, qt, pqt, kt, pkt, vt, kp, p0, p1, am_v, ot,
            macc, mb, bmask, gtab, g1tab, wrtab, ab_all, out_v, best_v, best_i, wrsum, beta_ref, wr_ref,
            sem_x, sem_w, sem_o):
    def x_copy(s):
        return pltpu.make_async_copy(x_hbm.at[0, :, pl.ds(s * L, L)],
                                     x_v.at[:, pl.ds(s * L, L)], sem_x.at[s])

    def out_copy(s):
        return pltpu.make_async_copy(out_v.at[:, pl.ds(s * L, L)],
                                     out_hbm.at[0, :, pl.ds(s * L, L)], sem_o.at[s])

    w_copies = [
        pltpu.make_async_copy(wq_hbm, w_in.at[0], sem_w.at[0]),
        pltpu.make_async_copy(wk_hbm, w_in.at[1], sem_w.at[1]),
        pltpu.make_async_copy(wv_hbm, w_in.at[2], sem_w.at[2]),
        pltpu.make_async_copy(wo_hbm, w_in.at[3], sem_w.at[3]),
        pltpu.make_async_copy(wg_hbm, wg_v, sem_w.at[4]),
        pltpu.make_async_copy(wu_hbm, wu_v, sem_w.at[5]),
        pltpu.make_async_copy(wd_hbm, wd_v, sem_w.at[6]),
    ]
    small_b = pltpu.make_async_copy(beta_hbm, beta_ref, sem_w.at[7])
    small_r = pltpu.make_async_copy(wr_hbm, wr_ref, sem_w.at[8])
    small_b.start()
    small_r.start()
    x_copy(0).start()
    w_copies[0].start()
    w_copies[1].start()

    def build_tables():
        gate = jax.nn.sigmoid(beta_ref[...].astype(f32).reshape(1, H))
        rr = lax.broadcasted_iota(jnp.int32, (D, H), 0)
        hh = lax.broadcasted_iota(jnp.int32, (D, H), 1)
        onehot = (rr >= hh * DH) & (rr < (hh + 1) * DH)
        gcol = jnp.sum(jnp.where(onehot, gate, 0.0), axis=1, keepdims=True)
        gtab[...] = jnp.broadcast_to(gcol, (D, T))
        hh8 = lax.broadcasted_iota(jnp.int32, (8, H), 1)
        for h in range(H):
            gh = jnp.sum(jnp.where(hh8 == h, gate, 0.0), axis=1, keepdims=True)
            g1tab[h] = jnp.broadcast_to(1.0 - gh, (8, T))
        wr_row = wr_ref[...].astype(f32).reshape(1, D)
        wr_pad = jnp.concatenate([wr_row, jnp.zeros((1, 5 * T - D), f32)], axis=1)
        wrtab[...] = jnp.broadcast_to(wr_pad, (T, 5 * T)).T[0:D]
        wrsum[...] = jnp.broadcast_to(jnp.sum(wr_row, axis=1, keepdims=True), wrsum.shape)

    mr = lax.broadcasted_iota(jnp.int32, (MROWS, T), 0)
    mc = lax.broadcasted_iota(jnp.int32, (MROWS, T), 1)
    for g in range(NG):
        ws = WIN * g
        m = jnp.zeros((MROWS, T), jnp.bool_)
        for i, h in enumerate(GROUPS[g]):
            lo = h * DH - ws
            cols = (mc >= lo) & (mc < lo + DH)
            rows = ((mr >= lo) & (mr < lo + DH) & (mr < T)) | (mr == T + i)
            m = m | (cols & rows)
        bmask[g] = jnp.where(m, 1.0, 0.0)
    macc[...] = jnp.zeros_like(macc)
    mb[...] = jnp.zeros_like(mb)
    best_v[...] = jnp.full(best_v.shape, -jnp.inf, f32)
    best_i[...] = jnp.zeros(best_i.shape, jnp.int32)

    ones_rows = jnp.ones((16, L), bf16)

    def ln1(s):
        col0 = pl.multiple_of(s * L, L)
        xs = x_v[:, pl.ds(col0, L)].astype(f32)
        m = _colsum(xs) * (1.0 / D)
        v = jnp.maximum(_colsum(xs * xs) * (1.0 / D) - m * m, 0.0)
        arow[:, pl.ds(col0, L)] = jnp.broadcast_to(lax.rsqrt(v + EPS), (8, L))
        m_hi = (-m).astype(bf16).astype(f32)
        m_lo = -m - m_hi
        r16 = lax.broadcasted_iota(jnp.int32, (16, L), 0)
        rows = jnp.where(r16 >= 4, 0.0, jnp.where((r16 & 1) == 0, m_hi, m_lo))
        aug[:, pl.ds(col0, L)] = rows.astype(bf16)

    def finalize(s, t0, nt, attn):
        w = nt * T
        col0 = pl.multiple_of(s * L + t0 * T, T)
        hres = x_v[:, pl.ds(col0, w)].astype(f32) + attn
        hbuf[:, pl.ds(col0, w)] = hres
        a, b = _ln_stats(hres)
        wr = jnp.concatenate([wrtab[...]] * nt, axis=1)
        r = _colsum(hres * wr) * a + b * wrsum[0:1, 0:1]
        ab_all[0:8, pl.ds(col0, w)] = jnp.broadcast_to(a, (8, w))
        ab_all[8:16, pl.ds(col0, w)] = jnp.broadcast_to(b, (8, w))
        out_v[:, pl.ds(col0, w)] = (hbuf[:, pl.ds(col0, w)] * (1.0 + a) + b).astype(bf16)
        r = r.astype(bf16).astype(f32)
        bv, bi = best_v[0:1, :], best_i[0:1, :]
        for t in range(nt):
            rt = r[:, t * T:(t + 1) * T]
            better = rt > bv
            bi = jnp.where(better, col0 + t * T, bi)
            bv = jnp.where(better, rt, bv)
        best_i[...] = jnp.broadcast_to(bi, best_i.shape)
        best_v[...] = jnp.broadcast_to(bv, best_v.shape)

    def proj_rhs(s):
        col0 = pl.multiple_of(s * L, L)
        return jnp.concatenate([x_v[:, pl.ds(col0, L)], aug[:, pl.ds(col0, L)],
                                jnp.zeros((KP - D - 16, L), bf16)], axis=0)

    def ln_scale(s):
        return arow[0:1, pl.ds(pl.multiple_of(s * L, L), L)]

    def store_q(raw, a, r0, r1, with_phi=True):
        qt[r0:r1, :] = (raw * (a * QSCALE)).astype(bf16)
        if with_phi:
            pqt[r0:r1, :] = _phi(raw * a).astype(bf16)

    def store_k_rows(raw, a, r0, r1):
        k = raw * a
        kt[r0:r1, :] = k.astype(bf16)
        pkt[r0:r1, :] = _phi(k).astype(bf16)

    def transpose_k():
        for g in range(NG):
            kp[g] = kt[WIN * g:WIN * g + T, :].T

    def store_k(raw, a):
        k = raw * a
        kb = k.astype(bf16)
        pkt[...] = _phi(k).astype(bf16)
        for g in range(NG):
            kp[g] = kb[WIN * g:WIN * g + T, :].T

    def store_v(raw, a):
        vt[...] = (raw * a).astype(bf16)

    def project(s):
        qkv = _dot(wt[...], proj_rhs(s))
        a = ln_scale(s)
        store_q(qkv[0:D], a, 0, D)
        store_k(qkv[D:2 * D], a)
        store_v(qkv[2 * D:3 * D], a)

    def mem_read():
        row128 = lax.broadcasted_iota(jnp.int32, (T, T), 0)
        row8 = lax.broadcasted_iota(jnp.int32, (8, T), 0)
        for g in range(NG):
            ws = WIN * g
            heads = GROUPS[g]
            lo_g, hi_g = heads[0] * DH - ws, (heads[-1] + 1) * DH - ws
            wmask = (row128 >= lo_g) & (row128 < hi_g)
            for j in range(NT):
                nd = _dot(mb[g], pqt[ws:ws + T, j * T:(j + 1) * T])
                rden = 1.0 / (nd[T:T + 8] + 1e-6)
                rb = [jnp.broadcast_to(rden[i:i + 1], (8, T)) for i in range(len(heads))]
                blocks = []
                for b in range(T // 8):
                    r_lo, r_hi = 8 * b, 8 * b + 7
                    i_lo = min(max((r_lo + ws) // DH - heads[0], 0), len(heads) - 1)
                    i_hi = min(max((r_hi + ws) // DH - heads[0], 0), len(heads) - 1)
                    if i_lo == i_hi:
                        blocks.append(rb[i_lo])
                    else:
                        cut = (heads[0] + i_hi) * DH - ws - r_lo
                        blocks.append(jnp.where(row8 < cut, rb[i_lo], rb[i_hi]))
                amv = nd[0:T] * jnp.concatenate(blocks, axis=0) * gtab[ws:ws + T, :]
                pltpu.store(am_v.at[ws:ws + T, j * T:(j + 1) * T], amv, mask=wmask)

    def attention(fast):
        ps = (p0, p1)
        if fast:
            _scores_fast(0, kp, qt, ps[0])
            for g in range(NG):
                if g + 1 < NG:
                    _scores_fast(g + 1, kp, qt, ps[(g + 1) % 2])
                _pv(g, vt, ps[g % 2], g1tab, am_v, ot)
        else:
            lax.fori_loop(0, H, lambda h, c: (_attention_safe(h, kp, qt, vt, g1tab, am_v, ot), c)[1], 0)

    def mem_update():
        for g in range(NG):
            ws = WIN * g
            lhs = jnp.concatenate([vt[ws:ws + T, :], ones_rows], axis=0)
            upd = macc[g] + _dot_nt(lhs, pkt[ws:ws + T, :])
            macc[g] = upd
            mb[g] = jnp.where(bmask[g] != 0.0, upd, 0.0).astype(bf16)

    def out_project():
        return _dot_tn(w_in[3], ot[...].astype(bf16))

    def load_weight(i):
        w = w_in[i]
        wf = w.astype(f32)
        c = jnp.sum(wf, axis=0, keepdims=True)
        c_hi = c.astype(bf16).astype(f32)
        r16 = lax.broadcasted_iota(jnp.int32, (16, D), 0)
        extra = jnp.where(r16 >= 4, 0.0, jnp.where(r16 < 2, c_hi, c - c_hi)).astype(bf16)
        w_aug = jnp.concatenate([w, extra, jnp.zeros((KP - D - 16, D), bf16)], axis=0)
        w_t = w_aug.T
        wt[i * D:(i + 1) * D, :] = w_t
        return w_t, jnp.max(jnp.sum(wf * wf, axis=0, keepdims=True))

    am_v[...] = jnp.zeros_like(am_v)
    with _scope("p_tables"):
        small_b.wait()
        small_r.wait()
        build_tables()
    with _scope("p_wq_wait"):
        w_copies[0].wait()
    w_copies[2].start()
    x_copy(1).start()
    w_copies[3].start()
    with _scope("p_wqT"):
        _, cq = load_weight(0)
    with _scope("p_x0_wait"):
        x_copy(0).wait()
    for s in range(2, NSEG):
        x_copy(s).start()
    for c in w_copies[4:]:
        c.start()
    HALF = 288
    with _scope("p_qlo"):
        ln1(0)
        store_q(_dot(wt[0:HALF, :], proj_rhs(0)), ln_scale(0), 0, HALF, False)
    with _scope("p_wk_wait"):
        w_copies[1].wait()
    with _scope("p_qhi_wkT_klo"):
        wk_t, ck = load_weight(1)
        store_q(_dot(wt[HALF:D, :], proj_rhs(0)), ln_scale(0), HALF, D, False)
        store_k_rows(_dot(wk_t[0:HALF], proj_rhs(0)), ln_scale(0), 0, HALF)
    with _scope("p_wv_wait"):
        w_copies[2].wait()
    with _scope("p_khi_wvT_v"):
        wv_t, cv = load_weight(2)
        store_k_rows(_dot(wt[D + HALF:2 * D, :], proj_rhs(0)), ln_scale(0), HALF, D)
        transpose_k()
        store_v(_dot(wv_t, proj_rhs(0)), ln_scale(0))
    slack = 1.05
    logit_bound2 = (cq * ck) * (slack * D * DH * QSCALE) ** 2
    v_bound2 = cv * (slack * D)
    safe = (logit_bound2 <= SAFE_LOGIT ** 2) & (v_bound2 <= SAFE_V ** 2)
    w_copies[3].wait()

    def body(s, carry):
        more = s + 1 < NSEG
        nxt = jnp.minimum(s + 1, NSEG - 1)

        @pl.when(more)
        def _():
            x_copy(nxt).wait()

        @pl.when(safe)
        def _():
            with _scope("attn"):
                attention(True)

        @pl.when(jnp.logical_not(safe))
        def _():
            attention(False)

        @pl.when(more)
        def _():
            with _scope("blockB"):
                hold = {}
                steps = {
                    "MU": mem_update,
                    "OP": lambda: hold.update(a=out_project()),
                    "LN1": lambda: ln1(nxt),
                    "PR": lambda: project(nxt),
                    "MR": mem_read,
                    "FIN": lambda: finalize(s, 0, NT, hold["a"]),
                }
                for n in _ORDER_B:
                    steps[n]()
            out_copy(s).start()
        return carry

    lax.fori_loop(0, NSEG, body, 0)
    with _scope("fin"):
        finalize(NSEG - 1, 0, NT, out_project())
        out_copy(NSEG - 1).start()

    bv = best_v[...]
    rmax = jnp.max(bv, axis=1, keepdims=True)
    cand = best_i[...] + lax.broadcasted_iota(jnp.int32, best_i.shape, 1)
    idx = jnp.clip(jnp.min(jnp.where(bv == rmax, cand, S)), 0, S - 1)
    base = pl.multiple_of((idx // T) * T, T)
    lane = idx - base
    blk = (hbuf[:, pl.ds(base, T)] * ab_all[0:1, pl.ds(base, T)]
           + ab_all[8:9, pl.ds(base, T)]).astype(bf16)
    pick = jnp.where(lax.broadcasted_iota(jnp.int32, (16, T), 1) == lane, 1.0, 0.0).astype(bf16)
    xg = _dot_nt(pick, blk).astype(bf16)
    for c in w_copies[4:]:
        c.wait()
    yacc = jnp.zeros((D, T), f32)
    FC = 4 * T
    for c in range(F // FC):
        gt = _dot(xg, wg_v[:, c * FC:(c + 1) * FC])
        up = _dot(xg, wu_v[:, c * FC:(c + 1) * FC])
        act = (gt * jax.nn.sigmoid(gt) * up)[0:1].astype(bf16).astype(f32)
        for t in range(FC // T):
            f0 = c * FC + t * T
            wd = jnp.concatenate([wd_v[r:r + 8, f0:f0 + T].astype(f32) for r in range(0, D, 8)], axis=0)
            yacc = yacc + wd * act[:, t * T:(t + 1) * T]
    y = jnp.sum(yacc, axis=1, keepdims=True) * jax.nn.sigmoid(rmax[0:1])
    for s in range(NSEG):
        out_copy(s).wait()
    sel = lax.broadcasted_iota(jnp.int32, (D, T), 1) == lane
    cur = out_v[:, pl.ds(base, T)].astype(f32)
    out_v[:, pl.ds(base, T)] = (cur + jnp.where(sel, y, 0.0)).astype(bf16)
    patch = pltpu.make_async_copy(out_v.at[:, pl.ds(base, T)],
                                  out_hbm.at[0, :, pl.ds(base, T)], sem_o.at[NSEG])
    patch.start()
    patch.wait()


@jax.jit
def pallas_sequential_preLN__memory_aug_infini_attn__moe_arch_mod__prompt_kernel(
    A_x: jax.Array,
    A_wq: jax.Array,
    A_wk: jax.Array,
    A_wv: jax.Array,
    A_wo: jax.Array,
    A_beta: jax.Array,
    B_x: jax.Array,
    B_w_r: jax.Array,
    B_w_gate: jax.Array,
    B_w_up: jax.Array,
    B_w_down: jax.Array,
):
    del B_x
    hbm_spec = pl.BlockSpec(memory_space=pltpu.HBM)
    scratch = [
        pltpu.VMEM((D, S), bf16),
        pltpu.VMEM((4, D, D), bf16),
        pltpu.VMEM((3 * D, KP), bf16),
        pltpu.VMEM((D, S), f32),
        pltpu.VMEM((D, F), bf16),
        pltpu.VMEM((D, F), bf16),
        pltpu.VMEM((D, F), bf16),
        pltpu.VMEM((16, S), bf16),
        pltpu.VMEM((8, S), f32),
        pltpu.VMEM((D, L), bf16),
        pltpu.VMEM((D, L), bf16),
        pltpu.VMEM((D, L), bf16),
        pltpu.VMEM((D, L), bf16),
        pltpu.VMEM((D, L), bf16),
        pltpu.VMEM((NG, L, T), bf16),
        pltpu.VMEM((7, NT, L, T), bf16),
        pltpu.VMEM((7, NT, L, T), bf16),
        pltpu.VMEM((D, L), f32),
        pltpu.VMEM((D, L), f32),
        pltpu.VMEM((NG, MROWS, T), f32),
        pltpu.VMEM((NG, MROWS, T), bf16),
        pltpu.VMEM((NG, MROWS, T), f32),
        pltpu.VMEM((D, T), f32),
        pltpu.VMEM((H, 8, T), f32),
        pltpu.VMEM((D, T), f32),
        pltpu.VMEM((16, S), f32),
        pltpu.VMEM((D, S), bf16),
        pltpu.VMEM((8, T), f32),
        pltpu.VMEM((8, T), jnp.int32),
        pltpu.VMEM((8, T), f32),
        pltpu.VMEM((H,), bf16),
        pltpu.VMEM((D,), bf16),
        pltpu.SemaphoreType.DMA((NSEG,)),
        pltpu.SemaphoreType.DMA((9,)),
        pltpu.SemaphoreType.DMA((NSEG + 1,)),
    ]
    out_t = pl.pallas_call(
        _kernel,
        out_shape=jax.ShapeDtypeStruct((1, D, S), bf16),
        in_specs=[hbm_spec] * 10,
        out_specs=hbm_spec,
        scratch_shapes=scratch,
        compiler_params=pltpu.CompilerParams(vmem_limit_bytes=100 * 1024 * 1024),
    )(jnp.transpose(A_x, (0, 2, 1)), A_wq, A_wk, A_wv, A_wo, A_beta,
      B_w_r, B_w_gate, B_w_up, B_w_down.T)
    return jnp.transpose(out_t, (0, 2, 1))
```

```python
import contextlib

import jax
import jax.numpy as jnp
from jax import lax
import jax.experimental.pallas as pl
import jax.experimental.pallas.tpu as pltpu

S = 2048
D = 576
H = 32
DH = 18
NSEG = 4
L = 512
F = 4608
T = 128
NT = L // T
EPS = 1e-5
LOG2E = 1.4426950408889634
QSCALE = (DH ** -0.5) * LOG2E
WIN = 112
GROUPS = (tuple(range(0, 7)), tuple(range(7, 13)), tuple(range(13, 19)),
          tuple(range(19, 25)), tuple(range(25, 32)))
NG = len(GROUPS)
KP = 640
MROWS = T + 16
SAFE_LOGIT = 60.0
SAFE_V = 2.0 ** 40

bf16 = jnp.bfloat16
f32 = jnp.float32
_ORDER_B = ["MU", "OP", "LN1", "PR", "MR", "FIN"]
_PROFILE = False


def _scope(name):
    return jax.named_scope(name) if _PROFILE else contextlib.nullcontext()


def _colsum(x):
    n = x.shape[0] // 4
    parts = [jnp.sum(x[i * n:(i + 1) * n].reshape(n // 8, 8, x.shape[1]), axis=0) for i in range(4)]
    return jnp.sum((parts[0] + parts[1]) + (parts[2] + parts[3]), axis=0, keepdims=True)


def _ln_stats(x):
    m = _colsum(x) * (1.0 / D)
    v = jnp.maximum(_colsum(x * x) * (1.0 / D) - m * m, 0.0)
    a = lax.rsqrt(v + EPS)
    return a, -m * a


def _phi(t):
    return jnp.where(t > 0, t + 1.0, jnp.exp(t))


def _dot(a, b):
    return jnp.dot(a, b, preferred_element_type=f32)


def _dot_nt(a, b):
    return lax.dot_general(a, b, (((1,), (1,)), ((), ())), preferred_element_type=f32)


def _dot_tn(a, b):
    return lax.dot_general(a, b, (((0,), (0,)), ((), ())), preferred_element_type=f32)


ROT = (0, 1, 2, 3, 0, 2, 1)
QW = T // 4


def _pack_plan(nh, c):
    tiles = []
    split = []
    for u in range(nh):
        need = [(a + ROT[u]) % 4 for a in range(c, 4)]
        for t in tiles:
            if all(t[q] is None for q in need):
                break
        else:
            bound = max(sum(q in [(a + ROT[v]) % 4 for a in range(c, 4)] for v in range(nh))
                        for q in range(4))
            if len(tiles) >= bound:
                split.append((u, need))
                continue
            t = [None] * 4
            tiles.append(t)
        for q in need:
            t[q] = u
    for u, need in split:
        for q in need:
            next(t for t in tiles if t[q] is None)[q] = u
    return tiles


def _masked_q(qt_ref, g, j):
    ws = WIN * g
    row64 = lax.broadcasted_iota(jnp.int32, (64, T), 0)
    qw32 = pltpu.bitcast(qt_ref[ws:ws + T, j * T:(j + 1) * T], jnp.uint32)
    rolled = {0: qw32}
    qms = []
    for u, h in enumerate(GROUPS[g]):
        if ROT[u] not in rolled:
            rolled[ROT[u]] = pltpu.roll(qw32, ROT[u] * QW, axis=1)
        lo2 = (h * DH - ws) // 2
        qmask = (row64 >= lo2) & (row64 < lo2 + DH // 2)
        qms.append(jnp.where(qmask, rolled[ROT[u]], jnp.uint32(0)))
    return qms


def _select_quarters(sources):
    distinct = []
    for x in sources:
        if x is not None and not any(x is y for y in distinct):
            distinct.append(x)
    distinct.sort(key=lambda y: -sum(x is y for x in sources))
    out = distinct[0]
    lane = lax.broadcasted_iota(jnp.int32, out.shape, 1)
    for y in distinct[1:]:
        mask = None
        for q, x in enumerate(sources):
            if x is y:
                m = (lane >= q * QW) & (lane < (q + 1) * QW)
                mask = m if mask is None else mask | m
        out = jnp.where(mask, y, out)
    return out


def _scores_fast(g, kp_ref, qt_ref, p_ref):
    nh = len(GROUPS[g])
    kk = lax.broadcasted_iota(jnp.int32, (T, T), 0)
    qq = lax.broadcasted_iota(jnp.int32, (T, T), 1)
    causal = {r: kk <= ((qq - r * QW) & (T - 1)) for r in set(ROT[:nh])}
    plans = {c: _pack_plan(nh, c) for c in range(1, 4)}
    for j in range(NT):
        qms = _masked_q(qt_ref, g, j)
        n0 = T * j + QW
        p0 = jnp.exp2(_dot(kp_ref[g, 0:n0, :],
                           jnp.concatenate([pltpu.bitcast(q, bf16) for q in qms], axis=1)))
        pc = {}
        for c in range(1, 4):
            w = [pltpu.bitcast(_select_quarters([None if u is None else qms[u] for u in t]), bf16)
                 for t in plans[c]]
            r0 = T * j + c * QW
            pc[c] = jnp.exp2(_dot(kp_ref[g, r0:r0 + QW, :], jnp.concatenate(w, axis=1)))
        for u in range(nh):
            pu = p0[:, u * T:(u + 1) * T]
            if j > 0:
                p_ref[u, j, 0:j * T, :] = pu[0:j * T].astype(bf16)
            rows = [pu[j * T:n0]]
            for c in range(1, 4):
                src = [None] * 4
                for i, t in enumerate(plans[c]):
                    for q in range(4):
                        if t[q] == u:
                            src[q] = i
                vals = {i: pc[c][:, i * T:(i + 1) * T] for i in set(src) if i is not None}
                rows.append(_select_quarters([None if i is None else vals[i] for i in src]))
            p_ref[u, j, j * T:(j + 1) * T, :] = jnp.where(
                causal[ROT[u]], jnp.concatenate(rows, axis=0), 0.0).astype(bf16)


def _attention_safe(h, kp_ref, qt_ref, vt_ref, g1_ref, am_ref, ot_ref):
    g = jnp.minimum(jnp.maximum(h - 1, 0) // 6, NG - 1)
    ws = pl.multiple_of(g * WIN, 16)
    lo = h * DH - ws
    row128 = lax.broadcasted_iota(jnp.int32, (T, T), 0)
    qmask = (row128 >= lo) & (row128 < lo + DH)
    vs = pl.multiple_of(((h * DH) // 16) * 16, 16)
    off = h * DH - vs
    row32 = lax.broadcasted_iota(jnp.int32, (32, T), 0)
    omask = (row32 >= off) & (row32 < off + DH)
    kk = lax.broadcasted_iota(jnp.int32, (L, T), 0)
    qq = lax.broadcasted_iota(jnp.int32, (L, T), 1)

    def tile(j, c):
        c0 = pl.multiple_of(j * T, T)
        qm = jnp.where(qmask, qt_ref[pl.ds(ws, T), pl.ds(c0, T)].astype(f32), 0.0).astype(bf16)
        s = _dot(kp_ref[g], qm)
        s = jnp.where(kk <= qq + c0, s, -jnp.inf)
        m = jnp.max(s, axis=0, keepdims=True)
        p = jnp.exp2(s - m).astype(bf16)
        acc = _dot(_v_rows(vt_ref, vs, off // 2, L), p)
        l8 = jnp.where(off <= 6, acc[24:32], acc[0:8])
        rl = g1_ref[h] / l8
        o = acc * jnp.concatenate([rl] * 4, axis=0) + am_ref[pl.ds(vs, 32), pl.ds(c0, T)]
        pltpu.store(ot_ref.at[pl.ds(vs, 32), pl.ds(c0, T)], o, mask=omask)
        return c

    lax.fori_loop(0, NT, tile, 0)


def _v_rows(vt_ref, vs, off2, nk):
    row16 = lax.broadcasted_iota(jnp.int32, (16, nk), 0)
    keep = (row16 >= off2) & (row16 < off2 + DH // 2)
    v32 = pltpu.bitcast(vt_ref[pl.ds(vs, 32), 0:nk], jnp.uint32)
    return pltpu.bitcast(jnp.where(keep, v32, jnp.uint32(0x3F803F80)), bf16)


def _pv(g, vt_ref, p_ref, g1_ref, am_ref, ot_ref):
    row32 = lax.broadcasted_iota(jnp.int32, (32, T), 0)
    for u, h in enumerate(GROUPS[g]):
        vs = ((h * DH) // 16) * 16
        off = h * DH - vs
        omask = (row32 >= off) & (row32 < off + DH)
        g1 = g1_ref[h]
        vrows = _v_rows(vt_ref, vs, off // 2, L)
        for j in range(NT):
            nk = T * (j + 1)
            acc = _dot(vrows[:, 0:nk], p_ref[u, j, 0:nk, :])
            l8 = acc[24:32] if off <= 6 else acc[0:8]
            rl = g1 / l8
            o = acc * jnp.concatenate([rl] * 4, axis=0)
            if ROT[u]:
                o = pltpu.roll(o, T - ROT[u] * QW, axis=1)
            o = o + am_ref[vs:vs + 32, j * T:(j + 1) * T]
            pltpu.store(ot_ref.at[vs:vs + 32, j * T:(j + 1) * T], o, mask=omask)


def _kernel(x_hbm, wq_hbm, wk_hbm, wv_hbm, wo_hbm, beta_hbm, wr_hbm, wg_hbm, wu_hbm, wd_hbm,
            out_hbm,
            x_v, w_in, wt, hbuf, wg_v, wu_v, wd_v,
            aug, arow, qt, pqt, kt, pkt, vt, kp, p0, p1, am_v, ot,
            macc, mb, bmask, gtab, g1tab, wrtab, ab_all, out_v, best_v, best_i, wrsum, beta_ref, wr_ref,
            sem_x, sem_w, sem_o):
    def x_copy(s):
        return pltpu.make_async_copy(x_hbm.at[0, :, pl.ds(s * L, L)],
                                     x_v.at[:, pl.ds(s * L, L)], sem_x.at[s])

    def out_copy(s):
        return pltpu.make_async_copy(out_v.at[:, pl.ds(s * L, L)],
                                     out_hbm.at[0, :, pl.ds(s * L, L)], sem_o.at[s])

    w_copies = [
        pltpu.make_async_copy(wq_hbm, w_in.at[0], sem_w.at[0]),
        pltpu.make_async_copy(wk_hbm, w_in.at[1], sem_w.at[1]),
        pltpu.make_async_copy(wv_hbm, w_in.at[2], sem_w.at[2]),
        pltpu.make_async_copy(wo_hbm, w_in.at[3], sem_w.at[3]),
        pltpu.make_async_copy(wg_hbm, wg_v, sem_w.at[4]),
        pltpu.make_async_copy(wu_hbm, wu_v, sem_w.at[5]),
        pltpu.make_async_copy(wd_hbm, wd_v, sem_w.at[6]),
    ]
    small_b = pltpu.make_async_copy(beta_hbm, beta_ref, sem_w.at[7])
    small_r = pltpu.make_async_copy(wr_hbm, wr_ref, sem_w.at[8])
    small_b.start()
    small_r.start()
    x_copy(0).start()
    w_copies[0].start()
    w_copies[1].start()

    def build_tables():
        gate = jax.nn.sigmoid(beta_ref[...].astype(f32).reshape(1, H))
        rr = lax.broadcasted_iota(jnp.int32, (D, H), 0)
        hh = lax.broadcasted_iota(jnp.int32, (D, H), 1)
        onehot = (rr >= hh * DH) & (rr < (hh + 1) * DH)
        gcol = jnp.sum(jnp.where(onehot, gate, 0.0), axis=1, keepdims=True)
        gtab[...] = jnp.broadcast_to(gcol, (D, T))
        hh8 = lax.broadcasted_iota(jnp.int32, (8, H), 1)
        for h in range(H):
            gh = jnp.sum(jnp.where(hh8 == h, gate, 0.0), axis=1, keepdims=True)
            g1tab[h] = jnp.broadcast_to(1.0 - gh, (8, T))
        wr_row = wr_ref[...].astype(f32).reshape(1, D)
        wr_pad = jnp.concatenate([wr_row, jnp.zeros((1, 5 * T - D), f32)], axis=1)
        wrtab[...] = jnp.broadcast_to(wr_pad, (T, 5 * T)).T[0:D]
        wrsum[...] = jnp.broadcast_to(jnp.sum(wr_row, axis=1, keepdims=True), wrsum.shape)

    mr = lax.broadcasted_iota(jnp.int32, (MROWS, T), 0)
    mc = lax.broadcasted_iota(jnp.int32, (MROWS, T), 1)
    for g in range(NG):
        ws = WIN * g
        m = jnp.zeros((MROWS, T), jnp.bool_)
        for i, h in enumerate(GROUPS[g]):
            lo = h * DH - ws
            cols = (mc >= lo) & (mc < lo + DH)
            rows = ((mr >= lo) & (mr < lo + DH) & (mr < T)) | (mr == T + i)
            m = m | (cols & rows)
        bmask[g] = jnp.where(m, 1.0, 0.0)
    macc[...] = jnp.zeros_like(macc)
    mb[...] = jnp.zeros_like(mb)
    best_v[...] = jnp.full(best_v.shape, -jnp.inf, f32)
    best_i[...] = jnp.zeros(best_i.shape, jnp.int32)

    ones_rows = jnp.ones((16, L), bf16)

    def ln1(s):
        col0 = pl.multiple_of(s * L, L)
        xs = x_v[:, pl.ds(col0, L)].astype(f32)
        m = _colsum(xs) * (1.0 / D)
        v = jnp.maximum(_colsum(xs * xs) * (1.0 / D) - m * m, 0.0)
        arow[:, pl.ds(col0, L)] = jnp.broadcast_to(lax.rsqrt(v + EPS), (8, L))
        m_hi = (-m).astype(bf16).astype(f32)
        m_lo = -m - m_hi
        r16 = lax.broadcasted_iota(jnp.int32, (16, L), 0)
        rows = jnp.where(r16 >= 4, 0.0, jnp.where((r16 & 1) == 0, m_hi, m_lo))
        aug[:, pl.ds(col0, L)] = rows.astype(bf16)

    def finalize(s, t0, nt, attn):
        w = nt * T
        col0 = pl.multiple_of(s * L + t0 * T, T)
        hres = x_v[:, pl.ds(col0, w)].astype(f32) + attn
        hbuf[:, pl.ds(col0, w)] = hres
        a, b = _ln_stats(hres)
        wr = jnp.concatenate([wrtab[...]] * nt, axis=1)
        r = _colsum(hres * wr) * a + b * wrsum[0:1, 0:1]
        ab_all[0:8, pl.ds(col0, w)] = jnp.broadcast_to(a, (8, w))
        ab_all[8:16, pl.ds(col0, w)] = jnp.broadcast_to(b, (8, w))
        out_v[:, pl.ds(col0, w)] = (hbuf[:, pl.ds(col0, w)] * (1.0 + a) + b).astype(bf16)
        r = r.astype(bf16).astype(f32)
        bv, bi = best_v[0:1, :], best_i[0:1, :]
        for t in range(nt):
            rt = r[:, t * T:(t + 1) * T]
            better = rt > bv
            bi = jnp.where(better, col0 + t * T, bi)
            bv = jnp.where(better, rt, bv)
        best_i[...] = jnp.broadcast_to(bi, best_i.shape)
        best_v[...] = jnp.broadcast_to(bv, best_v.shape)

    def proj_rhs(s):
        col0 = pl.multiple_of(s * L, L)
        return jnp.concatenate([x_v[:, pl.ds(col0, L)], aug[:, pl.ds(col0, L)],
                                jnp.zeros((KP - D - 16, L), bf16)], axis=0)

    def ln_scale(s):
        return arow[0:1, pl.ds(pl.multiple_of(s * L, L), L)]

    def store_q(raw, a, r0, r1, with_phi=True):
        qt[r0:r1, :] = (raw * (a * QSCALE)).astype(bf16)
        if with_phi:
            pqt[r0:r1, :] = _phi(raw * a).astype(bf16)

    def store_k_rows(raw, a, r0, r1):
        k = raw * a
        kt[r0:r1, :] = k.astype(bf16)
        pkt[r0:r1, :] = _phi(k).astype(bf16)

    def transpose_k():
        for g in range(NG):
            kp[g] = kt[WIN * g:WIN * g + T, :].T

    def store_k(raw, a):
        k = raw * a
        kb = k.astype(bf16)
        pkt[...] = _phi(k).astype(bf16)
        for g in range(NG):
            kp[g] = kb[WIN * g:WIN * g + T, :].T

    def store_v(raw, a):
        vt[...] = (raw * a).astype(bf16)

    def project(s):
        qkv = _dot(wt[...], proj_rhs(s))
        a = ln_scale(s)
        store_q(qkv[0:D], a, 0, D)
        store_k(qkv[D:2 * D], a)
        store_v(qkv[2 * D:3 * D], a)

    def mem_read():
        row128 = lax.broadcasted_iota(jnp.int32, (T, T), 0)
        row8 = lax.broadcasted_iota(jnp.int32, (8, T), 0)
        for g in range(NG):
            ws = WIN * g
            heads = GROUPS[g]
            lo_g, hi_g = heads[0] * DH - ws, (heads[-1] + 1) * DH - ws
            wmask = (row128 >= lo_g) & (row128 < hi_g)
            for j in range(NT):
                nd = _dot(mb[g], pqt[ws:ws + T, j * T:(j + 1) * T])
                rden = 1.0 / (nd[T:T + 8] + 1e-6)
                rb = [jnp.broadcast_to(rden[i:i + 1], (8, T)) for i in range(len(heads))]
                blocks = []
                for b in range(T // 8):
                    r_lo, r_hi = 8 * b, 8 * b + 7
                    i_lo = min(max((r_lo + ws) // DH - heads[0], 0), len(heads) - 1)
                    i_hi = min(max((r_hi + ws) // DH - heads[0], 0), len(heads) - 1)
                    if i_lo == i_hi:
                        blocks.append(rb[i_lo])
                    else:
                        cut = (heads[0] + i_hi) * DH - ws - r_lo
                        blocks.append(jnp.where(row8 < cut, rb[i_lo], rb[i_hi]))
                amv = nd[0:T] * jnp.concatenate(blocks, axis=0) * gtab[ws:ws + T, :]
                pltpu.store(am_v.at[ws:ws + T, j * T:(j + 1) * T], amv, mask=wmask)

    def attention(fast):
        ps = (p0, p1)
        if fast:
            _scores_fast(0, kp, qt, ps[0])
            for g in range(NG):
                if g + 1 < NG:
                    _scores_fast(g + 1, kp, qt, ps[(g + 1) % 2])
                _pv(g, vt, ps[g % 2], g1tab, am_v, ot)
        else:
            lax.fori_loop(0, H, lambda h, c: (_attention_safe(h, kp, qt, vt, g1tab, am_v, ot), c)[1], 0)

    def mem_update():
        for g in range(NG):
            ws = WIN * g
            lhs = jnp.concatenate([vt[ws:ws + T, :], ones_rows], axis=0)
            upd = macc[g] + _dot_nt(lhs, pkt[ws:ws + T, :])
            macc[g] = upd
            mb[g] = jnp.where(bmask[g] != 0.0, upd, 0.0).astype(bf16)

    def out_project():
        return _dot_tn(w_in[3], ot[...].astype(bf16))

    def load_weight(i):
        w = w_in[i]
        wf = w.astype(f32)
        c = jnp.sum(wf, axis=0, keepdims=True)
        c_hi = c.astype(bf16).astype(f32)
        r16 = lax.broadcasted_iota(jnp.int32, (16, D), 0)
        extra = jnp.where(r16 >= 4, 0.0, jnp.where(r16 < 2, c_hi, c - c_hi)).astype(bf16)
        w_aug = jnp.concatenate([w, extra, jnp.zeros((KP - D - 16, D), bf16)], axis=0)
        w_t = w_aug.T
        wt[i * D:(i + 1) * D, :] = w_t
        return w_t, jnp.max(jnp.sum(wf * wf, axis=0, keepdims=True))

    am_v[...] = jnp.zeros_like(am_v)
    with _scope("p_tables"):
        small_b.wait()
        small_r.wait()
        build_tables()
    with _scope("p_wq_wait"):
        w_copies[0].wait()
    w_copies[2].start()
    x_copy(1).start()
    w_copies[3].start()
    with _scope("p_wqT"):
        _, cq = load_weight(0)
    with _scope("p_x0_wait"):
        x_copy(0).wait()
    for s in range(2, NSEG):
        x_copy(s).start()
    for c in w_copies[4:]:
        c.start()
    HALF = 288
    with _scope("p_qlo"):
        ln1(0)
        store_q(_dot(wt[0:HALF, :], proj_rhs(0)), ln_scale(0), 0, HALF, False)
    with _scope("p_wk_wait"):
        w_copies[1].wait()
    with _scope("p_qhi_wkT_klo"):
        wk_t, ck = load_weight(1)
        store_q(_dot(wt[HALF:D, :], proj_rhs(0)), ln_scale(0), HALF, D, False)
        store_k_rows(_dot(wk_t[0:HALF], proj_rhs(0)), ln_scale(0), 0, HALF)
    with _scope("p_wv_wait"):
        w_copies[2].wait()
    with _scope("p_khi_wvT_v"):
        wv_t, cv = load_weight(2)
        store_k_rows(_dot(wt[D + HALF:2 * D, :], proj_rhs(0)), ln_scale(0), HALF, D)
        transpose_k()
        store_v(_dot(wv_t, proj_rhs(0)), ln_scale(0))
    slack = 1.05
    logit_bound2 = (cq * ck) * (slack * D * DH * QSCALE) ** 2
    v_bound2 = cv * (slack * D)
    safe = (logit_bound2 <= SAFE_LOGIT ** 2) & (v_bound2 <= SAFE_V ** 2)
    w_copies[3].wait()

    def body(s, carry):
        more = s + 1 < NSEG
        nxt = jnp.minimum(s + 1, NSEG - 1)

        @pl.when(more)
        def _():
            x_copy(nxt).wait()

        @pl.when(safe)
        def _():
            with _scope("attn"):
                attention(True)

        @pl.when(jnp.logical_not(safe))
        def _():
            attention(False)

        @pl.when(more)
        def _():
            with _scope("blockB"):
                hold = {}
                steps = {
                    "MU": mem_update,
                    "OP": lambda: hold.update(a=out_project()),
                    "LN1": lambda: ln1(nxt),
                    "PR": lambda: project(nxt),
                    "MR": mem_read,
                    "FIN": lambda: finalize(s, 0, NT, hold["a"]),
                }
                for n in _ORDER_B:
                    steps[n]()
            out_copy(s).start()
        return carry

    lax.fori_loop(0, NSEG, body, 0)
    with _scope("fin"):
        finalize(NSEG - 1, 0, NT, out_project())
        out_copy(NSEG - 1).start()

    bv = best_v[...]
    rmax = jnp.max(bv, axis=1, keepdims=True)
    cand = best_i[...] + lax.broadcasted_iota(jnp.int32, best_i.shape, 1)
    idx = jnp.clip(jnp.min(jnp.where(bv == rmax, cand, S)), 0, S - 1)
    base = pl.multiple_of((idx // T) * T, T)
    lane = idx - base
    blk = (hbuf[:, pl.ds(base, T)] * ab_all[0:1, pl.ds(base, T)]
           + ab_all[8:9, pl.ds(base, T)]).astype(bf16)
    pick = jnp.where(lax.broadcasted_iota(jnp.int32, (16, T), 1) == lane, 1.0, 0.0).astype(bf16)
    xg = _dot_nt(pick, blk).astype(bf16)
    for c in w_copies[4:]:
        c.wait()
    yacc = jnp.zeros((D, T), f32)
    FC = 4 * T
    for c in range(F // FC):
        gt = _dot(xg, wg_v[:, c * FC:(c + 1) * FC])
        up = _dot(xg, wu_v[:, c * FC:(c + 1) * FC])
        act = (gt * jax.nn.sigmoid(gt) * up)[0:1].astype(bf16).astype(f32)
        for t in range(FC // T):
            f0 = c * FC + t * T
            wd = jnp.concatenate([wd_v[r:r + 8, f0:f0 + T].astype(f32) for r in range(0, D, 8)], axis=0)
            yacc = yacc + wd * act[:, t * T:(t + 1) * T]
    y = jnp.sum(yacc, axis=1, keepdims=True) * jax.nn.sigmoid(rmax[0:1])
    for s in range(NSEG):
        out_copy(s).wait()
    sel = lax.broadcasted_iota(jnp.int32, (D, T), 1) == lane
    cur = out_v[:, pl.ds(base, T)].astype(f32)
    out_v[:, pl.ds(base, T)] = (cur + jnp.where(sel, y, 0.0)).astype(bf16)
    patch = pltpu.make_async_copy(out_v.at[:, pl.ds(base, T)],
                                  out_hbm.at[0, :, pl.ds(base, T)], sem_o.at[NSEG])
    patch.start()
    patch.wait()


@jax.jit
def pallas_sequential_preLN__memory_aug_infini_attn__moe_arch_mod__prompt_kernel(
    A_x: jax.Array,
    A_wq: jax.Array,
    A_wk: jax.Array,
    A_wv: jax.Array,
    A_wo: jax.Array,
    A_beta: jax.Array,
    B_x: jax.Array,
    B_w_r: jax.Array,
    B_w_gate: jax.Array,
    B_w_up: jax.Array,
    B_w_down: jax.Array,
):
    del B_x
    hbm_spec = pl.BlockSpec(memory_space=pltpu.HBM)
    scratch = [
        pltpu.VMEM((D, S), bf16),
        pltpu.VMEM((4, D, D), bf16),
        pltpu.VMEM((3 * D, KP), bf16),
        pltpu.VMEM((D, S), f32),
        pltpu.VMEM((D, F), bf16),
        pltpu.VMEM((D, F), bf16),
        pltpu.VMEM((D, F), bf16),
        pltpu.VMEM((16, S), bf16),
        pltpu.VMEM((8, S), f32),
        pltpu.VMEM((D, L), bf16),
        pltpu.VMEM((D, L), bf16),
        pltpu.VMEM((D, L), bf16),
        pltpu.VMEM((D, L), bf16),
        pltpu.VMEM((D, L), bf16),
        pltpu.VMEM((NG, L, T), bf16),
        pltpu.VMEM((7, NT, L, T), bf16),
        pltpu.VMEM((7, NT, L, T), bf16),
        pltpu.VMEM((D, L), f32),
        pltpu.VMEM((D, L), f32),
        pltpu.VMEM((NG, MROWS, T), f32),
        pltpu.VMEM((NG, MROWS, T), bf16),
        pltpu.VMEM((NG, MROWS, T), f32),
        pltpu.VMEM((D, T), f32),
        pltpu.VMEM((H, 8, T), f32),
        pltpu.VMEM((D, T), f32),
        pltpu.VMEM((16, S), f32),
        pltpu.VMEM((D, S), bf16),
        pltpu.VMEM((8, T), f32),
        pltpu.VMEM((8, T), jnp.int32),
        pltpu.VMEM((8, T), f32),
        pltpu.VMEM((H,), bf16),
        pltpu.VMEM((D,), bf16),
        pltpu.SemaphoreType.DMA((NSEG,)),
        pltpu.SemaphoreType.DMA((9,)),
        pltpu.SemaphoreType.DMA((NSEG + 1,)),
    ]
    out_t = pl.pallas_call(
        _kernel,
        out_shape=jax.ShapeDtypeStruct((1, D, S), bf16),
        in_specs=[hbm_spec] * 10,
        out_specs=hbm_spec,
        scratch_shapes=scratch,
        compiler_params=pltpu.CompilerParams(vmem_limit_bytes=100 * 1024 * 1024),
    )(jnp.transpose(A_x, (0, 2, 1)), A_wq, A_wk, A_wv, A_wo, A_beta,
      B_w_r, B_w_gate, B_w_up, B_w_down.T)
    return jnp.transpose(out_t, (0, 2, 1))
```

```python
import contextlib

import jax
import jax.numpy as jnp
from jax import lax
import jax.experimental.pallas as pl
import jax.experimental.pallas.tpu as pltpu

S = 2048
D = 576
H = 32
DH = 18
NSEG = 4
L = 512
F = 4608
T = 128
NT = L // T
EPS = 1e-5
LOG2E = 1.4426950408889634
QSCALE = (DH ** -0.5) * LOG2E
WIN = 112
GROUPS = (tuple(range(0, 7)), tuple(range(7, 13)), tuple(range(13, 19)),
          tuple(range(19, 25)), tuple(range(25, 32)))
NG = len(GROUPS)
KP = 640
MROWS = T + 16
SAFE_LOGIT = 60.0
SAFE_V = 2.0 ** 40

bf16 = jnp.bfloat16
f32 = jnp.float32
_ORDER_B = ["MU", "OP", "LN1", "PR", "MR", "FIN"]
_MOE_CHUNKS = (2,) * 18
_PROFILE = False


def _scope(name):
    return jax.named_scope(name) if _PROFILE else contextlib.nullcontext()


def _colsum(x):
    n = x.shape[0] // 4
    parts = [jnp.sum(x[i * n:(i + 1) * n].reshape(n // 8, 8, x.shape[1]), axis=0) for i in range(4)]
    return jnp.sum((parts[0] + parts[1]) + (parts[2] + parts[3]), axis=0, keepdims=True)


def _ln_stats(x):
    m = _colsum(x) * (1.0 / D)
    v = jnp.maximum(_colsum(x * x) * (1.0 / D) - m * m, 0.0)
    a = lax.rsqrt(v + EPS)
    return a, -m * a


def _phi(t):
    return jnp.where(t > 0, t + 1.0, jnp.exp(t))


def _dot(a, b):
    return jnp.dot(a, b, preferred_element_type=f32)


def _dot_nt(a, b):
    return lax.dot_general(a, b, (((1,), (1,)), ((), ())), preferred_element_type=f32)


def _dot_tn(a, b):
    return lax.dot_general(a, b, (((0,), (0,)), ((), ())), preferred_element_type=f32)


ROT = (0, 1, 2, 3, 0, 2, 1)
QW = T // 4


def _pack_plan(nh, c):
    tiles = []
    split = []
    for u in range(nh):
        need = [(a + ROT[u]) % 4 for a in range(c, 4)]
        for t in tiles:
            if all(t[q] is None for q in need):
                break
        else:
            bound = max(sum(q in [(a + ROT[v]) % 4 for a in range(c, 4)] for v in range(nh))
                        for q in range(4))
            if len(tiles) >= bound:
                split.append((u, need))
                continue
            t = [None] * 4
            tiles.append(t)
        for q in need:
            t[q] = u
    for u, need in split:
        for q in need:
            next(t for t in tiles if t[q] is None)[q] = u
    return tiles


def _masked_q(qt_ref, g, j):
    ws = WIN * g
    row64 = lax.broadcasted_iota(jnp.int32, (64, T), 0)
    qw32 = pltpu.bitcast(qt_ref[ws:ws + T, j * T:(j + 1) * T], jnp.uint32)
    rolled = {0: qw32}
    qms = []
    for u, h in enumerate(GROUPS[g]):
        if ROT[u] not in rolled:
            rolled[ROT[u]] = pltpu.roll(qw32, ROT[u] * QW, axis=1)
        lo2 = (h * DH - ws) // 2
        qmask = (row64 >= lo2) & (row64 < lo2 + DH // 2)
        qms.append(jnp.where(qmask, rolled[ROT[u]], jnp.uint32(0)))
    return qms


def _select_quarters(sources):
    distinct = []
    for x in sources:
        if x is not None and not any(x is y for y in distinct):
            distinct.append(x)
    distinct.sort(key=lambda y: -sum(x is y for x in sources))
    out = distinct[0]
    lane = lax.broadcasted_iota(jnp.int32, out.shape, 1)
    for y in distinct[1:]:
        mask = None
        for q, x in enumerate(sources):
            if x is y:
                m = (lane >= q * QW) & (lane < (q + 1) * QW)
                mask = m if mask is None else mask | m
        out = jnp.where(mask, y, out)
    return out


def _scores_fast(g, kp_ref, qt_ref, p_ref):
    nh = len(GROUPS[g])
    kk = lax.broadcasted_iota(jnp.int32, (T, T), 0)
    qq = lax.broadcasted_iota(jnp.int32, (T, T), 1)
    causal = {r: kk <= ((qq - r * QW) & (T - 1)) for r in set(ROT[:nh])}
    plans = {c: _pack_plan(nh, c) for c in range(1, 4)}
    for j in range(NT):
        qms = _masked_q(qt_ref, g, j)
        n0 = T * j + QW
        p0 = jnp.exp2(_dot(kp_ref[g, 0:n0, :],
                           jnp.concatenate([pltpu.bitcast(q, bf16) for q in qms], axis=1)))
        pc = {}
        for c in range(1, 4):
            w = [pltpu.bitcast(_select_quarters([None if u is None else qms[u] for u in t]), bf16)
                 for t in plans[c]]
            r0 = T * j + c * QW
            pc[c] = jnp.exp2(_dot(kp_ref[g, r0:r0 + QW, :], jnp.concatenate(w, axis=1)))
        for u in range(nh):
            pu = p0[:, u * T:(u + 1) * T]
            if j > 0:
                p_ref[u, j, 0:j * T, :] = pu[0:j * T].astype(bf16)
            rows = [pu[j * T:n0]]
            for c in range(1, 4):
                src = [None] * 4
                for i, t in enumerate(plans[c]):
                    for q in range(4):
                        if t[q] == u:
                            src[q] = i
                vals = {i: pc[c][:, i * T:(i + 1) * T] for i in set(src) if i is not None}
                rows.append(_select_quarters([None if i is None else vals[i] for i in src]))
            p_ref[u, j, j * T:(j + 1) * T, :] = jnp.where(
                causal[ROT[u]], jnp.concatenate(rows, axis=0), 0.0).astype(bf16)


def _attention_safe(h, kp_ref, qt_ref, vt_ref, g1_ref, am_ref, ot_ref):
    g = jnp.minimum(jnp.maximum(h - 1, 0) // 6, NG - 1)
    ws = pl.multiple_of(g * WIN, 16)
    lo = h * DH - ws
    row128 = lax.broadcasted_iota(jnp.int32, (T, T), 0)
    qmask = (row128 >= lo) & (row128 < lo + DH)
    vs = pl.multiple_of(((h * DH) // 16) * 16, 16)
    off = h * DH - vs
    row32 = lax.broadcasted_iota(jnp.int32, (32, T), 0)
    omask = (row32 >= off) & (row32 < off + DH)
    kk = lax.broadcasted_iota(jnp.int32, (L, T), 0)
    qq = lax.broadcasted_iota(jnp.int32, (L, T), 1)

    def tile(j, c):
        c0 = pl.multiple_of(j * T, T)
        qm = jnp.where(qmask, qt_ref[pl.ds(ws, T), pl.ds(c0, T)].astype(f32), 0.0).astype(bf16)
        s = _dot(kp_ref[g], qm)
        s = jnp.where(kk <= qq + c0, s, -jnp.inf)
        m = jnp.max(s, axis=0, keepdims=True)
        p = jnp.exp2(s - m).astype(bf16)
        acc = _dot(_v_rows(vt_ref, vs, off // 2, L), p)
        l8 = jnp.where(off <= 6, acc[24:32], acc[0:8])
        rl = g1_ref[h] / l8
        o = acc * jnp.concatenate([rl] * 4, axis=0) + am_ref[pl.ds(vs, 32), pl.ds(c0, T)]
        pltpu.store(ot_ref.at[pl.ds(vs, 32), pl.ds(c0, T)], o, mask=omask)
        return c

    lax.fori_loop(0, NT, tile, 0)


def _v_rows(vt_ref, vs, off2, nk):
    row16 = lax.broadcasted_iota(jnp.int32, (16, nk), 0)
    keep = (row16 >= off2) & (row16 < off2 + DH // 2)
    v32 = pltpu.bitcast(vt_ref[pl.ds(vs, 32), 0:nk], jnp.uint32)
    return pltpu.bitcast(jnp.where(keep, v32, jnp.uint32(0x3F803F80)), bf16)


def _pv(g, vt_ref, p_ref, g1_ref, am_ref, ot_ref):
    row32 = lax.broadcasted_iota(jnp.int32, (32, T), 0)
    for u, h in enumerate(GROUPS[g]):
        vs = ((h * DH) // 16) * 16
        off = h * DH - vs
        omask = (row32 >= off) & (row32 < off + DH)
        g1 = g1_ref[h]
        vrows = _v_rows(vt_ref, vs, off // 2, L)
        for j in range(NT):
            nk = T * (j + 1)
            acc = _dot(vrows[:, 0:nk], p_ref[u, j, 0:nk, :])
            l8 = acc[24:32] if off <= 6 else acc[0:8]
            rl = g1 / l8
            o = acc * jnp.concatenate([rl] * 4, axis=0)
            if ROT[u]:
                o = pltpu.roll(o, T - ROT[u] * QW, axis=1)
            o = o + am_ref[vs:vs + 32, j * T:(j + 1) * T]
            pltpu.store(ot_ref.at[vs:vs + 32, j * T:(j + 1) * T], o, mask=omask)


def _kernel(x_hbm, wq_hbm, wk_hbm, wv_hbm, wo_hbm, beta_hbm, wr_hbm, wg_hbm, wu_hbm, wd_hbm,
            out_hbm,
            x_v, w_in, wt, hbuf, wg_v, wu_v, wd_v,
            aug, arow, qt, pqt, kt, pkt, vt, kp, p0, p1, am_v, ot,
            macc, mb, bmask, gtab, g1tab, wrtab, ab_all, out_v, best_v, best_i, wrsum, beta_ref, wr_ref,
            sem_x, sem_w, sem_o):
    def x_copy(s):
        return pltpu.make_async_copy(x_hbm.at[0, :, pl.ds(s * L, L)],
                                     x_v.at[:, pl.ds(s * L, L)], sem_x.at[s])

    def out_copy(s):
        return pltpu.make_async_copy(out_v.at[:, pl.ds(s * L, L)],
                                     out_hbm.at[0, :, pl.ds(s * L, L)], sem_o.at[s])

    w_copies = [
        pltpu.make_async_copy(wq_hbm, w_in.at[0], sem_w.at[0]),
        pltpu.make_async_copy(wk_hbm, w_in.at[1], sem_w.at[1]),
        pltpu.make_async_copy(wv_hbm, w_in.at[2], sem_w.at[2]),
        pltpu.make_async_copy(wo_hbm, w_in.at[3], sem_w.at[3]),
        pltpu.make_async_copy(wg_hbm, wg_v, sem_w.at[4]),
        pltpu.make_async_copy(wu_hbm, wu_v, sem_w.at[5]),
        pltpu.make_async_copy(wd_hbm, wd_v, sem_w.at[6]),
    ]
    small_b = pltpu.make_async_copy(beta_hbm, beta_ref, sem_w.at[7])
    small_r = pltpu.make_async_copy(wr_hbm, wr_ref, sem_w.at[8])
    small_b.start()
    small_r.start()
    x_copy(0).start()
    w_copies[0].start()
    w_copies[1].start()

    def build_tables():
        gate = jax.nn.sigmoid(beta_ref[...].astype(f32).reshape(1, H))
        rr = lax.broadcasted_iota(jnp.int32, (D, H), 0)
        hh = lax.broadcasted_iota(jnp.int32, (D, H), 1)
        onehot = (rr >= hh * DH) & (rr < (hh + 1) * DH)
        gcol = jnp.sum(jnp.where(onehot, gate, 0.0), axis=1, keepdims=True)
        gtab[...] = jnp.broadcast_to(gcol, (D, T))
        hh8 = lax.broadcasted_iota(jnp.int32, (8, H), 1)
        for h in range(H):
            gh = jnp.sum(jnp.where(hh8 == h, gate, 0.0), axis=1, keepdims=True)
            g1tab[h] = jnp.broadcast_to(1.0 - gh, (8, T))
        wr_row = wr_ref[...].astype(f32).reshape(1, D)
        wr_pad = jnp.concatenate([wr_row, jnp.zeros((1, 5 * T - D), f32)], axis=1)
        wrtab[...] = jnp.broadcast_to(wr_pad, (T, 5 * T)).T[0:D]
        wrsum[...] = jnp.broadcast_to(jnp.sum(wr_row, axis=1, keepdims=True), wrsum.shape)

    mr = lax.broadcasted_iota(jnp.int32, (MROWS, T), 0)
    mc = lax.broadcasted_iota(jnp.int32, (MROWS, T), 1)
    for g in range(NG):
        ws = WIN * g
        m = jnp.zeros((MROWS, T), jnp.bool_)
        for i, h in enumerate(GROUPS[g]):
            lo = h * DH - ws
            cols = (mc >= lo) & (mc < lo + DH)
            rows = ((mr >= lo) & (mr < lo + DH) & (mr < T)) | (mr == T + i)
            m = m | (cols & rows)
        bmask[g] = jnp.where(m, 1.0, 0.0)
    macc[...] = jnp.zeros_like(macc)
    mb[...] = jnp.zeros_like(mb)
    best_v[...] = jnp.full(best_v.shape, -jnp.inf, f32)
    best_i[...] = jnp.zeros(best_i.shape, jnp.int32)

    ones_rows = jnp.ones((16, L), bf16)

    def ln1(s):
        col0 = pl.multiple_of(s * L, L)
        xs = x_v[:, pl.ds(col0, L)].astype(f32)
        m = _colsum(xs) * (1.0 / D)
        v = jnp.maximum(_colsum(xs * xs) * (1.0 / D) - m * m, 0.0)
        arow[:, pl.ds(col0, L)] = jnp.broadcast_to(lax.rsqrt(v + EPS), (8, L))
        m_hi = (-m).astype(bf16).astype(f32)
        m_lo = -m - m_hi
        r16 = lax.broadcasted_iota(jnp.int32, (16, L), 0)
        rows = jnp.where(r16 >= 4, 0.0, jnp.where((r16 & 1) == 0, m_hi, m_lo))
        aug[:, pl.ds(col0, L)] = rows.astype(bf16)

    def finalize(s, t0, nt, attn):
        w = nt * T
        col0 = pl.multiple_of(s * L + t0 * T, T)
        hres = x_v[:, pl.ds(col0, w)].astype(f32) + attn
        hbuf[:, pl.ds(col0, w)] = hres
        a, b = _ln_stats(hres)
        wr = jnp.concatenate([wrtab[...]] * nt, axis=1)
        r = _colsum(hres * wr) * a + b * wrsum[0:1, 0:1]
        ab_all[0:8, pl.ds(col0, w)] = jnp.broadcast_to(a, (8, w))
        ab_all[8:16, pl.ds(col0, w)] = jnp.broadcast_to(b, (8, w))
        out_v[:, pl.ds(col0, w)] = (hbuf[:, pl.ds(col0, w)] * (1.0 + a) + b).astype(bf16)
        r = r.astype(bf16).astype(f32)
        bv, bi = best_v[0:1, :], best_i[0:1, :]
        for t in range(nt):
            rt = r[:, t * T:(t + 1) * T]
            better = rt > bv
            bi = jnp.where(better, col0 + t * T, bi)
            bv = jnp.where(better, rt, bv)
        best_i[...] = jnp.broadcast_to(bi, best_i.shape)
        best_v[...] = jnp.broadcast_to(bv, best_v.shape)

    def proj_rhs(s):
        col0 = pl.multiple_of(s * L, L)
        return jnp.concatenate([x_v[:, pl.ds(col0, L)], aug[:, pl.ds(col0, L)],
                                jnp.zeros((KP - D - 16, L), bf16)], axis=0)

    def ln_scale(s):
        return arow[0:1, pl.ds(pl.multiple_of(s * L, L), L)]

    def store_q(raw, a, r0, r1, with_phi=True):
        qt[r0:r1, :] = (raw * (a * QSCALE)).astype(bf16)
        if with_phi:
            pqt[r0:r1, :] = _phi(raw * a).astype(bf16)

    def store_k_rows(raw, a, r0, r1):
        k = raw * a
        kt[r0:r1, :] = k.astype(bf16)
        pkt[r0:r1, :] = _phi(k).astype(bf16)

    def transpose_k():
        for g in range(NG):
            kp[g] = kt[WIN * g:WIN * g + T, :].T

    def store_k(raw, a):
        k = raw * a
        kb = k.astype(bf16)
        pkt[...] = _phi(k).astype(bf16)
        for g in range(NG):
            kp[g] = kb[WIN * g:WIN * g + T, :].T

    def store_v(raw, a):
        vt[...] = (raw * a).astype(bf16)

    def project(s):
        qkv = _dot(wt[...], proj_rhs(s))
        a = ln_scale(s)
        store_q(qkv[0:D], a, 0, D)
        store_k(qkv[D:2 * D], a)
        store_v(qkv[2 * D:3 * D], a)

    def mem_read():
        row128 = lax.broadcasted_iota(jnp.int32, (T, T), 0)
        row8 = lax.broadcasted_iota(jnp.int32, (8, T), 0)
        for g in range(NG):
            ws = WIN * g
            heads = GROUPS[g]
            lo_g, hi_g = heads[0] * DH - ws, (heads[-1] + 1) * DH - ws
            wmask = (row128 >= lo_g) & (row128 < hi_g)
            for j in range(NT):
                nd = _dot(mb[g], pqt[ws:ws + T, j * T:(j + 1) * T])
                rden = 1.0 / (nd[T:T + 8] + 1e-6)
                rb = [jnp.broadcast_to(rden[i:i + 1], (8, T)) for i in range(len(heads))]
                blocks = []
                for b in range(T // 8):
                    r_lo, r_hi = 8 * b, 8 * b + 7
                    i_lo = min(max((r_lo + ws) // DH - heads[0], 0), len(heads) - 1)
                    i_hi = min(max((r_hi + ws) // DH - heads[0], 0), len(heads) - 1)
                    if i_lo == i_hi:
                        blocks.append(rb[i_lo])
                    else:
                        cut = (heads[0] + i_hi) * DH - ws - r_lo
                        blocks.append(jnp.where(row8 < cut, rb[i_lo], rb[i_hi]))
                amv = nd[0:T] * jnp.concatenate(blocks, axis=0) * gtab[ws:ws + T, :]
                pltpu.store(am_v.at[ws:ws + T, j * T:(j + 1) * T], amv, mask=wmask)

    def attention(fast):
        ps = (p0, p1)
        if fast:
            _scores_fast(0, kp, qt, ps[0])
            for g in range(NG):
                if g + 1 < NG:
                    _scores_fast(g + 1, kp, qt, ps[(g + 1) % 2])
                _pv(g, vt, ps[g % 2], g1tab, am_v, ot)
        else:
            lax.fori_loop(0, H, lambda h, c: (_attention_safe(h, kp, qt, vt, g1tab, am_v, ot), c)[1], 0)

    def mem_update():
        for g in range(NG):
            ws = WIN * g
            lhs = jnp.concatenate([vt[ws:ws + T, :], ones_rows], axis=0)
            upd = macc[g] + _dot_nt(lhs, pkt[ws:ws + T, :])
            macc[g] = upd
            mb[g] = jnp.where(bmask[g] != 0.0, upd, 0.0).astype(bf16)

    def out_project():
        return _dot_tn(w_in[3], ot[...].astype(bf16))

    def load_weight(i):
        w = w_in[i]
        wf = w.astype(f32)
        c = jnp.sum(wf, axis=0, keepdims=True)
        c_hi = c.astype(bf16).astype(f32)
        r16 = lax.broadcasted_iota(jnp.int32, (16, D), 0)
        extra = jnp.where(r16 >= 4, 0.0, jnp.where(r16 < 2, c_hi, c - c_hi)).astype(bf16)
        w_aug = jnp.concatenate([w, extra, jnp.zeros((KP - D - 16, D), bf16)], axis=0)
        w_t = w_aug.T
        wt[i * D:(i + 1) * D, :] = w_t
        return w_t, jnp.max(jnp.sum(wf * wf, axis=0, keepdims=True))

    am_v[...] = jnp.zeros_like(am_v)
    with _scope("p_tables"):
        small_b.wait()
        small_r.wait()
        build_tables()
    with _scope("p_wq_wait"):
        w_copies[0].wait()
    w_copies[2].start()
    x_copy(1).start()
    w_copies[3].start()
    with _scope("p_wqT"):
        _, cq = load_weight(0)
    with _scope("p_x0_wait"):
        x_copy(0).wait()
    for s in range(2, NSEG):
        x_copy(s).start()
    for c in w_copies[4:]:
        c.start()
    HALF = 288
    with _scope("p_qlo"):
        ln1(0)
        store_q(_dot(wt[0:HALF, :], proj_rhs(0)), ln_scale(0), 0, HALF, False)
    with _scope("p_wk_wait"):
        w_copies[1].wait()
    with _scope("p_qhi_wkT_klo"):
        wk_t, ck = load_weight(1)
        store_q(_dot(wt[HALF:D, :], proj_rhs(0)), ln_scale(0), HALF, D, False)
        store_k_rows(_dot(wk_t[0:HALF], proj_rhs(0)), ln_scale(0), 0, HALF)
    with _scope("p_wv_wait"):
        w_copies[2].wait()
    with _scope("p_khi_wvT_v"):
        wv_t, cv = load_weight(2)
        store_k_rows(_dot(wt[D + HALF:2 * D, :], proj_rhs(0)), ln_scale(0), HALF, D)
        transpose_k()
        store_v(_dot(wv_t, proj_rhs(0)), ln_scale(0))
    slack = 1.05
    logit_bound2 = (cq * ck) * (slack * D * DH * QSCALE) ** 2
    v_bound2 = cv * (slack * D)
    safe = (logit_bound2 <= SAFE_LOGIT ** 2) & (v_bound2 <= SAFE_V ** 2)
    w_copies[3].wait()

    def body(s, carry):
        more = s + 1 < NSEG
        nxt = jnp.minimum(s + 1, NSEG - 1)

        @pl.when(more)
        def _():
            x_copy(nxt).wait()

        @pl.when(safe)
        def _():
            with _scope("attn"):
                attention(True)

        @pl.when(jnp.logical_not(safe))
        def _():
            attention(False)

        @pl.when(more)
        def _():
            with _scope("blockB"):
                hold = {}
                steps = {
                    "MU": mem_update,
                    "OP": lambda: hold.update(a=out_project()),
                    "LN1": lambda: ln1(nxt),
                    "PR": lambda: project(nxt),
                    "MR": mem_read,
                    "FIN": lambda: finalize(s, 0, NT, hold["a"]),
                }
                for n in _ORDER_B:
                    steps[n]()
            out_copy(s).start()
        return carry

    lax.fori_loop(0, NSEG, body, 0)
    with _scope("fin"):
        finalize(NSEG - 1, 0, NT, out_project())
        out_copy(NSEG - 1).start()

    bv = best_v[...]
    rmax = jnp.max(bv, axis=1, keepdims=True)
    cand = best_i[...] + lax.broadcasted_iota(jnp.int32, best_i.shape, 1)
    idx = jnp.clip(jnp.min(jnp.where(bv == rmax, cand, S)), 0, S - 1)
    base = pl.multiple_of((idx // T) * T, T)
    lane = idx - base
    blk = (hbuf[:, pl.ds(base, T)] * ab_all[0:1, pl.ds(base, T)]
           + ab_all[8:9, pl.ds(base, T)]).astype(bf16)
    pick = jnp.where(lax.broadcasted_iota(jnp.int32, (16, T), 1) == lane, 1.0, 0.0).astype(bf16)
    xg = _dot_nt(pick, blk).astype(bf16)
    for c in w_copies[4:]:
        c.wait()
    yacc = jnp.zeros((D, T), f32)
    f_lo = 0
    for nt in _MOE_CHUNKS:
        f_hi = f_lo + nt * T
        gt = _dot(xg, wg_v[:, f_lo:f_hi])
        up = _dot(xg, wu_v[:, f_lo:f_hi])
        act = (gt * jax.nn.sigmoid(gt) * up)[0:1].astype(bf16).astype(f32)
        for t in range(nt):
            f0 = f_lo + t * T
            yacc = yacc + wd_v[:, f0:f0 + T].astype(f32) * act[:, t * T:(t + 1) * T]
        f_lo = f_hi
    y = jnp.sum(yacc, axis=1, keepdims=True) * jax.nn.sigmoid(rmax[0:1])
    for s in range(NSEG):
        out_copy(s).wait()
    sel = lax.broadcasted_iota(jnp.int32, (D, T), 1) == lane
    cur = out_v[:, pl.ds(base, T)].astype(f32)
    out_v[:, pl.ds(base, T)] = (cur + jnp.where(sel, y, 0.0)).astype(bf16)
    patch = pltpu.make_async_copy(out_v.at[:, pl.ds(base, T)],
                                  out_hbm.at[0, :, pl.ds(base, T)], sem_o.at[NSEG])
    patch.start()
    patch.wait()


@jax.jit
def pallas_sequential_preLN__memory_aug_infini_attn__moe_arch_mod__prompt_kernel(
    A_x: jax.Array,
    A_wq: jax.Array,
    A_wk: jax.Array,
    A_wv: jax.Array,
    A_wo: jax.Array,
    A_beta: jax.Array,
    B_x: jax.Array,
    B_w_r: jax.Array,
    B_w_gate: jax.Array,
    B_w_up: jax.Array,
    B_w_down: jax.Array,
):
    del B_x
    hbm_spec = pl.BlockSpec(memory_space=pltpu.HBM)
    scratch = [
        pltpu.VMEM((D, S), bf16),
        pltpu.VMEM((4, D, D), bf16),
        pltpu.VMEM((3 * D, KP), bf16),
        pltpu.VMEM((D, S), f32),
        pltpu.VMEM((D, F), bf16),
        pltpu.VMEM((D, F), bf16),
        pltpu.VMEM((D, F), bf16),
        pltpu.VMEM((16, S), bf16),
        pltpu.VMEM((8, S), f32),
        pltpu.VMEM((D, L), bf16),
        pltpu.VMEM((D, L), bf16),
        pltpu.VMEM((D, L), bf16),
        pltpu.VMEM((D, L), bf16),
        pltpu.VMEM((D, L), bf16),
        pltpu.VMEM((NG, L, T), bf16),
        pltpu.VMEM((7, NT, L, T), bf16),
        pltpu.VMEM((7, NT, L, T), bf16),
        pltpu.VMEM((D, L), f32),
        pltpu.VMEM((D, L), f32),
        pltpu.VMEM((NG, MROWS, T), f32),
        pltpu.VMEM((NG, MROWS, T), bf16),
        pltpu.VMEM((NG, MROWS, T), f32),
        pltpu.VMEM((D, T), f32),
        pltpu.VMEM((H, 8, T), f32),
        pltpu.VMEM((D, T), f32),
        pltpu.VMEM((16, S), f32),
        pltpu.VMEM((D, S), bf16),
        pltpu.VMEM((8, T), f32),
        pltpu.VMEM((8, T), jnp.int32),
        pltpu.VMEM((8, T), f32),
        pltpu.VMEM((H,), bf16),
        pltpu.VMEM((D,), bf16),
        pltpu.SemaphoreType.DMA((NSEG,)),
        pltpu.SemaphoreType.DMA((9,)),
        pltpu.SemaphoreType.DMA((NSEG + 1,)),
    ]
    out_t = pl.pallas_call(
        _kernel,
        out_shape=jax.ShapeDtypeStruct((1, D, S), bf16),
        in_specs=[hbm_spec] * 10,
        out_specs=hbm_spec,
        scratch_shapes=scratch,
        compiler_params=pltpu.CompilerParams(vmem_limit_bytes=100 * 1024 * 1024),
    )(jnp.transpose(A_x, (0, 2, 1)), A_wq, A_wk, A_wv, A_wo, A_beta,
      B_w_r, B_w_gate, B_w_up, B_w_down.T)
    return jnp.transpose(out_t, (0, 2, 1))
```

```python
import contextlib

import jax
import jax.numpy as jnp
from jax import lax
import jax.experimental.pallas as pl
import jax.experimental.pallas.tpu as pltpu

S = 2048
D = 576
H = 32
DH = 18
NSEG = 4
L = 512
F = 4608
T = 128
NT = L // T
EPS = 1e-5
LOG2E = 1.4426950408889634
QSCALE = (DH ** -0.5) * LOG2E
WIN = 112
GROUPS = (tuple(range(0, 7)), tuple(range(7, 13)), tuple(range(13, 19)),
          tuple(range(19, 25)), tuple(range(25, 32)))
NG = len(GROUPS)
KP = 640
MROWS = T + 16
SAFE_LOGIT = 60.0
SAFE_V = 2.0 ** 40

bf16 = jnp.bfloat16
f32 = jnp.float32
_ORDER_B = ["MU", "OP", "LN1", "PR", "MR", "FIN"]
_MOE_CHUNKS = (2,) * 18
_PROFILE = False


def _scope(name):
    return jax.named_scope(name) if _PROFILE else contextlib.nullcontext()


def _colsum(x):
    n = x.shape[0] // 4
    parts = [jnp.sum(x[i * n:(i + 1) * n].reshape(n // 8, 8, x.shape[1]), axis=0) for i in range(4)]
    return jnp.sum((parts[0] + parts[1]) + (parts[2] + parts[3]), axis=0, keepdims=True)


def _ln_stats(x):
    m = _colsum(x) * (1.0 / D)
    v = jnp.maximum(_colsum(x * x) * (1.0 / D) - m * m, 0.0)
    a = lax.rsqrt(v + EPS)
    return a, -m * a


def _phi(t):
    return jnp.where(t > 0, t + 1.0, jnp.exp(t))


def _dot(a, b):
    return jnp.dot(a, b, preferred_element_type=f32)


def _dot_nt(a, b):
    return lax.dot_general(a, b, (((1,), (1,)), ((), ())), preferred_element_type=f32)


def _dot_tn(a, b):
    return lax.dot_general(a, b, (((0,), (0,)), ((), ())), preferred_element_type=f32)


ROT = (0, 1, 2, 3, 0, 2, 1)
QW = T // 4


def _pack_plan(nh, c):
    tiles = []
    split = []
    for u in range(nh):
        need = [(a + ROT[u]) % 4 for a in range(c, 4)]
        for t in tiles:
            if all(t[q] is None for q in need):
                break
        else:
            bound = max(sum(q in [(a + ROT[v]) % 4 for a in range(c, 4)] for v in range(nh))
                        for q in range(4))
            if len(tiles) >= bound:
                split.append((u, need))
                continue
            t = [None] * 4
            tiles.append(t)
        for q in need:
            t[q] = u
    for u, need in split:
        for q in need:
            next(t for t in tiles if t[q] is None)[q] = u
    return tiles


def _masked_q(qt_ref, g, j):
    ws = WIN * g
    row64 = lax.broadcasted_iota(jnp.int32, (64, T), 0)
    qw32 = pltpu.bitcast(qt_ref[ws:ws + T, j * T:(j + 1) * T], jnp.uint32)
    rolled = {0: qw32}
    qms = []
    for u, h in enumerate(GROUPS[g]):
        if ROT[u] not in rolled:
            rolled[ROT[u]] = pltpu.roll(qw32, ROT[u] * QW, axis=1)
        lo2 = (h * DH - ws) // 2
        qmask = (row64 >= lo2) & (row64 < lo2 + DH // 2)
        qms.append(jnp.where(qmask, rolled[ROT[u]], jnp.uint32(0)))
    return qms


def _select_quarters(sources):
    distinct = []
    for x in sources:
        if x is not None and not any(x is y for y in distinct):
            distinct.append(x)
    distinct.sort(key=lambda y: -sum(x is y for x in sources))
    out = distinct[0]
    lane = lax.broadcasted_iota(jnp.int32, out.shape, 1)
    for y in distinct[1:]:
        mask = None
        for q, x in enumerate(sources):
            if x is y:
                m = (lane >= q * QW) & (lane < (q + 1) * QW)
                mask = m if mask is None else mask | m
        out = jnp.where(mask, y, out)
    return out


def _scores_fast(g, kp_ref, qt_ref, p_ref):
    nh = len(GROUPS[g])
    kk = lax.broadcasted_iota(jnp.int32, (T, T), 0)
    qq = lax.broadcasted_iota(jnp.int32, (T, T), 1)
    causal = {r: kk <= ((qq - r * QW) & (T - 1)) for r in set(ROT[:nh])}
    plans = {c: _pack_plan(nh, c) for c in range(1, 4)}
    for j in range(NT):
        qms = _masked_q(qt_ref, g, j)
        n0 = T * j + QW
        p0 = jnp.exp2(_dot(kp_ref[g, 0:n0, :],
                           jnp.concatenate([pltpu.bitcast(q, bf16) for q in qms], axis=1)))
        pc = {}
        for c in range(1, 4):
            w = [pltpu.bitcast(_select_quarters([None if u is None else qms[u] for u in t]), bf16)
                 for t in plans[c]]
            r0 = T * j + c * QW
            pc[c] = jnp.exp2(_dot(kp_ref[g, r0:r0 + QW, :], jnp.concatenate(w, axis=1)))
        for u in range(nh):
            pu = p0[:, u * T:(u + 1) * T]
            if j > 0:
                p_ref[u, j, 0:j * T, :] = pu[0:j * T].astype(bf16)
            rows = [pu[j * T:n0]]
            for c in range(1, 4):
                src = [None] * 4
                for i, t in enumerate(plans[c]):
                    for q in range(4):
                        if t[q] == u:
                            src[q] = i
                vals = {i: pc[c][:, i * T:(i + 1) * T] for i in set(src) if i is not None}
                rows.append(_select_quarters([None if i is None else vals[i] for i in src]))
            p_ref[u, j, j * T:(j + 1) * T, :] = jnp.where(
                causal[ROT[u]], jnp.concatenate(rows, axis=0), 0.0).astype(bf16)


def _attention_safe(h, kp_ref, qt_ref, vt_ref, g1_ref, am_ref, ot_ref):
    g = jnp.minimum(jnp.maximum(h - 1, 0) // 6, NG - 1)
    ws = pl.multiple_of(g * WIN, 16)
    lo = h * DH - ws
    row128 = lax.broadcasted_iota(jnp.int32, (T, T), 0)
    qmask = (row128 >= lo) & (row128 < lo + DH)
    vs = pl.multiple_of(((h * DH) // 16) * 16, 16)
    off = h * DH - vs
    row32 = lax.broadcasted_iota(jnp.int32, (32, T), 0)
    omask = (row32 >= off) & (row32 < off + DH)
    kk = lax.broadcasted_iota(jnp.int32, (L, T), 0)
    qq = lax.broadcasted_iota(jnp.int32, (L, T), 1)

    def tile(j, c):
        c0 = pl.multiple_of(j * T, T)
        qm = jnp.where(qmask, qt_ref[pl.ds(ws, T), pl.ds(c0, T)].astype(f32), 0.0).astype(bf16)
        s = _dot(kp_ref[g], qm)
        s = jnp.where(kk <= qq + c0, s, -jnp.inf)
        m = jnp.max(s, axis=0, keepdims=True)
        p = jnp.exp2(s - m).astype(bf16)
        acc = _dot(_v_rows(vt_ref, vs, off // 2, L), p)
        l8 = jnp.where(off <= 6, acc[24:32], acc[0:8])
        rl = g1_ref[h] / l8
        o = acc * jnp.concatenate([rl] * 4, axis=0) + am_ref[pl.ds(vs, 32), pl.ds(c0, T)]
        pltpu.store(ot_ref.at[pl.ds(vs, 32), pl.ds(c0, T)], o, mask=omask)
        return c

    lax.fori_loop(0, NT, tile, 0)


def _v_rows(vt_ref, vs, off2, nk):
    row16 = lax.broadcasted_iota(jnp.int32, (16, nk), 0)
    keep = (row16 >= off2) & (row16 < off2 + DH // 2)
    v32 = pltpu.bitcast(vt_ref[pl.ds(vs, 32), 0:nk], jnp.uint32)
    return pltpu.bitcast(jnp.where(keep, v32, jnp.uint32(0x3F803F80)), bf16)


def _pv(g, vt_ref, p_ref, g1_ref, am_ref, ot_ref):
    row32 = lax.broadcasted_iota(jnp.int32, (32, T), 0)
    for u, h in enumerate(GROUPS[g]):
        vs = ((h * DH) // 16) * 16
        off = h * DH - vs
        omask = (row32 >= off) & (row32 < off + DH)
        g1 = g1_ref[h]
        vrows = _v_rows(vt_ref, vs, off // 2, L)
        for j in range(NT):
            nk = T * (j + 1)
            acc = _dot(vrows[:, 0:nk], p_ref[u, j, 0:nk, :])
            l8 = acc[24:32] if off <= 6 else acc[0:8]
            rl = g1 / l8
            o = acc * jnp.concatenate([rl] * 4, axis=0)
            if ROT[u]:
                o = pltpu.roll(o, T - ROT[u] * QW, axis=1)
            o = o + am_ref[vs:vs + 32, j * T:(j + 1) * T]
            pltpu.store(ot_ref.at[vs:vs + 32, j * T:(j + 1) * T], o, mask=omask)


def _kernel(x_hbm, wq_hbm, wk_hbm, wv_hbm, wo_hbm, beta_hbm, wr_hbm, wg_hbm, wu_hbm, wd_hbm,
            out_hbm,
            x_v, w_in, wt, hbuf, wg_v, wu_v, wd_v,
            aug, arow, qt, pqt, kt, pkt, vt, kp, p0, p1, am_v, ot,
            macc, mb, bmask, gtab, g1tab, wrtab, ab_all, out_v, best_v, best_i, wrsum, beta_ref, wr_ref,
            sem_x, sem_w, sem_o):
    def x_copy(s):
        return pltpu.make_async_copy(x_hbm.at[0, :, pl.ds(s * L, L)],
                                     x_v.at[:, pl.ds(s * L, L)], sem_x.at[s])

    def out_copy(s):
        return pltpu.make_async_copy(out_v.at[:, pl.ds(s * L, L)],
                                     out_hbm.at[0, :, pl.ds(s * L, L)], sem_o.at[s])

    w_copies = [
        None,
        pltpu.make_async_copy(wk_hbm, w_in.at[1], sem_w.at[1]),
        pltpu.make_async_copy(wv_hbm, w_in.at[2], sem_w.at[2]),
        pltpu.make_async_copy(wo_hbm, w_in.at[3], sem_w.at[3]),
        pltpu.make_async_copy(wg_hbm, wg_v, sem_w.at[4]),
        pltpu.make_async_copy(wu_hbm, wu_v, sem_w.at[5]),
        pltpu.make_async_copy(wd_hbm, wd_v, sem_w.at[6]),
    ]
    small_b = pltpu.make_async_copy(beta_hbm, beta_ref, sem_w.at[7])
    small_r = pltpu.make_async_copy(wr_hbm, wr_ref, sem_w.at[8])
    QLO = 256
    wq_lo = pltpu.make_async_copy(wq_hbm.at[:, 0:QLO], w_in.at[0, :, 0:QLO], sem_w.at[0])
    wq_hi = pltpu.make_async_copy(wq_hbm.at[:, QLO:D], w_in.at[0, :, QLO:D], sem_w.at[9])
    small_b.start()
    small_r.start()
    wq_lo.start()
    x_copy(0).start()

    def build_tables():
        gate = jax.nn.sigmoid(beta_ref[...].astype(f32).reshape(1, H))
        rr = lax.broadcasted_iota(jnp.int32, (D, H), 0)
        hh = lax.broadcasted_iota(jnp.int32, (D, H), 1)
        onehot = (rr >= hh * DH) & (rr < (hh + 1) * DH)
        gcol = jnp.sum(jnp.where(onehot, gate, 0.0), axis=1, keepdims=True)
        gtab[...] = jnp.broadcast_to(gcol, (D, T))
        hh8 = lax.broadcasted_iota(jnp.int32, (8, H), 1)
        for h in range(H):
            gh = jnp.sum(jnp.where(hh8 == h, gate, 0.0), axis=1, keepdims=True)
            g1tab[h] = jnp.broadcast_to(1.0 - gh, (8, T))
        wr_row = wr_ref[...].astype(f32).reshape(1, D)
        wr_pad = jnp.concatenate([wr_row, jnp.zeros((1, 5 * T - D), f32)], axis=1)
        wrtab[...] = jnp.broadcast_to(wr_pad, (T, 5 * T)).T[0:D]
        wrsum[...] = jnp.broadcast_to(jnp.sum(wr_row, axis=1, keepdims=True), wrsum.shape)

    mr = lax.broadcasted_iota(jnp.int32, (MROWS, T), 0)
    mc = lax.broadcasted_iota(jnp.int32, (MROWS, T), 1)
    for g in range(NG):
        ws = WIN * g
        m = jnp.zeros((MROWS, T), jnp.bool_)
        for i, h in enumerate(GROUPS[g]):
            lo = h * DH - ws
            cols = (mc >= lo) & (mc < lo + DH)
            rows = ((mr >= lo) & (mr < lo + DH) & (mr < T)) | (mr == T + i)
            m = m | (cols & rows)
        bmask[g] = jnp.where(m, 1.0, 0.0)
    macc[...] = jnp.zeros_like(macc)
    mb[...] = jnp.zeros_like(mb)
    best_v[...] = jnp.full(best_v.shape, -jnp.inf, f32)
    best_i[...] = jnp.zeros(best_i.shape, jnp.int32)

    ones_rows = jnp.ones((16, L), bf16)

    def ln1(s):
        col0 = pl.multiple_of(s * L, L)
        xs = x_v[:, pl.ds(col0, L)].astype(f32)
        m = _colsum(xs) * (1.0 / D)
        v = jnp.maximum(_colsum(xs * xs) * (1.0 / D) - m * m, 0.0)
        arow[:, pl.ds(col0, L)] = jnp.broadcast_to(lax.rsqrt(v + EPS), (8, L))
        m_hi = (-m).astype(bf16).astype(f32)
        m_lo = -m - m_hi
        r16 = lax.broadcasted_iota(jnp.int32, (16, L), 0)
        rows = jnp.where(r16 >= 4, 0.0, jnp.where((r16 & 1) == 0, m_hi, m_lo))
        aug[:, pl.ds(col0, L)] = rows.astype(bf16)

    def finalize(s, t0, nt, attn):
        w = nt * T
        col0 = pl.multiple_of(s * L + t0 * T, T)
        hres = x_v[:, pl.ds(col0, w)].astype(f32) + attn
        hbuf[:, pl.ds(col0, w)] = hres
        a, b = _ln_stats(hres)
        wr = jnp.concatenate([wrtab[...]] * nt, axis=1)
        r = _colsum(hres * wr) * a + b * wrsum[0:1, 0:1]
        ab_all[0:8, pl.ds(col0, w)] = jnp.broadcast_to(a, (8, w))
        ab_all[8:16, pl.ds(col0, w)] = jnp.broadcast_to(b, (8, w))
        out_v[:, pl.ds(col0, w)] = (hbuf[:, pl.ds(col0, w)] * (1.0 + a) + b).astype(bf16)
        r = r.astype(bf16).astype(f32)
        bv, bi = best_v[0:1, :], best_i[0:1, :]
        for t in range(nt):
            rt = r[:, t * T:(t + 1) * T]
            better = rt > bv
            bi = jnp.where(better, col0 + t * T, bi)
            bv = jnp.where(better, rt, bv)
        best_i[...] = jnp.broadcast_to(bi, best_i.shape)
        best_v[...] = jnp.broadcast_to(bv, best_v.shape)

    def proj_rhs(s):
        col0 = pl.multiple_of(s * L, L)
        return jnp.concatenate([x_v[:, pl.ds(col0, L)], aug[:, pl.ds(col0, L)],
                                jnp.zeros((KP - D - 16, L), bf16)], axis=0)

    def ln_scale(s):
        return arow[0:1, pl.ds(pl.multiple_of(s * L, L), L)]

    def store_q(raw, a, r0, r1, with_phi=True):
        qt[r0:r1, :] = (raw * (a * QSCALE)).astype(bf16)
        if with_phi:
            pqt[r0:r1, :] = _phi(raw * a).astype(bf16)

    def store_k_rows(raw, a, r0, r1):
        k = raw * a
        kt[r0:r1, :] = k.astype(bf16)
        pkt[r0:r1, :] = _phi(k).astype(bf16)

    def transpose_k():
        for g in range(NG):
            kp[g] = kt[WIN * g:WIN * g + T, :].T

    def store_k(raw, a):
        k = raw * a
        kb = k.astype(bf16)
        pkt[...] = _phi(k).astype(bf16)
        for g in range(NG):
            kp[g] = kb[WIN * g:WIN * g + T, :].T

    def store_v(raw, a):
        vt[...] = (raw * a).astype(bf16)

    def project(s):
        qkv = _dot(wt[...], proj_rhs(s))
        a = ln_scale(s)
        store_q(qkv[0:D], a, 0, D)
        store_k(qkv[D:2 * D], a)
        store_v(qkv[2 * D:3 * D], a)

    def mem_read():
        row128 = lax.broadcasted_iota(jnp.int32, (T, T), 0)
        row8 = lax.broadcasted_iota(jnp.int32, (8, T), 0)
        for g in range(NG):
            ws = WIN * g
            heads = GROUPS[g]
            lo_g, hi_g = heads[0] * DH - ws, (heads[-1] + 1) * DH - ws
            wmask = (row128 >= lo_g) & (row128 < hi_g)
            for j in range(NT):
                nd = _dot(mb[g], pqt[ws:ws + T, j * T:(j + 1) * T])
                rden = 1.0 / (nd[T:T + 8] + 1e-6)
                rb = [jnp.broadcast_to(rden[i:i + 1], (8, T)) for i in range(len(heads))]
                blocks = []
                for b in range(T // 8):
                    r_lo, r_hi = 8 * b, 8 * b + 7
                    i_lo = min(max((r_lo + ws) // DH - heads[0], 0), len(heads) - 1)
                    i_hi = min(max((r_hi + ws) // DH - heads[0], 0), len(heads) - 1)
                    if i_lo == i_hi:
                        blocks.append(rb[i_lo])
                    else:
                        cut = (heads[0] + i_hi) * DH - ws - r_lo
                        blocks.append(jnp.where(row8 < cut, rb[i_lo], rb[i_hi]))
                amv = nd[0:T] * jnp.concatenate(blocks, axis=0) * gtab[ws:ws + T, :]
                pltpu.store(am_v.at[ws:ws + T, j * T:(j + 1) * T], amv, mask=wmask)

    def attention(fast):
        ps = (p0, p1)
        if fast:
            _scores_fast(0, kp, qt, ps[0])
            for g in range(NG):
                if g + 1 < NG:
                    _scores_fast(g + 1, kp, qt, ps[(g + 1) % 2])
                _pv(g, vt, ps[g % 2], g1tab, am_v, ot)
        else:
            lax.fori_loop(0, H, lambda h, c: (_attention_safe(h, kp, qt, vt, g1tab, am_v, ot), c)[1], 0)

    def mem_update():
        for g in range(NG):
            ws = WIN * g
            lhs = jnp.concatenate([vt[ws:ws + T, :], ones_rows], axis=0)
            upd = macc[g] + _dot_nt(lhs, pkt[ws:ws + T, :])
            macc[g] = upd
            mb[g] = jnp.where(bmask[g] != 0.0, upd, 0.0).astype(bf16)

    def out_project():
        return _dot_tn(w_in[3], ot[...].astype(bf16))

    def load_weight(i, c0=0, c1=D):
        w = w_in[i, :, c0:c1]
        n = c1 - c0
        wf = w.astype(f32)
        c = jnp.sum(wf, axis=0, keepdims=True)
        c_hi = c.astype(bf16).astype(f32)
        r16 = lax.broadcasted_iota(jnp.int32, (16, n), 0)
        extra = jnp.where(r16 >= 4, 0.0, jnp.where(r16 < 2, c_hi, c - c_hi)).astype(bf16)
        w_aug = jnp.concatenate([w, extra, jnp.zeros((KP - D - 16, n), bf16)], axis=0)
        w_t = w_aug.T
        wt[i * D + c0:i * D + c1, :] = w_t
        return w_t, jnp.max(jnp.sum(wf * wf, axis=0, keepdims=True))

    am_v[...] = jnp.zeros_like(am_v)
    with _scope("p_tables"):
        small_b.wait()
        small_r.wait()
        build_tables()
    with _scope("p_wq_wait"):
        wq_lo.wait()
    wq_hi.start()
    w_copies[1].start()
    with _scope("p_wqT"):
        _, cq_lo = load_weight(0, 0, QLO)
    with _scope("p_x0_wait"):
        x_copy(0).wait()
    w_copies[2].start()
    x_copy(1).start()
    w_copies[3].start()
    HALF = 288
    with _scope("p_qlo"):
        ln1(0)
        store_q(_dot(wt[0:QLO, :], proj_rhs(0)), ln_scale(0), 0, QLO, False)
    with _scope("p_wqhi_wait"):
        wq_hi.wait()
    for s in range(2, NSEG):
        x_copy(s).start()
    for c in w_copies[4:]:
        c.start()
    with _scope("p_qmid"):
        wq_t, cq_hi = load_weight(0, QLO, D)
        cq = jnp.maximum(cq_lo, cq_hi)
    with _scope("p_wk_wait"):
        w_copies[1].wait()
    with _scope("p_qhi_wkT_klo"):
        wk_t, ck = load_weight(1)
        store_q(_dot(wt[QLO:D, :], proj_rhs(0)), ln_scale(0), QLO, D, False)
        store_k_rows(_dot(wk_t[0:HALF], proj_rhs(0)), ln_scale(0), 0, HALF)
    with _scope("p_wv_wait"):
        w_copies[2].wait()
    with _scope("p_khi_wvT_v"):
        wv_t, cv = load_weight(2)
        store_k_rows(_dot(wt[D + HALF:2 * D, :], proj_rhs(0)), ln_scale(0), HALF, D)
        transpose_k()
        store_v(_dot(wv_t, proj_rhs(0)), ln_scale(0))
    slack = 1.05
    logit_bound2 = (cq * ck) * (slack * D * DH * QSCALE) ** 2
    v_bound2 = cv * (slack * D)
    safe = (logit_bound2 <= SAFE_LOGIT ** 2) & (v_bound2 <= SAFE_V ** 2)
    w_copies[3].wait()

    def body(s, carry):
        more = s + 1 < NSEG
        nxt = jnp.minimum(s + 1, NSEG - 1)

        @pl.when(more)
        def _():
            x_copy(nxt).wait()

        @pl.when(safe)
        def _():
            with _scope("attn"):
                attention(True)

        @pl.when(jnp.logical_not(safe))
        def _():
            attention(False)

        @pl.when(more)
        def _():
            with _scope("blockB"):
                hold = {}
                steps = {
                    "MU": mem_update,
                    "OP": lambda: hold.update(a=out_project()),
                    "LN1": lambda: ln1(nxt),
                    "PR": lambda: project(nxt),
                    "MR": mem_read,
                    "FIN": lambda: finalize(s, 0, NT, hold["a"]),
                }
                for n in _ORDER_B:
                    steps[n]()
            out_copy(s).start()
        return carry

    lax.fori_loop(0, NSEG, body, 0)
    with _scope("fin"):
        finalize(NSEG - 1, 0, NT, out_project())
        out_copy(NSEG - 1).start()

    bv = best_v[...]
    rmax = jnp.max(bv, axis=1, keepdims=True)
    cand = best_i[...] + lax.broadcasted_iota(jnp.int32, best_i.shape, 1)
    idx = jnp.clip(jnp.min(jnp.where(bv == rmax, cand, S)), 0, S - 1)
    base = pl.multiple_of((idx // T) * T, T)
    lane = idx - base
    blk = (hbuf[:, pl.ds(base, T)] * ab_all[0:1, pl.ds(base, T)]
           + ab_all[8:9, pl.ds(base, T)]).astype(bf16)
    pick = jnp.where(lax.broadcasted_iota(jnp.int32, (16, T), 1) == lane, 1.0, 0.0).astype(bf16)
    xg = _dot_nt(pick, blk).astype(bf16)
    for c in w_copies[4:]:
        c.wait()
    yacc = jnp.zeros((D, T), f32)
    f_lo = 0
    for nt in _MOE_CHUNKS:
        f_hi = f_lo + nt * T
        gt = _dot(xg, wg_v[:, f_lo:f_hi])
        up = _dot(xg, wu_v[:, f_lo:f_hi])
        act = (gt * jax.nn.sigmoid(gt) * up)[0:1].astype(bf16).astype(f32)
        for t in range(nt):
            f0 = f_lo + t * T
            yacc = yacc + wd_v[:, f0:f0 + T].astype(f32) * act[:, t * T:(t + 1) * T]
        f_lo = f_hi
    y = jnp.sum(yacc, axis=1, keepdims=True) * jax.nn.sigmoid(rmax[0:1])
    for s in range(NSEG):
        out_copy(s).wait()
    sel = lax.broadcasted_iota(jnp.int32, (D, T), 1) == lane
    cur = out_v[:, pl.ds(base, T)].astype(f32)
    out_v[:, pl.ds(base, T)] = (cur + jnp.where(sel, y, 0.0)).astype(bf16)
    patch = pltpu.make_async_copy(out_v.at[:, pl.ds(base, T)],
                                  out_hbm.at[0, :, pl.ds(base, T)], sem_o.at[NSEG])
    patch.start()
    patch.wait()


@jax.jit
def pallas_sequential_preLN__memory_aug_infini_attn__moe_arch_mod__prompt_kernel(
    A_x: jax.Array,
    A_wq: jax.Array,
    A_wk: jax.Array,
    A_wv: jax.Array,
    A_wo: jax.Array,
    A_beta: jax.Array,
    B_x: jax.Array,
    B_w_r: jax.Array,
    B_w_gate: jax.Array,
    B_w_up: jax.Array,
    B_w_down: jax.Array,
):
    del B_x
    hbm_spec = pl.BlockSpec(memory_space=pltpu.HBM)
    scratch = [
        pltpu.VMEM((D, S), bf16),
        pltpu.VMEM((4, D, D), bf16),
        pltpu.VMEM((3 * D, KP), bf16),
        pltpu.VMEM((D, S), f32),
        pltpu.VMEM((D, F), bf16),
        pltpu.VMEM((D, F), bf16),
        pltpu.VMEM((D, F), bf16),
        pltpu.VMEM((16, S), bf16),
        pltpu.VMEM((8, S), f32),
        pltpu.VMEM((D, L), bf16),
        pltpu.VMEM((D, L), bf16),
        pltpu.VMEM((D, L), bf16),
        pltpu.VMEM((D, L), bf16),
        pltpu.VMEM((D, L), bf16),
        pltpu.VMEM((NG, L, T), bf16),
        pltpu.VMEM((7, NT, L, T), bf16),
        pltpu.VMEM((7, NT, L, T), bf16),
        pltpu.VMEM((D, L), f32),
        pltpu.VMEM((D, L), f32),
        pltpu.VMEM((NG, MROWS, T), f32),
        pltpu.VMEM((NG, MROWS, T), bf16),
        pltpu.VMEM((NG, MROWS, T), f32),
        pltpu.VMEM((D, T), f32),
        pltpu.VMEM((H, 8, T), f32),
        pltpu.VMEM((D, T), f32),
        pltpu.VMEM((16, S), f32),
        pltpu.VMEM((D, S), bf16),
        pltpu.VMEM((8, T), f32),
        pltpu.VMEM((8, T), jnp.int32),
        pltpu.VMEM((8, T), f32),
        pltpu.VMEM((H,), bf16),
        pltpu.VMEM((D,), bf16),
        pltpu.SemaphoreType.DMA((NSEG,)),
        pltpu.SemaphoreType.DMA((10,)),
        pltpu.SemaphoreType.DMA((NSEG + 1,)),
    ]
    out_t = pl.pallas_call(
        _kernel,
        out_shape=jax.ShapeDtypeStruct((1, D, S), bf16),
        in_specs=[hbm_spec] * 10,
        out_specs=hbm_spec,
        scratch_shapes=scratch,
        compiler_params=pltpu.CompilerParams(vmem_limit_bytes=100 * 1024 * 1024),
    )(jnp.transpose(A_x, (0, 2, 1)), A_wq, A_wk, A_wv, A_wo, A_beta,
      B_w_r, B_w_gate, B_w_up, B_w_down.T)
    return jnp.transpose(out_t, (0, 2, 1))
```

```python
import contextlib

import jax
import jax.numpy as jnp
from jax import lax
import jax.experimental.pallas as pl
import jax.experimental.pallas.tpu as pltpu

S = 2048
D = 576
H = 32
DH = 18
NSEG = 4
L = 512
F = 4608
T = 128
NT = L // T
EPS = 1e-5
LOG2E = 1.4426950408889634
QSCALE = (DH ** -0.5) * LOG2E
WIN = 112
GROUPS = (tuple(range(0, 7)), tuple(range(7, 13)), tuple(range(13, 19)),
          tuple(range(19, 25)), tuple(range(25, 32)))
NG = len(GROUPS)
KP = 640
MROWS = T + 16
SAFE_LOGIT = 60.0
SAFE_V = 2.0 ** 40

bf16 = jnp.bfloat16
f32 = jnp.float32
_ORDER_B = ["MU", "OP", "LN1", "PR", "MR", "FIN"]
_MOE_CHUNKS = (2,) * 18
_PROFILE = False


def _scope(name):
    return jax.named_scope(name) if _PROFILE else contextlib.nullcontext()


def _colsum(x):
    n = x.shape[0] // 4
    parts = [jnp.sum(x[i * n:(i + 1) * n].reshape(n // 8, 8, x.shape[1]), axis=0) for i in range(4)]
    return jnp.sum((parts[0] + parts[1]) + (parts[2] + parts[3]), axis=0, keepdims=True)


def _ln_stats(x):
    m = _colsum(x) * (1.0 / D)
    v = jnp.maximum(_colsum(x * x) * (1.0 / D) - m * m, 0.0)
    a = lax.rsqrt(v + EPS)
    return a, -m * a


def _phi(t):
    return jnp.where(t > 0, t + 1.0, jnp.exp(t))


def _dot(a, b):
    return jnp.dot(a, b, preferred_element_type=f32)


def _dot_nt(a, b):
    return lax.dot_general(a, b, (((1,), (1,)), ((), ())), preferred_element_type=f32)


def _dot_tn(a, b):
    return lax.dot_general(a, b, (((0,), (0,)), ((), ())), preferred_element_type=f32)


ROT = (0, 1, 2, 3, 0, 2, 1)
QW = T // 4


def _pack_plan(nh, c):
    tiles = []
    split = []
    for u in range(nh):
        need = [(a + ROT[u]) % 4 for a in range(c, 4)]
        for t in tiles:
            if all(t[q] is None for q in need):
                break
        else:
            bound = max(sum(q in [(a + ROT[v]) % 4 for a in range(c, 4)] for v in range(nh))
                        for q in range(4))
            if len(tiles) >= bound:
                split.append((u, need))
                continue
            t = [None] * 4
            tiles.append(t)
        for q in need:
            t[q] = u
    for u, need in split:
        for q in need:
            next(t for t in tiles if t[q] is None)[q] = u
    return tiles


def _masked_q(qt_ref, g, j):
    ws = WIN * g
    row64 = lax.broadcasted_iota(jnp.int32, (64, T), 0)
    qw32 = pltpu.bitcast(qt_ref[ws:ws + T, j * T:(j + 1) * T], jnp.uint32)
    rolled = {0: qw32}
    qms = []
    for u, h in enumerate(GROUPS[g]):
        if ROT[u] not in rolled:
            rolled[ROT[u]] = pltpu.roll(qw32, ROT[u] * QW, axis=1)
        lo2 = (h * DH - ws) // 2
        qmask = (row64 >= lo2) & (row64 < lo2 + DH // 2)
        qms.append(jnp.where(qmask, rolled[ROT[u]], jnp.uint32(0)))
    return qms


def _select_quarters(sources):
    distinct = []
    for x in sources:
        if x is not None and not any(x is y for y in distinct):
            distinct.append(x)
    distinct.sort(key=lambda y: -sum(x is y for x in sources))
    out = distinct[0]
    lane = lax.broadcasted_iota(jnp.int32, out.shape, 1)
    for y in distinct[1:]:
        mask = None
        for q, x in enumerate(sources):
            if x is y:
                m = (lane >= q * QW) & (lane < (q + 1) * QW)
                mask = m if mask is None else mask | m
        out = jnp.where(mask, y, out)
    return out


def _scores_fast(g, kp_ref, qt_ref, p_ref):
    nh = len(GROUPS[g])
    kk = lax.broadcasted_iota(jnp.int32, (T, T), 0)
    qq = lax.broadcasted_iota(jnp.int32, (T, T), 1)
    causal = {r: kk <= ((qq - r * QW) & (T - 1)) for r in set(ROT[:nh])}
    plans = {c: _pack_plan(nh, c) for c in range(1, 4)}
    for j in range(NT):
        qms = _masked_q(qt_ref, g, j)
        n0 = T * j + QW
        p0 = jnp.exp2(_dot(kp_ref[g, 0:n0, :],
                           jnp.concatenate([pltpu.bitcast(q, bf16) for q in qms], axis=1)))
        pc = {}
        for c in range(1, 4):
            w = [pltpu.bitcast(_select_quarters([None if u is None else qms[u] for u in t]), bf16)
                 for t in plans[c]]
            r0 = T * j + c * QW
            pc[c] = jnp.exp2(_dot(kp_ref[g, r0:r0 + QW, :], jnp.concatenate(w, axis=1)))
        for u in range(nh):
            pu = p0[:, u * T:(u + 1) * T]
            if j > 0:
                p_ref[u, j, 0:j * T, :] = pu[0:j * T].astype(bf16)
            rows = [pu[j * T:n0]]
            for c in range(1, 4):
                src = [None] * 4
                for i, t in enumerate(plans[c]):
                    for q in range(4):
                        if t[q] == u:
                            src[q] = i
                vals = {i: pc[c][:, i * T:(i + 1) * T] for i in set(src) if i is not None}
                rows.append(_select_quarters([None if i is None else vals[i] for i in src]))
            p_ref[u, j, j * T:(j + 1) * T, :] = jnp.where(
                causal[ROT[u]], jnp.concatenate(rows, axis=0), 0.0).astype(bf16)


def _attention_safe(h, kp_ref, qt_ref, vt_ref, g1_ref, am_ref, ot_ref):
    g = jnp.minimum(jnp.maximum(h - 1, 0) // 6, NG - 1)
    ws = pl.multiple_of(g * WIN, 16)
    lo = h * DH - ws
    row128 = lax.broadcasted_iota(jnp.int32, (T, T), 0)
    qmask = (row128 >= lo) & (row128 < lo + DH)
    vs = pl.multiple_of(((h * DH) // 16) * 16, 16)
    off = h * DH - vs
    row32 = lax.broadcasted_iota(jnp.int32, (32, T), 0)
    omask = (row32 >= off) & (row32 < off + DH)
    kk = lax.broadcasted_iota(jnp.int32, (L, T), 0)
    qq = lax.broadcasted_iota(jnp.int32, (L, T), 1)

    def tile(j, c):
        c0 = pl.multiple_of(j * T, T)
        qm = jnp.where(qmask, qt_ref[pl.ds(ws, T), pl.ds(c0, T)].astype(f32), 0.0).astype(bf16)
        s = _dot(kp_ref[g], qm)
        s = jnp.where(kk <= qq + c0, s, -jnp.inf)
        m = jnp.max(s, axis=0, keepdims=True)
        p = jnp.exp2(s - m).astype(bf16)
        acc = _dot(_v_rows(vt_ref, vs, off // 2, L), p)
        l8 = jnp.where(off <= 6, acc[24:32], acc[0:8])
        rl = g1_ref[h] / l8
        o = acc * jnp.concatenate([rl] * 4, axis=0) + am_ref[pl.ds(vs, 32), pl.ds(c0, T)]
        pltpu.store(ot_ref.at[pl.ds(vs, 32), pl.ds(c0, T)], o, mask=omask)
        return c

    lax.fori_loop(0, NT, tile, 0)


def _v_rows(vt_ref, vs, off2, nk):
    row16 = lax.broadcasted_iota(jnp.int32, (16, nk), 0)
    keep = (row16 >= off2) & (row16 < off2 + DH // 2)
    v32 = pltpu.bitcast(vt_ref[pl.ds(vs, 32), 0:nk], jnp.uint32)
    return pltpu.bitcast(jnp.where(keep, v32, jnp.uint32(0x3F803F80)), bf16)


def _pv(g, vt_ref, p_ref, g1_ref, am_ref, ot_ref):
    row32 = lax.broadcasted_iota(jnp.int32, (32, T), 0)
    for u, h in enumerate(GROUPS[g]):
        vs = ((h * DH) // 16) * 16
        off = h * DH - vs
        omask = (row32 >= off) & (row32 < off + DH)
        g1 = g1_ref[h]
        vrows = _v_rows(vt_ref, vs, off // 2, L)
        for j in range(NT):
            nk = T * (j + 1)
            acc = _dot(vrows[:, 0:nk], p_ref[u, j, 0:nk, :])
            l8 = acc[24:32] if off <= 6 else acc[0:8]
            rl = g1 / l8
            o = acc * jnp.concatenate([rl] * 4, axis=0)
            if ROT[u]:
                o = pltpu.roll(o, T - ROT[u] * QW, axis=1)
            o = o + am_ref[vs:vs + 32, j * T:(j + 1) * T]
            pltpu.store(ot_ref.at[vs:vs + 32, j * T:(j + 1) * T], o, mask=omask)


def _kernel(x_hbm, wq_hbm, wk_hbm, wv_hbm, wo_hbm, beta_hbm, wr_hbm, wg_hbm, wu_hbm, wd_hbm,
            out_hbm,
            x_v, w_in, wt, wot, hbuf, wg_v, wu_v, wd_v,
            aug, arow, qt, pqt, kt, pkt, vt, kp, p0, p1, am_v, ot,
            macc, mb, bmask, gtab, g1tab, wrtab, ab_all, out_v, best_v, best_i, wrsum, beta_ref, wr_ref,
            sem_x, sem_w, sem_o):
    def x_copy(s):
        return pltpu.make_async_copy(x_hbm.at[0, :, pl.ds(s * L, L)],
                                     x_v.at[:, pl.ds(s * L, L)], sem_x.at[s])

    def out_copy(s):
        return pltpu.make_async_copy(out_v.at[:, pl.ds(s * L, L)],
                                     out_hbm.at[0, :, pl.ds(s * L, L)], sem_o.at[s])

    w_copies = [
        None,
        pltpu.make_async_copy(wk_hbm, w_in.at[1], sem_w.at[1]),
        pltpu.make_async_copy(wv_hbm, w_in.at[2], sem_w.at[2]),
        pltpu.make_async_copy(wo_hbm, w_in.at[3], sem_w.at[3]),
        pltpu.make_async_copy(wg_hbm, wg_v, sem_w.at[4]),
        pltpu.make_async_copy(wu_hbm, wu_v, sem_w.at[5]),
        pltpu.make_async_copy(wd_hbm, wd_v, sem_w.at[6]),
    ]
    small_b = pltpu.make_async_copy(beta_hbm, beta_ref, sem_w.at[7])
    small_r = pltpu.make_async_copy(wr_hbm, wr_ref, sem_w.at[8])
    QLO = 256
    wq_lo = pltpu.make_async_copy(wq_hbm.at[:, 0:QLO], w_in.at[0, :, 0:QLO], sem_w.at[0])
    wq_hi = pltpu.make_async_copy(wq_hbm.at[:, QLO:D], w_in.at[0, :, QLO:D], sem_w.at[9])
    small_b.start()
    small_r.start()
    wq_lo.start()
    x_copy(0).start()

    def build_tables():
        gate = jax.nn.sigmoid(beta_ref[...].astype(f32).reshape(1, H))
        rr = lax.broadcasted_iota(jnp.int32, (D, H), 0)
        hh = lax.broadcasted_iota(jnp.int32, (D, H), 1)
        onehot = (rr >= hh * DH) & (rr < (hh + 1) * DH)
        gcol = jnp.sum(jnp.where(onehot, gate, 0.0), axis=1, keepdims=True)
        gtab[...] = jnp.broadcast_to(gcol, (D, T))
        hh8 = lax.broadcasted_iota(jnp.int32, (8, H), 1)
        for h in range(H):
            gh = jnp.sum(jnp.where(hh8 == h, gate, 0.0), axis=1, keepdims=True)
            g1tab[h] = jnp.broadcast_to(1.0 - gh, (8, T))
        wr_row = wr_ref[...].astype(f32).reshape(1, D)
        wr_pad = jnp.concatenate([wr_row, jnp.zeros((1, 5 * T - D), f32)], axis=1)
        wrtab[...] = jnp.broadcast_to(wr_pad, (T, 5 * T)).T[0:D]
        wrsum[...] = jnp.broadcast_to(jnp.sum(wr_row, axis=1, keepdims=True), wrsum.shape)

    mr = lax.broadcasted_iota(jnp.int32, (MROWS, T), 0)
    mc = lax.broadcasted_iota(jnp.int32, (MROWS, T), 1)
    for g in range(NG):
        ws = WIN * g
        m = jnp.zeros((MROWS, T), jnp.bool_)
        for i, h in enumerate(GROUPS[g]):
            lo = h * DH - ws
            cols = (mc >= lo) & (mc < lo + DH)
            rows = ((mr >= lo) & (mr < lo + DH) & (mr < T)) | (mr == T + i)
            m = m | (cols & rows)
        bmask[g] = jnp.where(m, 1.0, 0.0)
    macc[...] = jnp.zeros_like(macc)
    mb[...] = jnp.zeros_like(mb)
    best_v[...] = jnp.full(best_v.shape, -jnp.inf, f32)
    best_i[...] = jnp.zeros(best_i.shape, jnp.int32)

    ones_rows = jnp.ones((16, L), bf16)

    def ln1(s):
        col0 = pl.multiple_of(s * L, L)
        xs = x_v[:, pl.ds(col0, L)].astype(f32)
        m = _colsum(xs) * (1.0 / D)
        v = jnp.maximum(_colsum(xs * xs) * (1.0 / D) - m * m, 0.0)
        arow[:, pl.ds(col0, L)] = jnp.broadcast_to(lax.rsqrt(v + EPS), (8, L))
        m_hi = (-m).astype(bf16).astype(f32)
        m_lo = -m - m_hi
        r16 = lax.broadcasted_iota(jnp.int32, (16, L), 0)
        rows = jnp.where(r16 >= 4, 0.0, jnp.where((r16 & 1) == 0, m_hi, m_lo))
        aug[:, pl.ds(col0, L)] = rows.astype(bf16)

    def finalize(s, t0, nt, attn):
        w = nt * T
        col0 = pl.multiple_of(s * L + t0 * T, T)
        hres = x_v[:, pl.ds(col0, w)].astype(f32) + attn
        hbuf[:, pl.ds(col0, w)] = hres
        a, b = _ln_stats(hres)
        wr = jnp.concatenate([wrtab[...]] * nt, axis=1)
        r = _colsum(hres * wr) * a + b * wrsum[0:1, 0:1]
        ab_all[0:8, pl.ds(col0, w)] = jnp.broadcast_to(a, (8, w))
        ab_all[8:16, pl.ds(col0, w)] = jnp.broadcast_to(b, (8, w))
        out_v[:, pl.ds(col0, w)] = (hbuf[:, pl.ds(col0, w)] * (1.0 + a) + b).astype(bf16)
        r = r.astype(bf16).astype(f32)
        bv, bi = best_v[0:1, :], best_i[0:1, :]
        for t in range(nt):
            rt = r[:, t * T:(t + 1) * T]
            better = rt > bv
            bi = jnp.where(better, col0 + t * T, bi)
            bv = jnp.where(better, rt, bv)
        best_i[...] = jnp.broadcast_to(bi, best_i.shape)
        best_v[...] = jnp.broadcast_to(bv, best_v.shape)

    def proj_rhs(s):
        col0 = pl.multiple_of(s * L, L)
        return jnp.concatenate([x_v[:, pl.ds(col0, L)], aug[:, pl.ds(col0, L)],
                                jnp.zeros((KP - D - 16, L), bf16)], axis=0)

    def ln_scale(s):
        return arow[0:1, pl.ds(pl.multiple_of(s * L, L), L)]

    def store_q(raw, a, r0, r1, with_phi=True):
        qt[r0:r1, :] = (raw * (a * QSCALE)).astype(bf16)
        if with_phi:
            pqt[r0:r1, :] = _phi(raw * a).astype(bf16)

    def store_k_rows(raw, a, r0, r1):
        k = raw * a
        kt[r0:r1, :] = k.astype(bf16)
        pkt[r0:r1, :] = _phi(k).astype(bf16)

    def transpose_k():
        for g in range(NG):
            kp[g] = kt[WIN * g:WIN * g + T, :].T

    def store_k(raw, a):
        k = raw * a
        kb = k.astype(bf16)
        pkt[...] = _phi(k).astype(bf16)
        for g in range(NG):
            kp[g] = kb[WIN * g:WIN * g + T, :].T

    def store_v(raw, a):
        vt[...] = (raw * a).astype(bf16)

    def project(s):
        qkv = _dot(wt[...], proj_rhs(s))
        a = ln_scale(s)
        store_q(qkv[0:D], a, 0, D)
        store_k(qkv[D:2 * D], a)
        store_v(qkv[2 * D:3 * D], a)

    def mem_read():
        row128 = lax.broadcasted_iota(jnp.int32, (T, T), 0)
        row8 = lax.broadcasted_iota(jnp.int32, (8, T), 0)
        for g in range(NG):
            ws = WIN * g
            heads = GROUPS[g]
            lo_g, hi_g = heads[0] * DH - ws, (heads[-1] + 1) * DH - ws
            wmask = (row128 >= lo_g) & (row128 < hi_g)
            for j in range(NT):
                nd = _dot(mb[g], pqt[ws:ws + T, j * T:(j + 1) * T])
                rden = 1.0 / (nd[T:T + 8] + 1e-6)
                rb = [jnp.broadcast_to(rden[i:i + 1], (8, T)) for i in range(len(heads))]
                blocks = []
                for b in range(T // 8):
                    r_lo, r_hi = 8 * b, 8 * b + 7
                    i_lo = min(max((r_lo + ws) // DH - heads[0], 0), len(heads) - 1)
                    i_hi = min(max((r_hi + ws) // DH - heads[0], 0), len(heads) - 1)
                    if i_lo == i_hi:
                        blocks.append(rb[i_lo])
                    else:
                        cut = (heads[0] + i_hi) * DH - ws - r_lo
                        blocks.append(jnp.where(row8 < cut, rb[i_lo], rb[i_hi]))
                amv = nd[0:T] * jnp.concatenate(blocks, axis=0) * gtab[ws:ws + T, :]
                pltpu.store(am_v.at[ws:ws + T, j * T:(j + 1) * T], amv, mask=wmask)

    def attention(fast):
        ps = (p0, p1)
        if fast:
            _scores_fast(0, kp, qt, ps[0])
            for g in range(NG):
                if g + 1 < NG:
                    _scores_fast(g + 1, kp, qt, ps[(g + 1) % 2])
                _pv(g, vt, ps[g % 2], g1tab, am_v, ot)
        else:
            lax.fori_loop(0, H, lambda h, c: (_attention_safe(h, kp, qt, vt, g1tab, am_v, ot), c)[1], 0)

    def mem_update():
        for g in range(NG):
            ws = WIN * g
            lhs = jnp.concatenate([vt[ws:ws + T, :], ones_rows], axis=0)
            upd = macc[g] + _dot_nt(lhs, pkt[ws:ws + T, :])
            macc[g] = upd
            mb[g] = jnp.where(bmask[g] != 0.0, upd, 0.0).astype(bf16)

    def out_project():
        return _dot(wot[...], ot[...].astype(bf16))

    def load_weight(i, c0=0, c1=D):
        w = w_in[i, :, c0:c1]
        n = c1 - c0
        wf = w.astype(f32)
        c = jnp.sum(wf, axis=0, keepdims=True)
        c_hi = c.astype(bf16).astype(f32)
        r16 = lax.broadcasted_iota(jnp.int32, (16, n), 0)
        extra = jnp.where(r16 >= 4, 0.0, jnp.where(r16 < 2, c_hi, c - c_hi)).astype(bf16)
        w_aug = jnp.concatenate([w, extra, jnp.zeros((KP - D - 16, n), bf16)], axis=0)
        w_t = w_aug.T
        wt[i * D + c0:i * D + c1, :] = w_t
        return w_t, jnp.max(jnp.sum(wf * wf, axis=0, keepdims=True))

    am_v[...] = jnp.zeros_like(am_v)
    ot[...] = jnp.zeros_like(ot)
    with _scope("p_tables"):
        small_b.wait()
        small_r.wait()
        build_tables()
    with _scope("p_wq_wait"):
        wq_lo.wait()
    wq_hi.start()
    w_copies[1].start()
    with _scope("p_wqT"):
        _, cq_lo = load_weight(0, 0, QLO)
    with _scope("p_x0_wait"):
        x_copy(0).wait()
    w_copies[2].start()
    x_copy(1).start()
    w_copies[3].start()
    HALF = 288
    with _scope("p_qlo"):
        ln1(0)
        store_q(_dot(wt[0:QLO, :], proj_rhs(0)), ln_scale(0), 0, QLO, False)
    with _scope("p_wqhi_wait"):
        wq_hi.wait()
    for s in range(2, NSEG):
        x_copy(s).start()
    for c in w_copies[4:]:
        c.start()
    with _scope("p_qmid"):
        wq_t, cq_hi = load_weight(0, QLO, D)
        cq = jnp.maximum(cq_lo, cq_hi)
    with _scope("p_wk_wait"):
        w_copies[1].wait()
    with _scope("p_qhi_wkT_klo"):
        wk_t, ck = load_weight(1)
        store_q(_dot(wt[QLO:D, :], proj_rhs(0)), ln_scale(0), QLO, D, False)
        store_k_rows(_dot(wk_t[0:HALF], proj_rhs(0)), ln_scale(0), 0, HALF)
    with _scope("p_wv_wait"):
        w_copies[2].wait()
        w_copies[3].wait()
    with _scope("p_khi_wvT_v"):
        wv_t, cv = load_weight(2)
        wot[...] = w_in[3].T
        store_k_rows(_dot(wt[D + HALF:2 * D, :], proj_rhs(0)), ln_scale(0), HALF, D)
        transpose_k()
        store_v(_dot(wv_t, proj_rhs(0)), ln_scale(0))
    slack = 1.05
    logit_bound2 = (cq * ck) * (slack * D * DH * QSCALE) ** 2
    v_bound2 = cv * (slack * D)
    safe = (logit_bound2 <= SAFE_LOGIT ** 2) & (v_bound2 <= SAFE_V ** 2)

    def body(s, carry):
        more = s + 1 < NSEG
        nxt = jnp.minimum(s + 1, NSEG - 1)

        @pl.when(more)
        def _():
            x_copy(nxt).wait()

        @pl.when(safe)
        def _():
            with _scope("attn"):
                attention(True)

        @pl.when(jnp.logical_not(safe))
        def _():
            attention(False)

        @pl.when(more)
        def _():
            with _scope("blockB"):
                hold = {}
                steps = {
                    "MU": mem_update,
                    "OP": lambda: hold.update(a=out_project()),
                    "LN1": lambda: ln1(nxt),
                    "PR": lambda: project(nxt),
                    "MR": mem_read,
                    "FIN": lambda: finalize(s, 0, NT, hold["a"]),
                }
                for n in _ORDER_B:
                    steps[n]()
            out_copy(s).start()
        return carry

    lax.fori_loop(0, NSEG, body, 0)
    with _scope("fin"):
        otb = ot[...].astype(bf16)
        for t in range(NT):
            finalize(NSEG - 1, t, 1, _dot(wot[...], otb[:, t * T:(t + 1) * T]))
        out_copy(NSEG - 1).start()

    bv = best_v[...]
    rmax = jnp.max(bv, axis=1, keepdims=True)
    cand = best_i[...] + lax.broadcasted_iota(jnp.int32, best_i.shape, 1)
    idx = jnp.clip(jnp.min(jnp.where(bv == rmax, cand, S)), 0, S - 1)
    base = pl.multiple_of((idx // T) * T, T)
    lane = idx - base
    blk = (hbuf[:, pl.ds(base, T)] * ab_all[0:1, pl.ds(base, T)]
           + ab_all[8:9, pl.ds(base, T)]).astype(bf16)
    pick = jnp.where(lax.broadcasted_iota(jnp.int32, (16, T), 1) == lane, 1.0, 0.0).astype(bf16)
    xg = _dot_nt(pick, blk).astype(bf16)
    for c in w_copies[4:]:
        c.wait()
    yacc = jnp.zeros((D, T), f32)
    f_lo = 0
    for nt in _MOE_CHUNKS:
        f_hi = f_lo + nt * T
        gt = _dot(xg, wg_v[:, f_lo:f_hi])
        up = _dot(xg, wu_v[:, f_lo:f_hi])
        act = (gt * jax.nn.sigmoid(gt) * up)[0:1].astype(bf16).astype(f32)
        for t in range(nt):
            f0 = f_lo + t * T
            yacc = yacc + wd_v[:, f0:f0 + T].astype(f32) * act[:, t * T:(t + 1) * T]
        f_lo = f_hi
    y = jnp.sum(yacc, axis=1, keepdims=True) * jax.nn.sigmoid(rmax[0:1])
    for s in range(NSEG):
        out_copy(s).wait()
    sel = lax.broadcasted_iota(jnp.int32, (D, T), 1) == lane
    cur = out_v[:, pl.ds(base, T)].astype(f32)
    out_v[:, pl.ds(base, T)] = (cur + jnp.where(sel, y, 0.0)).astype(bf16)
    patch = pltpu.make_async_copy(out_v.at[:, pl.ds(base, T)],
                                  out_hbm.at[0, :, pl.ds(base, T)], sem_o.at[NSEG])
    patch.start()
    patch.wait()


@jax.jit
def pallas_sequential_preLN__memory_aug_infini_attn__moe_arch_mod__prompt_kernel(
    A_x: jax.Array,
    A_wq: jax.Array,
    A_wk: jax.Array,
    A_wv: jax.Array,
    A_wo: jax.Array,
    A_beta: jax.Array,
    B_x: jax.Array,
    B_w_r: jax.Array,
    B_w_gate: jax.Array,
    B_w_up: jax.Array,
    B_w_down: jax.Array,
):
    del B_x
    hbm_spec = pl.BlockSpec(memory_space=pltpu.HBM)
    scratch = [
        pltpu.VMEM((D, S), bf16),
        pltpu.VMEM((4, D, D), bf16),
        pltpu.VMEM((3 * D, KP), bf16),
        pltpu.VMEM((D, D), bf16),
        pltpu.VMEM((D, S), f32),
        pltpu.VMEM((D, F), bf16),
        pltpu.VMEM((D, F), bf16),
        pltpu.VMEM((D, F), bf16),
        pltpu.VMEM((16, S), bf16),
        pltpu.VMEM((8, S), f32),
        pltpu.VMEM((D, L), bf16),
        pltpu.VMEM((D, L), bf16),
        pltpu.VMEM((D, L), bf16),
        pltpu.VMEM((D, L), bf16),
        pltpu.VMEM((D, L), bf16),
        pltpu.VMEM((NG, L, T), bf16),
        pltpu.VMEM((7, NT, L, T), bf16),
        pltpu.VMEM((7, NT, L, T), bf16),
        pltpu.VMEM((D, L), f32),
        pltpu.VMEM((D, L), f32),
        pltpu.VMEM((NG, MROWS, T), f32),
        pltpu.VMEM((NG, MROWS, T), bf16),
        pltpu.VMEM((NG, MROWS, T), f32),
        pltpu.VMEM((D, T), f32),
        pltpu.VMEM((H, 8, T), f32),
        pltpu.VMEM((D, T), f32),
        pltpu.VMEM((16, S), f32),
        pltpu.VMEM((D, S), bf16),
        pltpu.VMEM((8, T), f32),
        pltpu.VMEM((8, T), jnp.int32),
        pltpu.VMEM((8, T), f32),
        pltpu.VMEM((H,), bf16),
        pltpu.VMEM((D,), bf16),
        pltpu.SemaphoreType.DMA((NSEG,)),
        pltpu.SemaphoreType.DMA((10,)),
        pltpu.SemaphoreType.DMA((NSEG + 1,)),
    ]
    out_t = pl.pallas_call(
        _kernel,
        out_shape=jax.ShapeDtypeStruct((1, D, S), bf16),
        in_specs=[hbm_spec] * 10,
        out_specs=hbm_spec,
        scratch_shapes=scratch,
        compiler_params=pltpu.CompilerParams(vmem_limit_bytes=100 * 1024 * 1024),
    )(jnp.transpose(A_x, (0, 2, 1)), A_wq, A_wk, A_wv, A_wo, A_beta,
      B_w_r, B_w_gate, B_w_up, B_w_down.T)
    return jnp.transpose(out_t, (0, 2, 1))
```

```python
import contextlib

import jax
import jax.numpy as jnp
from jax import lax
import jax.experimental.pallas as pl
import jax.experimental.pallas.tpu as pltpu

S = 2048
D = 576
H = 32
DH = 18
NSEG = 4
L = 512
F = 4608
T = 128
NT = L // T
EPS = 1e-5
LOG2E = 1.4426950408889634
QSCALE = (DH ** -0.5) * LOG2E
WIN = 112
GROUPS = (tuple(range(0, 7)), tuple(range(7, 13)), tuple(range(13, 19)),
          tuple(range(19, 25)), tuple(range(25, 32)))
NG = len(GROUPS)
KP = 640
MROWS = T + 16
SAFE_LOGIT = 60.0
SAFE_V = 2.0 ** 40

bf16 = jnp.bfloat16
f32 = jnp.float32
_ORDER_B = ["MU", "OP", "LN1", "PR", "MR", "FIN"]
_MOE_CHUNKS = (2,) * 18
_PCOLS = 2
_PROFILE = False


def _scope(name):
    return jax.named_scope(name) if _PROFILE else contextlib.nullcontext()


def _colsum(x):
    n = x.shape[0] // 4
    parts = [jnp.sum(x[i * n:(i + 1) * n].reshape(n // 8, 8, x.shape[1]), axis=0) for i in range(4)]
    return jnp.sum((parts[0] + parts[1]) + (parts[2] + parts[3]), axis=0, keepdims=True)


def _ln_stats(x):
    m = _colsum(x) * (1.0 / D)
    v = jnp.maximum(_colsum(x * x) * (1.0 / D) - m * m, 0.0)
    a = lax.rsqrt(v + EPS)
    return a, -m * a


def _phi(t):
    return jnp.where(t > 0, t + 1.0, jnp.exp(t))


def _dot(a, b):
    return jnp.dot(a, b, preferred_element_type=f32)


def _dot_nt(a, b):
    return lax.dot_general(a, b, (((1,), (1,)), ((), ())), preferred_element_type=f32)


def _dot_tn(a, b):
    return lax.dot_general(a, b, (((0,), (0,)), ((), ())), preferred_element_type=f32)


ROT = (0, 1, 2, 3, 0, 2, 1)
QW = T // 4


def _pack_plan(nh, c):
    tiles = []
    split = []
    for u in range(nh):
        need = [(a + ROT[u]) % 4 for a in range(c, 4)]
        for t in tiles:
            if all(t[q] is None for q in need):
                break
        else:
            bound = max(sum(q in [(a + ROT[v]) % 4 for a in range(c, 4)] for v in range(nh))
                        for q in range(4))
            if len(tiles) >= bound:
                split.append((u, need))
                continue
            t = [None] * 4
            tiles.append(t)
        for q in need:
            t[q] = u
    for u, need in split:
        for q in need:
            next(t for t in tiles if t[q] is None)[q] = u
    return tiles


def _masked_q(qt_ref, g, j):
    ws = WIN * g
    row64 = lax.broadcasted_iota(jnp.int32, (64, T), 0)
    qw32 = pltpu.bitcast(qt_ref[ws:ws + T, j * T:(j + 1) * T], jnp.uint32)
    rolled = {0: qw32}
    qms = []
    for u, h in enumerate(GROUPS[g]):
        if ROT[u] not in rolled:
            rolled[ROT[u]] = pltpu.roll(qw32, ROT[u] * QW, axis=1)
        lo2 = (h * DH - ws) // 2
        qmask = (row64 >= lo2) & (row64 < lo2 + DH // 2)
        qms.append(jnp.where(qmask, rolled[ROT[u]], jnp.uint32(0)))
    return qms


def _select_quarters(sources):
    distinct = []
    for x in sources:
        if x is not None and not any(x is y for y in distinct):
            distinct.append(x)
    distinct.sort(key=lambda y: -sum(x is y for x in sources))
    out = distinct[0]
    lane = lax.broadcasted_iota(jnp.int32, out.shape, 1)
    for y in distinct[1:]:
        mask = None
        for q, x in enumerate(sources):
            if x is y:
                m = (lane >= q * QW) & (lane < (q + 1) * QW)
                mask = m if mask is None else mask | m
        out = jnp.where(mask, y, out)
    return out


def _scores_fast(g, kp_ref, qt_ref, p_ref):
    nh = len(GROUPS[g])
    kk = lax.broadcasted_iota(jnp.int32, (T, T), 0)
    qq = lax.broadcasted_iota(jnp.int32, (T, T), 1)
    causal = {r: kk <= ((qq - r * QW) & (T - 1)) for r in set(ROT[:nh])}
    plans = {c: _pack_plan(nh, c) for c in range(1, 4)}
    for j in range(NT):
        qms = _masked_q(qt_ref, g, j)
        n0 = T * j + QW
        p0 = jnp.exp2(_dot(kp_ref[g, 0:n0, :],
                           jnp.concatenate([pltpu.bitcast(q, bf16) for q in qms], axis=1)))
        pc = {}
        for c in range(1, 4):
            w = [pltpu.bitcast(_select_quarters([None if u is None else qms[u] for u in t]), bf16)
                 for t in plans[c]]
            r0 = T * j + c * QW
            pc[c] = jnp.exp2(_dot(kp_ref[g, r0:r0 + QW, :], jnp.concatenate(w, axis=1)))
        for u in range(nh):
            pu = p0[:, u * T:(u + 1) * T]
            if j > 0:
                p_ref[u, j, 0:j * T, :] = pu[0:j * T].astype(bf16)
            rows = [pu[j * T:n0]]
            for c in range(1, 4):
                src = [None] * 4
                for i, t in enumerate(plans[c]):
                    for q in range(4):
                        if t[q] == u:
                            src[q] = i
                vals = {i: pc[c][:, i * T:(i + 1) * T] for i in set(src) if i is not None}
                rows.append(_select_quarters([None if i is None else vals[i] for i in src]))
            p_ref[u, j, j * T:(j + 1) * T, :] = jnp.where(
                causal[ROT[u]], jnp.concatenate(rows, axis=0), 0.0).astype(bf16)


def _attention_safe(h, kp_ref, qt_ref, vt_ref, g1_ref, am_ref, ot_ref):
    g = jnp.minimum(jnp.maximum(h - 1, 0) // 6, NG - 1)
    ws = pl.multiple_of(g * WIN, 16)
    lo = h * DH - ws
    row128 = lax.broadcasted_iota(jnp.int32, (T, T), 0)
    qmask = (row128 >= lo) & (row128 < lo + DH)
    vs = pl.multiple_of(((h * DH) // 16) * 16, 16)
    off = h * DH - vs
    row32 = lax.broadcasted_iota(jnp.int32, (32, T), 0)
    omask = (row32 >= off) & (row32 < off + DH)
    kk = lax.broadcasted_iota(jnp.int32, (L, T), 0)
    qq = lax.broadcasted_iota(jnp.int32, (L, T), 1)

    def tile(j, c):
        c0 = pl.multiple_of(j * T, T)
        qm = jnp.where(qmask, qt_ref[pl.ds(ws, T), pl.ds(c0, T)].astype(f32), 0.0).astype(bf16)
        s = _dot(kp_ref[g], qm)
        s = jnp.where(kk <= qq + c0, s, -jnp.inf)
        m = jnp.max(s, axis=0, keepdims=True)
        p = jnp.exp2(s - m).astype(bf16)
        acc = _dot(_v_rows(vt_ref, vs, off // 2, L), p)
        l8 = jnp.where(off <= 6, acc[24:32], acc[0:8])
        rl = g1_ref[h] / l8
        o = acc * jnp.concatenate([rl] * 4, axis=0) + am_ref[pl.ds(vs, 32), pl.ds(c0, T)]
        pltpu.store(ot_ref.at[pl.ds(vs, 32), pl.ds(c0, T)], o, mask=omask)
        return c

    lax.fori_loop(0, NT, tile, 0)


def _v_rows(vt_ref, vs, off2, nk):
    row16 = lax.broadcasted_iota(jnp.int32, (16, nk), 0)
    keep = (row16 >= off2) & (row16 < off2 + DH // 2)
    v32 = pltpu.bitcast(vt_ref[pl.ds(vs, 32), 0:nk], jnp.uint32)
    return pltpu.bitcast(jnp.where(keep, v32, jnp.uint32(0x3F803F80)), bf16)


def _pv(g, vt_ref, p_ref, g1_ref, am_ref, ot_ref):
    row32 = lax.broadcasted_iota(jnp.int32, (32, T), 0)
    for u, h in enumerate(GROUPS[g]):
        vs = ((h * DH) // 16) * 16
        off = h * DH - vs
        omask = (row32 >= off) & (row32 < off + DH)
        g1 = g1_ref[h]
        vrows = _v_rows(vt_ref, vs, off // 2, L)
        for j in range(NT):
            nk = T * (j + 1)
            acc = _dot(vrows[:, 0:nk], p_ref[u, j, 0:nk, :])
            l8 = acc[24:32] if off <= 6 else acc[0:8]
            rl = g1 / l8
            o = acc * jnp.concatenate([rl] * 4, axis=0)
            if ROT[u]:
                o = pltpu.roll(o, T - ROT[u] * QW, axis=1)
            o = o + am_ref[vs:vs + 32, j * T:(j + 1) * T]
            pltpu.store(ot_ref.at[vs:vs + 32, j * T:(j + 1) * T], o, mask=omask)


def _kernel(x_hbm, wq_hbm, wk_hbm, wv_hbm, wo_hbm, beta_hbm, wr_hbm, wg_hbm, wu_hbm, wd_hbm,
            out_hbm,
            x_v, w_in, wt, wot, hbuf, wg_v, wu_v, wd_v,
            aug, arow, qt, pqt, kt, pkt, vt, kp, p0, p1, am_v, ot,
            macc, mb, bmask, gtab, g1tab, wrtab, ab_all, out_v, best_v, best_i, wrsum, beta_ref, wr_ref,
            sem_x, sem_w, sem_o):
    def x_copy(s):
        return pltpu.make_async_copy(x_hbm.at[0, :, pl.ds(s * L, L)],
                                     x_v.at[:, pl.ds(s * L, L)], sem_x.at[s])

    def out_copy(s):
        return pltpu.make_async_copy(out_v.at[:, pl.ds(s * L, L)],
                                     out_hbm.at[0, :, pl.ds(s * L, L)], sem_o.at[s])

    w_copies = [
        None,
        pltpu.make_async_copy(wk_hbm, w_in.at[1], sem_w.at[1]),
        pltpu.make_async_copy(wv_hbm, w_in.at[2], sem_w.at[2]),
        pltpu.make_async_copy(wo_hbm, w_in.at[3], sem_w.at[3]),
        pltpu.make_async_copy(wg_hbm, wg_v, sem_w.at[4]),
        pltpu.make_async_copy(wu_hbm, wu_v, sem_w.at[5]),
        pltpu.make_async_copy(wd_hbm, wd_v, sem_w.at[6]),
    ]
    small_b = pltpu.make_async_copy(beta_hbm, beta_ref, sem_w.at[7])
    small_r = pltpu.make_async_copy(wr_hbm, wr_ref, sem_w.at[8])
    QLO = 256
    wq_lo = pltpu.make_async_copy(wq_hbm.at[:, 0:QLO], w_in.at[0, :, 0:QLO], sem_w.at[0])
    wq_hi = pltpu.make_async_copy(wq_hbm.at[:, QLO:D], w_in.at[0, :, QLO:D], sem_w.at[9])
    small_b.start()
    small_r.start()
    wq_lo.start()
    x_copy(0).start()

    def build_tables():
        gate = jax.nn.sigmoid(beta_ref[...].astype(f32).reshape(1, H))
        rr = lax.broadcasted_iota(jnp.int32, (D, H), 0)
        hh = lax.broadcasted_iota(jnp.int32, (D, H), 1)
        onehot = (rr >= hh * DH) & (rr < (hh + 1) * DH)
        gcol = jnp.sum(jnp.where(onehot, gate, 0.0), axis=1, keepdims=True)
        gtab[...] = jnp.broadcast_to(gcol, (D, T))
        hh8 = lax.broadcasted_iota(jnp.int32, (8, H), 1)
        for h in range(H):
            gh = jnp.sum(jnp.where(hh8 == h, gate, 0.0), axis=1, keepdims=True)
            g1tab[h] = jnp.broadcast_to(1.0 - gh, (8, T))
        wr_row = wr_ref[...].astype(f32).reshape(1, D)
        wr_pad = jnp.concatenate([wr_row, jnp.zeros((1, 5 * T - D), f32)], axis=1)
        wrtab[...] = jnp.broadcast_to(wr_pad, (T, 5 * T)).T[0:D]
        wrsum[...] = jnp.broadcast_to(jnp.sum(wr_row, axis=1, keepdims=True), wrsum.shape)

    mr = lax.broadcasted_iota(jnp.int32, (MROWS, T), 0)
    mc = lax.broadcasted_iota(jnp.int32, (MROWS, T), 1)
    for g in range(NG):
        ws = WIN * g
        m = jnp.zeros((MROWS, T), jnp.bool_)
        for i, h in enumerate(GROUPS[g]):
            lo = h * DH - ws
            cols = (mc >= lo) & (mc < lo + DH)
            rows = ((mr >= lo) & (mr < lo + DH) & (mr < T)) | (mr == T + i)
            m = m | (cols & rows)
        bmask[g] = jnp.where(m, 1.0, 0.0)
    macc[...] = jnp.zeros_like(macc)
    mb[...] = jnp.zeros_like(mb)
    best_v[...] = jnp.full(best_v.shape, -jnp.inf, f32)
    best_i[...] = jnp.zeros(best_i.shape, jnp.int32)

    ones_rows = jnp.ones((16, L), bf16)

    def ln1(s):
        col0 = pl.multiple_of(s * L, L)
        xs = x_v[:, pl.ds(col0, L)].astype(f32)
        m = _colsum(xs) * (1.0 / D)
        v = jnp.maximum(_colsum(xs * xs) * (1.0 / D) - m * m, 0.0)
        arow[:, pl.ds(col0, L)] = jnp.broadcast_to(lax.rsqrt(v + EPS), (8, L))
        m_hi = (-m).astype(bf16).astype(f32)
        m_lo = -m - m_hi
        r16 = lax.broadcasted_iota(jnp.int32, (16, L), 0)
        rows = jnp.where(r16 >= 4, 0.0, jnp.where((r16 & 1) == 0, m_hi, m_lo))
        aug[:, pl.ds(col0, L)] = rows.astype(bf16)

    def finalize(s, t0, nt, attn):
        w = nt * T
        col0 = pl.multiple_of(s * L + t0 * T, T)
        hres = x_v[:, pl.ds(col0, w)].astype(f32) + attn
        hbuf[:, pl.ds(col0, w)] = hres
        a, b = _ln_stats(hres)
        wr = jnp.concatenate([wrtab[...]] * nt, axis=1)
        r = _colsum(hres * wr) * a + b * wrsum[0:1, 0:1]
        ab_all[0:8, pl.ds(col0, w)] = jnp.broadcast_to(a, (8, w))
        ab_all[8:16, pl.ds(col0, w)] = jnp.broadcast_to(b, (8, w))
        out_v[:, pl.ds(col0, w)] = (hbuf[:, pl.ds(col0, w)] * (1.0 + a) + b).astype(bf16)
        r = r.astype(bf16).astype(f32)
        bv, bi = best_v[0:1, :], best_i[0:1, :]
        for t in range(nt):
            rt = r[:, t * T:(t + 1) * T]
            better = rt > bv
            bi = jnp.where(better, col0 + t * T, bi)
            bv = jnp.where(better, rt, bv)
        best_i[...] = jnp.broadcast_to(bi, best_i.shape)
        best_v[...] = jnp.broadcast_to(bv, best_v.shape)

    def proj_rhs(s):
        col0 = pl.multiple_of(s * L, L)
        return jnp.concatenate([x_v[:, pl.ds(col0, L)], aug[:, pl.ds(col0, L)],
                                jnp.zeros((KP - D - 16, L), bf16)], axis=0)

    def ln_scale(s):
        return arow[0:1, pl.ds(pl.multiple_of(s * L, L), L)]

    def store_q(raw, a, r0, r1, with_phi=True, cols=slice(None)):
        qt[r0:r1, cols] = (raw * (a * QSCALE)).astype(bf16)
        if with_phi:
            pqt[r0:r1, cols] = _phi(raw * a).astype(bf16)

    def store_k_rows(raw, a, r0, r1):
        k = raw * a
        kt[r0:r1, :] = k.astype(bf16)
        pkt[r0:r1, :] = _phi(k).astype(bf16)

    def transpose_k():
        for g in range(NG):
            kp[g] = kt[WIN * g:WIN * g + T, :].T

    def store_k(raw, a, cols):
        k = raw * a
        kb = k.astype(bf16)
        pkt[:, cols] = _phi(k).astype(bf16)
        for g in range(NG):
            kp[g, cols, :] = kb[WIN * g:WIN * g + T, :].T

    def store_v(raw, a, cols=slice(None)):
        vt[:, cols] = (raw * a).astype(bf16)

    def project(s):
        rhs = proj_rhs(s)
        a = ln_scale(s)
        w = _PCOLS * T
        for c0 in range(0, L, w):
            cols = slice(c0, c0 + w)
            qkv = _dot(wt[...], rhs[:, cols])
            store_q(qkv[0:D], a[:, cols], 0, D, True, cols)
            store_k(qkv[D:2 * D], a[:, cols], cols)
            store_v(qkv[2 * D:3 * D], a[:, cols], cols)

    def mem_read():
        row128 = lax.broadcasted_iota(jnp.int32, (T, T), 0)
        row8 = lax.broadcasted_iota(jnp.int32, (8, T), 0)
        for g in range(NG):
            ws = WIN * g
            heads = GROUPS[g]
            lo_g, hi_g = heads[0] * DH - ws, (heads[-1] + 1) * DH - ws
            wmask = (row128 >= lo_g) & (row128 < hi_g)
            for j in range(NT):
                nd = _dot(mb[g], pqt[ws:ws + T, j * T:(j + 1) * T])
                rden = 1.0 / (nd[T:T + 8] + 1e-6)
                rb = [jnp.broadcast_to(rden[i:i + 1], (8, T)) for i in range(len(heads))]
                blocks = []
                for b in range(T // 8):
                    r_lo, r_hi = 8 * b, 8 * b + 7
                    i_lo = min(max((r_lo + ws) // DH - heads[0], 0), len(heads) - 1)
                    i_hi = min(max((r_hi + ws) // DH - heads[0], 0), len(heads) - 1)
                    if i_lo == i_hi:
                        blocks.append(rb[i_lo])
                    else:
                        cut = (heads[0] + i_hi) * DH - ws - r_lo
                        blocks.append(jnp.where(row8 < cut, rb[i_lo], rb[i_hi]))
                amv = nd[0:T] * jnp.concatenate(blocks, axis=0) * gtab[ws:ws + T, :]
                pltpu.store(am_v.at[ws:ws + T, j * T:(j + 1) * T], amv, mask=wmask)

    def attention(fast):
        ps = (p0, p1)
        if fast:
            _scores_fast(0, kp, qt, ps[0])
            for g in range(NG):
                if g + 1 < NG:
                    _scores_fast(g + 1, kp, qt, ps[(g + 1) % 2])
                _pv(g, vt, ps[g % 2], g1tab, am_v, ot)
        else:
            lax.fori_loop(0, H, lambda h, c: (_attention_safe(h, kp, qt, vt, g1tab, am_v, ot), c)[1], 0)

    def mem_update():
        for g in range(NG):
            ws = WIN * g
            lhs = jnp.concatenate([vt[ws:ws + T, :], ones_rows], axis=0)
            upd = macc[g] + _dot_nt(lhs, pkt[ws:ws + T, :])
            macc[g] = upd
            mb[g] = jnp.where(bmask[g] != 0.0, upd, 0.0).astype(bf16)

    def load_weight(i, c0=0, c1=D):
        w = w_in[i, :, c0:c1]
        n = c1 - c0
        wf = w.astype(f32)
        c = jnp.sum(wf, axis=0, keepdims=True)
        c_hi = c.astype(bf16).astype(f32)
        r16 = lax.broadcasted_iota(jnp.int32, (16, n), 0)
        extra = jnp.where(r16 >= 4, 0.0, jnp.where(r16 < 2, c_hi, c - c_hi)).astype(bf16)
        w_aug = jnp.concatenate([w, extra, jnp.zeros((KP - D - 16, n), bf16)], axis=0)
        w_t = w_aug.T
        wt[i * D + c0:i * D + c1, :] = w_t
        return w_t, jnp.max(jnp.sum(wf * wf, axis=0, keepdims=True))

    am_v[...] = jnp.zeros_like(am_v)
    ot[...] = jnp.zeros_like(ot)
    with _scope("p_tables"):
        small_b.wait()
        small_r.wait()
        build_tables()
    with _scope("p_wq_wait"):
        wq_lo.wait()
    wq_hi.start()
    w_copies[1].start()
    with _scope("p_wqT"):
        _, cq_lo = load_weight(0, 0, QLO)
    with _scope("p_x0_wait"):
        x_copy(0).wait()
    w_copies[2].start()
    x_copy(1).start()
    w_copies[3].start()
    HALF = 288
    with _scope("p_qlo"):
        ln1(0)
        store_q(_dot(wt[0:QLO, :], proj_rhs(0)), ln_scale(0), 0, QLO, False)
    with _scope("p_wqhi_wait"):
        wq_hi.wait()
    for s in range(2, NSEG):
        x_copy(s).start()
    for c in w_copies[4:]:
        c.start()
    with _scope("p_qmid"):
        wq_t, cq_hi = load_weight(0, QLO, D)
        cq = jnp.maximum(cq_lo, cq_hi)
    with _scope("p_wk_wait"):
        w_copies[1].wait()
    with _scope("p_qhi_wkT_klo"):
        wk_t, ck = load_weight(1)
        store_q(_dot(wt[QLO:D, :], proj_rhs(0)), ln_scale(0), QLO, D, False)
        store_k_rows(_dot(wk_t[0:HALF], proj_rhs(0)), ln_scale(0), 0, HALF)
    with _scope("p_wv_wait"):
        w_copies[2].wait()
        w_copies[3].wait()
    with _scope("p_khi_wvT_v"):
        wv_t, cv = load_weight(2)
        wot[...] = w_in[3].T
        store_k_rows(_dot(wt[D + HALF:2 * D, :], proj_rhs(0)), ln_scale(0), HALF, D)
        transpose_k()
        store_v(_dot(wv_t, proj_rhs(0)), ln_scale(0))
    slack = 1.05
    logit_bound2 = (cq * ck) * (slack * D * DH * QSCALE) ** 2
    v_bound2 = cv * (slack * D)
    safe = (logit_bound2 <= SAFE_LOGIT ** 2) & (v_bound2 <= SAFE_V ** 2)

    def body(s, carry):
        more = s + 1 < NSEG
        nxt = jnp.minimum(s + 1, NSEG - 1)

        @pl.when(more)
        def _():
            x_copy(nxt).wait()

        @pl.when(safe)
        def _():
            with _scope("attn"):
                attention(True)

        @pl.when(jnp.logical_not(safe))
        def _():
            attention(False)

        @pl.when(more)
        def _():
            with _scope("blockB"):
                hold = {}
                steps = {
                    "MU": mem_update,
                    "OP": lambda: hold.update(a=[_dot(wot[...], ot[:, t * T:(t + 1) * T].astype(bf16))
                                                    for t in range(NT)]),
                    "LN1": lambda: ln1(nxt),
                    "PR": lambda: project(nxt),
                    "MR": mem_read,
                    "FIN": lambda: [finalize(s, t, 1, hold["a"][t]) for t in range(NT)],
                }
                for n in _ORDER_B:
                    steps[n]()
            out_copy(s).start()
        return carry

    lax.fori_loop(0, NSEG, body, 0)
    with _scope("fin"):
        otb = ot[...].astype(bf16)
        for t in range(NT):
            finalize(NSEG - 1, t, 1, _dot(wot[...], otb[:, t * T:(t + 1) * T]))
        out_copy(NSEG - 1).start()

    bv = best_v[...]
    rmax = jnp.max(bv, axis=1, keepdims=True)
    cand = best_i[...] + lax.broadcasted_iota(jnp.int32, best_i.shape, 1)
    idx = jnp.clip(jnp.min(jnp.where(bv == rmax, cand, S)), 0, S - 1)
    base = pl.multiple_of((idx // T) * T, T)
    lane = idx - base
    blk = (hbuf[:, pl.ds(base, T)] * ab_all[0:1, pl.ds(base, T)]
           + ab_all[8:9, pl.ds(base, T)]).astype(bf16)
    pick = jnp.where(lax.broadcasted_iota(jnp.int32, (16, T), 1) == lane, 1.0, 0.0).astype(bf16)
    xg = _dot_nt(pick, blk).astype(bf16)
    for c in w_copies[4:]:
        c.wait()
    yacc = jnp.zeros((D, T), f32)
    f_lo = 0
    for nt in _MOE_CHUNKS:
        f_hi = f_lo + nt * T
        gt = _dot(xg, wg_v[:, f_lo:f_hi])
        up = _dot(xg, wu_v[:, f_lo:f_hi])
        act = (gt * jax.nn.sigmoid(gt) * up)[0:1].astype(bf16).astype(f32)
        for t in range(nt):
            f0 = f_lo + t * T
            yacc = yacc + wd_v[:, f0:f0 + T].astype(f32) * act[:, t * T:(t + 1) * T]
        f_lo = f_hi
    y = jnp.sum(yacc, axis=1, keepdims=True) * jax.nn.sigmoid(rmax[0:1])
    for s in range(NSEG):
        out_copy(s).wait()
    sel = lax.broadcasted_iota(jnp.int32, (D, T), 1) == lane
    cur = out_v[:, pl.ds(base, T)].astype(f32)
    out_v[:, pl.ds(base, T)] = (cur + jnp.where(sel, y, 0.0)).astype(bf16)
    patch = pltpu.make_async_copy(out_v.at[:, pl.ds(base, T)],
                                  out_hbm.at[0, :, pl.ds(base, T)], sem_o.at[NSEG])
    patch.start()
    patch.wait()


@jax.jit
def pallas_sequential_preLN__memory_aug_infini_attn__moe_arch_mod__prompt_kernel(
    A_x: jax.Array,
    A_wq: jax.Array,
    A_wk: jax.Array,
    A_wv: jax.Array,
    A_wo: jax.Array,
    A_beta: jax.Array,
    B_x: jax.Array,
    B_w_r: jax.Array,
    B_w_gate: jax.Array,
    B_w_up: jax.Array,
    B_w_down: jax.Array,
):
    del B_x
    hbm_spec = pl.BlockSpec(memory_space=pltpu.HBM)
    scratch = [
        pltpu.VMEM((D, S), bf16),
        pltpu.VMEM((4, D, D), bf16),
        pltpu.VMEM((3 * D, KP), bf16),
        pltpu.VMEM((D, D), bf16),
        pltpu.VMEM((D, S), f32),
        pltpu.VMEM((D, F), bf16),
        pltpu.VMEM((D, F), bf16),
        pltpu.VMEM((D, F), bf16),
        pltpu.VMEM((16, S), bf16),
        pltpu.VMEM((8, S), f32),
        pltpu.VMEM((D, L), bf16),
        pltpu.VMEM((D, L), bf16),
        pltpu.VMEM((D, L), bf16),
        pltpu.VMEM((D, L), bf16),
        pltpu.VMEM((D, L), bf16),
        pltpu.VMEM((NG, L, T), bf16),
        pltpu.VMEM((7, NT, L, T), bf16),
        pltpu.VMEM((7, NT, L, T), bf16),
        pltpu.VMEM((D, L), f32),
        pltpu.VMEM((D, L), f32),
        pltpu.VMEM((NG, MROWS, T), f32),
        pltpu.VMEM((NG, MROWS, T), bf16),
        pltpu.VMEM((NG, MROWS, T), f32),
        pltpu.VMEM((D, T), f32),
        pltpu.VMEM((H, 8, T), f32),
        pltpu.VMEM((D, T), f32),
        pltpu.VMEM((16, S), f32),
        pltpu.VMEM((D, S), bf16),
        pltpu.VMEM((8, T), f32),
        pltpu.VMEM((8, T), jnp.int32),
        pltpu.VMEM((8, T), f32),
        pltpu.VMEM((H,), bf16),
        pltpu.VMEM((D,), bf16),
        pltpu.SemaphoreType.DMA((NSEG,)),
        pltpu.SemaphoreType.DMA((10,)),
        pltpu.SemaphoreType.DMA((NSEG + 1,)),
    ]
    out_t = pl.pallas_call(
        _kernel,
        out_shape=jax.ShapeDtypeStruct((1, D, S), bf16),
        in_specs=[hbm_spec] * 10,
        out_specs=hbm_spec,
        scratch_shapes=scratch,
        compiler_params=pltpu.CompilerParams(vmem_limit_bytes=100 * 1024 * 1024),
    )(jnp.transpose(A_x, (0, 2, 1)), A_wq, A_wk, A_wv, A_wo, A_beta,
      B_w_r, B_w_gate, B_w_up, B_w_down.T)
    return jnp.transpose(out_t, (0, 2, 1))
```

```python
import contextlib

import jax
import jax.numpy as jnp
from jax import lax
import jax.experimental.pallas as pl
import jax.experimental.pallas.tpu as pltpu

S = 2048
D = 576
H = 32
DH = 18
NSEG = 4
L = 512
F = 4608
T = 128
NT = L // T
EPS = 1e-5
LOG2E = 1.4426950408889634
QSCALE = (DH ** -0.5) * LOG2E
WIN = 112
GROUPS = (tuple(range(0, 7)), tuple(range(7, 13)), tuple(range(13, 19)),
          tuple(range(19, 25)), tuple(range(25, 32)))
NG = len(GROUPS)
KP = 640
MROWS = T + 16
SAFE_LOGIT = 60.0
SAFE_V = 2.0 ** 40

bf16 = jnp.bfloat16
f32 = jnp.float32
_ORDER_B = ["MU", "OP", "LN1", "PR", "MR", "FIN"]
_MOE_CHUNKS = (2,) * 18
_PCOLS = 2
_PRO_SPLITS = (128, 416)
_PROFILE = False


def _scope(name):
    return jax.named_scope(name) if _PROFILE else contextlib.nullcontext()


def _colsum(x):
    n = x.shape[0] // 4
    parts = [jnp.sum(x[i * n:(i + 1) * n].reshape(n // 8, 8, x.shape[1]), axis=0) for i in range(4)]
    return jnp.sum((parts[0] + parts[1]) + (parts[2] + parts[3]), axis=0, keepdims=True)


def _ln_stats(x):
    m = _colsum(x) * (1.0 / D)
    v = jnp.maximum(_colsum(x * x) * (1.0 / D) - m * m, 0.0)
    a = lax.rsqrt(v + EPS)
    return a, -m * a


def _phi(t):
    return jnp.where(t > 0, t + 1.0, jnp.exp(t))


def _dot(a, b):
    return jnp.dot(a, b, preferred_element_type=f32)


def _dot_nt(a, b):
    return lax.dot_general(a, b, (((1,), (1,)), ((), ())), preferred_element_type=f32)


def _dot_tn(a, b):
    return lax.dot_general(a, b, (((0,), (0,)), ((), ())), preferred_element_type=f32)


ROT = (0, 1, 2, 3, 0, 2, 1)
QW = T // 4


def _pack_plan(nh, c):
    tiles = []
    split = []
    for u in range(nh):
        need = [(a + ROT[u]) % 4 for a in range(c, 4)]
        for t in tiles:
            if all(t[q] is None for q in need):
                break
        else:
            bound = max(sum(q in [(a + ROT[v]) % 4 for a in range(c, 4)] for v in range(nh))
                        for q in range(4))
            if len(tiles) >= bound:
                split.append((u, need))
                continue
            t = [None] * 4
            tiles.append(t)
        for q in need:
            t[q] = u
    for u, need in split:
        for q in need:
            next(t for t in tiles if t[q] is None)[q] = u
    return tiles


def _masked_q(qt_ref, g, j):
    ws = WIN * g
    row64 = lax.broadcasted_iota(jnp.int32, (64, T), 0)
    qw32 = pltpu.bitcast(qt_ref[ws:ws + T, j * T:(j + 1) * T], jnp.uint32)
    rolled = {0: qw32}
    qms = []
    for u, h in enumerate(GROUPS[g]):
        if ROT[u] not in rolled:
            rolled[ROT[u]] = pltpu.roll(qw32, ROT[u] * QW, axis=1)
        lo2 = (h * DH - ws) // 2
        qmask = (row64 >= lo2) & (row64 < lo2 + DH // 2)
        qms.append(jnp.where(qmask, rolled[ROT[u]], jnp.uint32(0)))
    return qms


def _select_quarters(sources):
    distinct = []
    for x in sources:
        if x is not None and not any(x is y for y in distinct):
            distinct.append(x)
    distinct.sort(key=lambda y: -sum(x is y for x in sources))
    out = distinct[0]
    lane = lax.broadcasted_iota(jnp.int32, out.shape, 1)
    for y in distinct[1:]:
        mask = None
        for q, x in enumerate(sources):
            if x is y:
                m = (lane >= q * QW) & (lane < (q + 1) * QW)
                mask = m if mask is None else mask | m
        out = jnp.where(mask, y, out)
    return out


def _scores_fast(g, kp_ref, qt_ref, p_ref):
    nh = len(GROUPS[g])
    kk = lax.broadcasted_iota(jnp.int32, (T, T), 0)
    qq = lax.broadcasted_iota(jnp.int32, (T, T), 1)
    causal = {r: kk <= ((qq - r * QW) & (T - 1)) for r in set(ROT[:nh])}
    plans = {c: _pack_plan(nh, c) for c in range(1, 4)}
    for j in range(NT):
        qms = _masked_q(qt_ref, g, j)
        n0 = T * j + QW
        p0 = jnp.exp2(_dot(kp_ref[g, 0:n0, :],
                           jnp.concatenate([pltpu.bitcast(q, bf16) for q in qms], axis=1)))
        pc = {}
        for c in range(1, 4):
            w = [pltpu.bitcast(_select_quarters([None if u is None else qms[u] for u in t]), bf16)
                 for t in plans[c]]
            r0 = T * j + c * QW
            pc[c] = jnp.exp2(_dot(kp_ref[g, r0:r0 + QW, :], jnp.concatenate(w, axis=1)))
        for u in range(nh):
            pu = p0[:, u * T:(u + 1) * T]
            if j > 0:
                p_ref[u, j, 0:j * T, :] = pu[0:j * T].astype(bf16)
            rows = [pu[j * T:n0]]
            for c in range(1, 4):
                src = [None] * 4
                for i, t in enumerate(plans[c]):
                    for q in range(4):
                        if t[q] == u:
                            src[q] = i
                vals = {i: pc[c][:, i * T:(i + 1) * T] for i in set(src) if i is not None}
                rows.append(_select_quarters([None if i is None else vals[i] for i in src]))
            p_ref[u, j, j * T:(j + 1) * T, :] = jnp.where(
                causal[ROT[u]], jnp.concatenate(rows, axis=0), 0.0).astype(bf16)


def _attention_safe(h, kp_ref, qt_ref, vt_ref, g1_ref, am_ref, ot_ref):
    g = jnp.minimum(jnp.maximum(h - 1, 0) // 6, NG - 1)
    ws = pl.multiple_of(g * WIN, 16)
    lo = h * DH - ws
    row128 = lax.broadcasted_iota(jnp.int32, (T, T), 0)
    qmask = (row128 >= lo) & (row128 < lo + DH)
    vs = pl.multiple_of(((h * DH) // 16) * 16, 16)
    off = h * DH - vs
    row32 = lax.broadcasted_iota(jnp.int32, (32, T), 0)
    omask = (row32 >= off) & (row32 < off + DH)
    kk = lax.broadcasted_iota(jnp.int32, (L, T), 0)
    qq = lax.broadcasted_iota(jnp.int32, (L, T), 1)

    def tile(j, c):
        c0 = pl.multiple_of(j * T, T)
        qm = jnp.where(qmask, qt_ref[pl.ds(ws, T), pl.ds(c0, T)].astype(f32), 0.0).astype(bf16)
        s = _dot(kp_ref[g], qm)
        s = jnp.where(kk <= qq + c0, s, -jnp.inf)
        m = jnp.max(s, axis=0, keepdims=True)
        p = jnp.exp2(s - m).astype(bf16)
        acc = _dot(_v_rows(vt_ref, vs, off // 2, L), p)
        l8 = jnp.where(off <= 6, acc[24:32], acc[0:8])
        rl = g1_ref[h] / l8
        o = acc * jnp.concatenate([rl] * 4, axis=0) + am_ref[pl.ds(vs, 32), pl.ds(c0, T)]
        pltpu.store(ot_ref.at[pl.ds(vs, 32), pl.ds(c0, T)], o, mask=omask)
        return c

    lax.fori_loop(0, NT, tile, 0)


def _v_rows(vt_ref, vs, off2, nk):
    row16 = lax.broadcasted_iota(jnp.int32, (16, nk), 0)
    keep = (row16 >= off2) & (row16 < off2 + DH // 2)
    v32 = pltpu.bitcast(vt_ref[pl.ds(vs, 32), 0:nk], jnp.uint32)
    return pltpu.bitcast(jnp.where(keep, v32, jnp.uint32(0x3F803F80)), bf16)


def _pv(g, vt_ref, p_ref, g1_ref, am_ref, ot_ref):
    row32 = lax.broadcasted_iota(jnp.int32, (32, T), 0)
    for u, h in enumerate(GROUPS[g]):
        vs = ((h * DH) // 16) * 16
        off = h * DH - vs
        omask = (row32 >= off) & (row32 < off + DH)
        g1 = g1_ref[h]
        vrows = _v_rows(vt_ref, vs, off // 2, L)
        for j in range(NT):
            nk = T * (j + 1)
            acc = _dot(vrows[:, 0:nk], p_ref[u, j, 0:nk, :])
            l8 = acc[24:32] if off <= 6 else acc[0:8]
            rl = g1 / l8
            o = acc * jnp.concatenate([rl] * 4, axis=0)
            if ROT[u]:
                o = pltpu.roll(o, T - ROT[u] * QW, axis=1)
            o = o + am_ref[vs:vs + 32, j * T:(j + 1) * T]
            pltpu.store(ot_ref.at[vs:vs + 32, j * T:(j + 1) * T], o, mask=omask)


def _kernel(x_hbm, wq_hbm, wk_hbm, wv_hbm, wo_hbm, beta_hbm, wr_hbm, wg_hbm, wu_hbm, wd_hbm,
            out_hbm,
            x_v, w_in, wt, wot, hbuf, wg_v, wu_v, wd_v,
            aug, arow, qt, pqt, kt, pkt, vt, kp, p0, p1, am_v, ot,
            macc, mb, bmask, gtab, g1tab, wrtab, ab_all, out_v, best_v, best_i, wrsum, beta_ref, wr_ref,
            sem_x, sem_w, sem_o):
    def x_copy(s):
        return pltpu.make_async_copy(x_hbm.at[0, :, pl.ds(s * L, L)],
                                     x_v.at[:, pl.ds(s * L, L)], sem_x.at[s])

    def out_copy(s):
        return pltpu.make_async_copy(out_v.at[:, pl.ds(s * L, L)],
                                     out_hbm.at[0, :, pl.ds(s * L, L)], sem_o.at[s])

    w_copies = [
        None,
        pltpu.make_async_copy(wk_hbm, w_in.at[1], sem_w.at[1]),
        pltpu.make_async_copy(wv_hbm, w_in.at[2], sem_w.at[2]),
        pltpu.make_async_copy(wo_hbm, w_in.at[3], sem_w.at[3]),
        pltpu.make_async_copy(wg_hbm, wg_v, sem_w.at[4]),
        pltpu.make_async_copy(wu_hbm, wu_v, sem_w.at[5]),
        pltpu.make_async_copy(wd_hbm, wd_v, sem_w.at[6]),
    ]
    small_b = pltpu.make_async_copy(beta_hbm, beta_ref, sem_w.at[7])
    small_r = pltpu.make_async_copy(wr_hbm, wr_ref, sem_w.at[8])
    QLO = 256
    wq_lo = pltpu.make_async_copy(wq_hbm.at[:, 0:QLO], w_in.at[0, :, 0:QLO], sem_w.at[0])
    wq_hi = pltpu.make_async_copy(wq_hbm.at[:, QLO:D], w_in.at[0, :, QLO:D], sem_w.at[9])
    small_b.start()
    small_r.start()
    wq_lo.start()
    x_copy(0).start()

    def build_tables():
        gate = jax.nn.sigmoid(beta_ref[...].astype(f32).reshape(1, H))
        rr = lax.broadcasted_iota(jnp.int32, (D, H), 0)
        hh = lax.broadcasted_iota(jnp.int32, (D, H), 1)
        onehot = (rr >= hh * DH) & (rr < (hh + 1) * DH)
        gcol = jnp.sum(jnp.where(onehot, gate, 0.0), axis=1, keepdims=True)
        gtab[...] = jnp.broadcast_to(gcol, (D, T))
        hh8 = lax.broadcasted_iota(jnp.int32, (8, H), 1)
        for h in range(H):
            gh = jnp.sum(jnp.where(hh8 == h, gate, 0.0), axis=1, keepdims=True)
            g1tab[h] = jnp.broadcast_to(1.0 - gh, (8, T))
        wr_row = wr_ref[...].astype(f32).reshape(1, D)
        wr_pad = jnp.concatenate([wr_row, jnp.zeros((1, 5 * T - D), f32)], axis=1)
        wrtab[...] = jnp.broadcast_to(wr_pad, (T, 5 * T)).T[0:D]
        wrsum[...] = jnp.broadcast_to(jnp.sum(wr_row, axis=1, keepdims=True), wrsum.shape)

    mr = lax.broadcasted_iota(jnp.int32, (MROWS, T), 0)
    mc = lax.broadcasted_iota(jnp.int32, (MROWS, T), 1)
    for g in range(NG):
        ws = WIN * g
        m = jnp.zeros((MROWS, T), jnp.bool_)
        for i, h in enumerate(GROUPS[g]):
            lo = h * DH - ws
            cols = (mc >= lo) & (mc < lo + DH)
            rows = ((mr >= lo) & (mr < lo + DH) & (mr < T)) | (mr == T + i)
            m = m | (cols & rows)
        bmask[g] = jnp.where(m, 1.0, 0.0)
    macc[...] = jnp.zeros_like(macc)
    mb[...] = jnp.zeros_like(mb)
    best_v[...] = jnp.full(best_v.shape, -jnp.inf, f32)
    best_i[...] = jnp.zeros(best_i.shape, jnp.int32)

    ones_rows = jnp.ones((16, L), bf16)

    def ln1(s):
        col0 = pl.multiple_of(s * L, L)
        xs = x_v[:, pl.ds(col0, L)].astype(f32)
        m = _colsum(xs) * (1.0 / D)
        v = jnp.maximum(_colsum(xs * xs) * (1.0 / D) - m * m, 0.0)
        arow[:, pl.ds(col0, L)] = jnp.broadcast_to(lax.rsqrt(v + EPS), (8, L))
        m_hi = (-m).astype(bf16).astype(f32)
        m_lo = -m - m_hi
        r16 = lax.broadcasted_iota(jnp.int32, (16, L), 0)
        rows = jnp.where(r16 >= 4, 0.0, jnp.where((r16 & 1) == 0, m_hi, m_lo))
        aug[:, pl.ds(col0, L)] = rows.astype(bf16)

    def finalize(s, t0, nt, attn):
        w = nt * T
        col0 = pl.multiple_of(s * L + t0 * T, T)
        hres = x_v[:, pl.ds(col0, w)].astype(f32) + attn
        hbuf[:, pl.ds(col0, w)] = hres
        a, b = _ln_stats(hres)
        wr = jnp.concatenate([wrtab[...]] * nt, axis=1)
        r = _colsum(hres * wr) * a + b * wrsum[0:1, 0:1]
        ab_all[0:8, pl.ds(col0, w)] = jnp.broadcast_to(a, (8, w))
        ab_all[8:16, pl.ds(col0, w)] = jnp.broadcast_to(b, (8, w))
        out_v[:, pl.ds(col0, w)] = (hbuf[:, pl.ds(col0, w)] * (1.0 + a) + b).astype(bf16)
        r = r.astype(bf16).astype(f32)
        bv, bi = best_v[0:1, :], best_i[0:1, :]
        for t in range(nt):
            rt = r[:, t * T:(t + 1) * T]
            better = rt > bv
            bi = jnp.where(better, col0 + t * T, bi)
            bv = jnp.where(better, rt, bv)
        best_i[...] = jnp.broadcast_to(bi, best_i.shape)
        best_v[...] = jnp.broadcast_to(bv, best_v.shape)

    def proj_rhs(s):
        col0 = pl.multiple_of(s * L, L)
        return jnp.concatenate([x_v[:, pl.ds(col0, L)], aug[:, pl.ds(col0, L)],
                                jnp.zeros((KP - D - 16, L), bf16)], axis=0)

    def ln_scale(s):
        return arow[0:1, pl.ds(pl.multiple_of(s * L, L), L)]

    def store_q(raw, a, r0, r1, with_phi=True, cols=slice(None)):
        qt[r0:r1, cols] = (raw * (a * QSCALE)).astype(bf16)
        if with_phi:
            pqt[r0:r1, cols] = _phi(raw * a).astype(bf16)

    def store_k_rows(raw, a, r0, r1):
        k = raw * a
        kt[r0:r1, :] = k.astype(bf16)
        pkt[r0:r1, :] = _phi(k).astype(bf16)

    def transpose_k():
        for g in range(NG):
            kp[g] = kt[WIN * g:WIN * g + T, :].T

    def store_k(raw, a, cols):
        k = raw * a
        kb = k.astype(bf16)
        pkt[:, cols] = _phi(k).astype(bf16)
        for g in range(NG):
            kp[g, cols, :] = kb[WIN * g:WIN * g + T, :].T

    def store_v(raw, a, cols=slice(None)):
        vt[:, cols] = (raw * a).astype(bf16)

    def project(s):
        rhs = proj_rhs(s)
        a = ln_scale(s)
        w = _PCOLS * T
        for c0 in range(0, L, w):
            cols = slice(c0, c0 + w)
            qkv = _dot(wt[...], rhs[:, cols])
            store_q(qkv[0:D], a[:, cols], 0, D, True, cols)
            store_k(qkv[D:2 * D], a[:, cols], cols)
            store_v(qkv[2 * D:3 * D], a[:, cols], cols)

    def mem_read():
        row128 = lax.broadcasted_iota(jnp.int32, (T, T), 0)
        row8 = lax.broadcasted_iota(jnp.int32, (8, T), 0)
        for g in range(NG):
            ws = WIN * g
            heads = GROUPS[g]
            lo_g, hi_g = heads[0] * DH - ws, (heads[-1] + 1) * DH - ws
            wmask = (row128 >= lo_g) & (row128 < hi_g)
            for j in range(NT):
                nd = _dot(mb[g], pqt[ws:ws + T, j * T:(j + 1) * T])
                rden = 1.0 / (nd[T:T + 8] + 1e-6)
                rb = [jnp.broadcast_to(rden[i:i + 1], (8, T)) for i in range(len(heads))]
                blocks = []
                for b in range(T // 8):
                    r_lo, r_hi = 8 * b, 8 * b + 7
                    i_lo = min(max((r_lo + ws) // DH - heads[0], 0), len(heads) - 1)
                    i_hi = min(max((r_hi + ws) // DH - heads[0], 0), len(heads) - 1)
                    if i_lo == i_hi:
                        blocks.append(rb[i_lo])
                    else:
                        cut = (heads[0] + i_hi) * DH - ws - r_lo
                        blocks.append(jnp.where(row8 < cut, rb[i_lo], rb[i_hi]))
                amv = nd[0:T] * jnp.concatenate(blocks, axis=0) * gtab[ws:ws + T, :]
                pltpu.store(am_v.at[ws:ws + T, j * T:(j + 1) * T], amv, mask=wmask)

    def attention(fast):
        ps = (p0, p1)
        if fast:
            _scores_fast(0, kp, qt, ps[0])
            for g in range(NG):
                if g + 1 < NG:
                    _scores_fast(g + 1, kp, qt, ps[(g + 1) % 2])
                _pv(g, vt, ps[g % 2], g1tab, am_v, ot)
        else:
            lax.fori_loop(0, H, lambda h, c: (_attention_safe(h, kp, qt, vt, g1tab, am_v, ot), c)[1], 0)

    def mem_update():
        for g in range(NG):
            ws = WIN * g
            lhs = jnp.concatenate([vt[ws:ws + T, :], ones_rows], axis=0)
            upd = macc[g] + _dot_nt(lhs, pkt[ws:ws + T, :])
            macc[g] = upd
            mb[g] = jnp.where(bmask[g] != 0.0, upd, 0.0).astype(bf16)

    def load_weight(i, c0=0, c1=D):
        w = w_in[i, :, c0:c1]
        n = c1 - c0
        wf = w.astype(f32)
        c = jnp.sum(wf, axis=0, keepdims=True)
        c_hi = c.astype(bf16).astype(f32)
        r16 = lax.broadcasted_iota(jnp.int32, (16, n), 0)
        extra = jnp.where(r16 >= 4, 0.0, jnp.where(r16 < 2, c_hi, c - c_hi)).astype(bf16)
        w_aug = jnp.concatenate([w, extra, jnp.zeros((KP - D - 16, n), bf16)], axis=0)
        w_t = w_aug.T
        wt[i * D + c0:i * D + c1, :] = w_t
        return w_t, jnp.max(jnp.sum(wf * wf, axis=0, keepdims=True))

    am_v[...] = jnp.zeros_like(am_v)
    ot[...] = jnp.zeros_like(ot)
    with _scope("p_tables"):
        small_b.wait()
        small_r.wait()
        build_tables()
    with _scope("p_wq_wait"):
        wq_lo.wait()
    wq_hi.start()
    w_copies[1].start()
    with _scope("p_wqT"):
        _, cq_lo = load_weight(0, 0, QLO)
    with _scope("p_x0_wait"):
        x_copy(0).wait()
    w_copies[2].start()
    w_copies[3].start()
    HALF = 288
    def q_rows(lhs, r0, r1):
        store_q(_dot(lhs, proj_rhs(0)), ln_scale(0), r0, r1, False)

    QA, QB = _PRO_SPLITS
    with _scope("p_b1"):
        ln1(0)
        q_rows(wt[0:QA, :], 0, QA)
    with _scope("p_wqhi_wait"):
        wq_hi.wait()
    for s in range(1, NSEG):
        x_copy(s).start()
    for c in w_copies[4:]:
        c.start()
    with _scope("p_b2"):
        wq_t, cq_hi = load_weight(0, QLO, D)
        cq = jnp.maximum(cq_lo, cq_hi)
        q_rows(wt[QA:QLO, :], QA, QLO)
        q_rows(wq_t[0:QB - QLO], QLO, QB)
    with _scope("p_wk_wait"):
        w_copies[1].wait()
    with _scope("p_b3"):
        wk_t, ck = load_weight(1)
        q_rows(wt[QB:D, :], QB, D)
        store_k_rows(_dot(wk_t[0:HALF], proj_rhs(0)), ln_scale(0), 0, HALF)
    with _scope("p_wv_wait"):
        w_copies[2].wait()
        w_copies[3].wait()
    with _scope("p_khi_wvT_v"):
        wv_t, cv = load_weight(2)
        wot[...] = w_in[3].T
        store_k_rows(_dot(wt[D + HALF:2 * D, :], proj_rhs(0)), ln_scale(0), HALF, D)
        transpose_k()
        store_v(_dot(wv_t, proj_rhs(0)), ln_scale(0))
    slack = 1.05
    logit_bound2 = (cq * ck) * (slack * D * DH * QSCALE) ** 2
    v_bound2 = cv * (slack * D)
    safe = (logit_bound2 <= SAFE_LOGIT ** 2) & (v_bound2 <= SAFE_V ** 2)

    def body(s, carry):
        more = s + 1 < NSEG
        nxt = jnp.minimum(s + 1, NSEG - 1)

        @pl.when(more)
        def _():
            x_copy(nxt).wait()

        @pl.when(safe)
        def _():
            with _scope("attn"):
                attention(True)

        @pl.when(jnp.logical_not(safe))
        def _():
            attention(False)

        @pl.when(more)
        def _():
            with _scope("blockB"):
                hold = {}
                steps = {
                    "MU": mem_update,
                    "OP": lambda: hold.update(a=[_dot(wot[...], ot[:, t * T:(t + 1) * T].astype(bf16))
                                                    for t in range(NT)]),
                    "LN1": lambda: ln1(nxt),
                    "PR": lambda: project(nxt),
                    "MR": mem_read,
                    "FIN": lambda: [finalize(s, t, 1, hold["a"][t]) for t in range(NT)],
                }
                for n in _ORDER_B:
                    steps[n]()
            out_copy(s).start()
        return carry

    lax.fori_loop(0, NSEG, body, 0)
    with _scope("fin"):
        otb = ot[...].astype(bf16)
        for t in range(NT):
            finalize(NSEG - 1, t, 1, _dot(wot[...], otb[:, t * T:(t + 1) * T]))
        out_copy(NSEG - 1).start()

    bv = best_v[...]
    rmax = jnp.max(bv, axis=1, keepdims=True)
    cand = best_i[...] + lax.broadcasted_iota(jnp.int32, best_i.shape, 1)
    idx = jnp.clip(jnp.min(jnp.where(bv == rmax, cand, S)), 0, S - 1)
    base = pl.multiple_of((idx // T) * T, T)
    lane = idx - base
    blk = (hbuf[:, pl.ds(base, T)] * ab_all[0:1, pl.ds(base, T)]
           + ab_all[8:9, pl.ds(base, T)]).astype(bf16)
    pick = jnp.where(lax.broadcasted_iota(jnp.int32, (16, T), 1) == lane, 1.0, 0.0).astype(bf16)
    xg = _dot_nt(pick, blk).astype(bf16)
    for c in w_copies[4:]:
        c.wait()
    yacc = jnp.zeros((D, T), f32)
    f_lo = 0
    for nt in _MOE_CHUNKS:
        f_hi = f_lo + nt * T
        gt = _dot(xg, wg_v[:, f_lo:f_hi])
        up = _dot(xg, wu_v[:, f_lo:f_hi])
        act = (gt * jax.nn.sigmoid(gt) * up)[0:1].astype(bf16).astype(f32)
        for t in range(nt):
            f0 = f_lo + t * T
            yacc = yacc + wd_v[:, f0:f0 + T].astype(f32) * act[:, t * T:(t + 1) * T]
        f_lo = f_hi
    y = jnp.sum(yacc, axis=1, keepdims=True) * jax.nn.sigmoid(rmax[0:1])
    for s in range(NSEG):
        out_copy(s).wait()
    sel = lax.broadcasted_iota(jnp.int32, (D, T), 1) == lane
    cur = out_v[:, pl.ds(base, T)].astype(f32)
    out_v[:, pl.ds(base, T)] = (cur + jnp.where(sel, y, 0.0)).astype(bf16)
    patch = pltpu.make_async_copy(out_v.at[:, pl.ds(base, T)],
                                  out_hbm.at[0, :, pl.ds(base, T)], sem_o.at[NSEG])
    patch.start()
    patch.wait()


@jax.jit
def pallas_sequential_preLN__memory_aug_infini_attn__moe_arch_mod__prompt_kernel(
    A_x: jax.Array,
    A_wq: jax.Array,
    A_wk: jax.Array,
    A_wv: jax.Array,
    A_wo: jax.Array,
    A_beta: jax.Array,
    B_x: jax.Array,
    B_w_r: jax.Array,
    B_w_gate: jax.Array,
    B_w_up: jax.Array,
    B_w_down: jax.Array,
):
    del B_x
    hbm_spec = pl.BlockSpec(memory_space=pltpu.HBM)
    scratch = [
        pltpu.VMEM((D, S), bf16),
        pltpu.VMEM((4, D, D), bf16),
        pltpu.VMEM((3 * D, KP), bf16),
        pltpu.VMEM((D, D), bf16),
        pltpu.VMEM((D, S), f32),
        pltpu.VMEM((D, F), bf16),
        pltpu.VMEM((D, F), bf16),
        pltpu.VMEM((D, F), bf16),
        pltpu.VMEM((16, S), bf16),
        pltpu.VMEM((8, S), f32),
        pltpu.VMEM((D, L), bf16),
        pltpu.VMEM((D, L), bf16),
        pltpu.VMEM((D, L), bf16),
        pltpu.VMEM((D, L), bf16),
        pltpu.VMEM((D, L), bf16),
        pltpu.VMEM((NG, L, T), bf16),
        pltpu.VMEM((7, NT, L, T), bf16),
        pltpu.VMEM((7, NT, L, T), bf16),
        pltpu.VMEM((D, L), f32),
        pltpu.VMEM((D, L), f32),
        pltpu.VMEM((NG, MROWS, T), f32),
        pltpu.VMEM((NG, MROWS, T), bf16),
        pltpu.VMEM((NG, MROWS, T), f32),
        pltpu.VMEM((D, T), f32),
        pltpu.VMEM((H, 8, T), f32),
        pltpu.VMEM((D, T), f32),
        pltpu.VMEM((16, S), f32),
        pltpu.VMEM((D, S), bf16),
        pltpu.VMEM((8, T), f32),
        pltpu.VMEM((8, T), jnp.int32),
        pltpu.VMEM((8, T), f32),
        pltpu.VMEM((H,), bf16),
        pltpu.VMEM((D,), bf16),
        pltpu.SemaphoreType.DMA((NSEG,)),
        pltpu.SemaphoreType.DMA((10,)),
        pltpu.SemaphoreType.DMA((NSEG + 1,)),
    ]
    out_t = pl.pallas_call(
        _kernel,
        out_shape=jax.ShapeDtypeStruct((1, D, S), bf16),
        in_specs=[hbm_spec] * 10,
        out_specs=hbm_spec,
        scratch_shapes=scratch,
        compiler_params=pltpu.CompilerParams(vmem_limit_bytes=100 * 1024 * 1024),
    )(jnp.transpose(A_x, (0, 2, 1)), A_wq, A_wk, A_wv, A_wo, A_beta,
      B_w_r, B_w_gate, B_w_up, B_w_down.T)
    return jnp.transpose(out_t, (0, 2, 1))
```

```python
import contextlib

import jax
import jax.numpy as jnp
from jax import lax
import jax.experimental.pallas as pl
import jax.experimental.pallas.tpu as pltpu

S = 2048
D = 576
H = 32
DH = 18
NSEG = 4
L = 512
F = 4608
T = 128
NT = L // T
EPS = 1e-5
LOG2E = 1.4426950408889634
QSCALE = (DH ** -0.5) * LOG2E
WIN = 112
GROUPS = (tuple(range(0, 7)), tuple(range(7, 13)), tuple(range(13, 19)),
          tuple(range(19, 25)), tuple(range(25, 32)))
NG = len(GROUPS)
KP = 640
MROWS = T + 16
SAFE_LOGIT = 60.0
SAFE_V = 2.0 ** 40

bf16 = jnp.bfloat16
f32 = jnp.float32
_ORDER_B = ["MU", "OP", "LN1", "PR", "FIN"]
_MOE_CHUNKS = (2,) * 18
_PCOLS = 2
_PRO_SPLITS = (128, 416)
_PROFILE = False


def _scope(name):
    return jax.named_scope(name) if _PROFILE else contextlib.nullcontext()


def _colsum(x):
    return jnp.sum(x, axis=0, keepdims=True)


def _ln_stats(x):
    m = _colsum(x) * (1.0 / D)
    v = jnp.maximum(_colsum(x * x) * (1.0 / D) - m * m, 0.0)
    a = lax.rsqrt(v + EPS)
    return a, -m * a


def _phi(t):
    return jnp.where(t > 0, t + 1.0, jnp.exp(t))


def _dot(a, b):
    return jnp.dot(a, b, preferred_element_type=f32)


def _dot_nt(a, b):
    return lax.dot_general(a, b, (((1,), (1,)), ((), ())), preferred_element_type=f32)


def _dot_tn(a, b):
    return lax.dot_general(a, b, (((0,), (0,)), ((), ())), preferred_element_type=f32)


ROT = (0, 1, 2, 3, 0, 2, 1)
QW = T // 4


def _pack_plan(nh, c):
    tiles = []
    split = []
    for u in range(nh):
        need = [(a + ROT[u]) % 4 for a in range(c, 4)]
        for t in tiles:
            if all(t[q] is None for q in need):
                break
        else:
            bound = max(sum(q in [(a + ROT[v]) % 4 for a in range(c, 4)] for v in range(nh))
                        for q in range(4))
            if len(tiles) >= bound:
                split.append((u, need))
                continue
            t = [None] * 4
            tiles.append(t)
        for q in need:
            t[q] = u
    for u, need in split:
        for q in need:
            next(t for t in tiles if t[q] is None)[q] = u
    return tiles


def _masked_q(qt_ref, g, j):
    ws = WIN * g
    row64 = lax.broadcasted_iota(jnp.int32, (64, T), 0)
    qw32 = pltpu.bitcast(qt_ref[ws:ws + T, j * T:(j + 1) * T], jnp.uint32)
    rolled = {0: qw32}
    qms = []
    for u, h in enumerate(GROUPS[g]):
        if ROT[u] not in rolled:
            rolled[ROT[u]] = pltpu.roll(qw32, ROT[u] * QW, axis=1)
        lo2 = (h * DH - ws) // 2
        qmask = (row64 >= lo2) & (row64 < lo2 + DH // 2)
        qms.append(jnp.where(qmask, rolled[ROT[u]], jnp.uint32(0)))
    return qms


def _select_quarters(sources):
    distinct = []
    for x in sources:
        if x is not None and not any(x is y for y in distinct):
            distinct.append(x)
    distinct.sort(key=lambda y: -sum(x is y for x in sources))
    out = distinct[0]
    lane = lax.broadcasted_iota(jnp.int32, out.shape, 1)
    for y in distinct[1:]:
        mask = None
        for q, x in enumerate(sources):
            if x is y:
                m = (lane >= q * QW) & (lane < (q + 1) * QW)
                mask = m if mask is None else mask | m
        out = jnp.where(mask, y, out)
    return out


def _scores_fast(g, kp_ref, qt_ref, p_ref):
    nh = len(GROUPS[g])
    kk = lax.broadcasted_iota(jnp.int32, (T, T), 0)
    qq = lax.broadcasted_iota(jnp.int32, (T, T), 1)
    causal = {r: kk <= ((qq - r * QW) & (T - 1)) for r in set(ROT[:nh])}
    plans = {c: _pack_plan(nh, c) for c in range(1, 4)}
    for j in range(NT):
        qms = _masked_q(qt_ref, g, j)
        n0 = T * j + QW
        p0 = jnp.exp2(_dot(kp_ref[g, 0:n0, :],
                           jnp.concatenate([pltpu.bitcast(q, bf16) for q in qms], axis=1)))
        pc = {}
        for c in range(1, 4):
            w = [pltpu.bitcast(_select_quarters([None if u is None else qms[u] for u in t]), bf16)
                 for t in plans[c]]
            r0 = T * j + c * QW
            pc[c] = jnp.exp2(_dot(kp_ref[g, r0:r0 + QW, :], jnp.concatenate(w, axis=1)))
        for u in range(nh):
            pu = p0[:, u * T:(u + 1) * T]
            if j > 0:
                p_ref[u, j, 0:j * T, :] = pu[0:j * T].astype(bf16)
            rows = [pu[j * T:n0]]
            for c in range(1, 4):
                src = [None] * 4
                for i, t in enumerate(plans[c]):
                    for q in range(4):
                        if t[q] == u:
                            src[q] = i
                vals = {i: pc[c][:, i * T:(i + 1) * T] for i in set(src) if i is not None}
                rows.append(_select_quarters([None if i is None else vals[i] for i in src]))
            p_ref[u, j, j * T:(j + 1) * T, :] = jnp.where(
                causal[ROT[u]], jnp.concatenate(rows, axis=0), 0.0).astype(bf16)


def _attention_safe(h, kp_ref, qt_ref, vt_ref, g1_ref, am_ref, ot_ref):
    g = jnp.minimum(jnp.maximum(h - 1, 0) // 6, NG - 1)
    ws = pl.multiple_of(g * WIN, 16)
    lo = h * DH - ws
    row128 = lax.broadcasted_iota(jnp.int32, (T, T), 0)
    qmask = (row128 >= lo) & (row128 < lo + DH)
    vs = pl.multiple_of(((h * DH) // 16) * 16, 16)
    off = h * DH - vs
    row32 = lax.broadcasted_iota(jnp.int32, (32, T), 0)
    omask = (row32 >= off) & (row32 < off + DH)
    kk = lax.broadcasted_iota(jnp.int32, (L, T), 0)
    qq = lax.broadcasted_iota(jnp.int32, (L, T), 1)

    def tile(j, c):
        c0 = pl.multiple_of(j * T, T)
        qm = jnp.where(qmask, qt_ref[pl.ds(ws, T), pl.ds(c0, T)].astype(f32), 0.0).astype(bf16)
        s = _dot(kp_ref[g], qm)
        s = jnp.where(kk <= qq + c0, s, -jnp.inf)
        m = jnp.max(s, axis=0, keepdims=True)
        p = jnp.exp2(s - m).astype(bf16)
        acc = _dot(_v_rows(vt_ref, vs, off // 2, L), p)
        l8 = jnp.where(off <= 6, acc[24:32], acc[0:8])
        rl = g1_ref[h] / l8
        o = acc * jnp.concatenate([rl] * 4, axis=0) + am_ref[pl.ds(vs, 32), pl.ds(c0, T)]
        pltpu.store(ot_ref.at[pl.ds(vs, 32), pl.ds(c0, T)], o, mask=omask)
        return c

    lax.fori_loop(0, NT, tile, 0)


def _v_rows(vt_ref, vs, off2, nk):
    row16 = lax.broadcasted_iota(jnp.int32, (16, nk), 0)
    keep = (row16 >= off2) & (row16 < off2 + DH // 2)
    v32 = pltpu.bitcast(vt_ref[pl.ds(vs, 32), 0:nk], jnp.uint32)
    return pltpu.bitcast(jnp.where(keep, v32, jnp.uint32(0x3F803F80)), bf16)


def _pv(g, vt_ref, p_ref, g1_ref, am_ref, ot_ref):
    row32 = lax.broadcasted_iota(jnp.int32, (32, T), 0)
    for u, h in enumerate(GROUPS[g]):
        vs = ((h * DH) // 16) * 16
        off = h * DH - vs
        omask = (row32 >= off) & (row32 < off + DH)
        g1 = g1_ref[h]
        vrows = _v_rows(vt_ref, vs, off // 2, L)
        for j in range(NT):
            nk = T * (j + 1)
            acc = _dot(vrows[:, 0:nk], p_ref[u, j, 0:nk, :])
            l8 = acc[24:32] if off <= 6 else acc[0:8]
            rl = g1 / l8
            o = acc * jnp.concatenate([rl] * 4, axis=0)
            if ROT[u]:
                o = pltpu.roll(o, T - ROT[u] * QW, axis=1)
            o = o + am_ref[vs:vs + 32, j * T:(j + 1) * T]
            pltpu.store(ot_ref.at[vs:vs + 32, j * T:(j + 1) * T], o, mask=omask)


def _kernel(x_hbm, wq_hbm, wk_hbm, wv_hbm, wo_hbm, beta_hbm, wr_hbm, wg_hbm, wu_hbm, wd_hbm,
            out_hbm,
            x_v, w_in, wt, wot, hbuf, wg_v, wu_v, wd_v,
            aug, arow, qt, pqt, kt, pkt, vt, kp, p0, p1, am_v, ot,
            macc, mb, bmask, gtab, g1tab, wrtab, ab_all, out_v, best_v, best_i, wrsum, beta_ref, wr_ref,
            sem_x, sem_w, sem_o):
    def x_copy(s):
        return pltpu.make_async_copy(x_hbm.at[0, :, pl.ds(s * L, L)],
                                     x_v.at[:, pl.ds(s * L, L)], sem_x.at[s])

    def out_copy(s):
        return pltpu.make_async_copy(out_v.at[:, pl.ds(s * L, L)],
                                     out_hbm.at[0, :, pl.ds(s * L, L)], sem_o.at[s])

    w_copies = [
        None,
        pltpu.make_async_copy(wk_hbm, w_in.at[1], sem_w.at[1]),
        pltpu.make_async_copy(wv_hbm, w_in.at[2], sem_w.at[2]),
        pltpu.make_async_copy(wo_hbm, w_in.at[3], sem_w.at[3]),
        pltpu.make_async_copy(wg_hbm, wg_v, sem_w.at[4]),
        pltpu.make_async_copy(wu_hbm, wu_v, sem_w.at[5]),
        pltpu.make_async_copy(wd_hbm, wd_v, sem_w.at[6]),
    ]
    small_b = pltpu.make_async_copy(beta_hbm, beta_ref, sem_w.at[7])
    small_r = pltpu.make_async_copy(wr_hbm, wr_ref, sem_w.at[8])
    QLO = 256
    wq_lo = pltpu.make_async_copy(wq_hbm.at[:, 0:QLO], w_in.at[0, :, 0:QLO], sem_w.at[0])
    wq_hi = pltpu.make_async_copy(wq_hbm.at[:, QLO:D], w_in.at[0, :, QLO:D], sem_w.at[9])
    small_b.start()
    small_r.start()
    wq_lo.start()
    x_copy(0).start()

    def build_tables():
        gate = jax.nn.sigmoid(beta_ref[...].astype(f32).reshape(1, H))
        rr = lax.broadcasted_iota(jnp.int32, (D, H), 0)
        hh = lax.broadcasted_iota(jnp.int32, (D, H), 1)
        onehot = (rr >= hh * DH) & (rr < (hh + 1) * DH)
        gcol = jnp.sum(jnp.where(onehot, gate, 0.0), axis=1, keepdims=True)
        gtab[...] = jnp.broadcast_to(gcol, (D, T))
        hh8 = lax.broadcasted_iota(jnp.int32, (8, H), 1)
        for h in range(H):
            gh = jnp.sum(jnp.where(hh8 == h, gate, 0.0), axis=1, keepdims=True)
            g1tab[h] = jnp.broadcast_to(1.0 - gh, (8, T))
        wr_row = wr_ref[...].astype(f32).reshape(1, D)
        wr_pad = jnp.concatenate([wr_row, jnp.zeros((1, 5 * T - D), f32)], axis=1)
        wrtab[...] = jnp.broadcast_to(wr_pad, (T, 5 * T)).T[0:D]
        wrsum[...] = jnp.broadcast_to(jnp.sum(wr_row, axis=1, keepdims=True), wrsum.shape)

    mr = lax.broadcasted_iota(jnp.int32, (MROWS, T), 0)
    mc = lax.broadcasted_iota(jnp.int32, (MROWS, T), 1)
    for g in range(NG):
        ws = WIN * g
        m = jnp.zeros((MROWS, T), jnp.bool_)
        for i, h in enumerate(GROUPS[g]):
            lo = h * DH - ws
            cols = (mc >= lo) & (mc < lo + DH)
            rows = ((mr >= lo) & (mr < lo + DH) & (mr < T)) | (mr == T + i)
            m = m | (cols & rows)
        bmask[g] = jnp.where(m, 1.0, 0.0)
    macc[...] = jnp.zeros_like(macc)
    mb[...] = jnp.zeros_like(mb)
    best_v[...] = jnp.full(best_v.shape, -jnp.inf, f32)
    best_i[...] = jnp.zeros(best_i.shape, jnp.int32)

    ones_rows = jnp.ones((16, L), bf16)

    def ln1(s):
        col0 = pl.multiple_of(s * L, L)
        xs = x_v[:, pl.ds(col0, L)].astype(f32)
        m = _colsum(xs) * (1.0 / D)
        v = jnp.maximum(_colsum(xs * xs) * (1.0 / D) - m * m, 0.0)
        arow[:, pl.ds(col0, L)] = jnp.broadcast_to(lax.rsqrt(v + EPS), (8, L))
        m_hi = (-m).astype(bf16).astype(f32)
        m_lo = -m - m_hi
        r16 = lax.broadcasted_iota(jnp.int32, (16, L), 0)
        rows = jnp.where(r16 >= 4, 0.0, jnp.where((r16 & 1) == 0, m_hi, m_lo))
        aug[:, pl.ds(col0, L)] = rows.astype(bf16)

    def finalize(s, t0, nt, attn):
        w = nt * T
        col0 = pl.multiple_of(s * L + t0 * T, T)
        hres = x_v[:, pl.ds(col0, w)].astype(f32) + attn
        hbuf[:, pl.ds(col0, w)] = hres
        a, b = _ln_stats(hres)
        wr = jnp.concatenate([wrtab[...]] * nt, axis=1)
        r = _colsum(hres * wr) * a + b * wrsum[0:1, 0:1]
        ab_all[0:8, pl.ds(col0, w)] = jnp.broadcast_to(a, (8, w))
        ab_all[8:16, pl.ds(col0, w)] = jnp.broadcast_to(b, (8, w))
        out_v[:, pl.ds(col0, w)] = (hbuf[:, pl.ds(col0, w)] * (1.0 + a) + b).astype(bf16)
        r = r.astype(bf16).astype(f32)
        bv, bi = best_v[0:1, :], best_i[0:1, :]
        for t in range(nt):
            rt = r[:, t * T:(t + 1) * T]
            better = rt > bv
            bi = jnp.where(better, col0 + t * T, bi)
            bv = jnp.where(better, rt, bv)
        best_i[...] = jnp.broadcast_to(bi, best_i.shape)
        best_v[...] = jnp.broadcast_to(bv, best_v.shape)

    def proj_rhs(s):
        col0 = pl.multiple_of(s * L, L)
        return jnp.concatenate([x_v[:, pl.ds(col0, L)], aug[:, pl.ds(col0, L)],
                                jnp.zeros((KP - D - 16, L), bf16)], axis=0)

    def ln_scale(s):
        return arow[0:1, pl.ds(pl.multiple_of(s * L, L), L)]

    def store_q(raw, a, r0, r1, with_phi=True, cols=slice(None)):
        qt[r0:r1, cols] = (raw * (a * QSCALE)).astype(bf16)
        if with_phi:
            pqt[r0:r1, cols] = _phi(raw * a).astype(bf16)

    def store_k_rows(raw, a, r0, r1):
        k = raw * a
        kt[r0:r1, :] = k.astype(bf16)
        pkt[r0:r1, :] = _phi(k).astype(bf16)

    def transpose_k():
        for g in range(NG):
            kp[g] = kt[WIN * g:WIN * g + T, :].T

    def store_k(raw, a, cols):
        k = raw * a
        kb = k.astype(bf16)
        pkt[:, cols] = _phi(k).astype(bf16)
        for g in range(NG):
            kp[g, cols, :] = kb[WIN * g:WIN * g + T, :].T

    def store_v(raw, a, cols=slice(None)):
        vt[:, cols] = (raw * a).astype(bf16)

    def project(s):
        rhs = proj_rhs(s)
        a = ln_scale(s)
        w = _PCOLS * T
        halves = [slice(c0, c0 + w) for c0 in range(0, L, w)]
        for cols in halves:
            store_q(_dot(wt[0:D, :], rhs[:, cols]), a[:, cols], 0, D, True, cols)
        mem_read()
        for cols in halves:
            store_k(_dot(wt[D:2 * D, :], rhs[:, cols]), a[:, cols], cols)
        for cols in halves:
            store_v(_dot(wt[2 * D:3 * D, :], rhs[:, cols]), a[:, cols], cols)

    def mem_read():
        row128 = lax.broadcasted_iota(jnp.int32, (T, T), 0)
        row8 = lax.broadcasted_iota(jnp.int32, (8, T), 0)
        for g in range(NG):
            ws = WIN * g
            heads = GROUPS[g]
            lo_g, hi_g = heads[0] * DH - ws, (heads[-1] + 1) * DH - ws
            wmask = (row128 >= lo_g) & (row128 < hi_g)
            for j in range(NT):
                nd = _dot(mb[g], pqt[ws:ws + T, j * T:(j + 1) * T])
                rden = 1.0 / (nd[T:T + 8] + 1e-6)
                rb = [jnp.broadcast_to(rden[i:i + 1], (8, T)) for i in range(len(heads))]
                blocks = []
                for b in range(T // 8):
                    r_lo, r_hi = 8 * b, 8 * b + 7
                    i_lo = min(max((r_lo + ws) // DH - heads[0], 0), len(heads) - 1)
                    i_hi = min(max((r_hi + ws) // DH - heads[0], 0), len(heads) - 1)
                    if i_lo == i_hi:
                        blocks.append(rb[i_lo])
                    else:
                        cut = (heads[0] + i_hi) * DH - ws - r_lo
                        blocks.append(jnp.where(row8 < cut, rb[i_lo], rb[i_hi]))
                amv = nd[0:T] * jnp.concatenate(blocks, axis=0) * gtab[ws:ws + T, :]
                pltpu.store(am_v.at[ws:ws + T, j * T:(j + 1) * T], amv, mask=wmask)

    def attention(fast):
        ps = (p0, p1)
        if fast:
            _scores_fast(0, kp, qt, ps[0])
            for g in range(NG):
                if g + 1 < NG:
                    _scores_fast(g + 1, kp, qt, ps[(g + 1) % 2])
                _pv(g, vt, ps[g % 2], g1tab, am_v, ot)
        else:
            lax.fori_loop(0, H, lambda h, c: (_attention_safe(h, kp, qt, vt, g1tab, am_v, ot), c)[1], 0)

    def mem_update():
        for g in range(NG):
            ws = WIN * g
            lhs = jnp.concatenate([vt[ws:ws + T, :], ones_rows], axis=0)
            upd = macc[g] + _dot_nt(lhs, pkt[ws:ws + T, :])
            macc[g] = upd
            mb[g] = jnp.where(bmask[g] != 0.0, upd, 0.0).astype(bf16)

    def load_weight(i, c0=0, c1=D):
        w = w_in[i, :, c0:c1]
        n = c1 - c0
        wf = w.astype(f32)
        c = jnp.sum(wf, axis=0, keepdims=True)
        c_hi = c.astype(bf16).astype(f32)
        r16 = lax.broadcasted_iota(jnp.int32, (16, n), 0)
        extra = jnp.where(r16 >= 4, 0.0, jnp.where(r16 < 2, c_hi, c - c_hi)).astype(bf16)
        w_aug = jnp.concatenate([w, extra, jnp.zeros((KP - D - 16, n), bf16)], axis=0)
        w_t = w_aug.T
        wt[i * D + c0:i * D + c1, :] = w_t
        return w_t, jnp.max(jnp.sum(wf * wf, axis=0, keepdims=True))

    am_v[...] = jnp.zeros_like(am_v)
    ot[...] = jnp.zeros_like(ot)
    with _scope("p_tables"):
        small_b.wait()
        small_r.wait()
        build_tables()
    with _scope("p_wq_wait"):
        wq_lo.wait()
    wq_hi.start()
    w_copies[1].start()
    with _scope("p_wqT"):
        _, cq_lo = load_weight(0, 0, QLO)
    with _scope("p_x0_wait"):
        x_copy(0).wait()
    w_copies[2].start()
    w_copies[3].start()
    HALF = 288
    def q_rows(lhs, r0, r1):
        store_q(_dot(lhs, proj_rhs(0)), ln_scale(0), r0, r1, False)

    QA, QB = _PRO_SPLITS
    with _scope("p_b1"):
        ln1(0)
        q_rows(wt[0:QA, :], 0, QA)
    with _scope("p_wqhi_wait"):
        wq_hi.wait()
    for s in range(1, NSEG):
        x_copy(s).start()
    for c in w_copies[4:]:
        c.start()
    with _scope("p_b2"):
        wq_t, cq_hi = load_weight(0, QLO, D)
        cq = jnp.maximum(cq_lo, cq_hi)
        q_rows(wt[QA:QLO, :], QA, QLO)
        q_rows(wq_t[0:QB - QLO], QLO, QB)
    with _scope("p_wk_wait"):
        w_copies[1].wait()
    with _scope("p_b3"):
        wk_t, ck = load_weight(1)
        q_rows(wt[QB:D, :], QB, D)
        store_k_rows(_dot(wk_t[0:HALF], proj_rhs(0)), ln_scale(0), 0, HALF)
    with _scope("p_wv_wait"):
        w_copies[2].wait()
        w_copies[3].wait()
    with _scope("p_khi_wvT_v"):
        wv_t, cv = load_weight(2)
        wot[...] = w_in[3].T
        store_k_rows(_dot(wt[D + HALF:2 * D, :], proj_rhs(0)), ln_scale(0), HALF, D)
        transpose_k()
        store_v(_dot(wv_t, proj_rhs(0)), ln_scale(0))
    slack = 1.05
    logit_bound2 = (cq * ck) * (slack * D * DH * QSCALE) ** 2
    v_bound2 = cv * (slack * D)
    safe = (logit_bound2 <= SAFE_LOGIT ** 2) & (v_bound2 <= SAFE_V ** 2)

    def body(s, carry):
        more = s + 1 < NSEG
        nxt = jnp.minimum(s + 1, NSEG - 1)

        @pl.when(more)
        def _():
            x_copy(nxt).wait()

        @pl.when(safe)
        def _():
            with _scope("attn"):
                attention(True)

        @pl.when(jnp.logical_not(safe))
        def _():
            attention(False)

        @pl.when(more)
        def _():
            with _scope("blockB"):
                hold = {}
                steps = {
                    "MU": mem_update,
                    "OP": lambda: hold.update(a=[_dot(wot[...], ot[:, t * T:(t + 1) * T].astype(bf16))
                                                    for t in range(NT)]),
                    "LN1": lambda: ln1(nxt),
                    "PR": lambda: project(nxt),
                    "FIN": lambda: [finalize(s, t, 1, hold["a"][t]) for t in range(NT)],
                }
                for n in _ORDER_B:
                    steps[n]()
            out_copy(s).start()
        return carry

    lax.fori_loop(0, NSEG, body, 0)
    with _scope("fin"):
        otb = ot[...].astype(bf16)
        for t in range(NT):
            finalize(NSEG - 1, t, 1, _dot(wot[...], otb[:, t * T:(t + 1) * T]))
        out_copy(NSEG - 1).start()

    bv = best_v[...]
    rmax = jnp.max(bv, axis=1, keepdims=True)
    cand = best_i[...] + lax.broadcasted_iota(jnp.int32, best_i.shape, 1)
    idx = jnp.clip(jnp.min(jnp.where(bv == rmax, cand, S)), 0, S - 1)
    base = pl.multiple_of((idx // T) * T, T)
    lane = idx - base
    blk = (hbuf[:, pl.ds(base, T)] * ab_all[0:1, pl.ds(base, T)]
           + ab_all[8:9, pl.ds(base, T)]).astype(bf16)
    pick = jnp.where(lax.broadcasted_iota(jnp.int32, (16, T), 1) == lane, 1.0, 0.0).astype(bf16)
    xg = _dot_nt(pick, blk).astype(bf16)
    for c in w_copies[4:]:
        c.wait()
    yacc = jnp.zeros((D, T), f32)
    f_lo = 0
    for nt in _MOE_CHUNKS:
        f_hi = f_lo + nt * T
        gt = _dot(xg, wg_v[:, f_lo:f_hi])
        up = _dot(xg, wu_v[:, f_lo:f_hi])
        act = (gt * jax.nn.sigmoid(gt) * up)[0:1].astype(bf16).astype(f32)
        for t in range(nt):
            f0 = f_lo + t * T
            yacc = yacc + wd_v[:, f0:f0 + T].astype(f32) * act[:, t * T:(t + 1) * T]
        f_lo = f_hi
    y = jnp.sum(yacc, axis=1, keepdims=True) * jax.nn.sigmoid(rmax[0:1])
    for s in range(NSEG):
        out_copy(s).wait()
    sel = lax.broadcasted_iota(jnp.int32, (D, T), 1) == lane
    cur = out_v[:, pl.ds(base, T)].astype(f32)
    out_v[:, pl.ds(base, T)] = (cur + jnp.where(sel, y, 0.0)).astype(bf16)
    patch = pltpu.make_async_copy(out_v.at[:, pl.ds(base, T)],
                                  out_hbm.at[0, :, pl.ds(base, T)], sem_o.at[NSEG])
    patch.start()
    patch.wait()


@jax.jit
def pallas_sequential_preLN__memory_aug_infini_attn__moe_arch_mod__prompt_kernel(
    A_x: jax.Array,
    A_wq: jax.Array,
    A_wk: jax.Array,
    A_wv: jax.Array,
    A_wo: jax.Array,
    A_beta: jax.Array,
    B_x: jax.Array,
    B_w_r: jax.Array,
    B_w_gate: jax.Array,
    B_w_up: jax.Array,
    B_w_down: jax.Array,
):
    del B_x
    hbm_spec = pl.BlockSpec(memory_space=pltpu.HBM)
    scratch = [
        pltpu.VMEM((D, S), bf16),
        pltpu.VMEM((4, D, D), bf16),
        pltpu.VMEM((3 * D, KP), bf16),
        pltpu.VMEM((D, D), bf16),
        pltpu.VMEM((D, S), f32),
        pltpu.VMEM((D, F), bf16),
        pltpu.VMEM((D, F), bf16),
        pltpu.VMEM((D, F), bf16),
        pltpu.VMEM((16, S), bf16),
        pltpu.VMEM((8, S), f32),
        pltpu.VMEM((D, L), bf16),
        pltpu.VMEM((D, L), bf16),
        pltpu.VMEM((D, L), bf16),
        pltpu.VMEM((D, L), bf16),
        pltpu.VMEM((D, L), bf16),
        pltpu.VMEM((NG, L, T), bf16),
        pltpu.VMEM((7, NT, L, T), bf16),
        pltpu.VMEM((7, NT, L, T), bf16),
        pltpu.VMEM((D, L), f32),
        pltpu.VMEM((D, L), f32),
        pltpu.VMEM((NG, MROWS, T), f32),
        pltpu.VMEM((NG, MROWS, T), bf16),
        pltpu.VMEM((NG, MROWS, T), f32),
        pltpu.VMEM((D, T), f32),
        pltpu.VMEM((H, 8, T), f32),
        pltpu.VMEM((D, T), f32),
        pltpu.VMEM((16, S), f32),
        pltpu.VMEM((D, S), bf16),
        pltpu.VMEM((8, T), f32),
        pltpu.VMEM((8, T), jnp.int32),
        pltpu.VMEM((8, T), f32),
        pltpu.VMEM((H,), bf16),
        pltpu.VMEM((D,), bf16),
        pltpu.SemaphoreType.DMA((NSEG,)),
        pltpu.SemaphoreType.DMA((10,)),
        pltpu.SemaphoreType.DMA((NSEG + 1,)),
    ]
    out_t = pl.pallas_call(
        _kernel,
        out_shape=jax.ShapeDtypeStruct((1, D, S), bf16),
        in_specs=[hbm_spec] * 10,
        out_specs=hbm_spec,
        scratch_shapes=scratch,
        compiler_params=pltpu.CompilerParams(vmem_limit_bytes=100 * 1024 * 1024),
    )(jnp.transpose(A_x, (0, 2, 1)), A_wq, A_wk, A_wv, A_wo, A_beta,
      B_w_r, B_w_gate, B_w_up, B_w_down.T)
    return jnp.transpose(out_t, (0, 2, 1))
```

```python
import contextlib

import jax
import jax.numpy as jnp
from jax import lax
import jax.experimental.pallas as pl
import jax.experimental.pallas.tpu as pltpu

S = 2048
D = 576
H = 32
DH = 18
NSEG = 4
L = 512
F = 4608
T = 128
NT = L // T
EPS = 1e-5
LOG2E = 1.4426950408889634
QSCALE = (DH ** -0.5) * LOG2E
WIN = 112
GROUPS = (tuple(range(0, 7)), tuple(range(7, 13)), tuple(range(13, 19)),
          tuple(range(19, 25)), tuple(range(25, 32)))
NG = len(GROUPS)
KP = 640
MROWS = T + 16
SAFE_LOGIT = 60.0
SAFE_V = 2.0 ** 40

bf16 = jnp.bfloat16
f32 = jnp.float32
_ORDER_B = ["MU", "OP", "LN1", "PR", "FIN"]
_MOE_CHUNKS = (2,) * 18
_PCOLS = 2
_PRO_SPLITS = (128, 416)
_PROFILE = False


def _scope(name):
    return jax.named_scope(name) if _PROFILE else contextlib.nullcontext()


def _colsum(x):
    return jnp.sum(x, axis=0, keepdims=True)


def _ln_stats(x):
    m = _colsum(x) * (1.0 / D)
    v = jnp.maximum(_colsum(x * x) * (1.0 / D) - m * m, 0.0)
    a = lax.rsqrt(v + EPS)
    return a, -m * a


def _phi(t):
    return jnp.where(t > 0, t + 1.0, jnp.exp(t))


def _dot(a, b):
    return jnp.dot(a, b, preferred_element_type=f32)


def _dot_nt(a, b):
    return lax.dot_general(a, b, (((1,), (1,)), ((), ())), preferred_element_type=f32)


def _dot_tn(a, b):
    return lax.dot_general(a, b, (((0,), (0,)), ((), ())), preferred_element_type=f32)


ROT = (0, 1, 2, 3, 0, 2, 1)
QW = T // 4


def _pack_plan(nh, c):
    tiles = []
    split = []
    for u in range(nh):
        need = [(a + ROT[u]) % 4 for a in range(c, 4)]
        for t in tiles:
            if all(t[q] is None for q in need):
                break
        else:
            bound = max(sum(q in [(a + ROT[v]) % 4 for a in range(c, 4)] for v in range(nh))
                        for q in range(4))
            if len(tiles) >= bound:
                split.append((u, need))
                continue
            t = [None] * 4
            tiles.append(t)
        for q in need:
            t[q] = u
    for u, need in split:
        for q in need:
            next(t for t in tiles if t[q] is None)[q] = u
    return tiles


def _masked_q(qt_ref, g, j):
    ws = WIN * g
    row64 = lax.broadcasted_iota(jnp.int32, (64, T), 0)
    qw32 = pltpu.bitcast(qt_ref[ws:ws + T, j * T:(j + 1) * T], jnp.uint32)
    rolled = {0: qw32}
    qms = []
    for u, h in enumerate(GROUPS[g]):
        if ROT[u] not in rolled:
            rolled[ROT[u]] = pltpu.roll(qw32, ROT[u] * QW, axis=1)
        lo2 = (h * DH - ws) // 2
        qmask = (row64 >= lo2) & (row64 < lo2 + DH // 2)
        qms.append(jnp.where(qmask, rolled[ROT[u]], jnp.uint32(0)))
    return qms


def _select_quarters(sources):
    distinct = []
    for x in sources:
        if x is not None and not any(x is y for y in distinct):
            distinct.append(x)
    distinct.sort(key=lambda y: -sum(x is y for x in sources))
    out = distinct[0]
    lane = lax.broadcasted_iota(jnp.int32, out.shape, 1)
    for y in distinct[1:]:
        mask = None
        for q, x in enumerate(sources):
            if x is y:
                m = (lane >= q * QW) & (lane < (q + 1) * QW)
                mask = m if mask is None else mask | m
        out = jnp.where(mask, y, out)
    return out


def _scores_fast(g, kp_ref, qt_ref, cm_ref, p_ref):
    nh = len(GROUPS[g])
    plans = {c: _pack_plan(nh, c) for c in range(1, 4)}
    for j in range(NT):
        qms = _masked_q(qt_ref, g, j)
        n0 = T * j + QW
        p0 = jnp.exp2(_dot(kp_ref[g, 0:n0, :],
                           jnp.concatenate([pltpu.bitcast(q, bf16) for q in qms], axis=1)))
        pc = {}
        for c in range(1, 4):
            w = [pltpu.bitcast(_select_quarters([None if u is None else qms[u] for u in t]), bf16)
                 for t in plans[c]]
            r0 = T * j + c * QW
            pc[c] = jnp.exp2(_dot(kp_ref[g, r0:r0 + QW, :], jnp.concatenate(w, axis=1)))
        for u in range(nh):
            pu = p0[:, u * T:(u + 1) * T]
            if j > 0:
                p_ref[u, j, 0:j * T, :] = pu[0:j * T].astype(bf16)
            rows = [pu[j * T:n0]]
            for c in range(1, 4):
                src = [None] * 4
                for i, t in enumerate(plans[c]):
                    for q in range(4):
                        if t[q] == u:
                            src[q] = i
                vals = {i: pc[c][:, i * T:(i + 1) * T] for i in set(src) if i is not None}
                rows.append(_select_quarters([None if i is None else vals[i] for i in src]))
            p_ref[u, j, j * T:(j + 1) * T, :] = (
                jnp.concatenate(rows, axis=0) * cm_ref[ROT[u]]).astype(bf16)


def _attention_safe(h, kp_ref, qt_ref, vt_ref, g1_ref, am_ref, ot_ref):
    g = jnp.minimum(jnp.maximum(h - 1, 0) // 6, NG - 1)
    ws = pl.multiple_of(g * WIN, 16)
    lo = h * DH - ws
    row128 = lax.broadcasted_iota(jnp.int32, (T, T), 0)
    qmask = (row128 >= lo) & (row128 < lo + DH)
    vs = pl.multiple_of(((h * DH) // 16) * 16, 16)
    off = h * DH - vs
    row32 = lax.broadcasted_iota(jnp.int32, (32, T), 0)
    omask = (row32 >= off) & (row32 < off + DH)
    kk = lax.broadcasted_iota(jnp.int32, (L, T), 0)
    qq = lax.broadcasted_iota(jnp.int32, (L, T), 1)

    def tile(j, c):
        c0 = pl.multiple_of(j * T, T)
        qm = jnp.where(qmask, qt_ref[pl.ds(ws, T), pl.ds(c0, T)].astype(f32), 0.0).astype(bf16)
        s = _dot(kp_ref[g], qm)
        s = jnp.where(kk <= qq + c0, s, -jnp.inf)
        m = jnp.max(s, axis=0, keepdims=True)
        p = jnp.exp2(s - m).astype(bf16)
        acc = _dot(_v_rows(vt_ref, vs, off // 2, L), p)
        l8 = jnp.where(off <= 6, acc[24:32], acc[0:8])
        rl = g1_ref[h] / l8
        o = acc * jnp.concatenate([rl] * 4, axis=0) + am_ref[pl.ds(vs, 32), pl.ds(c0, T)]
        pltpu.store(ot_ref.at[pl.ds(vs, 32), pl.ds(c0, T)], o, mask=omask)
        return c

    lax.fori_loop(0, NT, tile, 0)


def _v_rows(vt_ref, vs, off2, nk):
    row16 = lax.broadcasted_iota(jnp.int32, (16, nk), 0)
    keep = (row16 >= off2) & (row16 < off2 + DH // 2)
    v32 = pltpu.bitcast(vt_ref[pl.ds(vs, 32), 0:nk], jnp.uint32)
    return pltpu.bitcast(jnp.where(keep, v32, jnp.uint32(0x3F803F80)), bf16)


def _pv(g, vt_ref, p_ref, g1_ref, am_ref, ot_ref):
    row32 = lax.broadcasted_iota(jnp.int32, (32, T), 0)
    for u, h in enumerate(GROUPS[g]):
        vs = ((h * DH) // 16) * 16
        off = h * DH - vs
        omask = (row32 >= off) & (row32 < off + DH)
        g1 = g1_ref[h]
        vrows = _v_rows(vt_ref, vs, off // 2, L)
        for j in range(NT):
            nk = T * (j + 1)
            acc = _dot(vrows[:, 0:nk], p_ref[u, j, 0:nk, :])
            l8 = acc[24:32] if off <= 6 else acc[0:8]
            rl = g1 / l8
            o = acc * jnp.concatenate([rl] * 4, axis=0)
            if ROT[u]:
                o = pltpu.roll(o, T - ROT[u] * QW, axis=1)
            o = o + am_ref[vs:vs + 32, j * T:(j + 1) * T]
            pltpu.store(ot_ref.at[vs:vs + 32, j * T:(j + 1) * T], o, mask=omask)


def _kernel(x_hbm, wq_hbm, wk_hbm, wv_hbm, wo_hbm, beta_hbm, wr_hbm, wg_hbm, wu_hbm, wd_hbm,
            out_hbm,
            x_v, w_in, wt, wot, hbuf, wg_v, wu_v, wd_v,
            aug, arow, qt, pqt, kt, pkt, vt, kp, p0, p1, am_v, ot,
            macc, mb, bmask, cmask, gtab, g1tab, wrtab, ab_all, out_v, best_v, best_i, wrsum, beta_ref, wr_ref,
            sem_x, sem_w, sem_o):
    def x_copy(s):
        return pltpu.make_async_copy(x_hbm.at[0, :, pl.ds(s * L, L)],
                                     x_v.at[:, pl.ds(s * L, L)], sem_x.at[s])

    def out_copy(s):
        return pltpu.make_async_copy(out_v.at[:, pl.ds(s * L, L)],
                                     out_hbm.at[0, :, pl.ds(s * L, L)], sem_o.at[s])

    w_copies = [
        None,
        pltpu.make_async_copy(wk_hbm, w_in.at[1], sem_w.at[1]),
        pltpu.make_async_copy(wv_hbm, w_in.at[2], sem_w.at[2]),
        pltpu.make_async_copy(wo_hbm, w_in.at[3], sem_w.at[3]),
        pltpu.make_async_copy(wg_hbm, wg_v, sem_w.at[4]),
        pltpu.make_async_copy(wu_hbm, wu_v, sem_w.at[5]),
        pltpu.make_async_copy(wd_hbm, wd_v, sem_w.at[6]),
    ]
    small_b = pltpu.make_async_copy(beta_hbm, beta_ref, sem_w.at[7])
    small_r = pltpu.make_async_copy(wr_hbm, wr_ref, sem_w.at[8])
    QLO = 256
    wq_lo = pltpu.make_async_copy(wq_hbm.at[:, 0:QLO], w_in.at[0, :, 0:QLO], sem_w.at[0])
    wq_hi = pltpu.make_async_copy(wq_hbm.at[:, QLO:D], w_in.at[0, :, QLO:D], sem_w.at[9])
    small_b.start()
    small_r.start()
    wq_lo.start()
    x_copy(0).start()

    def build_tables():
        gate = jax.nn.sigmoid(beta_ref[...].astype(f32).reshape(1, H))
        rr = lax.broadcasted_iota(jnp.int32, (D, H), 0)
        hh = lax.broadcasted_iota(jnp.int32, (D, H), 1)
        onehot = (rr >= hh * DH) & (rr < (hh + 1) * DH)
        gcol = jnp.sum(jnp.where(onehot, gate, 0.0), axis=1, keepdims=True)
        gtab[...] = jnp.broadcast_to(gcol, (D, T))
        hh8 = lax.broadcasted_iota(jnp.int32, (8, H), 1)
        for h in range(H):
            gh = jnp.sum(jnp.where(hh8 == h, gate, 0.0), axis=1, keepdims=True)
            g1tab[h] = jnp.broadcast_to(1.0 - gh, (8, T))
        wr_row = wr_ref[...].astype(f32).reshape(1, D)
        wr_pad = jnp.concatenate([wr_row, jnp.zeros((1, 5 * T - D), f32)], axis=1)
        wrtab[...] = jnp.broadcast_to(wr_pad, (T, 5 * T)).T[0:D]
        wrsum[...] = jnp.broadcast_to(jnp.sum(wr_row, axis=1, keepdims=True), wrsum.shape)

    mr = lax.broadcasted_iota(jnp.int32, (MROWS, T), 0)
    mc = lax.broadcasted_iota(jnp.int32, (MROWS, T), 1)
    for g in range(NG):
        ws = WIN * g
        m = jnp.zeros((MROWS, T), jnp.bool_)
        for i, h in enumerate(GROUPS[g]):
            lo = h * DH - ws
            cols = (mc >= lo) & (mc < lo + DH)
            rows = ((mr >= lo) & (mr < lo + DH) & (mr < T)) | (mr == T + i)
            m = m | (cols & rows)
        bmask[g] = jnp.where(m, 1.0, 0.0)
    kk = lax.broadcasted_iota(jnp.int32, (T, T), 0)
    qq = lax.broadcasted_iota(jnp.int32, (T, T), 1)
    for r in range(4):
        cmask[r] = jnp.where(kk <= ((qq - r * QW) & (T - 1)), 1.0, 0.0)
    macc[...] = jnp.zeros_like(macc)
    mb[...] = jnp.zeros_like(mb)
    best_v[...] = jnp.full(best_v.shape, -jnp.inf, f32)
    best_i[...] = jnp.zeros(best_i.shape, jnp.int32)

    ones_rows = jnp.ones((16, L), bf16)

    def ln1(s):
        col0 = pl.multiple_of(s * L, L)
        xs = x_v[:, pl.ds(col0, L)].astype(f32)
        m = _colsum(xs) * (1.0 / D)
        v = jnp.maximum(_colsum(xs * xs) * (1.0 / D) - m * m, 0.0)
        arow[:, pl.ds(col0, L)] = jnp.broadcast_to(lax.rsqrt(v + EPS), (8, L))
        m_hi = (-m).astype(bf16).astype(f32)
        m_lo = -m - m_hi
        r16 = lax.broadcasted_iota(jnp.int32, (16, L), 0)
        rows = jnp.where(r16 >= 4, 0.0, jnp.where((r16 & 1) == 0, m_hi, m_lo))
        aug[:, pl.ds(col0, L)] = rows.astype(bf16)

    def finalize(s, t0, nt, attn):
        w = nt * T
        col0 = pl.multiple_of(s * L + t0 * T, T)
        hres = x_v[:, pl.ds(col0, w)].astype(f32) + attn
        hbuf[:, pl.ds(col0, w)] = hres
        a, b = _ln_stats(hres)
        wr = jnp.concatenate([wrtab[...]] * nt, axis=1)
        r = _colsum(hres * wr) * a + b * wrsum[0:1, 0:1]
        ab_all[0:8, pl.ds(col0, w)] = jnp.broadcast_to(a, (8, w))
        ab_all[8:16, pl.ds(col0, w)] = jnp.broadcast_to(b, (8, w))
        out_v[:, pl.ds(col0, w)] = (hbuf[:, pl.ds(col0, w)] * (1.0 + a) + b).astype(bf16)
        r = r.astype(bf16).astype(f32)
        bv, bi = best_v[0:1, :], best_i[0:1, :]
        for t in range(nt):
            rt = r[:, t * T:(t + 1) * T]
            better = rt > bv
            bi = jnp.where(better, col0 + t * T, bi)
            bv = jnp.where(better, rt, bv)
        best_i[...] = jnp.broadcast_to(bi, best_i.shape)
        best_v[...] = jnp.broadcast_to(bv, best_v.shape)

    def proj_rhs(s):
        col0 = pl.multiple_of(s * L, L)
        return jnp.concatenate([x_v[:, pl.ds(col0, L)], aug[:, pl.ds(col0, L)],
                                jnp.zeros((KP - D - 16, L), bf16)], axis=0)

    def ln_scale(s):
        return arow[0:1, pl.ds(pl.multiple_of(s * L, L), L)]

    def store_q(raw, a, r0, r1, with_phi=True, cols=slice(None)):
        qt[r0:r1, cols] = (raw * (a * QSCALE)).astype(bf16)
        if with_phi:
            pqt[r0:r1, cols] = _phi(raw * a).astype(bf16)

    def store_k_rows(raw, a, r0, r1):
        k = raw * a
        kt[r0:r1, :] = k.astype(bf16)
        pkt[r0:r1, :] = _phi(k).astype(bf16)

    def transpose_k():
        for g in range(NG):
            kp[g] = kt[WIN * g:WIN * g + T, :].T

    def store_k(raw, a, cols):
        k = raw * a
        kb = k.astype(bf16)
        pkt[:, cols] = _phi(k).astype(bf16)
        for g in range(NG):
            kp[g, cols, :] = kb[WIN * g:WIN * g + T, :].T

    def store_v(raw, a, cols=slice(None)):
        vt[:, cols] = (raw * a).astype(bf16)

    def project(s):
        rhs = proj_rhs(s)
        a = ln_scale(s)
        w = _PCOLS * T
        halves = [slice(c0, c0 + w) for c0 in range(0, L, w)]
        for cols in halves:
            store_q(_dot(wt[0:D, :], rhs[:, cols]), a[:, cols], 0, D, True, cols)
        mem_read()
        for cols in halves:
            store_k(_dot(wt[D:2 * D, :], rhs[:, cols]), a[:, cols], cols)
        for cols in halves:
            store_v(_dot(wt[2 * D:3 * D, :], rhs[:, cols]), a[:, cols], cols)

    def mem_read():
        row128 = lax.broadcasted_iota(jnp.int32, (T, T), 0)
        row8 = lax.broadcasted_iota(jnp.int32, (8, T), 0)
        for g in range(NG):
            ws = WIN * g
            heads = GROUPS[g]
            lo_g, hi_g = heads[0] * DH - ws, (heads[-1] + 1) * DH - ws
            wmask = (row128 >= lo_g) & (row128 < hi_g)
            for j in range(NT):
                nd = _dot(mb[g], pqt[ws:ws + T, j * T:(j + 1) * T])
                rden = 1.0 / (nd[T:T + 8] + 1e-6)
                rb = [jnp.broadcast_to(rden[i:i + 1], (8, T)) for i in range(len(heads))]
                blocks = []
                for b in range(T // 8):
                    r_lo, r_hi = 8 * b, 8 * b + 7
                    i_lo = min(max((r_lo + ws) // DH - heads[0], 0), len(heads) - 1)
                    i_hi = min(max((r_hi + ws) // DH - heads[0], 0), len(heads) - 1)
                    if i_lo == i_hi:
                        blocks.append(rb[i_lo])
                    else:
                        cut = (heads[0] + i_hi) * DH - ws - r_lo
                        blocks.append(jnp.where(row8 < cut, rb[i_lo], rb[i_hi]))
                amv = nd[0:T] * jnp.concatenate(blocks, axis=0) * gtab[ws:ws + T, :]
                pltpu.store(am_v.at[ws:ws + T, j * T:(j + 1) * T], amv, mask=wmask)

    def attention(fast):
        ps = (p0, p1)
        if fast:
            _scores_fast(0, kp, qt, cmask, ps[0])
            for g in range(NG):
                if g + 1 < NG:
                    _scores_fast(g + 1, kp, qt, cmask, ps[(g + 1) % 2])
                _pv(g, vt, ps[g % 2], g1tab, am_v, ot)
        else:
            lax.fori_loop(0, H, lambda h, c: (_attention_safe(h, kp, qt, vt, g1tab, am_v, ot), c)[1], 0)

    def mem_update():
        for g in range(NG):
            ws = WIN * g
            lhs = jnp.concatenate([vt[ws:ws + T, :], ones_rows], axis=0)
            upd = macc[g] + _dot_nt(lhs, pkt[ws:ws + T, :])
            macc[g] = upd
            mb[g] = jnp.where(bmask[g] != 0.0, upd, 0.0).astype(bf16)

    def load_weight(i, c0=0, c1=D):
        w = w_in[i, :, c0:c1]
        n = c1 - c0
        wf = w.astype(f32)
        c = jnp.sum(wf, axis=0, keepdims=True)
        c_hi = c.astype(bf16).astype(f32)
        r16 = lax.broadcasted_iota(jnp.int32, (16, n), 0)
        extra = jnp.where(r16 >= 4, 0.0, jnp.where(r16 < 2, c_hi, c - c_hi)).astype(bf16)
        w_aug = jnp.concatenate([w, extra, jnp.zeros((KP - D - 16, n), bf16)], axis=0)
        w_t = w_aug.T
        wt[i * D + c0:i * D + c1, :] = w_t
        return w_t, jnp.max(jnp.sum(wf * wf, axis=0, keepdims=True))

    am_v[...] = jnp.zeros_like(am_v)
    ot[...] = jnp.zeros_like(ot)
    with _scope("p_tables"):
        small_b.wait()
        small_r.wait()
        build_tables()
    with _scope("p_wq_wait"):
        wq_lo.wait()
    wq_hi.start()
    w_copies[1].start()
    with _scope("p_wqT"):
        _, cq_lo = load_weight(0, 0, QLO)
    with _scope("p_x0_wait"):
        x_copy(0).wait()
    w_copies[2].start()
    w_copies[3].start()
    HALF = 288
    def q_rows(lhs, r0, r1):
        store_q(_dot(lhs, proj_rhs(0)), ln_scale(0), r0, r1, False)

    QA, QB = _PRO_SPLITS
    with _scope("p_b1"):
        ln1(0)
        q_rows(wt[0:QA, :], 0, QA)
    with _scope("p_wqhi_wait"):
        wq_hi.wait()
    for s in range(1, NSEG):
        x_copy(s).start()
    for c in w_copies[4:]:
        c.start()
    with _scope("p_b2"):
        wq_t, cq_hi = load_weight(0, QLO, D)
        cq = jnp.maximum(cq_lo, cq_hi)
        q_rows(wt[QA:QLO, :], QA, QLO)
        q_rows(wq_t[0:QB - QLO], QLO, QB)
    with _scope("p_wk_wait"):
        w_copies[1].wait()
    with _scope("p_b3"):
        wk_t, ck = load_weight(1)
        q_rows(wt[QB:D, :], QB, D)
        store_k_rows(_dot(wk_t[0:HALF], proj_rhs(0)), ln_scale(0), 0, HALF)
    with _scope("p_wv_wait"):
        w_copies[2].wait()
        w_copies[3].wait()
    with _scope("p_khi_wvT_v"):
        wv_t, cv = load_weight(2)
        wot[...] = w_in[3].T
        store_k_rows(_dot(wt[D + HALF:2 * D, :], proj_rhs(0)), ln_scale(0), HALF, D)
        transpose_k()
        store_v(_dot(wv_t, proj_rhs(0)), ln_scale(0))
    slack = 1.05
    logit_bound2 = (cq * ck) * (slack * D * DH * QSCALE) ** 2
    v_bound2 = cv * (slack * D)
    safe = (logit_bound2 <= SAFE_LOGIT ** 2) & (v_bound2 <= SAFE_V ** 2)

    def body(s, carry):
        more = s + 1 < NSEG
        nxt = jnp.minimum(s + 1, NSEG - 1)

        @pl.when(more)
        def _():
            x_copy(nxt).wait()

        @pl.when(safe)
        def _():
            with _scope("attn"):
                attention(True)

        @pl.when(jnp.logical_not(safe))
        def _():
            attention(False)

        @pl.when(more)
        def _():
            with _scope("blockB"):
                hold = {}
                steps = {
                    "MU": mem_update,
                    "OP": lambda: hold.update(a=[_dot(wot[...], ot[:, t * T:(t + 1) * T].astype(bf16))
                                                    for t in range(NT)]),
                    "LN1": lambda: ln1(nxt),
                    "PR": lambda: project(nxt),
                    "FIN": lambda: [finalize(s, t, 1, hold["a"][t]) for t in range(NT)],
                }
                for n in _ORDER_B:
                    steps[n]()
            out_copy(s).start()
        return carry

    lax.fori_loop(0, NSEG, body, 0)
    with _scope("fin"):
        otb = ot[...].astype(bf16)
        for t in range(NT):
            finalize(NSEG - 1, t, 1, _dot(wot[...], otb[:, t * T:(t + 1) * T]))
        out_copy(NSEG - 1).start()

    bv = best_v[...]
    rmax = jnp.max(bv, axis=1, keepdims=True)
    cand = best_i[...] + lax.broadcasted_iota(jnp.int32, best_i.shape, 1)
    idx = jnp.clip(jnp.min(jnp.where(bv == rmax, cand, S)), 0, S - 1)
    base = pl.multiple_of((idx // T) * T, T)
    lane = idx - base
    blk = (hbuf[:, pl.ds(base, T)] * ab_all[0:1, pl.ds(base, T)]
           + ab_all[8:9, pl.ds(base, T)]).astype(bf16)
    pick = jnp.where(lax.broadcasted_iota(jnp.int32, (16, T), 1) == lane, 1.0, 0.0).astype(bf16)
    xg = _dot_nt(pick, blk).astype(bf16)
    for c in w_copies[4:]:
        c.wait()
    yacc = jnp.zeros((D, T), f32)
    f_lo = 0
    for nt in _MOE_CHUNKS:
        f_hi = f_lo + nt * T
        gt = _dot(xg, wg_v[:, f_lo:f_hi])
        up = _dot(xg, wu_v[:, f_lo:f_hi])
        act = (gt * jax.nn.sigmoid(gt) * up)[0:1].astype(bf16).astype(f32)
        for t in range(nt):
            f0 = f_lo + t * T
            yacc = yacc + wd_v[:, f0:f0 + T].astype(f32) * act[:, t * T:(t + 1) * T]
        f_lo = f_hi
    y = jnp.sum(yacc, axis=1, keepdims=True) * jax.nn.sigmoid(rmax[0:1])
    for s in range(NSEG):
        out_copy(s).wait()
    sel = lax.broadcasted_iota(jnp.int32, (D, T), 1) == lane
    cur = out_v[:, pl.ds(base, T)].astype(f32)
    out_v[:, pl.ds(base, T)] = (cur + jnp.where(sel, y, 0.0)).astype(bf16)
    patch = pltpu.make_async_copy(out_v.at[:, pl.ds(base, T)],
                                  out_hbm.at[0, :, pl.ds(base, T)], sem_o.at[NSEG])
    patch.start()
    patch.wait()


@jax.jit
def pallas_sequential_preLN__memory_aug_infini_attn__moe_arch_mod__prompt_kernel(
    A_x: jax.Array,
    A_wq: jax.Array,
    A_wk: jax.Array,
    A_wv: jax.Array,
    A_wo: jax.Array,
    A_beta: jax.Array,
    B_x: jax.Array,
    B_w_r: jax.Array,
    B_w_gate: jax.Array,
    B_w_up: jax.Array,
    B_w_down: jax.Array,
):
    del B_x
    hbm_spec = pl.BlockSpec(memory_space=pltpu.HBM)
    scratch = [
        pltpu.VMEM((D, S), bf16),
        pltpu.VMEM((4, D, D), bf16),
        pltpu.VMEM((3 * D, KP), bf16),
        pltpu.VMEM((D, D), bf16),
        pltpu.VMEM((D, S), f32),
        pltpu.VMEM((D, F), bf16),
        pltpu.VMEM((D, F), bf16),
        pltpu.VMEM((D, F), bf16),
        pltpu.VMEM((16, S), bf16),
        pltpu.VMEM((8, S), f32),
        pltpu.VMEM((D, L), bf16),
        pltpu.VMEM((D, L), bf16),
        pltpu.VMEM((D, L), bf16),
        pltpu.VMEM((D, L), bf16),
        pltpu.VMEM((D, L), bf16),
        pltpu.VMEM((NG, L, T), bf16),
        pltpu.VMEM((7, NT, L, T), bf16),
        pltpu.VMEM((7, NT, L, T), bf16),
        pltpu.VMEM((D, L), f32),
        pltpu.VMEM((D, L), f32),
        pltpu.VMEM((NG, MROWS, T), f32),
        pltpu.VMEM((NG, MROWS, T), bf16),
        pltpu.VMEM((NG, MROWS, T), f32),
        pltpu.VMEM((4, T, T), f32),
        pltpu.VMEM((D, T), f32),
        pltpu.VMEM((H, 8, T), f32),
        pltpu.VMEM((D, T), f32),
        pltpu.VMEM((16, S), f32),
        pltpu.VMEM((D, S), bf16),
        pltpu.VMEM((8, T), f32),
        pltpu.VMEM((8, T), jnp.int32),
        pltpu.VMEM((8, T), f32),
        pltpu.VMEM((H,), bf16),
        pltpu.VMEM((D,), bf16),
        pltpu.SemaphoreType.DMA((NSEG,)),
        pltpu.SemaphoreType.DMA((10,)),
        pltpu.SemaphoreType.DMA((NSEG + 1,)),
    ]
    out_t = pl.pallas_call(
        _kernel,
        out_shape=jax.ShapeDtypeStruct((1, D, S), bf16),
        in_specs=[hbm_spec] * 10,
        out_specs=hbm_spec,
        scratch_shapes=scratch,
        compiler_params=pltpu.CompilerParams(vmem_limit_bytes=100 * 1024 * 1024),
    )(jnp.transpose(A_x, (0, 2, 1)), A_wq, A_wk, A_wv, A_wo, A_beta,
      B_w_r, B_w_gate, B_w_up, B_w_down.T)
    return jnp.transpose(out_t, (0, 2, 1))
```

```python
import contextlib

import jax
import jax.numpy as jnp
from jax import lax
import jax.experimental.pallas as pl
import jax.experimental.pallas.tpu as pltpu

S = 2048
D = 576
H = 32
DH = 18
NSEG = 4
L = 512
F = 4608
T = 128
NT = L // T
EPS = 1e-5
LOG2E = 1.4426950408889634
QSCALE = (DH ** -0.5) * LOG2E
WIN = 112
GROUPS = (tuple(range(0, 7)), tuple(range(7, 13)), tuple(range(13, 19)),
          tuple(range(19, 25)), tuple(range(25, 32)))
NG = len(GROUPS)
KP = 640
MROWS = T + 16
SAFE_LOGIT = 60.0
SAFE_V = 2.0 ** 40

bf16 = jnp.bfloat16
f32 = jnp.float32
_ORDER_B = ["MU", "OP", "LN1", "PR", "FIN"]
_MOE_CHUNKS = (2,) * 18
_PCOLS = 2
_PRO_SPLITS = (128, 416)
_PROFILE = False


def _scope(name):
    return jax.named_scope(name) if _PROFILE else contextlib.nullcontext()


def _colsum(x):
    return jnp.sum(x, axis=0, keepdims=True)


def _ln_stats(x):
    m = _colsum(x) * (1.0 / D)
    v = jnp.maximum(_colsum(x * x) * (1.0 / D) - m * m, 0.0)
    a = lax.rsqrt(v + EPS)
    return a, -m * a


def _phi(t):
    return jnp.where(t > 0, t + 1.0, jnp.exp(t))


def _dot(a, b):
    return jnp.dot(a, b, preferred_element_type=f32)


def _dot_nt(a, b):
    return lax.dot_general(a, b, (((1,), (1,)), ((), ())), preferred_element_type=f32)


def _dot_tn(a, b):
    return lax.dot_general(a, b, (((0,), (0,)), ((), ())), preferred_element_type=f32)


ROT = (0, 1, 2, 3, 0, 2, 1)
QW = T // 4


def _pack_plan(nh, c):
    tiles = []
    split = []
    for u in range(nh):
        need = [(a + ROT[u]) % 4 for a in range(c, 4)]
        for t in tiles:
            if all(t[q] is None for q in need):
                break
        else:
            bound = max(sum(q in [(a + ROT[v]) % 4 for a in range(c, 4)] for v in range(nh))
                        for q in range(4))
            if len(tiles) >= bound:
                split.append((u, need))
                continue
            t = [None] * 4
            tiles.append(t)
        for q in need:
            t[q] = u
    for u, need in split:
        for q in need:
            next(t for t in tiles if t[q] is None)[q] = u
    return tiles


def _masked_q(qt_ref, g, j):
    ws = WIN * g
    row64 = lax.broadcasted_iota(jnp.int32, (64, T), 0)
    qw32 = pltpu.bitcast(qt_ref[ws:ws + T, j * T:(j + 1) * T], jnp.uint32)
    rolled = {0: qw32}
    qms = []
    for u, h in enumerate(GROUPS[g]):
        if ROT[u] not in rolled:
            rolled[ROT[u]] = pltpu.roll(qw32, ROT[u] * QW, axis=1)
        lo2 = (h * DH - ws) // 2
        qmask = (row64 >= lo2) & (row64 < lo2 + DH // 2)
        qms.append(jnp.where(qmask, rolled[ROT[u]], jnp.uint32(0)))
    return qms


def _select_quarters(sources):
    distinct = []
    for x in sources:
        if x is not None and not any(x is y for y in distinct):
            distinct.append(x)
    distinct.sort(key=lambda y: -sum(x is y for x in sources))
    out = distinct[0]
    lane = lax.broadcasted_iota(jnp.int32, out.shape, 1)
    for y in distinct[1:]:
        mask = None
        for q, x in enumerate(sources):
            if x is y:
                m = (lane >= q * QW) & (lane < (q + 1) * QW)
                mask = m if mask is None else mask | m
        out = jnp.where(mask, y, out)
    return out


def _scores_fast(g, kp_ref, qt_ref, cm_ref, p_ref):
    nh = len(GROUPS[g])
    plans = {c: _pack_plan(nh, c) for c in range(1, 4)}
    for j in range(NT):
        qms = _masked_q(qt_ref, g, j)
        n0 = T * j + QW
        p0 = jnp.exp2(_dot(kp_ref[g, 0:n0, :],
                           jnp.concatenate([pltpu.bitcast(q, bf16) for q in qms], axis=1)))
        pc = {}
        for c in range(1, 4):
            w = [pltpu.bitcast(_select_quarters([None if u is None else qms[u] for u in t]), bf16)
                 for t in plans[c]]
            r0 = T * j + c * QW
            pc[c] = jnp.exp2(_dot(kp_ref[g, r0:r0 + QW, :], jnp.concatenate(w, axis=1)))
        for u in range(nh):
            pu = p0[:, u * T:(u + 1) * T]
            if j > 0:
                p_ref[u, j, 0:j * T, :] = pu[0:j * T].astype(bf16)
            rows = [pu[j * T:n0]]
            for c in range(1, 4):
                src = [None] * 4
                for i, t in enumerate(plans[c]):
                    for q in range(4):
                        if t[q] == u:
                            src[q] = i
                vals = {i: pc[c][:, i * T:(i + 1) * T] for i in set(src) if i is not None}
                rows.append(_select_quarters([None if i is None else vals[i] for i in src]))
            p_ref[u, j, j * T:(j + 1) * T, :] = (
                jnp.concatenate(rows, axis=0) * cm_ref[ROT[u]]).astype(bf16)


def _attention_safe(h, kp_ref, qt_ref, vt_ref, g1_ref, am_ref, ot_ref):
    g = jnp.minimum(jnp.maximum(h - 1, 0) // 6, NG - 1)
    ws = pl.multiple_of(g * WIN, 16)
    lo = h * DH - ws
    row128 = lax.broadcasted_iota(jnp.int32, (T, T), 0)
    qmask = (row128 >= lo) & (row128 < lo + DH)
    vs = pl.multiple_of(((h * DH) // 16) * 16, 16)
    off = h * DH - vs
    row32 = lax.broadcasted_iota(jnp.int32, (32, T), 0)
    omask = (row32 >= off) & (row32 < off + DH)
    kk = lax.broadcasted_iota(jnp.int32, (L, T), 0)
    qq = lax.broadcasted_iota(jnp.int32, (L, T), 1)

    def tile(j, c):
        c0 = pl.multiple_of(j * T, T)
        qm = jnp.where(qmask, qt_ref[pl.ds(ws, T), pl.ds(c0, T)].astype(f32), 0.0).astype(bf16)
        s = _dot(kp_ref[g], qm)
        s = jnp.where(kk <= qq + c0, s, -jnp.inf)
        m = jnp.max(s, axis=0, keepdims=True)
        p = jnp.exp2(s - m).astype(bf16)
        acc = _dot(_v_rows(vt_ref, vs, off // 2, L), p)
        l8 = jnp.where(off <= 6, acc[24:32], acc[0:8])
        rl = g1_ref[h] / l8
        o = acc * jnp.concatenate([rl] * 4, axis=0) + am_ref[pl.ds(vs, 32), pl.ds(c0, T)]
        pltpu.store(ot_ref.at[pl.ds(vs, 32), pl.ds(c0, T)], o, mask=omask)
        return c

    lax.fori_loop(0, NT, tile, 0)


def _v_rows(vt_ref, vs, off2, nk):
    row16 = lax.broadcasted_iota(jnp.int32, (16, nk), 0)
    keep = (row16 >= off2) & (row16 < off2 + DH // 2)
    v32 = pltpu.bitcast(vt_ref[pl.ds(vs, 32), 0:nk], jnp.uint32)
    return pltpu.bitcast(jnp.where(keep, v32, jnp.uint32(0x3F803F80)), bf16)


def _pv(g, vt_ref, p_ref, g1_ref, am_ref, ot_ref):
    row32 = lax.broadcasted_iota(jnp.int32, (32, T), 0)
    for u, h in enumerate(GROUPS[g]):
        vs = ((h * DH) // 16) * 16
        off = h * DH - vs
        omask = (row32 >= off) & (row32 < off + DH)
        g1 = g1_ref[h]
        vrows = _v_rows(vt_ref, vs, off // 2, L)
        for j in range(NT):
            nk = T * (j + 1)
            acc = _dot(vrows[:, 0:nk], p_ref[u, j, 0:nk, :])
            l8 = acc[24:32] if off <= 6 else acc[0:8]
            rl = g1 / l8
            o = acc * jnp.concatenate([rl] * 4, axis=0)
            if ROT[u]:
                o = pltpu.roll(o, T - ROT[u] * QW, axis=1)
            o = o + am_ref[vs:vs + 32, j * T:(j + 1) * T]
            pltpu.store(ot_ref.at[vs:vs + 32, j * T:(j + 1) * T], o, mask=omask)


def _kernel(x_hbm, wq_hbm, wk_hbm, wv_hbm, wo_hbm, beta_hbm, wr_hbm, wg_hbm, wu_hbm, wd_hbm,
            out_hbm,
            x_v, w_in, wt, wot, hbuf, wg_v, wu_v, wd_v,
            aug, arow, qt, pqt, kt, pkt, vt, kp, p0, p1, am_v, ot,
            macc, mb, bmask, cmask, g1tab, wrtab, ab_all, out_v, best_v, best_i, wrsum, beta_ref, wr_ref,
            sem_x, sem_w, sem_o):
    def x_copy(s):
        return pltpu.make_async_copy(x_hbm.at[0, :, pl.ds(s * L, L)],
                                     x_v.at[:, pl.ds(s * L, L)], sem_x.at[s])

    def out_copy(s):
        return pltpu.make_async_copy(out_v.at[:, pl.ds(s * L, L)],
                                     out_hbm.at[0, :, pl.ds(s * L, L)], sem_o.at[s])

    w_copies = [
        None,
        pltpu.make_async_copy(wk_hbm, w_in.at[1], sem_w.at[1]),
        pltpu.make_async_copy(wv_hbm, w_in.at[2], sem_w.at[2]),
        pltpu.make_async_copy(wo_hbm, w_in.at[3], sem_w.at[3]),
        pltpu.make_async_copy(wg_hbm, wg_v, sem_w.at[4]),
        pltpu.make_async_copy(wu_hbm, wu_v, sem_w.at[5]),
        pltpu.make_async_copy(wd_hbm, wd_v, sem_w.at[6]),
    ]
    small_b = pltpu.make_async_copy(beta_hbm, beta_ref, sem_w.at[7])
    small_r = pltpu.make_async_copy(wr_hbm, wr_ref, sem_w.at[8])
    QLO = 256
    wq_lo = pltpu.make_async_copy(wq_hbm.at[:, 0:QLO], w_in.at[0, :, 0:QLO], sem_w.at[0])
    wq_hi = pltpu.make_async_copy(wq_hbm.at[:, QLO:D], w_in.at[0, :, QLO:D], sem_w.at[9])
    small_b.start()
    small_r.start()
    wq_lo.start()
    x_copy(0).start()

    def build_tables():
        gate = jax.nn.sigmoid(beta_ref[...].astype(f32).reshape(1, H))
        hh8 = lax.broadcasted_iota(jnp.int32, (8, H), 1)
        for h in range(H):
            gh = jnp.sum(jnp.where(hh8 == h, gate, 0.0), axis=1, keepdims=True)
            g1tab[h] = jnp.broadcast_to(1.0 - gh, (8, T))
        wr_row = wr_ref[...].astype(f32).reshape(1, D)
        wr_pad = jnp.concatenate([wr_row, jnp.zeros((1, 5 * T - D), f32)], axis=1)
        wrtab[...] = jnp.broadcast_to(wr_pad, (T, 5 * T)).T[0:D]
        wrsum[...] = jnp.broadcast_to(jnp.sum(wr_row, axis=1, keepdims=True), wrsum.shape)

    mr = lax.broadcasted_iota(jnp.int32, (MROWS, T), 0)
    mc = lax.broadcasted_iota(jnp.int32, (MROWS, T), 1)
    for g in range(NG):
        ws = WIN * g
        m = jnp.zeros((MROWS, T), jnp.bool_)
        for i, h in enumerate(GROUPS[g]):
            lo = h * DH - ws
            cols = (mc >= lo) & (mc < lo + DH)
            rows = ((mr >= lo) & (mr < lo + DH) & (mr < T)) | (mr == T + i)
            m = m | (cols & rows)
        bmask[g] = jnp.where(m, 1.0, 0.0)
    kk = lax.broadcasted_iota(jnp.int32, (T, T), 0)
    qq = lax.broadcasted_iota(jnp.int32, (T, T), 1)
    for r in range(4):
        cmask[r] = jnp.where(kk <= ((qq - r * QW) & (T - 1)), 1.0, 0.0)
    macc[...] = jnp.zeros_like(macc)
    mb[...] = jnp.zeros_like(mb)
    best_v[...] = jnp.full(best_v.shape, -jnp.inf, f32)
    best_i[...] = jnp.zeros(best_i.shape, jnp.int32)

    ones_rows = jnp.ones((16, L), bf16)

    def ln1(s):
        col0 = pl.multiple_of(s * L, L)
        xs = x_v[:, pl.ds(col0, L)].astype(f32)
        m = _colsum(xs) * (1.0 / D)
        v = jnp.maximum(_colsum(xs * xs) * (1.0 / D) - m * m, 0.0)
        arow[:, pl.ds(col0, L)] = jnp.broadcast_to(lax.rsqrt(v + EPS), (8, L))
        m_hi = (-m).astype(bf16).astype(f32)
        m_lo = -m - m_hi
        r16 = lax.broadcasted_iota(jnp.int32, (16, L), 0)
        rows = jnp.where(r16 >= 4, 0.0, jnp.where((r16 & 1) == 0, m_hi, m_lo))
        aug[:, pl.ds(col0, L)] = rows.astype(bf16)

    def finalize(s, t0, nt, attn):
        w = nt * T
        col0 = pl.multiple_of(s * L + t0 * T, T)
        hres = x_v[:, pl.ds(col0, w)].astype(f32) + attn
        hbuf[:, pl.ds(col0, w)] = hres
        a, b = _ln_stats(hres)
        wr = jnp.concatenate([wrtab[...]] * nt, axis=1)
        r = _colsum(hres * wr) * a + b * wrsum[0:1, 0:1]
        ab_all[0:8, pl.ds(col0, w)] = jnp.broadcast_to(a, (8, w))
        ab_all[8:16, pl.ds(col0, w)] = jnp.broadcast_to(b, (8, w))
        out_v[:, pl.ds(col0, w)] = (hbuf[:, pl.ds(col0, w)] * (1.0 + a) + b).astype(bf16)
        r = r.astype(bf16).astype(f32)
        bv, bi = best_v[0:1, :], best_i[0:1, :]
        for t in range(nt):
            rt = r[:, t * T:(t + 1) * T]
            better = rt > bv
            bi = jnp.where(better, col0 + t * T, bi)
            bv = jnp.where(better, rt, bv)
        best_i[...] = jnp.broadcast_to(bi, best_i.shape)
        best_v[...] = jnp.broadcast_to(bv, best_v.shape)

    def proj_rhs(s):
        col0 = pl.multiple_of(s * L, L)
        return jnp.concatenate([x_v[:, pl.ds(col0, L)], aug[:, pl.ds(col0, L)],
                                jnp.zeros((KP - D - 16, L), bf16)], axis=0)

    def ln_scale(s):
        return arow[0:1, pl.ds(pl.multiple_of(s * L, L), L)]

    def store_q(raw, a, r0, r1, with_phi=True, cols=slice(None)):
        qt[r0:r1, cols] = (raw * (a * QSCALE)).astype(bf16)
        if with_phi:
            pqt[r0:r1, cols] = _phi(raw * a).astype(bf16)

    def store_k_rows(raw, a, r0, r1):
        k = raw * a
        kt[r0:r1, :] = k.astype(bf16)
        pkt[r0:r1, :] = _phi(k).astype(bf16)

    def transpose_k():
        for g in range(NG):
            kp[g] = kt[WIN * g:WIN * g + T, :].T

    def store_k(raw, a, cols):
        k = raw * a
        kb = k.astype(bf16)
        pkt[:, cols] = _phi(k).astype(bf16)
        for g in range(NG):
            kp[g, cols, :] = kb[WIN * g:WIN * g + T, :].T

    def store_v(raw, a, cols=slice(None)):
        vt[:, cols] = (raw * a).astype(bf16)

    def project(s):
        rhs = proj_rhs(s)
        a = ln_scale(s)
        w = _PCOLS * T
        halves = [slice(c0, c0 + w) for c0 in range(0, L, w)]
        for cols in halves:
            store_q(_dot(wt[0:D, :], rhs[:, cols]), a[:, cols], 0, D, True, cols)
        mem_read()
        for cols in halves:
            store_k(_dot(wt[D:2 * D, :], rhs[:, cols]), a[:, cols], cols)
        for cols in halves:
            store_v(_dot(wt[2 * D:3 * D, :], rhs[:, cols]), a[:, cols], cols)

    def mem_read():
        row128 = lax.broadcasted_iota(jnp.int32, (T, T), 0)
        row8 = lax.broadcasted_iota(jnp.int32, (8, T), 0)
        for g in range(NG):
            ws = WIN * g
            heads = GROUPS[g]
            lo_g, hi_g = heads[0] * DH - ws, (heads[-1] + 1) * DH - ws
            wmask = (row128 >= lo_g) & (row128 < hi_g)
            for j in range(NT):
                nd = _dot(mb[g], pqt[ws:ws + T, j * T:(j + 1) * T])
                rden = 1.0 / (nd[T:T + 8] + 1e-6)
                rb = [jnp.broadcast_to(rden[i:i + 1], (8, T)) * (1.0 - g1tab[h])
                      for i, h in enumerate(heads)]
                blocks = []
                for b in range(T // 8):
                    r_lo, r_hi = 8 * b, 8 * b + 7
                    i_lo = min(max((r_lo + ws) // DH - heads[0], 0), len(heads) - 1)
                    i_hi = min(max((r_hi + ws) // DH - heads[0], 0), len(heads) - 1)
                    if i_lo == i_hi:
                        blocks.append(rb[i_lo])
                    else:
                        cut = (heads[0] + i_hi) * DH - ws - r_lo
                        blocks.append(jnp.where(row8 < cut, rb[i_lo], rb[i_hi]))
                amv = nd[0:T] * jnp.concatenate(blocks, axis=0)
                pltpu.store(am_v.at[ws:ws + T, j * T:(j + 1) * T], amv, mask=wmask)

    def attention(fast):
        ps = (p0, p1)
        if fast:
            _scores_fast(0, kp, qt, cmask, ps[0])
            for g in range(NG):
                if g + 1 < NG:
                    _scores_fast(g + 1, kp, qt, cmask, ps[(g + 1) % 2])
                _pv(g, vt, ps[g % 2], g1tab, am_v, ot)
        else:
            lax.fori_loop(0, H, lambda h, c: (_attention_safe(h, kp, qt, vt, g1tab, am_v, ot), c)[1], 0)

    def mem_update():
        for g in range(NG):
            ws = WIN * g
            lhs = jnp.concatenate([vt[ws:ws + T, :], ones_rows], axis=0)
            upd = macc[g] + _dot_nt(lhs, pkt[ws:ws + T, :])
            macc[g] = upd
            mb[g] = jnp.where(bmask[g] != 0.0, upd, 0.0).astype(bf16)

    def load_weight(i, c0=0, c1=D):
        w = w_in[i, :, c0:c1]
        n = c1 - c0
        wf = w.astype(f32)
        c = jnp.sum(wf, axis=0, keepdims=True)
        c_hi = c.astype(bf16).astype(f32)
        r16 = lax.broadcasted_iota(jnp.int32, (16, n), 0)
        extra = jnp.where(r16 >= 4, 0.0, jnp.where(r16 < 2, c_hi, c - c_hi)).astype(bf16)
        w_aug = jnp.concatenate([w, extra, jnp.zeros((KP - D - 16, n), bf16)], axis=0)
        w_t = w_aug.T
        wt[i * D + c0:i * D + c1, :] = w_t
        return w_t, jnp.max(jnp.sum(wf * wf, axis=0, keepdims=True))

    am_v[...] = jnp.zeros_like(am_v)
    ot[...] = jnp.zeros_like(ot)
    with _scope("p_tables"):
        small_b.wait()
        small_r.wait()
        build_tables()
    with _scope("p_wq_wait"):
        wq_lo.wait()
    wq_hi.start()
    w_copies[1].start()
    with _scope("p_wqT"):
        _, cq_lo = load_weight(0, 0, QLO)
    with _scope("p_x0_wait"):
        x_copy(0).wait()
    w_copies[2].start()
    w_copies[3].start()
    HALF = 288
    def q_rows(lhs, r0, r1):
        store_q(_dot(lhs, proj_rhs(0)), ln_scale(0), r0, r1, False)

    QA, QB = _PRO_SPLITS
    with _scope("p_b1"):
        ln1(0)
        q_rows(wt[0:QA, :], 0, QA)
    with _scope("p_wqhi_wait"):
        wq_hi.wait()
    for s in range(1, NSEG):
        x_copy(s).start()
    for c in w_copies[4:]:
        c.start()
    with _scope("p_b2"):
        wq_t, cq_hi = load_weight(0, QLO, D)
        cq = jnp.maximum(cq_lo, cq_hi)
        q_rows(wt[QA:QLO, :], QA, QLO)
        q_rows(wq_t[0:QB - QLO], QLO, QB)
    with _scope("p_wk_wait"):
        w_copies[1].wait()
    with _scope("p_b3"):
        wk_t, ck = load_weight(1)
        q_rows(wt[QB:D, :], QB, D)
        store_k_rows(_dot(wk_t[0:HALF], proj_rhs(0)), ln_scale(0), 0, HALF)
    with _scope("p_wv_wait"):
        w_copies[2].wait()
        w_copies[3].wait()
    with _scope("p_khi_wvT_v"):
        wv_t, cv = load_weight(2)
        wot[...] = w_in[3].T
        store_k_rows(_dot(wt[D + HALF:2 * D, :], proj_rhs(0)), ln_scale(0), HALF, D)
        transpose_k()
        store_v(_dot(wv_t, proj_rhs(0)), ln_scale(0))
    slack = 1.05
    logit_bound2 = (cq * ck) * (slack * D * DH * QSCALE) ** 2
    v_bound2 = cv * (slack * D)
    safe = (logit_bound2 <= SAFE_LOGIT ** 2) & (v_bound2 <= SAFE_V ** 2)

    def body(s, carry):
        more = s + 1 < NSEG
        nxt = jnp.minimum(s + 1, NSEG - 1)

        @pl.when(more)
        def _():
            x_copy(nxt).wait()

        @pl.when(safe)
        def _():
            with _scope("attn"):
                attention(True)

        @pl.when(jnp.logical_not(safe))
        def _():
            attention(False)

        @pl.when(more)
        def _():
            with _scope("blockB"):
                hold = {}
                steps = {
                    "MU": mem_update,
                    "OP": lambda: hold.update(a=[_dot(wot[...], ot[:, t * T:(t + 1) * T].astype(bf16))
                                                    for t in range(NT)]),
                    "LN1": lambda: ln1(nxt),
                    "PR": lambda: project(nxt),
                    "FIN": lambda: [finalize(s, t, 1, hold["a"][t]) for t in range(NT)],
                }
                for n in _ORDER_B:
                    steps[n]()
            out_copy(s).start()
        return carry

    lax.fori_loop(0, NSEG, body, 0)
    with _scope("fin"):
        otb = ot[...].astype(bf16)
        for t in range(NT):
            finalize(NSEG - 1, t, 1, _dot(wot[...], otb[:, t * T:(t + 1) * T]))
        out_copy(NSEG - 1).start()

    bv = best_v[...]
    rmax = jnp.max(bv, axis=1, keepdims=True)
    cand = best_i[...] + lax.broadcasted_iota(jnp.int32, best_i.shape, 1)
    idx = jnp.clip(jnp.min(jnp.where(bv == rmax, cand, S)), 0, S - 1)
    base = pl.multiple_of((idx // T) * T, T)
    lane = idx - base
    blk = (hbuf[:, pl.ds(base, T)] * ab_all[0:1, pl.ds(base, T)]
           + ab_all[8:9, pl.ds(base, T)]).astype(bf16)
    pick = jnp.where(lax.broadcasted_iota(jnp.int32, (16, T), 1) == lane, 1.0, 0.0).astype(bf16)
    xg = _dot_nt(pick, blk).astype(bf16)
    for c in w_copies[4:]:
        c.wait()
    yacc = jnp.zeros((D, T), f32)
    f_lo = 0
    for nt in _MOE_CHUNKS:
        f_hi = f_lo + nt * T
        gt = _dot(xg, wg_v[:, f_lo:f_hi])
        up = _dot(xg, wu_v[:, f_lo:f_hi])
        act = (gt * jax.nn.sigmoid(gt) * up)[0:1].astype(bf16).astype(f32)
        for t in range(nt):
            f0 = f_lo + t * T
            yacc = yacc + wd_v[:, f0:f0 + T].astype(f32) * act[:, t * T:(t + 1) * T]
        f_lo = f_hi
    y = jnp.sum(yacc, axis=1, keepdims=True) * jax.nn.sigmoid(rmax[0:1])
    for s in range(NSEG):
        out_copy(s).wait()
    sel = lax.broadcasted_iota(jnp.int32, (D, T), 1) == lane
    cur = out_v[:, pl.ds(base, T)].astype(f32)
    out_v[:, pl.ds(base, T)] = (cur + jnp.where(sel, y, 0.0)).astype(bf16)
    patch = pltpu.make_async_copy(out_v.at[:, pl.ds(base, T)],
                                  out_hbm.at[0, :, pl.ds(base, T)], sem_o.at[NSEG])
    patch.start()
    patch.wait()


@jax.jit
def pallas_sequential_preLN__memory_aug_infini_attn__moe_arch_mod__prompt_kernel(
    A_x: jax.Array,
    A_wq: jax.Array,
    A_wk: jax.Array,
    A_wv: jax.Array,
    A_wo: jax.Array,
    A_beta: jax.Array,
    B_x: jax.Array,
    B_w_r: jax.Array,
    B_w_gate: jax.Array,
    B_w_up: jax.Array,
    B_w_down: jax.Array,
):
    del B_x
    hbm_spec = pl.BlockSpec(memory_space=pltpu.HBM)
    scratch = [
        pltpu.VMEM((D, S), bf16),
        pltpu.VMEM((4, D, D), bf16),
        pltpu.VMEM((3 * D, KP), bf16),
        pltpu.VMEM((D, D), bf16),
        pltpu.VMEM((D, S), f32),
        pltpu.VMEM((D, F), bf16),
        pltpu.VMEM((D, F), bf16),
        pltpu.VMEM((D, F), bf16),
        pltpu.VMEM((16, S), bf16),
        pltpu.VMEM((8, S), f32),
        pltpu.VMEM((D, L), bf16),
        pltpu.VMEM((D, L), bf16),
        pltpu.VMEM((D, L), bf16),
        pltpu.VMEM((D, L), bf16),
        pltpu.VMEM((D, L), bf16),
        pltpu.VMEM((NG, L, T), bf16),
        pltpu.VMEM((7, NT, L, T), bf16),
        pltpu.VMEM((7, NT, L, T), bf16),
        pltpu.VMEM((D, L), f32),
        pltpu.VMEM((D, L), f32),
        pltpu.VMEM((NG, MROWS, T), f32),
        pltpu.VMEM((NG, MROWS, T), bf16),
        pltpu.VMEM((NG, MROWS, T), f32),
        pltpu.VMEM((4, T, T), f32),
        pltpu.VMEM((H, 8, T), f32),
        pltpu.VMEM((D, T), f32),
        pltpu.VMEM((16, S), f32),
        pltpu.VMEM((D, S), bf16),
        pltpu.VMEM((8, T), f32),
        pltpu.VMEM((8, T), jnp.int32),
        pltpu.VMEM((8, T), f32),
        pltpu.VMEM((H,), bf16),
        pltpu.VMEM((D,), bf16),
        pltpu.SemaphoreType.DMA((NSEG,)),
        pltpu.SemaphoreType.DMA((10,)),
        pltpu.SemaphoreType.DMA((NSEG + 1,)),
    ]
    out_t = pl.pallas_call(
        _kernel,
        out_shape=jax.ShapeDtypeStruct((1, D, S), bf16),
        in_specs=[hbm_spec] * 10,
        out_specs=hbm_spec,
        scratch_shapes=scratch,
        compiler_params=pltpu.CompilerParams(vmem_limit_bytes=100 * 1024 * 1024),
    )(jnp.transpose(A_x, (0, 2, 1)), A_wq, A_wk, A_wv, A_wo, A_beta,
      B_w_r, B_w_gate, B_w_up, B_w_down.T)
    return jnp.transpose(out_t, (0, 2, 1))
```

```python
import contextlib

import jax
import jax.numpy as jnp
from jax import lax
import jax.experimental.pallas as pl
import jax.experimental.pallas.tpu as pltpu

S = 2048
D = 576
H = 32
DH = 18
NSEG = 4
L = 512
F = 4608
T = 128
NT = L // T
EPS = 1e-5
LOG2E = 1.4426950408889634
QSCALE = (DH ** -0.5) * LOG2E
WIN = 112
GROUPS = (tuple(range(0, 7)), tuple(range(7, 13)), tuple(range(13, 19)),
          tuple(range(19, 25)), tuple(range(25, 32)))
NG = len(GROUPS)
KP = 640
MROWS = T + 16
SAFE_LOGIT = 60.0
SAFE_V = 2.0 ** 40

bf16 = jnp.bfloat16
f32 = jnp.float32
_ORDER_B = ["MU", "OP", "LN1", "PR", "FIN"]
_MOE_CHUNKS = (2,) * 18
_PCOLS = 2
_PRO_SPLITS = (128, 416)
_PROFILE = False


def _scope(name):
    return jax.named_scope(name) if _PROFILE else contextlib.nullcontext()


def _colsum(x):
    return jnp.sum(x, axis=0, keepdims=True)


def _ln_stats(x):
    m = _colsum(x) * (1.0 / D)
    v = jnp.maximum(_colsum(x * x) * (1.0 / D) - m * m, 0.0)
    a = lax.rsqrt(v + EPS)
    return a, -m * a


def _phi(t):
    return jnp.where(t > 0, t + 1.0, jnp.exp(t))


def _dot(a, b):
    return jnp.dot(a, b, preferred_element_type=f32)


def _dot_nt(a, b):
    return lax.dot_general(a, b, (((1,), (1,)), ((), ())), preferred_element_type=f32)


def _dot_tn(a, b):
    return lax.dot_general(a, b, (((0,), (0,)), ((), ())), preferred_element_type=f32)


ROT = (0, 1, 2, 3, 0, 2, 1)
QW = T // 4


def _pack_plan(nh, c):
    tiles = []
    split = []
    for u in range(nh):
        need = [(a + ROT[u]) % 4 for a in range(c, 4)]
        for t in tiles:
            if all(t[q] is None for q in need):
                break
        else:
            bound = max(sum(q in [(a + ROT[v]) % 4 for a in range(c, 4)] for v in range(nh))
                        for q in range(4))
            if len(tiles) >= bound:
                split.append((u, need))
                continue
            t = [None] * 4
            tiles.append(t)
        for q in need:
            t[q] = u
    for u, need in split:
        for q in need:
            next(t for t in tiles if t[q] is None)[q] = u
    return tiles


def _masked_q(qt_ref, g, j):
    ws = WIN * g
    row64 = lax.broadcasted_iota(jnp.int32, (64, T), 0)
    qw32 = pltpu.bitcast(qt_ref[ws:ws + T, j * T:(j + 1) * T], jnp.uint32)
    rolled = {0: qw32}
    qms = []
    for u, h in enumerate(GROUPS[g]):
        if ROT[u] not in rolled:
            rolled[ROT[u]] = pltpu.roll(qw32, ROT[u] * QW, axis=1)
        lo2 = (h * DH - ws) // 2
        qmask = (row64 >= lo2) & (row64 < lo2 + DH // 2)
        qms.append(jnp.where(qmask, rolled[ROT[u]], jnp.uint32(0)))
    return qms


def _select_quarters(sources):
    distinct = []
    for x in sources:
        if x is not None and not any(x is y for y in distinct):
            distinct.append(x)
    distinct.sort(key=lambda y: -sum(x is y for x in sources))
    out = distinct[0]
    lane = lax.broadcasted_iota(jnp.int32, out.shape, 1)
    for y in distinct[1:]:
        mask = None
        for q, x in enumerate(sources):
            if x is y:
                m = (lane >= q * QW) & (lane < (q + 1) * QW)
                mask = m if mask is None else mask | m
        out = jnp.where(mask, y, out)
    return out


def _scores_fast(g, kp_ref, qt_ref, cm_ref, p_ref):
    nh = len(GROUPS[g])
    plans = {c: _pack_plan(nh, c) for c in range(1, 4)}
    for j in range(NT):
        qms = _masked_q(qt_ref, g, j)
        n0 = T * j + QW
        p0 = jnp.exp2(_dot(kp_ref[g, 0:n0, :],
                           jnp.concatenate([pltpu.bitcast(q, bf16) for q in qms], axis=1)))
        pc = {}
        for c in range(1, 4):
            w = [pltpu.bitcast(_select_quarters([None if u is None else qms[u] for u in t]), bf16)
                 for t in plans[c]]
            r0 = T * j + c * QW
            pc[c] = jnp.exp2(_dot(kp_ref[g, r0:r0 + QW, :], jnp.concatenate(w, axis=1)))
        for u in range(nh):
            pu = p0[:, u * T:(u + 1) * T]
            if j > 0:
                p_ref[u, j, 0:j * T, :] = pu[0:j * T].astype(bf16)
            rows = [pu[j * T:n0]]
            for c in range(1, 4):
                src = [None] * 4
                for i, t in enumerate(plans[c]):
                    for q in range(4):
                        if t[q] == u:
                            src[q] = i
                vals = {i: pc[c][:, i * T:(i + 1) * T] for i in set(src) if i is not None}
                rows.append(_select_quarters([None if i is None else vals[i] for i in src]))
            p_ref[u, j, j * T:(j + 1) * T, :] = (
                jnp.concatenate(rows, axis=0) * cm_ref[ROT[u]]).astype(bf16)


def _attention_safe(h, kp_ref, qt_ref, vt_ref, g1_ref, am_ref, ot_ref):
    g = jnp.minimum(jnp.maximum(h - 1, 0) // 6, NG - 1)
    ws = pl.multiple_of(g * WIN, 16)
    lo = h * DH - ws
    row128 = lax.broadcasted_iota(jnp.int32, (T, T), 0)
    qmask = (row128 >= lo) & (row128 < lo + DH)
    vs = pl.multiple_of(((h * DH) // 16) * 16, 16)
    off = h * DH - vs
    row32 = lax.broadcasted_iota(jnp.int32, (32, T), 0)
    omask = (row32 >= off) & (row32 < off + DH)
    kk = lax.broadcasted_iota(jnp.int32, (L, T), 0)
    qq = lax.broadcasted_iota(jnp.int32, (L, T), 1)

    def tile(j, c):
        c0 = pl.multiple_of(j * T, T)
        qm = jnp.where(qmask, qt_ref[pl.ds(ws, T), pl.ds(c0, T)].astype(f32), 0.0).astype(bf16)
        s = _dot(kp_ref[g], qm)
        s = jnp.where(kk <= qq + c0, s, -jnp.inf)
        m = jnp.max(s, axis=0, keepdims=True)
        p = jnp.exp2(s - m).astype(bf16)
        acc = _dot(_v_rows(vt_ref, vs, off // 2, L), p)
        l8 = jnp.where(off <= 6, acc[24:32], acc[0:8])
        rl = g1_ref[h] / l8
        o = acc * jnp.concatenate([rl] * 4, axis=0) + am_ref[pl.ds(vs, 32), pl.ds(c0, T)]
        pltpu.store(ot_ref.at[pl.ds(vs, 32), pl.ds(c0, T)], o, mask=omask)
        return c

    lax.fori_loop(0, NT, tile, 0)


def _v_rows(vt_ref, vs, off2, nk):
    row16 = lax.broadcasted_iota(jnp.int32, (16, nk), 0)
    keep = (row16 >= off2) & (row16 < off2 + DH // 2)
    v32 = pltpu.bitcast(vt_ref[pl.ds(vs, 32), 0:nk], jnp.uint32)
    return pltpu.bitcast(jnp.where(keep, v32, jnp.uint32(0x3F803F80)), bf16)


def _pv(g, vt_ref, p_ref, g1_ref, am_ref, ot_ref):
    row32 = lax.broadcasted_iota(jnp.int32, (32, T), 0)
    for u, h in enumerate(GROUPS[g]):
        vs = ((h * DH) // 16) * 16
        off = h * DH - vs
        omask = (row32 >= off) & (row32 < off + DH)
        g1 = g1_ref[h]
        vrows = _v_rows(vt_ref, vs, off // 2, L)
        for j in range(NT):
            nk = T * (j + 1)
            acc = _dot(vrows[:, 0:nk], p_ref[u, j, 0:nk, :])
            l8 = acc[24:32] if off <= 6 else acc[0:8]
            rl = g1 / l8
            o = acc * jnp.concatenate([rl] * 4, axis=0)
            if ROT[u]:
                o = pltpu.roll(o, T - ROT[u] * QW, axis=1)
            o = o + am_ref[vs:vs + 32, j * T:(j + 1) * T]
            pltpu.store(ot_ref.at[vs:vs + 32, j * T:(j + 1) * T], o, mask=omask)


def _kernel(x_hbm, wq_hbm, wk_hbm, wv_hbm, wo_hbm, beta_hbm, wr_hbm, wg_hbm, wu_hbm, wd_hbm,
            out_hbm,
            x_v, w_in, wt, wot, hbuf, wg_v, wu_v, wd_v,
            aug, arow, qt, pqt, kt, pkt, vt, kp, p0, p1, am_v, ot,
            macc, mb, bmask, cmask, g1tab, wrtab, ab_all, out_v, best_v, best_i, wrsum, beta_ref, wr_ref,
            sem_x, sem_w, sem_o):
    def x_copy(s):
        return pltpu.make_async_copy(x_hbm.at[0, :, pl.ds(s * L, L)],
                                     x_v.at[:, pl.ds(s * L, L)], sem_x.at[s])

    def out_copy(s):
        return pltpu.make_async_copy(out_v.at[:, pl.ds(s * L, L)],
                                     out_hbm.at[0, :, pl.ds(s * L, L)], sem_o.at[s])

    w_copies = [
        None,
        pltpu.make_async_copy(wk_hbm, w_in.at[1], sem_w.at[1]),
        pltpu.make_async_copy(wv_hbm, w_in.at[2], sem_w.at[2]),
        pltpu.make_async_copy(wo_hbm, w_in.at[3], sem_w.at[3]),
        pltpu.make_async_copy(wg_hbm, wg_v, sem_w.at[4]),
        pltpu.make_async_copy(wu_hbm, wu_v, sem_w.at[5]),
        pltpu.make_async_copy(wd_hbm, wd_v, sem_w.at[6]),
    ]
    small_b = pltpu.make_async_copy(beta_hbm, beta_ref, sem_w.at[7])
    small_r = pltpu.make_async_copy(wr_hbm, wr_ref, sem_w.at[8])
    QLO = 256
    wq_lo = pltpu.make_async_copy(wq_hbm.at[:, 0:QLO], w_in.at[0, :, 0:QLO], sem_w.at[0])
    wq_hi = pltpu.make_async_copy(wq_hbm.at[:, QLO:D], w_in.at[0, :, QLO:D], sem_w.at[9])
    small_b.start()
    small_r.start()
    wq_lo.start()
    x_copy(0).start()

    def build_tables():
        gate = jax.nn.sigmoid(beta_ref[...].astype(f32).reshape(1, H))
        hh8 = lax.broadcasted_iota(jnp.int32, (8, H), 1)
        for h in range(H):
            gh = jnp.sum(jnp.where(hh8 == h, gate, 0.0), axis=1, keepdims=True)
            g1tab[h] = jnp.broadcast_to(1.0 - gh, (8, T))
        wr_row = wr_ref[...].astype(f32).reshape(1, D)
        wr_pad = jnp.concatenate([wr_row, jnp.zeros((1, 5 * T - D), f32)], axis=1)
        wrtab[...] = jnp.broadcast_to(wr_pad, (T, 5 * T)).T[0:D]
        wrsum[...] = jnp.broadcast_to(jnp.sum(wr_row, axis=1, keepdims=True), wrsum.shape)

    mr = lax.broadcasted_iota(jnp.int32, (MROWS, T), 0)
    mc = lax.broadcasted_iota(jnp.int32, (MROWS, T), 1)
    for g in range(NG):
        ws = WIN * g
        m = jnp.zeros((MROWS, T), jnp.bool_)
        for i, h in enumerate(GROUPS[g]):
            lo = h * DH - ws
            cols = (mc >= lo) & (mc < lo + DH)
            rows = ((mr >= lo) & (mr < lo + DH) & (mr < T)) | (mr == T + i)
            m = m | (cols & rows)
        bmask[g] = jnp.where(m, 1.0, 0.0)
    kk = lax.broadcasted_iota(jnp.int32, (T, T), 0)
    qq = lax.broadcasted_iota(jnp.int32, (T, T), 1)
    for r in range(4):
        cmask[r] = jnp.where(kk <= ((qq - r * QW) & (T - 1)), 1.0, 0.0)
    macc[...] = jnp.zeros_like(macc)
    mb[...] = jnp.zeros_like(mb)
    best_v[...] = jnp.full(best_v.shape, -jnp.inf, f32)
    best_i[...] = jnp.zeros(best_i.shape, jnp.int32)

    ones_rows = jnp.ones((16, L), bf16)

    def ln1(s):
        col0 = pl.multiple_of(s * L, L)
        xs = x_v[:, pl.ds(col0, L)].astype(f32)
        m = _colsum(xs) * (1.0 / D)
        v = jnp.maximum(_colsum(xs * xs) * (1.0 / D) - m * m, 0.0)
        arow[:, pl.ds(col0, L)] = jnp.broadcast_to(lax.rsqrt(v + EPS), (8, L))
        m_hi = (-m).astype(bf16).astype(f32)
        m_lo = -m - m_hi
        r16 = lax.broadcasted_iota(jnp.int32, (16, L), 0)
        rows = jnp.where(r16 >= 4, 0.0, jnp.where((r16 & 1) == 0, m_hi, m_lo))
        aug[:, pl.ds(col0, L)] = rows.astype(bf16)

    def finalize(s, t0, nt, attn):
        w = nt * T
        col0 = pl.multiple_of(s * L + t0 * T, T)
        hres = x_v[:, pl.ds(col0, w)].astype(f32) + attn
        hbuf[:, pl.ds(col0, w)] = hres
        a, b = _ln_stats(hres)
        wr = jnp.concatenate([wrtab[...]] * nt, axis=1)
        r = _colsum(hres * wr) * a + b * wrsum[0:1, 0:1]
        ab_all[0:8, pl.ds(col0, w)] = jnp.broadcast_to(a, (8, w))
        ab_all[8:16, pl.ds(col0, w)] = jnp.broadcast_to(b, (8, w))
        out_v[:, pl.ds(col0, w)] = (hbuf[:, pl.ds(col0, w)] * (1.0 + a) + b).astype(bf16)
        r = r.astype(bf16).astype(f32)
        bv, bi = best_v[0:1, :], best_i[0:1, :]
        for t in range(nt):
            rt = r[:, t * T:(t + 1) * T]
            better = rt > bv
            bi = jnp.where(better, col0 + t * T, bi)
            bv = jnp.where(better, rt, bv)
        best_i[...] = jnp.broadcast_to(bi, best_i.shape)
        best_v[...] = jnp.broadcast_to(bv, best_v.shape)

    def proj_rhs(s):
        col0 = pl.multiple_of(s * L, L)
        return jnp.concatenate([x_v[:, pl.ds(col0, L)], aug[:, pl.ds(col0, L)],
                                jnp.zeros((KP - D - 16, L), bf16)], axis=0)

    def ln_scale(s):
        return arow[0:1, pl.ds(pl.multiple_of(s * L, L), L)]

    def store_q(raw, a, r0, r1, with_phi=True, cols=slice(None)):
        qt[r0:r1, cols] = (raw * (a * QSCALE)).astype(bf16)
        if with_phi:
            pqt[r0:r1, cols] = _phi(raw * a).astype(bf16)

    def store_k_rows(raw, a, r0, r1):
        k = raw * a
        kt[r0:r1, :] = k.astype(bf16)
        pkt[r0:r1, :] = _phi(k).astype(bf16)

    def transpose_k():
        for g in range(NG):
            kp[g] = kt[WIN * g:WIN * g + T, :].T

    def store_k(raw, a, cols):
        k = raw * a
        kb = k.astype(bf16)
        pkt[:, cols] = _phi(k).astype(bf16)
        for g in range(NG):
            kp[g, cols, :] = kb[WIN * g:WIN * g + T, :].T

    def store_v(raw, a, cols=slice(None)):
        vt[:, cols] = (raw * a).astype(bf16)

    def project(s):
        rhs = proj_rhs(s)
        a = ln_scale(s)
        w = _PCOLS * T
        halves = [slice(c0, c0 + w) for c0 in range(0, L, w)]
        for cols in halves:
            store_q(_dot(wt[0:D, :], rhs[:, cols]), a[:, cols], 0, D, True, cols)
        mem_read()
        for cols in halves:
            store_k(_dot(wt[D:2 * D, :], rhs[:, cols]), a[:, cols], cols)
        for cols in halves:
            store_v(_dot(wt[2 * D:3 * D, :], rhs[:, cols]), a[:, cols], cols)

    def mem_read():
        row128 = lax.broadcasted_iota(jnp.int32, (T, T), 0)
        row8 = lax.broadcasted_iota(jnp.int32, (8, T), 0)
        for g in range(NG):
            ws = WIN * g
            heads = GROUPS[g]
            lo_g, hi_g = heads[0] * DH - ws, (heads[-1] + 1) * DH - ws
            wmask = (row128 >= lo_g) & (row128 < hi_g)
            for j in range(NT):
                nd = _dot(mb[g], pqt[ws:ws + T, j * T:(j + 1) * T])
                rden = 1.0 / (nd[T:T + 8] + 1e-6)
                rb = [jnp.broadcast_to(rden[i:i + 1], (8, T)) * (1.0 - g1tab[h])
                      for i, h in enumerate(heads)]
                blocks = []
                for b in range(T // 8):
                    r_lo, r_hi = 8 * b, 8 * b + 7
                    i_lo = min(max((r_lo + ws) // DH - heads[0], 0), len(heads) - 1)
                    i_hi = min(max((r_hi + ws) // DH - heads[0], 0), len(heads) - 1)
                    if i_lo == i_hi:
                        blocks.append(rb[i_lo])
                    else:
                        cut = (heads[0] + i_hi) * DH - ws - r_lo
                        blocks.append(jnp.where(row8 < cut, rb[i_lo], rb[i_hi]))
                amv = nd[0:T] * jnp.concatenate(blocks, axis=0)
                pltpu.store(am_v.at[ws:ws + T, j * T:(j + 1) * T], amv, mask=wmask)

    def attention(fast):
        ps = (p0, p1)
        if fast:
            _scores_fast(0, kp, qt, cmask, ps[0])
            for g in range(NG):
                if g + 1 < NG:
                    _scores_fast(g + 1, kp, qt, cmask, ps[(g + 1) % 2])
                _pv(g, vt, ps[g % 2], g1tab, am_v, ot)
        else:
            lax.fori_loop(0, H, lambda h, c: (_attention_safe(h, kp, qt, vt, g1tab, am_v, ot), c)[1], 0)

    def mem_update():
        for g in range(NG):
            ws = WIN * g
            lhs = jnp.concatenate([vt[ws:ws + T, :], ones_rows], axis=0)
            upd = macc[g] + _dot_nt(lhs, pkt[ws:ws + T, :])
            macc[g] = upd
            mb[g] = jnp.where(bmask[g] != 0.0, upd, 0.0).astype(bf16)

    def load_weight(i, c0=0, c1=D):
        w = w_in[i, :, c0:c1]
        n = c1 - c0
        wf = w.astype(f32)
        ones = jnp.ones((16, D), bf16)
        c = _dot(ones, w)[0:1]
        c_hi = c.astype(bf16).astype(f32)
        r16 = lax.broadcasted_iota(jnp.int32, (16, n), 0)
        extra = jnp.where(r16 >= 4, 0.0, jnp.where(r16 < 2, c_hi, c - c_hi)).astype(bf16)
        w_aug = jnp.concatenate([w, extra, jnp.zeros((KP - D - 16, n), bf16)], axis=0)
        w_t = w_aug.T
        wt[i * D + c0:i * D + c1, :] = w_t
        return w_t, jnp.max(_dot(ones, (wf * wf).astype(bf16)))

    am_v[...] = jnp.zeros_like(am_v)
    ot[...] = jnp.zeros_like(ot)
    with _scope("p_tables"):
        small_b.wait()
        small_r.wait()
        build_tables()
    with _scope("p_wq_wait"):
        wq_lo.wait()
    wq_hi.start()
    w_copies[1].start()
    with _scope("p_wqT"):
        _, cq_lo = load_weight(0, 0, QLO)
    with _scope("p_x0_wait"):
        x_copy(0).wait()
    w_copies[2].start()
    w_copies[3].start()
    HALF = 288
    def q_rows(lhs, r0, r1):
        store_q(_dot(lhs, proj_rhs(0)), ln_scale(0), r0, r1, False)

    QA, QB = _PRO_SPLITS
    with _scope("p_b1"):
        ln1(0)
        q_rows(wt[0:QA, :], 0, QA)
    with _scope("p_wqhi_wait"):
        wq_hi.wait()
    for s in range(1, NSEG):
        x_copy(s).start()
    for c in w_copies[4:]:
        c.start()
    with _scope("p_b2"):
        wq_t, cq_hi = load_weight(0, QLO, D)
        cq = jnp.maximum(cq_lo, cq_hi)
        q_rows(wt[QA:QLO, :], QA, QLO)
        q_rows(wq_t[0:QB - QLO], QLO, QB)
    with _scope("p_wk_wait"):
        w_copies[1].wait()
    with _scope("p_b3"):
        wk_t, ck = load_weight(1)
        q_rows(wt[QB:D, :], QB, D)
        store_k_rows(_dot(wk_t[0:HALF], proj_rhs(0)), ln_scale(0), 0, HALF)
    with _scope("p_wv_wait"):
        w_copies[2].wait()
        w_copies[3].wait()
    with _scope("p_khi_wvT_v"):
        wv_t, cv = load_weight(2)
        wot[...] = w_in[3].T
        store_k_rows(_dot(wt[D + HALF:2 * D, :], proj_rhs(0)), ln_scale(0), HALF, D)
        transpose_k()
        store_v(_dot(wv_t, proj_rhs(0)), ln_scale(0))
    slack = 1.06
    logit_bound2 = (cq * ck) * (slack * D * DH * QSCALE) ** 2
    v_bound2 = cv * (slack * D)
    safe = (logit_bound2 <= SAFE_LOGIT ** 2) & (v_bound2 <= SAFE_V ** 2)

    def body(s, carry):
        more = s + 1 < NSEG
        nxt = jnp.minimum(s + 1, NSEG - 1)

        @pl.when(more)
        def _():
            x_copy(nxt).wait()

        @pl.when(safe)
        def _():
            with _scope("attn"):
                attention(True)

        @pl.when(jnp.logical_not(safe))
        def _():
            attention(False)

        @pl.when(more)
        def _():
            with _scope("blockB"):
                hold = {}
                steps = {
                    "MU": mem_update,
                    "OP": lambda: hold.update(a=[_dot(wot[...], ot[:, t * T:(t + 1) * T].astype(bf16))
                                                    for t in range(NT)]),
                    "LN1": lambda: ln1(nxt),
                    "PR": lambda: project(nxt),
                    "FIN": lambda: [finalize(s, t, 1, hold["a"][t]) for t in range(NT)],
                }
                for n in _ORDER_B:
                    steps[n]()
            out_copy(s).start()
        return carry

    lax.fori_loop(0, NSEG, body, 0)
    with _scope("fin"):
        otb = ot[...].astype(bf16)
        for t in range(NT):
            finalize(NSEG - 1, t, 1, _dot(wot[...], otb[:, t * T:(t + 1) * T]))
        out_copy(NSEG - 1).start()

    bv = best_v[...]
    rmax = jnp.max(bv, axis=1, keepdims=True)
    cand = best_i[...] + lax.broadcasted_iota(jnp.int32, best_i.shape, 1)
    idx = jnp.clip(jnp.min(jnp.where(bv == rmax, cand, S)), 0, S - 1)
    base = pl.multiple_of((idx // T) * T, T)
    lane = idx - base
    blk = (hbuf[:, pl.ds(base, T)] * ab_all[0:1, pl.ds(base, T)]
           + ab_all[8:9, pl.ds(base, T)]).astype(bf16)
    pick = jnp.where(lax.broadcasted_iota(jnp.int32, (16, T), 1) == lane, 1.0, 0.0).astype(bf16)
    xg = _dot_nt(pick, blk).astype(bf16)
    for c in w_copies[4:]:
        c.wait()
    yacc = jnp.zeros((D, T), f32)
    f_lo = 0
    for nt in _MOE_CHUNKS:
        f_hi = f_lo + nt * T
        gt = _dot(xg, wg_v[:, f_lo:f_hi])
        up = _dot(xg, wu_v[:, f_lo:f_hi])
        act = (gt * jax.nn.sigmoid(gt) * up)[0:1].astype(bf16).astype(f32)
        for t in range(nt):
            f0 = f_lo + t * T
            yacc = yacc + wd_v[:, f0:f0 + T].astype(f32) * act[:, t * T:(t + 1) * T]
        f_lo = f_hi
    y = jnp.sum(yacc, axis=1, keepdims=True) * jax.nn.sigmoid(rmax[0:1])
    for s in range(NSEG):
        out_copy(s).wait()
    sel = lax.broadcasted_iota(jnp.int32, (D, T), 1) == lane
    cur = out_v[:, pl.ds(base, T)].astype(f32)
    out_v[:, pl.ds(base, T)] = (cur + jnp.where(sel, y, 0.0)).astype(bf16)
    patch = pltpu.make_async_copy(out_v.at[:, pl.ds(base, T)],
                                  out_hbm.at[0, :, pl.ds(base, T)], sem_o.at[NSEG])
    patch.start()
    patch.wait()


@jax.jit
def pallas_sequential_preLN__memory_aug_infini_attn__moe_arch_mod__prompt_kernel(
    A_x: jax.Array,
    A_wq: jax.Array,
    A_wk: jax.Array,
    A_wv: jax.Array,
    A_wo: jax.Array,
    A_beta: jax.Array,
    B_x: jax.Array,
    B_w_r: jax.Array,
    B_w_gate: jax.Array,
    B_w_up: jax.Array,
    B_w_down: jax.Array,
):
    del B_x
    hbm_spec = pl.BlockSpec(memory_space=pltpu.HBM)
    scratch = [
        pltpu.VMEM((D, S), bf16),
        pltpu.VMEM((4, D, D), bf16),
        pltpu.VMEM((3 * D, KP), bf16),
        pltpu.VMEM((D, D), bf16),
        pltpu.VMEM((D, S), f32),
        pltpu.VMEM((D, F), bf16),
        pltpu.VMEM((D, F), bf16),
        pltpu.VMEM((D, F), bf16),
        pltpu.VMEM((16, S), bf16),
        pltpu.VMEM((8, S), f32),
        pltpu.VMEM((D, L), bf16),
        pltpu.VMEM((D, L), bf16),
        pltpu.VMEM((D, L), bf16),
        pltpu.VMEM((D, L), bf16),
        pltpu.VMEM((D, L), bf16),
        pltpu.VMEM((NG, L, T), bf16),
        pltpu.VMEM((7, NT, L, T), bf16),
        pltpu.VMEM((7, NT, L, T), bf16),
        pltpu.VMEM((D, L), f32),
        pltpu.VMEM((D, L), f32),
        pltpu.VMEM((NG, MROWS, T), f32),
        pltpu.VMEM((NG, MROWS, T), bf16),
        pltpu.VMEM((NG, MROWS, T), f32),
        pltpu.VMEM((4, T, T), f32),
        pltpu.VMEM((H, 8, T), f32),
        pltpu.VMEM((D, T), f32),
        pltpu.VMEM((16, S), f32),
        pltpu.VMEM((D, S), bf16),
        pltpu.VMEM((8, T), f32),
        pltpu.VMEM((8, T), jnp.int32),
        pltpu.VMEM((8, T), f32),
        pltpu.VMEM((H,), bf16),
        pltpu.VMEM((D,), bf16),
        pltpu.SemaphoreType.DMA((NSEG,)),
        pltpu.SemaphoreType.DMA((10,)),
        pltpu.SemaphoreType.DMA((NSEG + 1,)),
    ]
    out_t = pl.pallas_call(
        _kernel,
        out_shape=jax.ShapeDtypeStruct((1, D, S), bf16),
        in_specs=[hbm_spec] * 10,
        out_specs=hbm_spec,
        scratch_shapes=scratch,
        compiler_params=pltpu.CompilerParams(vmem_limit_bytes=100 * 1024 * 1024),
    )(jnp.transpose(A_x, (0, 2, 1)), A_wq, A_wk, A_wv, A_wo, A_beta,
      B_w_r, B_w_gate, B_w_up, B_w_down.T)
    return jnp.transpose(out_t, (0, 2, 1))
```

```python
import contextlib

import jax
import jax.numpy as jnp
from jax import lax
import jax.experimental.pallas as pl
import jax.experimental.pallas.tpu as pltpu

S = 2048
D = 576
H = 32
DH = 18
NSEG = 4
L = 512
F = 4608
T = 128
NT = L // T
EPS = 1e-5
LOG2E = 1.4426950408889634
QSCALE = (DH ** -0.5) * LOG2E
WIN = 112
GROUPS = (tuple(range(0, 7)), tuple(range(7, 13)), tuple(range(13, 19)),
          tuple(range(19, 25)), tuple(range(25, 32)))
NG = len(GROUPS)
KP = 640
MROWS = T + 16
Z_ROW = (126, 0, 0, 0, 0)
DEN_ROW = tuple(T if len(g) == 7 else 0 for g in GROUPS)
SAFE_LOGIT = 60.0
SAFE_V = 2.0 ** 40

bf16 = jnp.bfloat16
f32 = jnp.float32
_ORDER_B = ["MU", "OP", "LN1", "PR", "FIN"]
_MOE_CHUNKS = (2,) * 18
_PCOLS = 2
_PRO_SPLITS = (128, 416)
_PROFILE = False


def _scope(name):
    return jax.named_scope(name) if _PROFILE else contextlib.nullcontext()


def _colsum(x):
    return jnp.sum(x, axis=0, keepdims=True)


def _ln_stats(x):
    m = _colsum(x) * (1.0 / D)
    v = jnp.maximum(_colsum(x * x) * (1.0 / D) - m * m, 0.0)
    a = lax.rsqrt(v + EPS)
    return a, -m * a


def _phi(t):
    return jnp.where(t > 0, t + 1.0, jnp.exp(t))


def _dot(a, b):
    return jnp.dot(a, b, preferred_element_type=f32)


def _dot_nt(a, b):
    return lax.dot_general(a, b, (((1,), (1,)), ((), ())), preferred_element_type=f32)


def _dot_tn(a, b):
    return lax.dot_general(a, b, (((0,), (0,)), ((), ())), preferred_element_type=f32)


ROT = (0, 1, 2, 3, 0, 2, 1)
QW = T // 4


def _pack_plan(nh, c):
    tiles = []
    split = []
    for u in range(nh):
        need = [(a + ROT[u]) % 4 for a in range(c, 4)]
        for t in tiles:
            if all(t[q] is None for q in need):
                break
        else:
            bound = max(sum(q in [(a + ROT[v]) % 4 for a in range(c, 4)] for v in range(nh))
                        for q in range(4))
            if len(tiles) >= bound:
                split.append((u, need))
                continue
            t = [None] * 4
            tiles.append(t)
        for q in need:
            t[q] = u
    for u, need in split:
        for q in need:
            next(t for t in tiles if t[q] is None)[q] = u
    return tiles


def _masked_q(qt_ref, g, j):
    ws = WIN * g
    row64 = lax.broadcasted_iota(jnp.int32, (64, T), 0)
    qw32 = pltpu.bitcast(qt_ref[ws:ws + T, j * T:(j + 1) * T], jnp.uint32)
    rolled = {0: qw32}
    qms = []
    for u, h in enumerate(GROUPS[g]):
        if ROT[u] not in rolled:
            rolled[ROT[u]] = pltpu.roll(qw32, ROT[u] * QW, axis=1)
        lo2 = (h * DH - ws) // 2
        qmask = (row64 >= lo2) & (row64 < lo2 + DH // 2)
        qms.append(jnp.where(qmask, rolled[ROT[u]], jnp.uint32(0)))
    return qms


def _select_quarters(sources):
    distinct = []
    for x in sources:
        if x is not None and not any(x is y for y in distinct):
            distinct.append(x)
    distinct.sort(key=lambda y: -sum(x is y for x in sources))
    out = distinct[0]
    lane = lax.broadcasted_iota(jnp.int32, out.shape, 1)
    for y in distinct[1:]:
        mask = None
        for q, x in enumerate(sources):
            if x is y:
                m = (lane >= q * QW) & (lane < (q + 1) * QW)
                mask = m if mask is None else mask | m
        out = jnp.where(mask, y, out)
    return out


def _scores_fast(g, kp_ref, qt_ref, cm_ref, p_ref):
    nh = len(GROUPS[g])
    plans = {c: _pack_plan(nh, c) for c in range(1, 4)}
    for j in range(NT):
        qms = _masked_q(qt_ref, g, j)
        n0 = T * j + QW
        p0 = jnp.exp2(_dot(kp_ref[g, 0:n0, :],
                           jnp.concatenate([pltpu.bitcast(q, bf16) for q in qms], axis=1)))
        pc = {}
        for c in range(1, 4):
            w = [pltpu.bitcast(_select_quarters([None if u is None else qms[u] for u in t]), bf16)
                 for t in plans[c]]
            r0 = T * j + c * QW
            pc[c] = jnp.exp2(_dot(kp_ref[g, r0:r0 + QW, :], jnp.concatenate(w, axis=1)))
        for u in range(nh):
            pu = p0[:, u * T:(u + 1) * T]
            if j > 0:
                p_ref[u, j, 0:j * T, :] = pu[0:j * T].astype(bf16)
            rows = [pu[j * T:n0]]
            for c in range(1, 4):
                src = [None] * 4
                for i, t in enumerate(plans[c]):
                    for q in range(4):
                        if t[q] == u:
                            src[q] = i
                vals = {i: pc[c][:, i * T:(i + 1) * T] for i in set(src) if i is not None}
                rows.append(_select_quarters([None if i is None else vals[i] for i in src]))
            p_ref[u, j, j * T:(j + 1) * T, :] = (
                jnp.concatenate(rows, axis=0) * cm_ref[ROT[u]]).astype(bf16)


def _attention_safe(h, kp_ref, qt_ref, vt_ref, g1_ref, am_ref, ot_ref):
    g = jnp.minimum(jnp.maximum(h - 1, 0) // 6, NG - 1)
    ws = pl.multiple_of(g * WIN, 16)
    lo = h * DH - ws
    row128 = lax.broadcasted_iota(jnp.int32, (T, T), 0)
    qmask = (row128 >= lo) & (row128 < lo + DH)
    vs = pl.multiple_of(((h * DH) // 16) * 16, 16)
    off = h * DH - vs
    row32 = lax.broadcasted_iota(jnp.int32, (32, T), 0)
    omask = (row32 >= off) & (row32 < off + DH)
    kk = lax.broadcasted_iota(jnp.int32, (L, T), 0)
    qq = lax.broadcasted_iota(jnp.int32, (L, T), 1)

    def tile(j, c):
        c0 = pl.multiple_of(j * T, T)
        qm = jnp.where(qmask, qt_ref[pl.ds(ws, T), pl.ds(c0, T)].astype(f32), 0.0).astype(bf16)
        s = _dot(kp_ref[g], qm)
        s = jnp.where(kk <= qq + c0, s, -jnp.inf)
        m = jnp.max(s, axis=0, keepdims=True)
        p = jnp.exp2(s - m).astype(bf16)
        acc = _dot(_v_rows(vt_ref, vs, off // 2, L), p)
        l8 = jnp.where(off <= 6, acc[24:32], acc[0:8])
        rl = g1_ref[h] / l8
        o = acc * jnp.concatenate([rl] * 4, axis=0) + am_ref[pl.ds(vs, 32), pl.ds(c0, T)]
        pltpu.store(ot_ref.at[pl.ds(vs, 32), pl.ds(c0, T)], o, mask=omask)
        return c

    lax.fori_loop(0, NT, tile, 0)


def _v_rows(vt_ref, vs, off2, nk):
    row16 = lax.broadcasted_iota(jnp.int32, (16, nk), 0)
    keep = (row16 >= off2) & (row16 < off2 + DH // 2)
    v32 = pltpu.bitcast(vt_ref[pl.ds(vs, 32), 0:nk], jnp.uint32)
    return pltpu.bitcast(jnp.where(keep, v32, jnp.uint32(0x3F803F80)), bf16)


def _pv(g, vt_ref, p_ref, g1_ref, am_ref, ot_ref):
    row32 = lax.broadcasted_iota(jnp.int32, (32, T), 0)
    for u, h in enumerate(GROUPS[g]):
        vs = ((h * DH) // 16) * 16
        off = h * DH - vs
        omask = (row32 >= off) & (row32 < off + DH)
        g1 = g1_ref[h]
        vrows = _v_rows(vt_ref, vs, off // 2, L)
        for j in range(NT):
            nk = T * (j + 1)
            acc = _dot(vrows[:, 0:nk], p_ref[u, j, 0:nk, :])
            l8 = acc[24:32] if off <= 6 else acc[0:8]
            rl = g1 / l8
            o = acc * jnp.concatenate([rl] * 4, axis=0)
            if ROT[u]:
                o = pltpu.roll(o, T - ROT[u] * QW, axis=1)
            o = o + am_ref[vs:vs + 32, j * T:(j + 1) * T]
            pltpu.store(ot_ref.at[vs:vs + 32, j * T:(j + 1) * T], o, mask=omask)


def _kernel(x_hbm, wq_hbm, wk_hbm, wv_hbm, wo_hbm, beta_hbm, wr_hbm, wg_hbm, wu_hbm, wd_hbm,
            out_hbm,
            x_v, w_in, wt, wot, hbuf, wg_v, wu_v, wd_v,
            aug, arow, qt, pqt, kt, pkt, vt, kp, p0, p1, am_v, ot,
            macc, mb, bmask, cmask, g1tab, wrtab, ab_all, out_v, best_v, best_i, wrsum, beta_ref, wr_ref,
            sem_x, sem_w, sem_o):
    def x_copy(s):
        return pltpu.make_async_copy(x_hbm.at[0, :, pl.ds(s * L, L)],
                                     x_v.at[:, pl.ds(s * L, L)], sem_x.at[s])

    def out_copy(s):
        return pltpu.make_async_copy(out_v.at[:, pl.ds(s * L, L)],
                                     out_hbm.at[0, :, pl.ds(s * L, L)], sem_o.at[s])

    w_copies = [
        None,
        pltpu.make_async_copy(wk_hbm, w_in.at[1], sem_w.at[1]),
        pltpu.make_async_copy(wv_hbm, w_in.at[2], sem_w.at[2]),
        pltpu.make_async_copy(wo_hbm, w_in.at[3], sem_w.at[3]),
        pltpu.make_async_copy(wg_hbm, wg_v, sem_w.at[4]),
        pltpu.make_async_copy(wu_hbm, wu_v, sem_w.at[5]),
        pltpu.make_async_copy(wd_hbm, wd_v, sem_w.at[6]),
    ]
    small_b = pltpu.make_async_copy(beta_hbm, beta_ref, sem_w.at[7])
    small_r = pltpu.make_async_copy(wr_hbm, wr_ref, sem_w.at[8])
    QLO = 256
    wq_lo = pltpu.make_async_copy(wq_hbm.at[:, 0:QLO], w_in.at[0, :, 0:QLO], sem_w.at[0])
    wq_hi = pltpu.make_async_copy(wq_hbm.at[:, QLO:D], w_in.at[0, :, QLO:D], sem_w.at[9])
    small_b.start()
    small_r.start()
    wq_lo.start()
    x_copy(0).start()

    def build_tables():
        gate = jax.nn.sigmoid(beta_ref[...].astype(f32).reshape(1, H))
        hh8 = lax.broadcasted_iota(jnp.int32, (8, H), 1)
        for h in range(H):
            gh = jnp.sum(jnp.where(hh8 == h, gate, 0.0), axis=1, keepdims=True)
            g1tab[h] = jnp.broadcast_to(1.0 - gh, (8, T))
        wr_row = wr_ref[...].astype(f32).reshape(1, D)
        wr_pad = jnp.concatenate([wr_row, jnp.zeros((1, 5 * T - D), f32)], axis=1)
        wrtab[...] = jnp.broadcast_to(wr_pad, (T, 5 * T)).T[0:D]
        wrsum[...] = jnp.broadcast_to(jnp.sum(wr_row, axis=1, keepdims=True), wrsum.shape)

    mr = lax.broadcasted_iota(jnp.int32, (MROWS, T), 0)
    mc = lax.broadcasted_iota(jnp.int32, (MROWS, T), 1)
    for g in range(NG):
        ws = WIN * g
        code = jnp.zeros((MROWS, T), f32)
        for i, h in enumerate(GROUPS[g]):
            lo = h * DH - ws
            cols = (mc >= lo) & (mc < lo + DH)
            code = jnp.where(cols & (mr >= lo) & (mr < lo + DH) & (mr < T), 1.0, code)
            code = jnp.where(cols & (mr == DEN_ROW[g] + i), 2.0, code)
        bmask[g] = code
    kk = lax.broadcasted_iota(jnp.int32, (T, T), 0)
    qq = lax.broadcasted_iota(jnp.int32, (T, T), 1)
    for r in range(4):
        cmask[r] = jnp.where(kk <= ((qq - r * QW) & (T - 1)), 1.0, 0.0)
    macc[...] = jnp.zeros_like(macc)
    mb[...] = jnp.zeros_like(mb)
    best_v[...] = jnp.full(best_v.shape, -jnp.inf, f32)
    best_i[...] = jnp.zeros(best_i.shape, jnp.int32)


    def ln1(s):
        col0 = pl.multiple_of(s * L, L)
        xs = x_v[:, pl.ds(col0, L)].astype(f32)
        m = _colsum(xs) * (1.0 / D)
        v = jnp.maximum(_colsum(xs * xs) * (1.0 / D) - m * m, 0.0)
        arow[:, pl.ds(col0, L)] = jnp.broadcast_to(lax.rsqrt(v + EPS), (8, L))
        m_hi = (-m).astype(bf16).astype(f32)
        m_lo = -m - m_hi
        r16 = lax.broadcasted_iota(jnp.int32, (16, L), 0)
        rows = jnp.where(r16 >= 4, 0.0, jnp.where((r16 & 1) == 0, m_hi, m_lo))
        aug[:, pl.ds(col0, L)] = rows.astype(bf16)

    def finalize(s, t0, nt, attn):
        w = nt * T
        col0 = pl.multiple_of(s * L + t0 * T, T)
        hres = x_v[:, pl.ds(col0, w)].astype(f32) + attn
        hbuf[:, pl.ds(col0, w)] = hres
        a, b = _ln_stats(hres)
        wr = jnp.concatenate([wrtab[...]] * nt, axis=1)
        r = _colsum(hres * wr) * a + b * wrsum[0:1, 0:1]
        ab_all[0:8, pl.ds(col0, w)] = jnp.broadcast_to(a, (8, w))
        ab_all[8:16, pl.ds(col0, w)] = jnp.broadcast_to(b, (8, w))
        out_v[:, pl.ds(col0, w)] = (hbuf[:, pl.ds(col0, w)] * (1.0 + a) + b).astype(bf16)
        r = r.astype(bf16).astype(f32)
        bv, bi = best_v[0:1, :], best_i[0:1, :]
        for t in range(nt):
            rt = r[:, t * T:(t + 1) * T]
            better = rt > bv
            bi = jnp.where(better, col0 + t * T, bi)
            bv = jnp.where(better, rt, bv)
        best_i[...] = jnp.broadcast_to(bi, best_i.shape)
        best_v[...] = jnp.broadcast_to(bv, best_v.shape)

    def proj_rhs(s):
        col0 = pl.multiple_of(s * L, L)
        return jnp.concatenate([x_v[:, pl.ds(col0, L)], aug[:, pl.ds(col0, L)],
                                jnp.zeros((KP - D - 16, L), bf16)], axis=0)

    def ln_scale(s):
        return arow[0:1, pl.ds(pl.multiple_of(s * L, L), L)]

    def store_q(raw, a, r0, r1, with_phi=True, cols=slice(None)):
        qt[r0:r1, cols] = (raw * (a * QSCALE)).astype(bf16)
        if with_phi:
            pqt[r0:r1, cols] = _phi(raw * a).astype(bf16)

    def store_k_rows(raw, a, r0, r1):
        k = raw * a
        kt[r0:r1, :] = k.astype(bf16)
        pkt[r0:r1, :] = _phi(k).astype(bf16)

    def transpose_k():
        for g in range(NG):
            kp[g] = kt[WIN * g:WIN * g + T, :].T

    def store_k(raw, a, cols):
        k = raw * a
        kb = k.astype(bf16)
        pkt[:, cols] = _phi(k).astype(bf16)
        for g in range(NG):
            kp[g, cols, :] = kb[WIN * g:WIN * g + T, :].T

    def store_v(raw, a, cols=slice(None)):
        vt[:, cols] = (raw * a).astype(bf16)

    def project(s):
        rhs = proj_rhs(s)
        a = ln_scale(s)
        w = _PCOLS * T
        halves = [slice(c0, c0 + w) for c0 in range(0, L, w)]
        for cols in halves:
            store_q(_dot(wt[0:D, :], rhs[:, cols]), a[:, cols], 0, D, True, cols)
        mem_read()
        for cols in halves:
            store_k(_dot(wt[D:2 * D, :], rhs[:, cols]), a[:, cols], cols)
        for cols in halves:
            store_v(_dot(wt[2 * D:3 * D, :], rhs[:, cols]), a[:, cols], cols)

    def mem_read():
        row128 = lax.broadcasted_iota(jnp.int32, (T, T), 0)
        row8 = lax.broadcasted_iota(jnp.int32, (8, T), 0)
        for g in range(NG):
            ws = WIN * g
            heads = GROUPS[g]
            lo_g, hi_g = heads[0] * DH - ws, (heads[-1] + 1) * DH - ws
            wmask = (row128 >= lo_g) & (row128 < hi_g)
            for j in range(NT):
                nrows = MROWS if DEN_ROW[g] == T else T
                nd = _dot(mb[g, 0:nrows], pqt[ws:ws + T, j * T:(j + 1) * T])
                rden = 1.0 / (nd[DEN_ROW[g]:DEN_ROW[g] + 8] + 1e-6)
                rb = [jnp.broadcast_to(rden[i:i + 1], (8, T)) * (1.0 - g1tab[h])
                      for i, h in enumerate(heads)]
                blocks = []
                for b in range(T // 8):
                    r_lo, r_hi = 8 * b, 8 * b + 7
                    i_lo = min(max((r_lo + ws) // DH - heads[0], 0), len(heads) - 1)
                    i_hi = min(max((r_hi + ws) // DH - heads[0], 0), len(heads) - 1)
                    if i_lo == i_hi:
                        blocks.append(rb[i_lo])
                    else:
                        cut = (heads[0] + i_hi) * DH - ws - r_lo
                        blocks.append(jnp.where(row8 < cut, rb[i_lo], rb[i_hi]))
                amv = nd[0:T] * jnp.concatenate(blocks, axis=0)
                pltpu.store(am_v.at[ws:ws + T, j * T:(j + 1) * T], amv, mask=wmask)

    def attention(fast):
        ps = (p0, p1)
        if fast:
            _scores_fast(0, kp, qt, cmask, ps[0])
            for g in range(NG):
                if g + 1 < NG:
                    _scores_fast(g + 1, kp, qt, cmask, ps[(g + 1) % 2])
                _pv(g, vt, ps[g % 2], g1tab, am_v, ot)
        else:
            lax.fori_loop(0, H, lambda h, c: (_attention_safe(h, kp, qt, vt, g1tab, am_v, ot), c)[1], 0)

    def mem_update():
        word = lax.broadcasted_iota(jnp.int32, (T // 2, L), 0)
        for g in range(NG):
            ws = WIN * g
            v32 = pltpu.bitcast(vt[ws:ws + T, :], jnp.uint32)
            lhs = pltpu.bitcast(jnp.where(word == Z_ROW[g] // 2, jnp.uint32(0x3F803F80), v32), bf16)
            upd = macc[g] + _dot_nt(lhs, pkt[ws:ws + T, :])
            macc[g] = upd
            nrows = MROWS if DEN_ROW[g] == T else T
            z = jnp.broadcast_to(upd[Z_ROW[g]:Z_ROW[g] + 1], (nrows, T))
            m = upd if nrows == T else jnp.concatenate([upd, jnp.zeros((nrows - T, T), f32)], axis=0)
            code = bmask[g, 0:nrows]
            mb[g, 0:nrows] = jnp.where(code == 1.0, m, jnp.where(code == 2.0, z, 0.0)).astype(bf16)

    def load_weight(i, c0=0, c1=D):
        w = w_in[i, :, c0:c1]
        n = c1 - c0
        wf = w.astype(f32)
        ones = jnp.ones((16, D), bf16)
        c = _dot(ones, w)[0:1]
        c_hi = c.astype(bf16).astype(f32)
        r16 = lax.broadcasted_iota(jnp.int32, (16, n), 0)
        extra = jnp.where(r16 >= 4, 0.0, jnp.where(r16 < 2, c_hi, c - c_hi)).astype(bf16)
        w_aug = jnp.concatenate([w, extra, jnp.zeros((KP - D - 16, n), bf16)], axis=0)
        w_t = w_aug.T
        wt[i * D + c0:i * D + c1, :] = w_t
        return w_t, jnp.max(_dot(ones, (wf * wf).astype(bf16)))

    am_v[...] = jnp.zeros_like(am_v)
    ot[...] = jnp.zeros_like(ot)
    with _scope("p_tables"):
        small_b.wait()
        small_r.wait()
        build_tables()
    with _scope("p_wq_wait"):
        wq_lo.wait()
    wq_hi.start()
    w_copies[1].start()
    with _scope("p_wqT"):
        _, cq_lo = load_weight(0, 0, QLO)
    with _scope("p_x0_wait"):
        x_copy(0).wait()
    w_copies[2].start()
    w_copies[3].start()
    HALF = 288
    def q_rows(lhs, r0, r1):
        store_q(_dot(lhs, proj_rhs(0)), ln_scale(0), r0, r1, False)

    QA, QB = _PRO_SPLITS
    with _scope("p_b1"):
        ln1(0)
        q_rows(wt[0:QA, :], 0, QA)
    with _scope("p_wqhi_wait"):
        wq_hi.wait()
    for s in range(1, NSEG):
        x_copy(s).start()
    for c in w_copies[4:]:
        c.start()
    with _scope("p_b2"):
        wq_t, cq_hi = load_weight(0, QLO, D)
        cq = jnp.maximum(cq_lo, cq_hi)
        q_rows(wt[QA:QLO, :], QA, QLO)
        q_rows(wq_t[0:QB - QLO], QLO, QB)
    with _scope("p_wk_wait"):
        w_copies[1].wait()
    with _scope("p_b3"):
        wk_t, ck = load_weight(1)
        q_rows(wt[QB:D, :], QB, D)
        store_k_rows(_dot(wk_t[0:HALF], proj_rhs(0)), ln_scale(0), 0, HALF)
    with _scope("p_wv_wait"):
        w_copies[2].wait()
        w_copies[3].wait()
    with _scope("p_khi_wvT_v"):
        wv_t, cv = load_weight(2)
        wot[...] = w_in[3].T
        store_k_rows(_dot(wt[D + HALF:2 * D, :], proj_rhs(0)), ln_scale(0), HALF, D)
        transpose_k()
        store_v(_dot(wv_t, proj_rhs(0)), ln_scale(0))
    slack = 1.06
    logit_bound2 = (cq * ck) * (slack * D * DH * QSCALE) ** 2
    v_bound2 = cv * (slack * D)
    safe = (logit_bound2 <= SAFE_LOGIT ** 2) & (v_bound2 <= SAFE_V ** 2)

    def body(s, carry):
        more = s + 1 < NSEG
        nxt = jnp.minimum(s + 1, NSEG - 1)

        @pl.when(more)
        def _():
            x_copy(nxt).wait()

        @pl.when(safe)
        def _():
            with _scope("attn"):
                attention(True)

        @pl.when(jnp.logical_not(safe))
        def _():
            attention(False)

        @pl.when(more)
        def _():
            with _scope("blockB"):
                hold = {}
                steps = {
                    "MU": mem_update,
                    "OP": lambda: hold.update(a=[_dot(wot[...], ot[:, t * T:(t + 1) * T].astype(bf16))
                                                    for t in range(NT)]),
                    "LN1": lambda: ln1(nxt),
                    "PR": lambda: project(nxt),
                    "FIN": lambda: [finalize(s, t, 1, hold["a"][t]) for t in range(NT)],
                }
                for n in _ORDER_B:
                    steps[n]()
            out_copy(s).start()
        return carry

    lax.fori_loop(0, NSEG, body, 0)
    with _scope("fin"):
        otb = ot[...].astype(bf16)
        for t in range(NT):
            finalize(NSEG - 1, t, 1, _dot(wot[...], otb[:, t * T:(t + 1) * T]))
        out_copy(NSEG - 1).start()

    bv = best_v[...]
    rmax = jnp.max(bv, axis=1, keepdims=True)
    cand = best_i[...] + lax.broadcasted_iota(jnp.int32, best_i.shape, 1)
    idx = jnp.clip(jnp.min(jnp.where(bv == rmax, cand, S)), 0, S - 1)
    base = pl.multiple_of((idx // T) * T, T)
    lane = idx - base
    blk = (hbuf[:, pl.ds(base, T)] * ab_all[0:1, pl.ds(base, T)]
           + ab_all[8:9, pl.ds(base, T)]).astype(bf16)
    pick = jnp.where(lax.broadcasted_iota(jnp.int32, (16, T), 1) == lane, 1.0, 0.0).astype(bf16)
    xg = _dot_nt(pick, blk).astype(bf16)
    for c in w_copies[4:]:
        c.wait()
    yacc = jnp.zeros((D, T), f32)
    f_lo = 0
    for nt in _MOE_CHUNKS:
        f_hi = f_lo + nt * T
        gt = _dot(xg, wg_v[:, f_lo:f_hi])
        up = _dot(xg, wu_v[:, f_lo:f_hi])
        act = (gt * jax.nn.sigmoid(gt) * up)[0:1].astype(bf16).astype(f32)
        for t in range(nt):
            f0 = f_lo + t * T
            yacc = yacc + wd_v[:, f0:f0 + T].astype(f32) * act[:, t * T:(t + 1) * T]
        f_lo = f_hi
    y = jnp.sum(yacc, axis=1, keepdims=True) * jax.nn.sigmoid(rmax[0:1])
    for s in range(NSEG):
        out_copy(s).wait()
    sel = lax.broadcasted_iota(jnp.int32, (D, T), 1) == lane
    cur = out_v[:, pl.ds(base, T)].astype(f32)
    out_v[:, pl.ds(base, T)] = (cur + jnp.where(sel, y, 0.0)).astype(bf16)
    patch = pltpu.make_async_copy(out_v.at[:, pl.ds(base, T)],
                                  out_hbm.at[0, :, pl.ds(base, T)], sem_o.at[NSEG])
    patch.start()
    patch.wait()


@jax.jit
def pallas_sequential_preLN__memory_aug_infini_attn__moe_arch_mod__prompt_kernel(
    A_x: jax.Array,
    A_wq: jax.Array,
    A_wk: jax.Array,
    A_wv: jax.Array,
    A_wo: jax.Array,
    A_beta: jax.Array,
    B_x: jax.Array,
    B_w_r: jax.Array,
    B_w_gate: jax.Array,
    B_w_up: jax.Array,
    B_w_down: jax.Array,
):
    del B_x
    hbm_spec = pl.BlockSpec(memory_space=pltpu.HBM)
    scratch = [
        pltpu.VMEM((D, S), bf16),
        pltpu.VMEM((4, D, D), bf16),
        pltpu.VMEM((3 * D, KP), bf16),
        pltpu.VMEM((D, D), bf16),
        pltpu.VMEM((D, S), f32),
        pltpu.VMEM((D, F), bf16),
        pltpu.VMEM((D, F), bf16),
        pltpu.VMEM((D, F), bf16),
        pltpu.VMEM((16, S), bf16),
        pltpu.VMEM((8, S), f32),
        pltpu.VMEM((D, L), bf16),
        pltpu.VMEM((D, L), bf16),
        pltpu.VMEM((D, L), bf16),
        pltpu.VMEM((D, L), bf16),
        pltpu.VMEM((D, L), bf16),
        pltpu.VMEM((NG, L, T), bf16),
        pltpu.VMEM((7, NT, L, T), bf16),
        pltpu.VMEM((7, NT, L, T), bf16),
        pltpu.VMEM((D, L), f32),
        pltpu.VMEM((D, L), f32),
        pltpu.VMEM((NG, T, T), f32),
        pltpu.VMEM((NG, MROWS, T), bf16),
        pltpu.VMEM((NG, MROWS, T), f32),
        pltpu.VMEM((4, T, T), f32),
        pltpu.VMEM((H, 8, T), f32),
        pltpu.VMEM((D, T), f32),
        pltpu.VMEM((16, S), f32),
        pltpu.VMEM((D, S), bf16),
        pltpu.VMEM((8, T), f32),
        pltpu.VMEM((8, T), jnp.int32),
        pltpu.VMEM((8, T), f32),
        pltpu.VMEM((H,), bf16),
        pltpu.VMEM((D,), bf16),
        pltpu.SemaphoreType.DMA((NSEG,)),
        pltpu.SemaphoreType.DMA((10,)),
        pltpu.SemaphoreType.DMA((NSEG + 1,)),
    ]
    out_t = pl.pallas_call(
        _kernel,
        out_shape=jax.ShapeDtypeStruct((1, D, S), bf16),
        in_specs=[hbm_spec] * 10,
        out_specs=hbm_spec,
        scratch_shapes=scratch,
        compiler_params=pltpu.CompilerParams(vmem_limit_bytes=100 * 1024 * 1024),
    )(jnp.transpose(A_x, (0, 2, 1)), A_wq, A_wk, A_wv, A_wo, A_beta,
      B_w_r, B_w_gate, B_w_up, B_w_down.T)
    return jnp.transpose(out_t, (0, 2, 1))
```

```python
import contextlib

import jax
import jax.numpy as jnp
from jax import lax
import jax.experimental.pallas as pl
import jax.experimental.pallas.tpu as pltpu

S = 2048
D = 576
H = 32
DH = 18
NSEG = 4
L = 512
F = 4608
T = 128
NT = L // T
EPS = 1e-5
LOG2E = 1.4426950408889634
QSCALE = (DH ** -0.5) * LOG2E
WIN = 112
GROUPS = (tuple(range(0, 7)), tuple(range(7, 13)), tuple(range(13, 19)),
          tuple(range(19, 25)), tuple(range(25, 32)))
NG = len(GROUPS)
KP = 640
MROWS = T + 16
Z_ROW = (126, 0, 0, 0, 0)
DEN_ROW = tuple(T if len(g) == 7 else 0 for g in GROUPS)
SAFE_LOGIT = 60.0
SAFE_V = 2.0 ** 40

bf16 = jnp.bfloat16
f32 = jnp.float32
MOE_CHUNK = 2
PROJ_COLS = 2
Q_SPLITS = (128, 256, 416)
K_SPLIT = 288
_PROFILE = False


def _scope(name):
    return jax.named_scope(name) if _PROFILE else contextlib.nullcontext()


def _colsum(x):
    return jnp.sum(x, axis=0, keepdims=True)


def _ln_stats(x):
    m = _colsum(x) * (1.0 / D)
    v = jnp.maximum(_colsum(x * x) * (1.0 / D) - m * m, 0.0)
    a = lax.rsqrt(v + EPS)
    return a, -m * a


def _phi(t):
    return jnp.where(t > 0, t + 1.0, jnp.exp(t))


def _dot(a, b):
    return jnp.dot(a, b, preferred_element_type=f32)


def _dot_nt(a, b):
    return lax.dot_general(a, b, (((1,), (1,)), ((), ())), preferred_element_type=f32)


ROT = (0, 1, 2, 3, 0, 2, 1)
QW = T // 4


def _pack_plan(nh, c):
    tiles = []
    split = []
    for u in range(nh):
        need = [(a + ROT[u]) % 4 for a in range(c, 4)]
        for t in tiles:
            if all(t[q] is None for q in need):
                break
        else:
            bound = max(sum(q in [(a + ROT[v]) % 4 for a in range(c, 4)] for v in range(nh))
                        for q in range(4))
            if len(tiles) >= bound:
                split.append((u, need))
                continue
            t = [None] * 4
            tiles.append(t)
        for q in need:
            t[q] = u
    for u, need in split:
        for q in need:
            next(t for t in tiles if t[q] is None)[q] = u
    return tiles


def _masked_q(qt_ref, g, j):
    ws = WIN * g
    row64 = lax.broadcasted_iota(jnp.int32, (64, T), 0)
    qw32 = pltpu.bitcast(qt_ref[ws:ws + T, j * T:(j + 1) * T], jnp.uint32)
    rolled = {0: qw32}
    qms = []
    for u, h in enumerate(GROUPS[g]):
        if ROT[u] not in rolled:
            rolled[ROT[u]] = pltpu.roll(qw32, ROT[u] * QW, axis=1)
        lo2 = (h * DH - ws) // 2
        qmask = (row64 >= lo2) & (row64 < lo2 + DH // 2)
        qms.append(jnp.where(qmask, rolled[ROT[u]], jnp.uint32(0)))
    return qms


def _select_quarters(sources):
    distinct = []
    for x in sources:
        if x is not None and not any(x is y for y in distinct):
            distinct.append(x)
    distinct.sort(key=lambda y: -sum(x is y for x in sources))
    out = distinct[0]
    lane = lax.broadcasted_iota(jnp.int32, out.shape, 1)
    for y in distinct[1:]:
        mask = None
        for q, x in enumerate(sources):
            if x is y:
                m = (lane >= q * QW) & (lane < (q + 1) * QW)
                mask = m if mask is None else mask | m
        out = jnp.where(mask, y, out)
    return out


def _scores_fast(g, kp_ref, qt_ref, cm_ref, p_ref):
    nh = len(GROUPS[g])
    plans = {c: _pack_plan(nh, c) for c in range(1, 4)}
    for j in range(NT):
        qms = _masked_q(qt_ref, g, j)
        n0 = T * j + QW
        p0 = jnp.exp2(_dot(kp_ref[g, 0:n0, :],
                           jnp.concatenate([pltpu.bitcast(q, bf16) for q in qms], axis=1)))
        pc = {}
        for c in range(1, 4):
            w = [pltpu.bitcast(_select_quarters([None if u is None else qms[u] for u in t]), bf16)
                 for t in plans[c]]
            r0 = T * j + c * QW
            pc[c] = jnp.exp2(_dot(kp_ref[g, r0:r0 + QW, :], jnp.concatenate(w, axis=1)))
        for u in range(nh):
            pu = p0[:, u * T:(u + 1) * T]
            if j > 0:
                p_ref[u, j, 0:j * T, :] = pu[0:j * T].astype(bf16)
            rows = [pu[j * T:n0]]
            for c in range(1, 4):
                src = [None] * 4
                for i, t in enumerate(plans[c]):
                    for q in range(4):
                        if t[q] == u:
                            src[q] = i
                vals = {i: pc[c][:, i * T:(i + 1) * T] for i in set(src) if i is not None}
                rows.append(_select_quarters([None if i is None else vals[i] for i in src]))
            p_ref[u, j, j * T:(j + 1) * T, :] = (
                jnp.concatenate(rows, axis=0) * cm_ref[ROT[u]]).astype(bf16)


def _attention_safe(h, kp_ref, qt_ref, vt_ref, g1_ref, am_ref, ot_ref):
    g = jnp.minimum(jnp.maximum(h - 1, 0) // 6, NG - 1)
    ws = pl.multiple_of(g * WIN, 16)
    lo = h * DH - ws
    row128 = lax.broadcasted_iota(jnp.int32, (T, T), 0)
    qmask = (row128 >= lo) & (row128 < lo + DH)
    vs = pl.multiple_of(((h * DH) // 16) * 16, 16)
    off = h * DH - vs
    row32 = lax.broadcasted_iota(jnp.int32, (32, T), 0)
    omask = (row32 >= off) & (row32 < off + DH)
    kk = lax.broadcasted_iota(jnp.int32, (L, T), 0)
    qq = lax.broadcasted_iota(jnp.int32, (L, T), 1)

    def tile(j, c):
        c0 = pl.multiple_of(j * T, T)
        qm = jnp.where(qmask, qt_ref[pl.ds(ws, T), pl.ds(c0, T)].astype(f32), 0.0).astype(bf16)
        s = _dot(kp_ref[g], qm)
        s = jnp.where(kk <= qq + c0, s, -jnp.inf)
        m = jnp.max(s, axis=0, keepdims=True)
        p = jnp.exp2(s - m).astype(bf16)
        acc = _dot(_v_rows(vt_ref, vs, off // 2, L), p)
        l8 = jnp.where(off <= 6, acc[24:32], acc[0:8])
        rl = g1_ref[h] / l8
        o = acc * jnp.concatenate([rl] * 4, axis=0) + am_ref[pl.ds(vs, 32), pl.ds(c0, T)]
        pltpu.store(ot_ref.at[pl.ds(vs, 32), pl.ds(c0, T)], o, mask=omask)
        return c

    lax.fori_loop(0, NT, tile, 0)


def _v_rows(vt_ref, vs, off2, nk):
    row16 = lax.broadcasted_iota(jnp.int32, (16, nk), 0)
    keep = (row16 >= off2) & (row16 < off2 + DH // 2)
    v32 = pltpu.bitcast(vt_ref[pl.ds(vs, 32), 0:nk], jnp.uint32)
    return pltpu.bitcast(jnp.where(keep, v32, jnp.uint32(0x3F803F80)), bf16)


def _pv(g, vt_ref, p_ref, g1_ref, am_ref, ot_ref):
    row32 = lax.broadcasted_iota(jnp.int32, (32, T), 0)
    for u, h in enumerate(GROUPS[g]):
        vs = ((h * DH) // 16) * 16
        off = h * DH - vs
        omask = (row32 >= off) & (row32 < off + DH)
        g1 = g1_ref[h]
        vrows = _v_rows(vt_ref, vs, off // 2, L)
        for j in range(NT):
            nk = T * (j + 1)
            acc = _dot(vrows[:, 0:nk], p_ref[u, j, 0:nk, :])
            l8 = acc[24:32] if off <= 6 else acc[0:8]
            rl = g1 / l8
            o = acc * jnp.concatenate([rl] * 4, axis=0)
            if ROT[u]:
                o = pltpu.roll(o, T - ROT[u] * QW, axis=1)
            o = o + am_ref[vs:vs + 32, j * T:(j + 1) * T]
            pltpu.store(ot_ref.at[vs:vs + 32, j * T:(j + 1) * T], o, mask=omask)


def _kernel(x_hbm, wq_hbm, wk_hbm, wv_hbm, wo_hbm, beta_hbm, wr_hbm, wg_hbm, wu_hbm, wd_hbm,
            out_hbm,
            x_v, w_in, wt, wot, hbuf, wg_v, wu_v, wd_v,
            aug, arow, qt, pqt, kt, pkt, vt, kp, p0, p1, am_v, ot,
            macc, mb, bmask, cmask, g1tab, wrtab, ab_all, out_v, best_v, best_i, wrsum, beta_ref, wr_ref,
            sem_x, sem_w, sem_o):
    def x_copy(s):
        return pltpu.make_async_copy(x_hbm.at[0, :, pl.ds(s * L, L)],
                                     x_v.at[:, pl.ds(s * L, L)], sem_x.at[s])

    def out_copy(s):
        return pltpu.make_async_copy(out_v.at[:, pl.ds(s * L, L)],
                                     out_hbm.at[0, :, pl.ds(s * L, L)], sem_o.at[s])

    w_copies = [
        None,
        pltpu.make_async_copy(wk_hbm, w_in.at[1], sem_w.at[1]),
        pltpu.make_async_copy(wv_hbm, w_in.at[2], sem_w.at[2]),
        pltpu.make_async_copy(wo_hbm, w_in.at[3], sem_w.at[3]),
        pltpu.make_async_copy(wg_hbm, wg_v, sem_w.at[4]),
        pltpu.make_async_copy(wu_hbm, wu_v, sem_w.at[5]),
        pltpu.make_async_copy(wd_hbm, wd_v, sem_w.at[6]),
    ]
    small_b = pltpu.make_async_copy(beta_hbm, beta_ref, sem_w.at[7])
    small_r = pltpu.make_async_copy(wr_hbm, wr_ref, sem_w.at[8])
    QA, QLO, QB = Q_SPLITS
    wq_lo = pltpu.make_async_copy(wq_hbm.at[:, 0:QLO], w_in.at[0, :, 0:QLO], sem_w.at[0])
    wq_hi = pltpu.make_async_copy(wq_hbm.at[:, QLO:D], w_in.at[0, :, QLO:D], sem_w.at[9])
    small_b.start()
    small_r.start()
    wq_lo.start()
    x_copy(0).start()

    def build_tables():
        gate = jax.nn.sigmoid(beta_ref[...].astype(f32).reshape(1, H))
        hh8 = lax.broadcasted_iota(jnp.int32, (8, H), 1)
        for h in range(H):
            gh = jnp.sum(jnp.where(hh8 == h, gate, 0.0), axis=1, keepdims=True)
            g1tab[h] = jnp.broadcast_to(1.0 - gh, (8, T))
        wr_row = wr_ref[...].astype(f32).reshape(1, D)
        wr_pad = jnp.concatenate([wr_row, jnp.zeros((1, 5 * T - D), f32)], axis=1)
        wrtab[...] = jnp.broadcast_to(wr_pad, (T, 5 * T)).T[0:D]
        wrsum[...] = jnp.broadcast_to(jnp.sum(wr_row, axis=1, keepdims=True), wrsum.shape)

    mr = lax.broadcasted_iota(jnp.int32, (MROWS, T), 0)
    mc = lax.broadcasted_iota(jnp.int32, (MROWS, T), 1)
    for g in range(NG):
        ws = WIN * g
        code = jnp.zeros((MROWS, T), f32)
        for i, h in enumerate(GROUPS[g]):
            lo = h * DH - ws
            cols = (mc >= lo) & (mc < lo + DH)
            code = jnp.where(cols & (mr >= lo) & (mr < lo + DH) & (mr < T), 1.0, code)
            code = jnp.where(cols & (mr == DEN_ROW[g] + i), 2.0, code)
        bmask[g] = code
    kk = lax.broadcasted_iota(jnp.int32, (T, T), 0)
    qq = lax.broadcasted_iota(jnp.int32, (T, T), 1)
    for r in range(4):
        cmask[r] = jnp.where(kk <= ((qq - r * QW) & (T - 1)), 1.0, 0.0)
    macc[...] = jnp.zeros_like(macc)
    mb[...] = jnp.zeros_like(mb)
    best_v[...] = jnp.full(best_v.shape, -jnp.inf, f32)
    best_i[...] = jnp.zeros(best_i.shape, jnp.int32)

    def ln1(s):
        col0 = pl.multiple_of(s * L, L)
        xs = x_v[:, pl.ds(col0, L)].astype(f32)
        m = _colsum(xs) * (1.0 / D)
        v = jnp.maximum(_colsum(xs * xs) * (1.0 / D) - m * m, 0.0)
        arow[:, pl.ds(col0, L)] = jnp.broadcast_to(lax.rsqrt(v + EPS), (8, L))
        m_hi = (-m).astype(bf16).astype(f32)
        m_lo = -m - m_hi
        r16 = lax.broadcasted_iota(jnp.int32, (16, L), 0)
        rows = jnp.where(r16 >= 4, 0.0, jnp.where((r16 & 1) == 0, m_hi, m_lo))
        aug[:, pl.ds(col0, L)] = rows.astype(bf16)

    def finalize(s, t0, nt, attn):
        w = nt * T
        col0 = pl.multiple_of(s * L + t0 * T, T)
        hres = x_v[:, pl.ds(col0, w)].astype(f32) + attn
        hbuf[:, pl.ds(col0, w)] = hres
        a, b = _ln_stats(hres)
        wr = jnp.concatenate([wrtab[...]] * nt, axis=1)
        r = _colsum(hres * wr) * a + b * wrsum[0:1, 0:1]
        ab_all[0:8, pl.ds(col0, w)] = jnp.broadcast_to(a, (8, w))
        ab_all[8:16, pl.ds(col0, w)] = jnp.broadcast_to(b, (8, w))
        out_v[:, pl.ds(col0, w)] = (hbuf[:, pl.ds(col0, w)] * (1.0 + a) + b).astype(bf16)
        r = r.astype(bf16).astype(f32)
        bv, bi = best_v[0:1, :], best_i[0:1, :]
        for t in range(nt):
            rt = r[:, t * T:(t + 1) * T]
            better = rt > bv
            bi = jnp.where(better, col0 + t * T, bi)
            bv = jnp.where(better, rt, bv)
        best_i[...] = jnp.broadcast_to(bi, best_i.shape)
        best_v[...] = jnp.broadcast_to(bv, best_v.shape)

    def proj_rhs(s):
        col0 = pl.multiple_of(s * L, L)
        return jnp.concatenate([x_v[:, pl.ds(col0, L)], aug[:, pl.ds(col0, L)],
                                jnp.zeros((KP - D - 16, L), bf16)], axis=0)

    def ln_scale(s):
        return arow[0:1, pl.ds(pl.multiple_of(s * L, L), L)]

    def store_q(raw, a, r0, r1, with_phi=True, cols=slice(None)):
        qt[r0:r1, cols] = (raw * (a * QSCALE)).astype(bf16)
        if with_phi:
            pqt[r0:r1, cols] = _phi(raw * a).astype(bf16)

    def store_k_rows(raw, a, r0, r1):
        k = raw * a
        kt[r0:r1, :] = k.astype(bf16)
        pkt[r0:r1, :] = _phi(k).astype(bf16)

    def transpose_k():
        for g in range(NG):
            kp[g] = kt[WIN * g:WIN * g + T, :].T

    def store_k(raw, a, cols):
        k = raw * a
        kb = k.astype(bf16)
        pkt[:, cols] = _phi(k).astype(bf16)
        for g in range(NG):
            kp[g, cols, :] = kb[WIN * g:WIN * g + T, :].T

    def store_v(raw, a, cols=slice(None)):
        vt[:, cols] = (raw * a).astype(bf16)

    def project(s):
        rhs = proj_rhs(s)
        a = ln_scale(s)
        w = PROJ_COLS * T
        halves = [slice(c0, c0 + w) for c0 in range(0, L, w)]
        for cols in halves:
            store_q(_dot(wt[0:D, :], rhs[:, cols]), a[:, cols], 0, D, True, cols)
        mem_read()
        for cols in halves:
            store_k(_dot(wt[D:2 * D, :], rhs[:, cols]), a[:, cols], cols)
        for cols in halves:
            store_v(_dot(wt[2 * D:3 * D, :], rhs[:, cols]), a[:, cols], cols)

    def mem_read():
        row128 = lax.broadcasted_iota(jnp.int32, (T, T), 0)
        row8 = lax.broadcasted_iota(jnp.int32, (8, T), 0)
        for g in range(NG):
            ws = WIN * g
            heads = GROUPS[g]
            lo_g, hi_g = heads[0] * DH - ws, (heads[-1] + 1) * DH - ws
            wmask = (row128 >= lo_g) & (row128 < hi_g)
            for j in range(NT):
                nrows = MROWS if DEN_ROW[g] == T else T
                nd = _dot(mb[g, 0:nrows], pqt[ws:ws + T, j * T:(j + 1) * T])
                rden = 1.0 / (nd[DEN_ROW[g]:DEN_ROW[g] + 8] + 1e-6)
                rb = [jnp.broadcast_to(rden[i:i + 1], (8, T)) * (1.0 - g1tab[h])
                      for i, h in enumerate(heads)]
                blocks = []
                for b in range(T // 8):
                    r_lo, r_hi = 8 * b, 8 * b + 7
                    i_lo = min(max((r_lo + ws) // DH - heads[0], 0), len(heads) - 1)
                    i_hi = min(max((r_hi + ws) // DH - heads[0], 0), len(heads) - 1)
                    if i_lo == i_hi:
                        blocks.append(rb[i_lo])
                    else:
                        cut = (heads[0] + i_hi) * DH - ws - r_lo
                        blocks.append(jnp.where(row8 < cut, rb[i_lo], rb[i_hi]))
                amv = nd[0:T] * jnp.concatenate(blocks, axis=0)
                pltpu.store(am_v.at[ws:ws + T, j * T:(j + 1) * T], amv, mask=wmask)

    def attention(fast):
        ps = (p0, p1)
        if fast:
            _scores_fast(0, kp, qt, cmask, ps[0])
            for g in range(NG):
                if g + 1 < NG:
                    _scores_fast(g + 1, kp, qt, cmask, ps[(g + 1) % 2])
                _pv(g, vt, ps[g % 2], g1tab, am_v, ot)
        else:
            lax.fori_loop(0, H, lambda h, c: (_attention_safe(h, kp, qt, vt, g1tab, am_v, ot), c)[1], 0)

    def mem_update():
        word = lax.broadcasted_iota(jnp.int32, (T // 2, L), 0)
        for g in range(NG):
            ws = WIN * g
            v32 = pltpu.bitcast(vt[ws:ws + T, :], jnp.uint32)
            lhs = pltpu.bitcast(jnp.where(word == Z_ROW[g] // 2, jnp.uint32(0x3F803F80), v32), bf16)
            upd = macc[g] + _dot_nt(lhs, pkt[ws:ws + T, :])
            macc[g] = upd
            nrows = MROWS if DEN_ROW[g] == T else T
            z = jnp.broadcast_to(upd[Z_ROW[g]:Z_ROW[g] + 1], (nrows, T))
            m = upd if nrows == T else jnp.concatenate([upd, jnp.zeros((nrows - T, T), f32)], axis=0)
            code = bmask[g, 0:nrows]
            mb[g, 0:nrows] = jnp.where(code == 1.0, m, jnp.where(code == 2.0, z, 0.0)).astype(bf16)

    def load_weight(i, c0=0, c1=D):
        w = w_in[i, :, c0:c1]
        n = c1 - c0
        wf = w.astype(f32)
        ones = jnp.ones((16, D), bf16)
        c = _dot(ones, w)[0:1]
        c_hi = c.astype(bf16).astype(f32)
        r16 = lax.broadcasted_iota(jnp.int32, (16, n), 0)
        extra = jnp.where(r16 >= 4, 0.0, jnp.where(r16 < 2, c_hi, c - c_hi)).astype(bf16)
        w_aug = jnp.concatenate([w, extra, jnp.zeros((KP - D - 16, n), bf16)], axis=0)
        w_t = w_aug.T
        wt[i * D + c0:i * D + c1, :] = w_t
        return w_t, jnp.max(_dot(ones, (wf * wf).astype(bf16)))

    am_v[...] = jnp.zeros_like(am_v)
    ot[...] = jnp.zeros_like(ot)
    with _scope("p_tables"):
        small_b.wait()
        small_r.wait()
        build_tables()
    with _scope("p_wq_wait"):
        wq_lo.wait()
    wq_hi.start()
    w_copies[1].start()
    with _scope("p_wqT"):
        _, cq_lo = load_weight(0, 0, QLO)
    with _scope("p_x0_wait"):
        x_copy(0).wait()
    w_copies[2].start()
    w_copies[3].start()
    HALF = K_SPLIT

    def q_rows(lhs, r0, r1):
        store_q(_dot(lhs, proj_rhs(0)), ln_scale(0), r0, r1, False)

    with _scope("p_b1"):
        ln1(0)
        q_rows(wt[0:QA, :], 0, QA)
    with _scope("p_wqhi_wait"):
        wq_hi.wait()
    for s in range(1, NSEG):
        x_copy(s).start()
    for c in w_copies[4:]:
        c.start()
    with _scope("p_b2"):
        wq_t, cq_hi = load_weight(0, QLO, D)
        cq = jnp.maximum(cq_lo, cq_hi)
        q_rows(wt[QA:QLO, :], QA, QLO)
        q_rows(wq_t[0:QB - QLO], QLO, QB)
    with _scope("p_wk_wait"):
        w_copies[1].wait()
    with _scope("p_b3"):
        wk_t, ck = load_weight(1)
        q_rows(wt[QB:D, :], QB, D)
        store_k_rows(_dot(wk_t[0:HALF], proj_rhs(0)), ln_scale(0), 0, HALF)
    with _scope("p_wv_wait"):
        w_copies[2].wait()
        w_copies[3].wait()
    with _scope("p_khi_wvT_v"):
        wv_t, cv = load_weight(2)
        wot[...] = w_in[3].T
        store_k_rows(_dot(wt[D + HALF:2 * D, :], proj_rhs(0)), ln_scale(0), HALF, D)
        transpose_k()
        store_v(_dot(wv_t, proj_rhs(0)), ln_scale(0))
    slack = 1.06
    logit_bound2 = (cq * ck) * (slack * D * DH * QSCALE) ** 2
    v_bound2 = cv * (slack * D)
    safe = (logit_bound2 <= SAFE_LOGIT ** 2) & (v_bound2 <= SAFE_V ** 2)

    def body(s, carry):
        more = s + 1 < NSEG
        nxt = jnp.minimum(s + 1, NSEG - 1)

        @pl.when(more)
        def _():
            x_copy(nxt).wait()

        @pl.when(safe)
        def _():
            with _scope("attn"):
                attention(True)

        @pl.when(jnp.logical_not(safe))
        def _():
            attention(False)

        @pl.when(more)
        def _():
            with _scope("blockB"):
                mem_update()
                attn = [_dot(wot[...], ot[:, t * T:(t + 1) * T].astype(bf16)) for t in range(NT)]
                ln1(nxt)
                project(nxt)
                for t in range(NT):
                    finalize(s, t, 1, attn[t])
            out_copy(s).start()
        return carry

    lax.fori_loop(0, NSEG, body, 0)
    with _scope("fin"):
        otb = ot[...].astype(bf16)
        for t in range(NT):
            finalize(NSEG - 1, t, 1, _dot(wot[...], otb[:, t * T:(t + 1) * T]))
        out_copy(NSEG - 1).start()

    bv = best_v[...]
    rmax = jnp.max(bv, axis=1, keepdims=True)
    cand = best_i[...] + lax.broadcasted_iota(jnp.int32, best_i.shape, 1)
    idx = jnp.clip(jnp.min(jnp.where(bv == rmax, cand, S)), 0, S - 1)
    base = pl.multiple_of((idx // T) * T, T)
    lane = idx - base
    blk = (hbuf[:, pl.ds(base, T)] * ab_all[0:1, pl.ds(base, T)]
           + ab_all[8:9, pl.ds(base, T)]).astype(bf16)
    pick = jnp.where(lax.broadcasted_iota(jnp.int32, (16, T), 1) == lane, 1.0, 0.0).astype(bf16)
    xg = _dot_nt(pick, blk).astype(bf16)
    for c in w_copies[4:]:
        c.wait()
    yacc = jnp.zeros((D, T), f32)
    for f_lo in range(0, F, MOE_CHUNK * T):
        f_hi = f_lo + MOE_CHUNK * T
        gt = _dot(xg, wg_v[:, f_lo:f_hi])
        up = _dot(xg, wu_v[:, f_lo:f_hi])
        act = (gt * jax.nn.sigmoid(gt) * up)[0:1].astype(bf16).astype(f32)
        for t in range(MOE_CHUNK):
            f0 = f_lo + t * T
            yacc = yacc + wd_v[:, f0:f0 + T].astype(f32) * act[:, t * T:(t + 1) * T]
    y = jnp.sum(yacc, axis=1, keepdims=True) * jax.nn.sigmoid(rmax[0:1])
    for s in range(NSEG):
        out_copy(s).wait()
    sel = lax.broadcasted_iota(jnp.int32, (D, T), 1) == lane
    cur = out_v[:, pl.ds(base, T)].astype(f32)
    out_v[:, pl.ds(base, T)] = (cur + jnp.where(sel, y, 0.0)).astype(bf16)
    patch = pltpu.make_async_copy(out_v.at[:, pl.ds(base, T)],
                                  out_hbm.at[0, :, pl.ds(base, T)], sem_o.at[NSEG])
    patch.start()
    patch.wait()


@jax.jit
def pallas_sequential_preLN__memory_aug_infini_attn__moe_arch_mod__prompt_kernel(
    A_x: jax.Array,
    A_wq: jax.Array,
    A_wk: jax.Array,
    A_wv: jax.Array,
    A_wo: jax.Array,
    A_beta: jax.Array,
    B_x: jax.Array,
    B_w_r: jax.Array,
    B_w_gate: jax.Array,
    B_w_up: jax.Array,
    B_w_down: jax.Array,
):
    del B_x
    hbm_spec = pl.BlockSpec(memory_space=pltpu.HBM)
    scratch = [
        pltpu.VMEM((D, S), bf16),
        pltpu.VMEM((4, D, D), bf16),
        pltpu.VMEM((3 * D, KP), bf16),
        pltpu.VMEM((D, D), bf16),
        pltpu.VMEM((D, S), f32),
        pltpu.VMEM((D, F), bf16),
        pltpu.VMEM((D, F), bf16),
        pltpu.VMEM((D, F), bf16),
        pltpu.VMEM((16, S), bf16),
        pltpu.VMEM((8, S), f32),
        pltpu.VMEM((D, L), bf16),
        pltpu.VMEM((D, L), bf16),
        pltpu.VMEM((D, L), bf16),
        pltpu.VMEM((D, L), bf16),
        pltpu.VMEM((D, L), bf16),
        pltpu.VMEM((NG, L, T), bf16),
        pltpu.VMEM((7, NT, L, T), bf16),
        pltpu.VMEM((7, NT, L, T), bf16),
        pltpu.VMEM((D, L), f32),
        pltpu.VMEM((D, L), f32),
        pltpu.VMEM((NG, T, T), f32),
        pltpu.VMEM((NG, MROWS, T), bf16),
        pltpu.VMEM((NG, MROWS, T), f32),
        pltpu.VMEM((4, T, T), f32),
        pltpu.VMEM((H, 8, T), f32),
        pltpu.VMEM((D, T), f32),
        pltpu.VMEM((16, S), f32),
        pltpu.VMEM((D, S), bf16),
        pltpu.VMEM((8, T), f32),
        pltpu.VMEM((8, T), jnp.int32),
        pltpu.VMEM((8, T), f32),
        pltpu.VMEM((H,), bf16),
        pltpu.VMEM((D,), bf16),
        pltpu.SemaphoreType.DMA((NSEG,)),
        pltpu.SemaphoreType.DMA((10,)),
        pltpu.SemaphoreType.DMA((NSEG + 1,)),
    ]
    out_t = pl.pallas_call(
        _kernel,
        out_shape=jax.ShapeDtypeStruct((1, D, S), bf16),
        in_specs=[hbm_spec] * 10,
        out_specs=hbm_spec,
        scratch_shapes=scratch,
        compiler_params=pltpu.CompilerParams(vmem_limit_bytes=100 * 1024 * 1024),
    )(jnp.transpose(A_x, (0, 2, 1)), A_wq, A_wk, A_wv, A_wo, A_beta,
      B_w_r, B_w_gate, B_w_up, B_w_down.T)
    return jnp.transpose(out_t, (0, 2, 1))
```
